```python
import jax
import jax.numpy as jnp

def _softmax(x, axis=-1):
    return jax.nn.softmax(x, axis=axis)

def _gelu(x):
    return jax.nn.gelu(x, approximate=True)

def _silu(x):
    return jax.nn.silu(x)

def _sigmoid(x):
    return jax.nn.sigmoid(x)

def _layernorm(x, axis=-1, eps=1e-05):
    m = jnp.mean(x, axis=axis, keepdims=True)
    v = jnp.var(x, axis=axis, keepdims=True)
    return (x - m) / jnp.sqrt(v + eps)

def _scatter_add(tgt, idx, src, axis=0):
    return tgt.at[idx].add(src)

def _segment_sum(src, seg, n):
    return jax.ops.segment_sum(src, seg, n)

class _Rng:

    def __init__(self, key):
        self._k = key

    def _next(self):
        self._k, sub = jax.random.split(self._k)
        return sub

    def normal(self, shape):
        return jax.random.normal(self._next(), shape, dtype=jnp.bfloat16)

    def randint(self, lo, hi, shape):
        return jax.random.randint(self._next(), shape, lo, hi, dtype=jnp.int32)

    def uniform(self, shape, lo=0.0, hi=1.0):
        return jax.random.uniform(self._next(), shape, jnp.bfloat16, lo, hi)

    def permutation(self, n):
        return jax.random.permutation(self._next(), n)
kernel_name = 'interleave_layers__memory_aug_infini_attn__mixer_s_mlp__prompt'

def setup_inputs():
    _rng = _Rng(jax.random.key(int.from_bytes(__import__("os").urandom(4), "little")))
    _w = lambda a: (lambda t: t.astype(jnp.bfloat16) if jnp.issubdtype(t.dtype, jnp.floating) else t)(jnp.asarray(a))

    def _A_setup():
        B, S, D, H = (1, 2048, 1024, 32)
        N = 4
        L = max(1, S // N)
        sc = D ** (-0.5)
        return {'x': _w((lambda *s: _rng.normal(s) * 0.05)(B, N * L, D)), 'wq': _w((lambda *s: _rng.normal(s) * 0.05)(D, D) * sc), 'wk': _w((lambda *s: _rng.normal(s) * 0.05)(D, D) * sc), 'wv': _w((lambda *s: _rng.normal(s) * 0.05)(D, D) * sc), 'wo': _w((lambda *s: _rng.normal(s) * 0.05)(D, D) * sc), 'beta': _w((lambda *s: _rng.normal(s) * 0.05)(H))}
    _A_in = _A_setup()

    def _B_setup():
        B, S, D, F = (1, 2048, 1024, 3584)
        return {'x': _w((lambda *s: _rng.normal(s) * 0.05)(B, S, D)), 'w1': _w((lambda *s: _rng.normal(s) * 0.05)(D, D) * D ** (-0.5)), 'w2': _w((lambda *s: _rng.normal(s) * 0.05)(D, D) * D ** (-0.5)), 'w3': _w((lambda *s: _rng.normal(s) * 0.05)(D, F) * D ** (-0.5)), 'w4': _w((lambda *s: _rng.normal(s) * 0.05)(F, D) * F ** (-0.5))}
    _B_in = _B_setup()
    return {'A_x': _A_in['x'], 'A_wq': _A_in['wq'], 'A_wk': _A_in['wk'], 'A_wv': _A_in['wv'], 'A_wo': _A_in['wo'], 'A_beta': _A_in['beta'], 'B_x': _B_in['x'], 'B_w1': _B_in['w1'], 'B_w2': _B_in['w2'], 'B_w3': _B_in['w3'], 'B_w4': _B_in['w4']}

def reference(A_x, A_wq, A_wk, A_wv, A_wo, A_beta, B_x, B_w1, B_w2, B_w3, B_w4):

    def _A_ref(x, wq, wk, wv, wo, beta):
        B, S, D = x.shape
        H = 32
        Dh = D // H
        N = 4
        L = S // N
        q = (lambda x, *d: x.transpose(*d))((x @ wq).reshape(B, S, H, Dh), 0, 2, 1, 3).reshape(B, H, N, L, Dh)
        k = (lambda x, *d: x.transpose(*d))((x @ wk).reshape(B, S, H, Dh), 0, 2, 1, 3).reshape(B, H, N, L, Dh)
        v = (lambda x, *d: x.transpose(*d))((x @ wv).reshape(B, S, H, Dh), 0, 2, 1, 3).reshape(B, H, N, L, Dh)
        phi = lambda t: jnp.where(t > 0, t + 1.0, jnp.exp(t))
        scale = Dh ** (-0.5)
        ar = jnp.arange(L)
        mask = (lambda x, dt: x.astype(dt))(ar[:, None] < ar[None, :], x.dtype) * -1000000000.0
        g = _sigmoid(beta).reshape(1, H, 1, 1)
        M = jnp.einsum('bhd,bhe->bhde', q[:, :, 0, 0, :] * 0.0, q[:, :, 0, 0, :] * 0.0)
        z = q[:, :, 0, 0, :] * 0.0
        outs = []
        for s in range(N):
            qs, ks, vs = (q[:, :, s].copy(), k[:, :, s].copy(), v[:, :, s].copy())
            logits = jnp.einsum('bhqd,bhkd->bhqk', qs, ks) * scale + mask
            p = _softmax(logits, axis=-1)
            a_dot = jnp.einsum('bhqk,bhkd->bhqd', p, vs)
            pq = phi(qs)
            num = jnp.einsum('bhld,bhde->bhle', pq, M)
            den = jnp.einsum('bhld,bhd->bhl', pq, z)[..., None] + 1e-06
            a_mem = num / den
            o = g * a_mem + (1.0 - g) * a_dot
            outs.append(o)
            pk = phi(ks)
            M = M + jnp.einsum('bhld,bhle->bhde', pk, vs)
            z = z + jnp.einsum('bhld->bhd', pk)
        o = (lambda x, *d: x.transpose(*d))(jnp.stack(outs, 2).reshape(B, H, S, Dh), 0, 2, 1, 3).reshape(B, S, D)
        return o @ wo

    def _B_ref(x, w1, w2, w3, w4):
        B, S, D = x.shape
        h = _gelu(_layernorm(x, axis=-1) @ w1)
        c = D // 4
        g0 = jnp.pad(h[:, :, 0 * c:1 * c], ((0, 0), (1, 0), (0, 0)))[:, :S, :]
        g1 = jnp.pad(h[:, :, 1 * c:2 * c], ((0, 0), (0, 1), (0, 0)))[:, 1:, :]
        g2 = jnp.pad(h[:, :, 2 * c:3 * c], ((0, 0), (2, 0), (0, 0)))[:, :S, :]
        g3 = jnp.pad(h[:, :, 3 * c:], ((0, 0), (0, 2), (0, 0)))[:, 2:, :]
        hs = jnp.concatenate([g0, g1, g2, g3], axis=-1) @ w2
        x1 = x + hs
        h2 = _gelu(_layernorm(x1, axis=-1) @ w3) @ w4
        return x1 + h2
    x = A_x
    x = x + _A_ref(_layernorm(x, axis=-1), A_wq, A_wk, A_wv, A_wo, A_beta)
    x = x + _B_ref(_layernorm(x, axis=-1), B_w1, B_w2, B_w3, B_w4)
    x = x + _A_ref(_layernorm(x, axis=-1), A_wq, A_wk, A_wv, A_wo, A_beta)
    x = x + _B_ref(_layernorm(x, axis=-1), B_w1, B_w2, B_w3, B_w4)
    return x
```

```python
import functools
import math

import jax
import jax.numpy as jnp
import jax.experimental.pallas as pl
import jax.experimental.pallas.tpu as pltpu

S = 2048
D = 1024
F = 3584
H = 32
DH = 32
L = 512
NSEG = S // L
NG = D // 128
NT_TILES = L // 128
FC = 256
HALO = 8

LOG2E = math.log2(math.e)
QSCALE = DH ** -0.5 * LOG2E
MASK_BIAS = -1e9 * LOG2E
EPS = 1e-5

f32 = jnp.float32
bf16 = jnp.bfloat16
NT_DIMS = (((1,), (1,)), ((), ()))


def _ln(x):
    m = jnp.mean(x, axis=-1, keepdims=True)
    xc = x - m
    v = jnp.mean(xc * xc, axis=-1, keepdims=True)
    return xc * jax.lax.rsqrt(v + EPS)


def _gelu(x):
    c = math.sqrt(2.0 / math.pi)
    inner = x * (c + (c * 0.044715) * (x * x))
    hx = 0.5 * x
    return hx + hx * jnp.tanh(inner)


def _phi(t):
    return jnp.where(t > 0, t + 1.0, jnp.exp(t))


def _red8(x, op):
    return functools.reduce(op, [x[i * 8:(i + 1) * 8] for i in range(x.shape[0] // 8)])


def _dot(a, b):
    return jnp.dot(a, b, preferred_element_type=f32)


def _kernel(x_hbm, wq_hbm, wk_hbm, wv_hbm, wo_hbm, beta_ref, w1_hbm, w2_hbm, w3_hbm, w4_hbm,
            out_hbm,
            xin, stage, wqvt, wk, wo, w1, w2, w3, w4,
            xres, yres, hbuf, xn, qt, pqt, kb, pkb, vt, ob, amem,
            mt, zrow, gate, bias,
            s0, s1, s2, s3, m0, m1, m2, m3,
            acc, obuf, sems, osems):
    sbuf = (s0, s1, s2, s3)
    mbuf = (m0, m1, m2, m3)

    cp_x = pltpu.make_async_copy(x_hbm.at[0], xin, sems.at[0])
    cp_wq = pltpu.make_async_copy(wq_hbm, stage.at[0], sems.at[1])
    cp_wv = pltpu.make_async_copy(wv_hbm, stage.at[1], sems.at[2])
    cp_wk = pltpu.make_async_copy(wk_hbm, wk, sems.at[3])
    cp_wo = pltpu.make_async_copy(wo_hbm, wo, sems.at[4])
    cp_w1 = pltpu.make_async_copy(w1_hbm, w1, sems.at[5])
    cp_w2 = pltpu.make_async_copy(w2_hbm, w2, sems.at[6])
    cp_w3 = [pltpu.make_async_copy(w3_hbm.at[:, pl.ds(c * FC, FC)], w3.at[c], sems.at[7])
             for c in range(F // FC)]
    cp_w4 = pltpu.make_async_copy(w4_hbm, w4, sems.at[8])

    cp_wq.start()
    cp_wv.start()
    cp_x.start()
    cp_wk.start()

    kk = jax.lax.broadcasted_iota(jnp.int32, (128, 512), 0)
    qq = jax.lax.broadcasted_iota(jnp.int32, (128, 512), 1) % 128
    bias[...] = jnp.where(kk > qq, MASK_BIAS, 0.0).astype(f32)
    bt = jnp.broadcast_to(beta_ref[...].astype(f32), (H, H))
    eye = (jax.lax.broadcasted_iota(jnp.int32, (H, H), 0)
           == jax.lax.broadcasted_iota(jnp.int32, (H, H), 1))
    bcol = jnp.sum(jnp.where(eye, bt, 0.0), axis=1, keepdims=True)
    gate[...] = jnp.broadcast_to(jax.nn.sigmoid(bcol), (H, 128))
    hbuf[0:HALO, :] = jnp.zeros((HALO, D), f32)
    hbuf[S + HALO:S + 2 * HALO, :] = jnp.zeros((HALO, D), f32)

    def transpose_w(i):
        def body(c, _):
            r = pl.multiple_of(c * 128, 128)
            blk = stage[i, pl.ds(r, 128), :].astype(f32)
            wqvt[i, c] = blk.T.astype(bf16)
            return 0
        jax.lax.fori_loop(0, D // 128, body, 0)

    cp_wq.wait()
    transpose_w(0)
    cp_wv.wait()
    transpose_w(1)
    cp_x.wait()
    cp_wk.wait()
    cp_wo.start()
    cp_w1.start()
    cp_w2.start()
    for c in cp_w3:
        c.start()
    cp_w4.start()

    def init_x(i, _):
        r = pl.multiple_of(i * 256, 256)
        xres[pl.ds(r, 256), :] = xin[pl.ds(r, 256), :].astype(f32)
        return 0
    jax.lax.fori_loop(0, S // 256, init_x, 0)

    def qmask(g, t):
        z = jnp.zeros((DH, 128), bf16)
        cols = []
        for h in range(4):
            qh = qt[g, h * DH:(h + 1) * DH, t * 128:(t + 1) * 128]
            cols.append(jnp.concatenate([qh if i == h else z for i in range(4)], axis=0))
        return jnp.concatenate(cols, axis=1)

    def attn_step(g, gn):
        pr = None if g is None else g % 2
        pw = None if gn is None else gn % 2
        for t in range(NT_TILES):
            macc = None
            oacc = [None] * 4
            lacc = [None] * 4
            for j in range(t + 1):
                ks = slice(j * 128, (j + 1) * 128)
                if gn is not None:
                    s = _dot(kb[gn, ks, :], qmask(gn, t))
                    if j == t:
                        s = s + bias[...]
                    sbuf[t][pw, ks, :] = s
                    mx = _red8(s, jnp.maximum)
                    macc = mx if macc is None else jnp.maximum(macc, mx)
                if g is not None:
                    for h in range(4):
                        sl = slice(h * 128, (h + 1) * 128)
                        p = jnp.exp2(sbuf[t][pr, ks, sl] - mbuf[t][pr, :, sl])
                        lt = _red8(p, jnp.add)
                        lacc[h] = lt if lacc[h] is None else lacc[h] + lt
                        o = _dot(vt[g, h * DH:(h + 1) * DH, ks], p.astype(bf16))
                        oacc[h] = o if oacc[h] is None else oacc[h] + o
            if gn is not None:
                mbuf[t][pw] = jnp.max(macc, axis=0, keepdims=True)
            if g is not None:
                parts = []
                for h in range(4):
                    l = jnp.sum(lacc[h], axis=0, keepdims=True)
                    gh = gate[g * 4 + h:g * 4 + h + 1, :]
                    parts.append(oacc[h] * ((1.0 - gh) / l))
                ot = jnp.concatenate(parts, axis=0) + amem[g, :, t * 128:(t + 1) * 128]
                ob[g, t * 128:(t + 1) * 128, :] = ot.T.astype(bf16)

    rowh = jax.lax.broadcasted_iota(jnp.int32, (128, 128), 0) // DH
    colh = jax.lax.broadcasted_iota(jnp.int32, (128, 128), 1) // DH
    row16 = jax.lax.broadcasted_iota(jnp.int32, (16, 128), 0)
    col16 = jax.lax.broadcasted_iota(jnp.int32, (16, 128), 1) // DH

    def phase_a(layer, seg):
        r0 = pl.multiple_of(seg * L, L)
        rows = pl.ds(r0, L)
        xn[...] = _ln(xres[rows, :]).astype(bf16)

        wq_t = jnp.concatenate([wqvt[0, c] for c in range(NG)], axis=1)
        q_t = jax.lax.dot_general(wq_t, xn[...], NT_DIMS, preferred_element_type=f32)
        for g in range(NG):
            qg = q_t[g * 128:(g + 1) * 128, :]
            qt[g] = (qg * QSCALE).astype(bf16)
            pqt[g] = _phi(qg).astype(bf16)
        k = _dot(xn[...], wk[...])
        pk = _phi(k)
        for g in range(NG):
            kb[g] = k[:, g * 128:(g + 1) * 128].astype(bf16)
            pkb[g] = pk[:, g * 128:(g + 1) * 128].astype(bf16)
        zsum = jnp.sum(pk, axis=0, keepdims=True)
        wv_t = jnp.concatenate([wqvt[1, c] for c in range(NG)], axis=1)
        v_t = jax.lax.dot_general(wv_t, xn[...], NT_DIMS, preferred_element_type=f32)
        for g in range(NG):
            vt[g] = v_t[g * 128:(g + 1) * 128, :].astype(bf16)

        for g in range(NG):
            mbd = jnp.where(rowh == colh, mt[g], 0.0)
            zg = jnp.broadcast_to(zrow[:, g * 128:(g + 1) * 128], (16, 128))
            zx = jnp.where(row16 == col16, zg, 0.0)
            lhs = jnp.concatenate([mbd, zx], axis=0).astype(bf16)
            ret = _dot(lhs, pqt[g])
            parts = []
            for h in range(4):
                gh = gate[g * 4 + h:g * 4 + h + 1, 0:1]
                den = ret[128 + h:129 + h, :] + 1e-6
                parts.append(ret[h * DH:(h + 1) * DH, :] * (gh / den))
            amem[g] = jnp.concatenate(parts, axis=0)
            mt[g] = mt[g] + _dot(vt[g], pkb[g])
        zrow[...] = zrow[...] + zsum

        attn_step(None, 0)
        for g in range(NG):
            attn_step(g, g + 1 if g + 1 < NG else None)

        @pl.when(jnp.logical_and(layer == 0, seg == 0))
        def _():
            cp_wo.wait()
            cp_w1.wait()

        o = jnp.concatenate([ob[g] for g in range(NG)], axis=1)
        xa = xres[rows, :] + _dot(o, wo[...])
        xres[rows, :] = xa
        y = _ln(xa)
        yres[rows, :] = y
        hh = _gelu(_dot(_ln(y).astype(bf16), w1[...]))
        hbuf[pl.ds(r0 + HALO, L), :] = hh

    def out_copy(blk, slot):
        return pltpu.make_async_copy(
            obuf.at[slot], out_hbm.at[0, pl.ds(blk * L, L), :], osems.at[slot])

    def phase_b(layer, blk):
        r0 = pl.multiple_of(blk * L, L)
        rows = pl.ds(r0, L)

        @pl.when(jnp.logical_and(layer == 0, blk == 0))
        def _():
            cp_w2.wait()
            for c in cp_w3:
                c.wait()
            cp_w4.wait()

        hw = hbuf.at[pl.ds(r0, L + 2 * HALO), :]
        c4 = D // 4
        hs = jnp.concatenate([
            hw[HALO - 1:HALO - 1 + L, 0 * c4:1 * c4],
            hw[HALO + 1:HALO + 1 + L, 1 * c4:2 * c4],
            hw[HALO - 2:HALO - 2 + L, 2 * c4:3 * c4],
            hw[HALO + 2:HALO + 2 + L, 3 * c4:4 * c4]], axis=1).astype(bf16)
        x1 = yres[rows, :] + _dot(hs, w2[...])
        acc[...] = xres[rows, :] + x1
        xn[...] = _ln(x1).astype(bf16)

        def ffn(c, _):
            ha = _dot(xn[...], w3[2 * c])
            hb = _dot(xn[...], w3[2 * c + 1])
            ra = pl.multiple_of(c * (2 * FC), 2 * FC)
            da = _dot(_gelu(ha).astype(bf16), w4[pl.ds(ra, FC), :])
            db = _dot(_gelu(hb).astype(bf16), w4[pl.ds(ra + FC, FC), :])
            acc[...] = acc[...] + da + db
            return 0
        jax.lax.fori_loop(0, F // (2 * FC), ffn, 0)

        @pl.when(layer == 0)
        def _():
            xres[rows, :] = acc[...]

        @pl.when(layer == 1)
        def _():
            slot = blk % 2

            @pl.when(blk >= 2)
            def _():
                out_copy(blk - 2, slot).wait()
            obuf[slot] = acc[...].astype(bf16)
            out_copy(blk, slot).start()

    def layer_body(layer, _):
        mt[...] = jnp.zeros(mt.shape, f32)
        zrow[...] = jnp.zeros(zrow.shape, f32)

        def a_body(seg, _):
            phase_a(layer, seg)
            return 0
        jax.lax.fori_loop(0, NSEG, a_body, 0)

        def b_body(blk, _):
            phase_b(layer, blk)
            return 0
        jax.lax.fori_loop(0, NSEG, b_body, 0)
        return 0
    jax.lax.fori_loop(0, 2, layer_body, 0)

    out_copy(NSEG - 2, 0).wait()
    out_copy(NSEG - 1, 1).wait()


@jax.jit
def pallas_interleave_layers__memory_aug_infini_attn__mixer_s_mlp__prompt_kernel(
    A_x: jax.Array,
    A_wq: jax.Array,
    A_wk: jax.Array,
    A_wv: jax.Array,
    A_wo: jax.Array,
    A_beta: jax.Array,
    B_x: jax.Array,
    B_w1: jax.Array,
    B_w2: jax.Array,
    B_w3: jax.Array,
    B_w4: jax.Array,
):
    del B_x
    hbm = pl.BlockSpec(memory_space=pl.ANY)
    vm = pltpu.VMEM
    scratch = [
        vm((S, D), bf16),
        vm((2, D, D), bf16),
        vm((2, NG, D, 128), bf16),
        vm((D, D), bf16),
        vm((D, D), bf16),
        vm((D, D), bf16),
        vm((D, D), bf16),
        vm((F // FC, D, FC), bf16),
        vm((F, D), bf16),
        vm((S, D), f32),
        vm((S, D), f32),
        vm((S + 2 * HALO, D), f32),
        vm((L, D), bf16),
        vm((NG, 128, L), bf16),
        vm((NG, 128, L), bf16),
        vm((NG, L, 128), bf16),
        vm((NG, L, 128), bf16),
        vm((NG, 128, L), bf16),
        vm((NG, L, 128), bf16),
        vm((NG, 128, L), f32),
        vm((NG, 128, 128), f32),
        vm((1, D), f32),
        vm((H, 128), f32),
        vm((128, 512), f32),
    ]
    scratch += [vm((2, 128 * (t + 1), 512), f32) for t in range(NT_TILES)]
    scratch += [vm((2, 1, 512), f32) for _ in range(NT_TILES)]
    scratch += [
        vm((L, D), f32),
        vm((2, L, D), bf16),
        pltpu.SemaphoreType.DMA((9,)),
        pltpu.SemaphoreType.DMA((2,)),
    ]
    return pl.pallas_call(
        _kernel,
        out_shape=jax.ShapeDtypeStruct((1, S, D), bf16),
        in_specs=[hbm, hbm, hbm, hbm, hbm, pl.BlockSpec(memory_space=pltpu.VMEM),
                  hbm, hbm, hbm, hbm],
        out_specs=hbm,
        scratch_shapes=scratch,
        compiler_params=pltpu.CompilerParams(vmem_limit_bytes=120 * 1024 * 1024),
    )(A_x, A_wq, A_wk, A_wv, A_wo, A_beta.reshape(1, H), B_w1, B_w2, B_w3, B_w4)
```

```python
import functools
import math

import jax
import jax.numpy as jnp
import jax.experimental.pallas as pl
import jax.experimental.pallas.tpu as pltpu

S = 2048
D = 1024
F = 3584
H = 32
DH = 32
L = 512
NSEG = S // L
NG = D // 128
NT_TILES = L // 128
FC = 256
HALO = 8
GH = NG // 2
DHALF = D // 2
TAIL_CHUNKS = (256, 256)
MIX_CHUNKS = (256, 256)

LOG2E = math.log2(math.e)
QSCALE = DH ** -0.5 * LOG2E
MASK_BIAS = -1e9 * LOG2E
EPS = 1e-5

f32 = jnp.float32
bf16 = jnp.bfloat16
NT_DIMS = (((1,), (1,)), ((), ()))


def _ln(x):
    m = jnp.mean(x, axis=-1, keepdims=True)
    xc = x - m
    v = jnp.mean(xc * xc, axis=-1, keepdims=True)
    return xc * jax.lax.rsqrt(v + EPS)


def _gelu(x):
    c = math.sqrt(2.0 / math.pi)
    inner = x * (c + (c * 0.044715) * (x * x))
    hx = 0.5 * x
    return hx + hx * jnp.tanh(inner)


def _phi(t):
    return jnp.where(t > 0, t + 1.0, jnp.exp(t))


def _red8(x, op):
    return functools.reduce(op, [x[i * 8:(i + 1) * 8] for i in range(x.shape[0] // 8)])


def _dot(a, b):
    return jnp.dot(a, b, preferred_element_type=f32)


def _dot_nt(a, b):
    return jax.lax.dot_general(a, b, NT_DIMS, preferred_element_type=f32)


def _kernel(x_hbm, wq_hbm, wk_hbm, wv_hbm, wo_hbm, beta_ref, w1_hbm, w2_hbm, w3_hbm, w4_hbm,
            out_hbm,
            xin, stage, wt, wk, wo, w1, w2, w3, w4,
            xres, yres, hbuf, xna, xnb, qt, pqt, kb, pkb, vt, ob, amem,
            mt, zrow, gate, bias,
            s0, s1, s2, s3, m0, m1, m2, m3,
            obuf, sems, tsems, osems):
    sbuf = (s0, s1, s2, s3)
    mbuf = (m0, m1, m2, m3)

    def seg_rows(s):
        return pl.ds(s * L, L)

    cp_x0 = pltpu.make_async_copy(x_hbm.at[0, seg_rows(0)], xin.at[seg_rows(0)], sems.at[0])
    cp_xr = pltpu.make_async_copy(x_hbm.at[0, pl.ds(L, S - L)], xin.at[pl.ds(L, S - L)], sems.at[1])
    cp_wk = [pltpu.make_async_copy(wk_hbm.at[:, pl.ds(i * DHALF, DHALF)], wk.at[i], sems.at[2 + i])
             for i in range(2)]
    cp_wo = [pltpu.make_async_copy(wo_hbm.at[pl.ds(i * DHALF, DHALF)], wo.at[i], sems.at[4 + i])
             for i in range(2)]
    cp_w1 = pltpu.make_async_copy(w1_hbm, w1, sems.at[6])
    cp_w2 = pltpu.make_async_copy(w2_hbm, w2, sems.at[7])
    cp_w3 = [pltpu.make_async_copy(w3_hbm.at[:, pl.ds(c * FC, FC)], w3.at[c], sems.at[8])
             for c in range(F // FC)]
    cp_w4 = pltpu.make_async_copy(w4_hbm, w4, sems.at[9])

    TC = 256
    NTC = D // TC

    def cp_stage(i, c):
        src = (wq_hbm, wv_hbm)[i]
        return pltpu.make_async_copy(src.at[pl.ds(c * TC, TC)], stage.at[i * NTC + c],
                                     tsems.at[i * NTC + c])

    cp_x0.start()
    for i in range(2):
        for c in range(NTC):
            cp_stage(i, c).start()
    cp_wk[0].start()
    cp_wo[0].start()

    kk = jax.lax.broadcasted_iota(jnp.int32, (128, 512), 0)
    qq = jax.lax.broadcasted_iota(jnp.int32, (128, 512), 1) % 128
    bias[...] = jnp.where(kk > qq, MASK_BIAS, 0.0).astype(f32)
    bt = jnp.broadcast_to(beta_ref[...].astype(f32), (H, H))
    eye = (jax.lax.broadcasted_iota(jnp.int32, (H, H), 0)
           == jax.lax.broadcasted_iota(jnp.int32, (H, H), 1))
    bcol = jnp.sum(jnp.where(eye, bt, 0.0), axis=1, keepdims=True)
    gsig = jnp.broadcast_to(jax.nn.sigmoid(bcol), (H, 128))
    gate[0] = gsig[0:H // 2]
    gate[1] = gsig[H // 2:H]
    hbuf[0:HALO, :] = jnp.zeros((HALO, D), f32)
    hbuf[S + HALO:S + 2 * HALO, :] = jnp.zeros((HALO, D), f32)

    cp_x0.wait()

    def init_x(i, _):
        r = pl.ds(pl.multiple_of(i * 128, 128), 128)
        xv = xin[r, :].astype(f32)
        xres[r, :] = xv
        xna[r, :] = _ln(xv).astype(bf16)
        return 0
    jax.lax.fori_loop(0, L // 128, init_x, 0)

    ident = (jax.lax.broadcasted_iota(jnp.int32, (128, 128), 0)
             == jax.lax.broadcasted_iota(jnp.int32, (128, 128), 1)).astype(f32).astype(bf16)

    def transpose_chunk(ic, _):
        pltpu.make_async_copy(stage.at[ic], stage.at[ic], tsems.at[ic]).wait()
        i = ic // NTC
        c = ic % NTC
        ro = pl.multiple_of(i * DHALF, DHALF)
        for n in range(D // 128):
            tile = _dot_nt(ident, stage[ic, :, n * 128:(n + 1) * 128]).astype(bf16)
            wt[n // 4, c, pl.ds(ro + (n % 4) * 128, 128), :] = tile
        return 0
    jax.lax.fori_loop(0, 2 * NTC, transpose_chunk, 0)

    cp_wk[1].start()
    cp_wo[1].start()
    cp_w1.start()
    cp_xr.start()
    cp_w2.start()
    for c in cp_w3:
        c.start()
    cp_w4.start()
    cp_wk[0].wait()
    cp_wo[0].wait()

    def qmask(g, t):
        z = jnp.zeros((DH, 128), bf16)
        cols = []
        for h in range(4):
            qh = qt[g, h * DH:(h + 1) * DH, t * 128:(t + 1) * 128]
            cols.append(jnp.concatenate([qh if i == h else z for i in range(4)], axis=0))
        return jnp.concatenate(cols, axis=1)

    def attn_step(half, g, gn):
        pr = None if g is None else g % 2
        pw = None if gn is None else gn % 2
        for t in range(NT_TILES):
            macc = None
            oacc = [None] * 4
            lacc = [None] * 4
            for j in range(t + 1):
                ks = slice(j * 128, (j + 1) * 128)
                if gn is not None:
                    s = _dot(kb[gn, ks, :], qmask(gn, t))
                    if j == t:
                        s = s + bias[...]
                    sbuf[t][pw, ks, :] = s
                    mx = _red8(s, jnp.maximum)
                    macc = mx if macc is None else jnp.maximum(macc, mx)
                if g is not None:
                    for h in range(4):
                        sl = slice(h * 128, (h + 1) * 128)
                        p = jnp.exp2(sbuf[t][pr, ks, sl] - mbuf[t][pr, :, sl])
                        lt = _red8(p, jnp.add)
                        lacc[h] = lt if lacc[h] is None else lacc[h] + lt
                        o = _dot(vt[g, h * DH:(h + 1) * DH, ks], p.astype(bf16))
                        oacc[h] = o if oacc[h] is None else oacc[h] + o
            if gn is not None:
                mbuf[t][pw] = jnp.max(macc, axis=0, keepdims=True)
            if g is not None:
                parts = []
                for h in range(4):
                    l = jnp.sum(lacc[h], axis=0, keepdims=True)
                    gh = gate[half, g * 4 + h:g * 4 + h + 1, :]
                    parts.append(oacc[h] * ((1.0 - gh) / l))
                ot = jnp.concatenate(parts, axis=0) + amem[g, :, t * 128:(t + 1) * 128]
                ob[g, t * 128:(t + 1) * 128, :] = ot.T.astype(bf16)

    rowh = jax.lax.broadcasted_iota(jnp.int32, (128, 128), 0) // DH
    colh = jax.lax.broadcasted_iota(jnp.int32, (128, 128), 1) // DH
    row16 = jax.lax.broadcasted_iota(jnp.int32, (16, 128), 0)
    col16 = jax.lax.broadcasted_iota(jnp.int32, (16, 128), 1) // DH

    def attn_half(layer, seg, half):
        rows = pl.ds(pl.multiple_of(seg * L, L), L)

        @pl.when(jnp.logical_and(jnp.logical_and(layer == 0, seg == 0), half == 1))
        def _():
            cp_wk[1].wait()
            cp_wo[1].wait()
            cp_w1.wait()
            cp_xr.wait()

        k = _dot(xna[...], wk[half])
        pk = _phi(k)
        for g in range(GH):
            kb[g] = k[:, g * 128:(g + 1) * 128].astype(bf16)
            pkb[g] = pk[:, g * 128:(g + 1) * 128].astype(bf16)
        zsum = jnp.sum(pk, axis=0, keepdims=True)
        w_t = jnp.concatenate([wt[half, c] for c in range(NTC)], axis=1)
        qv_t = _dot_nt(w_t, xna[...])
        for g in range(GH):
            qg = qv_t[g * 128:(g + 1) * 128, :]
            qt[g] = (qg * QSCALE).astype(bf16)
            pqt[g] = _phi(qg).astype(bf16)
            vt[g] = qv_t[DHALF + g * 128:DHALF + (g + 1) * 128, :].astype(bf16)

        zold = zrow[half]
        for g in range(GH):
            mold = mt[half, g]
            mbd = jnp.where(rowh == colh, mold, 0.0)
            zg = jnp.broadcast_to(zold[:, g * 128:(g + 1) * 128], (16, 128))
            zx = jnp.where(row16 == col16, zg, 0.0)
            lhs = jnp.concatenate([mbd, zx], axis=0).astype(bf16)
            ret = _dot(lhs, pqt[g])
            parts = []
            for h in range(4):
                gh = gate[half, g * 4 + h:g * 4 + h + 1, 0:1]
                den = ret[128 + h:129 + h, :] + 1e-6
                parts.append(ret[h * DH:(h + 1) * DH, :] * (gh / den))
            amem[g] = jnp.concatenate(parts, axis=0)
            mt[half, g] = mold + _dot(vt[g], pkb[g])
        zrow[half] = zold + zsum

        attn_step(half, None, 0)
        for g in range(GH - 1):
            attn_step(half, g, g + 1)
        o = jnp.concatenate([ob[g] for g in range(GH - 1)], axis=1)
        part = xres[rows, :] + _dot(o, wo[half, 0:(GH - 1) * 128, :])
        attn_step(half, GH - 1, None)
        xres[rows, :] = part + _dot(ob[GH - 1], wo[half, (GH - 1) * 128:GH * 128, :])

    def phase_a(layer, seg):
        r0 = pl.multiple_of(seg * L, L)

        def half_body(half, _):
            attn_half(layer, seg, half)
            return 0
        jax.lax.fori_loop(0, 2, half_body, 0)

        off = 0
        for n in TAIL_CHUNKS:
            rr = pl.ds(r0 + off, n)
            y = _ln(xres[rr, :])
            yres[rr, :] = y
            hh = _gelu(_dot(_ln(y).astype(bf16), w1[...]))
            hbuf[pl.ds(r0 + off + HALO, n), :] = hh
            off += n

        nxt = pl.ds(pl.multiple_of(jnp.minimum(seg + 1, NSEG - 1) * L, L), L)
        fresh = jnp.logical_and(layer == 0, seg < NSEG - 1)
        xv = jnp.where(fresh, xin[nxt, :].astype(f32), xres[nxt, :])
        xres[nxt, :] = xv
        xna[...] = _ln(xv).astype(bf16)

    def out_copy(blk, slot):
        return pltpu.make_async_copy(
            obuf.at[slot], out_hbm.at[0, pl.ds(blk * L, L), :], osems.at[slot])

    def phase_b(layer, blk):
        r0 = pl.multiple_of(blk * L, L)
        rows = pl.ds(r0, L)

        @pl.when(jnp.logical_and(layer == 0, blk == 0))
        def _():
            cp_w2.wait()
            for c in cp_w3:
                c.wait()
            cp_w4.wait()

        xna[...] = _ln(xres[0:L, :]).astype(bf16)

        hw = hbuf.at[pl.ds(r0, L + 2 * HALO), :]
        c4 = D // 4
        off = 0
        for n in MIX_CHUNKS:
            b = HALO + off
            hs = jnp.concatenate([
                hw[b - 1:b - 1 + n, 0 * c4:1 * c4],
                hw[b + 1:b + 1 + n, 1 * c4:2 * c4],
                hw[b - 2:b - 2 + n, 2 * c4:3 * c4],
                hw[b + 2:b + 2 + n, 3 * c4:4 * c4]], axis=1).astype(bf16)
            rr = pl.ds(r0 + off, n)
            x1 = yres[rr, :] + _dot(hs, w2[...])
            xres[rr, :] = xres[rr, :] + x1
            xnb[off:off + n, :] = _ln(x1).astype(bf16)
            off += n

        def ffn(c, _):
            ha = _dot(xnb[...], w3[2 * c])
            hb = _dot(xnb[...], w3[2 * c + 1])
            ra = pl.multiple_of(c * (2 * FC), 2 * FC)
            da = _dot(_gelu(ha).astype(bf16), w4[pl.ds(ra, FC), :])
            db = _dot(_gelu(hb).astype(bf16), w4[pl.ds(ra + FC, FC), :])
            xres[rows, :] = xres[rows, :] + da + db
            return 0
        jax.lax.fori_loop(0, F // (2 * FC), ffn, 0)

        @pl.when(layer == 1)
        def _():
            slot = blk % 2

            @pl.when(blk >= 2)
            def _():
                out_copy(blk - 2, slot).wait()
            obuf[slot] = xres[rows, :].astype(bf16)
            out_copy(blk, slot).start()

    def layer_body(layer, _):
        mt[...] = jnp.zeros(mt.shape, f32)
        zrow[...] = jnp.zeros(zrow.shape, f32)

        def a_body(seg, _):
            phase_a(layer, seg)
            return 0
        jax.lax.fori_loop(0, NSEG, a_body, 0)

        def b_body(blk, _):
            phase_b(layer, blk)
            return 0
        jax.lax.fori_loop(0, NSEG, b_body, 0)
        return 0
    jax.lax.fori_loop(0, 2, layer_body, 0)

    out_copy(NSEG - 2, 0).wait()
    out_copy(NSEG - 1, 1).wait()


@jax.jit
def pallas_interleave_layers__memory_aug_infini_attn__mixer_s_mlp__prompt_kernel(
    A_x: jax.Array,
    A_wq: jax.Array,
    A_wk: jax.Array,
    A_wv: jax.Array,
    A_wo: jax.Array,
    A_beta: jax.Array,
    B_x: jax.Array,
    B_w1: jax.Array,
    B_w2: jax.Array,
    B_w3: jax.Array,
    B_w4: jax.Array,
):
    del B_x
    hbm = pl.BlockSpec(memory_space=pl.ANY)
    vm = pltpu.VMEM
    scratch = [
        vm((S, D), bf16),
        vm((8, 256, D), bf16),
        vm((2, 4, D, 256), bf16),
        vm((2, D, DHALF), bf16),
        vm((2, DHALF, D), bf16),
        vm((D, D), bf16),
        vm((D, D), bf16),
        vm((F // FC, D, FC), bf16),
        vm((F, D), bf16),
        vm((S, D), f32),
        vm((S, D), f32),
        vm((S + 2 * HALO, D), f32),
        vm((L, D), bf16),
        vm((L, D), bf16),
        vm((GH, 128, L), bf16),
        vm((GH, 128, L), bf16),
        vm((GH, L, 128), bf16),
        vm((GH, L, 128), bf16),
        vm((GH, 128, L), bf16),
        vm((GH, L, 128), bf16),
        vm((GH, 128, L), f32),
        vm((2, GH, 128, 128), f32),
        vm((2, 1, DHALF), f32),
        vm((2, H // 2, 128), f32),
        vm((128, 512), f32),
    ]
    scratch += [vm((2, 128 * (t + 1), 512), f32) for t in range(NT_TILES)]
    scratch += [vm((2, 1, 512), f32) for _ in range(NT_TILES)]
    scratch += [
        vm((2, L, D), bf16),
        pltpu.SemaphoreType.DMA((10,)),
        pltpu.SemaphoreType.DMA((8,)),
        pltpu.SemaphoreType.DMA((2,)),
    ]
    return pl.pallas_call(
        _kernel,
        out_shape=jax.ShapeDtypeStruct((1, S, D), bf16),
        in_specs=[hbm, hbm, hbm, hbm, hbm, pl.BlockSpec(memory_space=pltpu.VMEM),
                  hbm, hbm, hbm, hbm],
        out_specs=hbm,
        scratch_shapes=scratch,
        compiler_params=pltpu.CompilerParams(vmem_limit_bytes=120 * 1024 * 1024),
    )(A_x, A_wq, A_wk, A_wv, A_wo, A_beta.reshape(1, H), B_w1, B_w2, B_w3, B_w4)
```

```python
import functools
import math

import jax
import jax.numpy as jnp
import jax.experimental.pallas as pl
import jax.experimental.pallas.tpu as pltpu

S = 2048
D = 1024
F = 3584
H = 32
DH = 32
L = 512
NSEG = S // L
NG = D // 128
NT_TILES = L // 128
FC = 256
HALO = 8
GH = NG // 2
DHALF = D // 2
XA = S
PIN = XA + L
BIG_ROWS = PIN + 8 * NSEG
SHIFTS = (1, -1, 2, -2)

LOG2E = math.log2(math.e)
QSCALE = DH ** -0.5 * LOG2E
MASK_BIAS = -1e9 * LOG2E
EPS = 1e-5

f32 = jnp.float32
bf16 = jnp.bfloat16
NT_DIMS = (((1,), (1,)), ((), ()))


def _ln(x):
    m = jnp.mean(x, axis=-1, keepdims=True)
    xc = x - m
    v = jnp.mean(xc * xc, axis=-1, keepdims=True)
    return xc * jax.lax.rsqrt(v + EPS)


def _gelu(x):
    c = math.sqrt(2.0 / math.pi)
    inner = x * (c + (c * 0.044715) * (x * x))
    hx = 0.5 * x
    return hx + hx * jnp.tanh(inner)


def _phi(t):
    return jnp.where(t > 0, t + 1.0, jnp.exp(t))


def _red8(x, op):
    return functools.reduce(op, [x[i * 8:(i + 1) * 8] for i in range(x.shape[0] // 8)])


def _dot(a, b):
    return jnp.dot(a, b, preferred_element_type=f32)


def _dot_nt(a, b):
    return jax.lax.dot_general(a, b, NT_DIMS, preferred_element_type=f32)


def _kernel(x_hbm, wq_hbm, wk_hbm, wv_hbm, wo_hbm, beta_ref, w1_hbm, w2_hbm, w3_hbm, w4_hbm,
            out_hbm,
            xin, stage, wt, wk, wo, w1, w2, w3, w4,
            big, yres, hbuf, xnb, gh, qt, pqt, kb, pkb, vt, ob, obl, amem,
            mt, zrow, gate, bias,
            s0, s1, s2, s3, m0, m1, m2, m3,
            obuf, sems, tsems, osems):
    sbuf = (s0, s1, s2, s3)
    mbuf = (m0, m1, m2, m3)

    def seg_rows(s):
        return pl.ds(s * L, L)

    cp_x0 = pltpu.make_async_copy(x_hbm.at[0, seg_rows(0)], xin.at[seg_rows(0)], sems.at[0])
    cp_xr = pltpu.make_async_copy(x_hbm.at[0, pl.ds(L, S - L)], xin.at[pl.ds(L, S - L)], sems.at[1])
    cp_wk = [pltpu.make_async_copy(wk_hbm.at[:, pl.ds(i * DHALF, DHALF)], wk.at[i], sems.at[2 + i])
             for i in range(2)]
    cp_wo = [pltpu.make_async_copy(wo_hbm.at[pl.ds(i * DHALF, DHALF)], wo.at[i], sems.at[4 + i])
             for i in range(2)]
    cp_w1 = pltpu.make_async_copy(w1_hbm, w1, sems.at[6])
    cp_w2 = pltpu.make_async_copy(w2_hbm, w2, sems.at[7])
    cp_w3 = [pltpu.make_async_copy(w3_hbm.at[:, pl.ds(c * FC, FC)], w3.at[c], sems.at[8])
             for c in range(F // FC)]
    cp_w4 = pltpu.make_async_copy(w4_hbm, w4, sems.at[9])

    TC = 256
    NTC = D // TC

    def cp_stage(i, c):
        src = (wq_hbm, wv_hbm)[i]
        return pltpu.make_async_copy(src.at[pl.ds(c * TC, TC)], stage.at[i * NTC + c],
                                     tsems.at[i * NTC + c])

    cp_x0.start()
    for i in range(2):
        for c in range(NTC):
            cp_stage(i, c).start()
    cp_wk[0].start()
    cp_wo[0].start()

    kk = jax.lax.broadcasted_iota(jnp.int32, (128, 512), 0)
    qq = jax.lax.broadcasted_iota(jnp.int32, (128, 512), 1) % 128
    bias[...] = jnp.where(kk > qq, MASK_BIAS, 0.0).astype(f32)
    bt = jnp.broadcast_to(beta_ref[...].astype(f32), (H, H))
    eye = (jax.lax.broadcasted_iota(jnp.int32, (H, H), 0)
           == jax.lax.broadcasted_iota(jnp.int32, (H, H), 1))
    bcol = jnp.sum(jnp.where(eye, bt, 0.0), axis=1, keepdims=True)
    gsig = jnp.broadcast_to(jax.nn.sigmoid(bcol), (H, 128))
    gate[0] = gsig[0:H // 2]
    gate[1] = gsig[H // 2:H]
    hbuf[HALO:2 * HALO, :] = jnp.zeros((HALO, D), f32)
    hbuf[S:S + HALO, :] = jnp.zeros((HALO, D), f32)

    ident = (jax.lax.broadcasted_iota(jnp.int32, (128, 128), 0)
             == jax.lax.broadcasted_iota(jnp.int32, (128, 128), 1)).astype(f32).astype(bf16)

    def transpose_chunk(ic, _):
        pltpu.make_async_copy(stage.at[ic], stage.at[ic], tsems.at[ic]).wait()
        i = ic // NTC
        c = ic % NTC
        ro = pl.multiple_of(i * DHALF, DHALF)
        for n in range(D // 128):
            tile = _dot_nt(ident, stage[ic, :, n * 128:(n + 1) * 128]).astype(bf16)
            wt[n // 4, c, pl.ds(ro + (n % 4) * 128, 128), :] = tile
        return 0
    jax.lax.fori_loop(0, 2 * NTC, transpose_chunk, 0)

    cp_wk[1].start()
    cp_wo[1].start()
    cp_w1.start()
    cp_xr.start()
    cp_w2.start()
    for c in cp_w3:
        c.start()
    cp_w4.start()
    cp_x0.wait()
    cp_wk[0].wait()
    cp_wo[0].wait()

    def qmask(g, t):
        z = jnp.zeros((DH, 128), bf16)
        cols = []
        for h in range(4):
            qh = qt[g, h * DH:(h + 1) * DH, t * 128:(t + 1) * 128]
            cols.append(jnp.concatenate([qh if i == h else z for i in range(4)], axis=0))
        return jnp.concatenate(cols, axis=1)

    def attn_step(half, g, gn, fill=()):
        pr = None if g is None else g % 2
        pw = None if gn is None else gn % 2
        fill = list(fill)
        for t in range(NT_TILES):
            macc = None
            oacc = [None] * 4
            lacc = [None] * 4
            for j in range(t + 1):
                ks = slice(j * 128, (j + 1) * 128)
                if fill and (t, j) != (0, 0):
                    fill.pop(0)()
                if gn is not None:
                    s = _dot(kb[gn, ks, :], qmask(gn, t))
                    if j == t:
                        s = s + bias[...]
                    sbuf[t][pw, ks, :] = s
                    mx = _red8(s, jnp.maximum)
                    macc = mx if macc is None else jnp.maximum(macc, mx)
                if g is not None:
                    for h in range(4):
                        sl = slice(h * 128, (h + 1) * 128)
                        p = jnp.exp2(sbuf[t][pr, ks, sl] - mbuf[t][pr, :, sl])
                        lt = _red8(p, jnp.add)
                        lacc[h] = lt if lacc[h] is None else lacc[h] + lt
                        o = _dot(vt[g, h * DH:(h + 1) * DH, ks], p.astype(bf16))
                        oacc[h] = o if oacc[h] is None else oacc[h] + o
            if gn is not None:
                mbuf[t][pw] = jnp.max(macc, axis=0, keepdims=True)
            if g is not None:
                parts = []
                for h in range(4):
                    l = jnp.sum(lacc[h], axis=0, keepdims=True)
                    gh = gate[half, g * 4 + h:g * 4 + h + 1, :]
                    parts.append(oacc[h] * ((1.0 - gh) / l))
                ot = jnp.concatenate(parts, axis=0) + amem[g, :, t * 128:(t + 1) * 128]
                if g < GH - 1:
                    ob[g, t * 128:(t + 1) * 128, :] = ot.T.astype(bf16)
                else:
                    obl[half, t * 128:(t + 1) * 128, :] = ot.T.astype(bf16)

    rowh = jax.lax.broadcasted_iota(jnp.int32, (128, 128), 0) // DH
    colh = jax.lax.broadcasted_iota(jnp.int32, (128, 128), 1) // DH
    row16 = jax.lax.broadcasted_iota(jnp.int32, (16, 128), 0)
    col16 = jax.lax.broadcasted_iota(jnp.int32, (16, 128), 1) // DH

    def attn_half(layer, seg, half):
        r0 = pl.multiple_of(seg * L, L)

        @pl.when(jnp.logical_and(jnp.logical_and(layer == 0, seg == 0), half == 1))
        def _():
            cp_wk[1].wait()
            cp_wo[1].wait()
            cp_w1.wait()
            cp_xr.wait()

        xn = big[XA:XA + L, :].astype(bf16)
        k = _dot(xn, wk[half])
        pk = _phi(k)
        for g in range(GH):
            kb[g] = k[:, g * 128:(g + 1) * 128].astype(bf16)
            pkb[g] = pk[:, g * 128:(g + 1) * 128].astype(bf16)
        zsum = jnp.sum(pk, axis=0, keepdims=True)
        w_t = jnp.concatenate([wt[half, c] for c in range(NTC)], axis=1)
        qv_t = _dot_nt(w_t, xn)
        for g in range(GH):
            qg = qv_t[g * 128:(g + 1) * 128, :]
            qt[g] = (qg * QSCALE).astype(bf16)
            pqt[g] = _phi(qg).astype(bf16)
            vt[g] = qv_t[DHALF + g * 128:DHALF + (g + 1) * 128, :].astype(bf16)

        zold = zrow[half]
        for g in range(GH):
            mold = mt[half, g]
            mbd = jnp.where(rowh == colh, mold, 0.0)
            zg = jnp.broadcast_to(zold[:, g * 128:(g + 1) * 128], (16, 128))
            zx = jnp.where(row16 == col16, zg, 0.0)
            lhs = jnp.concatenate([mbd, zx], axis=0).astype(bf16)
            ret = _dot(lhs, pqt[g])
            parts = []
            for h in range(4):
                gh = gate[half, g * 4 + h:g * 4 + h + 1, 0:1]
                den = ret[128 + h:129 + h, :] + 1e-6
                parts.append(ret[h * DH:(h + 1) * DH, :] * (gh / den))
            amem[g] = jnp.concatenate(parts, axis=0)
            mt[half, g] = mold + _dot(vt[g], pkb[g])
        zrow[half] = zold + zsum

        attn_step(half, None, 0)
        for g in range(GH - 1):
            attn_step(half, g, g + 1)
        kp = (GH - 1) * 128

        def wo_piece(i):
            off = (i // 2) * 128
            cs = slice((i % 2) * DHALF, (i % 2 + 1) * DHALF)
            rr = pl.ds(r0 + off, 128)
            o = jnp.concatenate([ob[g, off:off + 128, :] for g in range(GH - 1)], axis=1)
            big[rr, cs] = big[rr, cs] + _dot(o, wo[half, 0:kp, cs])

        attn_step(half, GH - 1, None, fill=[functools.partial(wo_piece, i) for i in range(8)])

    def phase_a(layer, seg):
        r0 = pl.multiple_of(seg * L, L)

        def half_body(half, _):
            attn_half(layer, seg, half)
            return 0
        jax.lax.fori_loop(0, 2, half_body, 0)

        hl = L // 2
        kp = (GH - 1) * 128

        def wo_rest(off, n):
            rr = pl.ds(r0 + off, n)
            o = jnp.concatenate([obl[0, off:off + n, :], obl[1, off:off + n, :]], axis=1)
            w = jnp.concatenate([wo[0, kp:DHALF, :], wo[1, kp:DHALF, :]], axis=0)
            big[rr, :] = big[rr, :] + _dot(o, w)

        def lnln(off, n):
            y = _ln(big[pl.ds(r0 + off, n), :])
            yres[pl.ds(r0 + off, n), :] = y
            xnb[off:off + n, :] = _ln(y).astype(bf16)

        def up(off, n):
            cs = slice(n * 256, (n + 1) * 256)
            hh = _gelu(_dot(xnb[off:off + hl, :], w1[:, cs]))
            win = hbuf.at[pl.ds(r0 + off, hl + 2 * HALO), :]
            b = HALO + SHIFTS[n]
            win[b:b + hl, cs] = hh
            big[pl.ds(PIN + pl.multiple_of(seg * 8, 8), 8), 0:128] = hh[hl - 8:hl, 128:256]

        n0 = pl.multiple_of(jnp.minimum(seg + 1, NSEG - 1) * L, L)
        fresh = jnp.logical_and(layer == 0, seg < NSEG - 1)

        def ln_next(off, n):
            rr = pl.ds(n0 + off, n)
            xv = jnp.where(fresh, xin[pl.ds(n0 + off, n), :].astype(f32), big[rr, :])
            big[rr, :] = xv
            big[XA + off:XA + off + n, :] = _ln(xv)

        wo_rest(0, 128)
        lnln(0, 128)
        wo_rest(128, 128)
        lnln(128, 128)
        wo_rest(hl, hl)
        for n in range(4):
            lnln(hl + n * 64, 64)
            up(0, n)
        for n in range(4):
            ln_next(n * 128, 128)
            up(hl, n)

    def out_copy(blk, slot):
        return pltpu.make_async_copy(
            obuf.at[slot], out_hbm.at[0, pl.ds(blk * L, L), :], osems.at[slot])

    def phase_b(layer, blk):
        r0 = pl.multiple_of(blk * L, L)
        rows = pl.ds(r0, L)

        @pl.when(jnp.logical_and(layer == 0, blk == 0))
        def _():
            cp_w2.wait()
            for c in cp_w3:
                c.wait()
            cp_w4.wait()

        hl = L // 2

        def mix(off, cs):
            hs = hbuf[pl.ds(HALO + r0 + off, hl), :].astype(bf16)
            rr = pl.ds(r0 + off, hl)
            x1 = yres[rr, cs] + _dot(hs, w2[:, cs])
            yres[rr, cs] = x1
            big[rr, cs] = big[rr, cs] + x1

        def ln_mid(off, n):
            xnb[off:off + n, :] = _ln(yres[pl.ds(r0 + off, n), :]).astype(bf16)

        def ffn_up(c, slot, off=0, n=L):
            gh[slot, off:off + n, :] = _gelu(_dot(xnb[off:off + n, :], w3[c])).astype(bf16)

        def ffn_down(c, slot, cs=slice(0, D)):
            w = w4[pl.ds(pl.multiple_of(c * FC, FC), FC), cs]
            big[rows, cs] = big[rows, cs] + _dot(gh[slot], w)

        mix(0, slice(0, D))
        for n in range(4):
            ln_mid(n * 64, 64)
            mix(hl, slice(n * 256, (n + 1) * 256))
        ln_mid(hl, hl)
        ffn_up(0, 0, 0, hl)
        ffn_up(0, 0, hl, hl)

        def ffn(i, _):
            ffn_up(2 * i + 1, 1)
            ffn_down(2 * i, 0)
            ffn_up(2 * i + 2, 0)
            ffn_down(2 * i + 1, 1)
            return 0
        nc = F // FC
        jax.lax.fori_loop(0, nc // 2 - 1, ffn, 0)
        ffn_up(nc - 1, 1)
        ffn_down(nc - 2, 0)
        ffn_down(nc - 1, 1)

        @pl.when(layer == 1)
        def _():
            slot = blk % 2

            @pl.when(blk >= 2)
            def _():
                out_copy(blk - 2, slot).wait()
            obuf[slot] = big[rows, :].astype(bf16)
            out_copy(blk, slot).start()

    def layer_body(layer, _):
        mt[...] = jnp.zeros(mt.shape, f32)
        zrow[...] = jnp.zeros(zrow.shape, f32)

        def init_x(i, _):
            r = pl.multiple_of(i * 256, 256)
            xv = jnp.where(layer == 0, xin[pl.ds(r, 256), :].astype(f32), big[pl.ds(r, 256), :])
            big[pl.ds(r, 256), :] = xv
            big[pl.ds(XA + r, 256), :] = _ln(xv)
            return 0
        jax.lax.fori_loop(0, L // 256, init_x, 0)

        def a_body(seg, _):
            phase_a(layer, seg)
            return 0
        jax.lax.fori_loop(0, NSEG, a_body, 0)

        def b_body(blk, _):
            phase_b(layer, blk)
            return 0
        jax.lax.fori_loop(0, NSEG, b_body, 0)
        return 0
    jax.lax.fori_loop(0, 2, layer_body, 0)

    out_copy(NSEG - 2, 0).wait()
    out_copy(NSEG - 1, 1).wait()


@jax.jit
def pallas_interleave_layers__memory_aug_infini_attn__mixer_s_mlp__prompt_kernel(
    A_x: jax.Array,
    A_wq: jax.Array,
    A_wk: jax.Array,
    A_wv: jax.Array,
    A_wo: jax.Array,
    A_beta: jax.Array,
    B_x: jax.Array,
    B_w1: jax.Array,
    B_w2: jax.Array,
    B_w3: jax.Array,
    B_w4: jax.Array,
):
    del B_x
    hbm = pl.BlockSpec(memory_space=pl.ANY)
    vm = pltpu.VMEM
    scratch = [
        vm((S, D), bf16),
        vm((8, 256, D), bf16),
        vm((2, 4, D, 256), bf16),
        vm((2, D, DHALF), bf16),
        vm((2, DHALF, D), bf16),
        vm((D, D), bf16),
        vm((D, D), bf16),
        vm((F // FC, D, FC), bf16),
        vm((F, D), bf16),
        vm((BIG_ROWS, D), f32),
        vm((S, D), f32),
        vm((S + 2 * HALO, D), f32),
        vm((L, D), bf16),
        vm((2, L, FC), bf16),
        vm((GH, 128, L), bf16),
        vm((GH, 128, L), bf16),
        vm((GH, L, 128), bf16),
        vm((GH, L, 128), bf16),
        vm((GH, 128, L), bf16),
        vm((GH - 1, L, 128), bf16),
        vm((2, L, 128), bf16),
        vm((GH, 128, L), f32),
        vm((2, GH, 128, 128), f32),
        vm((2, 1, DHALF), f32),
        vm((2, H // 2, 128), f32),
        vm((128, 512), f32),
    ]
    scratch += [vm((2, 128 * (t + 1), 512), f32) for t in range(NT_TILES)]
    scratch += [vm((2, 1, 512), f32) for _ in range(NT_TILES)]
    scratch += [
        vm((2, L, D), bf16),
        pltpu.SemaphoreType.DMA((10,)),
        pltpu.SemaphoreType.DMA((8,)),
        pltpu.SemaphoreType.DMA((2,)),
    ]
    return pl.pallas_call(
        _kernel,
        out_shape=jax.ShapeDtypeStruct((1, S, D), bf16),
        in_specs=[hbm, hbm, hbm, hbm, hbm, pl.BlockSpec(memory_space=pltpu.VMEM),
                  hbm, hbm, hbm, hbm],
        out_specs=hbm,
        scratch_shapes=scratch,
        compiler_params=pltpu.CompilerParams(vmem_limit_bytes=120 * 1024 * 1024),
    )(A_x, A_wq, A_wk, A_wv, A_wo, A_beta.reshape(1, H), B_w1, B_w2, B_w3, B_w4)
```

```python
import functools
import math

import jax
import jax.numpy as jnp
import jax.experimental.pallas as pl
import jax.experimental.pallas.tpu as pltpu

S = 2048
D = 1024
F = 3584
H = 32
DH = 32
L = 512
NSEG = S // L
NG = D // 128
NT_TILES = L // 128
FC = 256
HALO = 8
GH = NG // 2
DHALF = D // 2
PIN = S
BIG_ROWS = PIN + 8 * NSEG
SHIFTS = (1, -1, 2, -2)

LOG2E = math.log2(math.e)
QSCALE = DH ** -0.5 * LOG2E
MASK_BIAS = -1e9 * LOG2E
EPS = 1e-5

f32 = jnp.float32
bf16 = jnp.bfloat16
NT_DIMS = (((1,), (1,)), ((), ()))


def _stats(x):
    m = jnp.mean(x, axis=-1, keepdims=True)
    xc = x - m
    return m, jnp.mean(xc * xc, axis=-1, keepdims=True)


def _ln(x):
    m, v = _stats(x)
    r = jax.lax.rsqrt(v + EPS)
    return x * r - m * r


def _ln_ln(x):
    m, v = _stats(x)
    r1 = jax.lax.rsqrt(v + EPS)
    y = x * r1 - m * r1
    return y, y * jax.lax.rsqrt(v * r1 * r1 + EPS)


def _gelu(x):
    c = math.sqrt(2.0 / math.pi)
    inner = x * (c + (c * 0.044715) * (x * x))
    hx = 0.5 * x
    return hx + hx * jnp.tanh(inner)


def _phi(t):
    return jnp.where(t > 0, t + 1.0, jnp.exp(t))


def _red8(x, op):
    return functools.reduce(op, [x[i * 8:(i + 1) * 8] for i in range(x.shape[0] // 8)])


def _dot(a, b):
    return jnp.dot(a, b, preferred_element_type=f32)


def _dot_nt(a, b):
    return jax.lax.dot_general(a, b, NT_DIMS, preferred_element_type=f32)


def _kernel(x_hbm, wq_hbm, wk_hbm, wv_hbm, wo_hbm, beta_ref, w1_hbm, w2_hbm, w3_hbm, w4_hbm,
            out_hbm,
            xin, stage, wt, wk, wo, w1, w2, w3, w4,
            big, yres, hbuf, xna, xnb, gh, qt, pqt, kb, pkb, vt, ob, obl, amem,
            mt, zrow, gate, bias,
            s0, s1, s2, s3, m0, m1, m2, m3,
            obuf, sems, tsems, osems):
    sbuf = (s0, s1, s2, s3)
    mbuf = (m0, m1, m2, m3)

    def seg_rows(s):
        return pl.ds(s * L, L)

    cp_x0 = pltpu.make_async_copy(x_hbm.at[0, seg_rows(0)], xin.at[seg_rows(0)], sems.at[0])
    cp_xr = pltpu.make_async_copy(x_hbm.at[0, pl.ds(L, S - L)], xin.at[pl.ds(L, S - L)], sems.at[1])
    cp_wk = [pltpu.make_async_copy(wk_hbm.at[:, pl.ds(i * DHALF, DHALF)], wk.at[i], sems.at[2 + i])
             for i in range(2)]
    cp_wo = [pltpu.make_async_copy(wo_hbm.at[pl.ds(i * DHALF, DHALF)], wo.at[i], sems.at[4 + i])
             for i in range(2)]
    cp_w1 = pltpu.make_async_copy(w1_hbm, w1, sems.at[6])
    cp_w2 = pltpu.make_async_copy(w2_hbm, w2, sems.at[7])
    cp_w3 = [pltpu.make_async_copy(w3_hbm.at[:, pl.ds(c * FC, FC)], w3.at[c], sems.at[8])
             for c in range(F // FC)]
    cp_w4 = pltpu.make_async_copy(w4_hbm, w4, sems.at[9])

    TC = 256
    NTC = D // TC

    def cp_stage(i, c):
        src = (wq_hbm, wv_hbm)[i]
        return pltpu.make_async_copy(src.at[pl.ds(c * TC, TC)], stage.at[i * NTC + c],
                                     tsems.at[i * NTC + c])

    cp_x0.start()
    for i in range(2):
        for c in range(NTC):
            cp_stage(i, c).start()
    cp_wk[0].start()
    cp_wo[0].start()

    kk = jax.lax.broadcasted_iota(jnp.int32, (128, 512), 0)
    qq = jax.lax.broadcasted_iota(jnp.int32, (128, 512), 1) % 128
    bias[...] = jnp.where(kk > qq, MASK_BIAS, 0.0).astype(f32)
    bt = jnp.broadcast_to(beta_ref[...].astype(f32), (H, H))
    eye = (jax.lax.broadcasted_iota(jnp.int32, (H, H), 0)
           == jax.lax.broadcasted_iota(jnp.int32, (H, H), 1))
    bcol = jnp.sum(jnp.where(eye, bt, 0.0), axis=1, keepdims=True)
    gsig = jnp.broadcast_to(jax.nn.sigmoid(bcol), (H, 128))
    gate[0] = gsig[0:H // 2]
    gate[1] = gsig[H // 2:H]
    hbuf[HALO:2 * HALO, :] = jnp.zeros((HALO, D), f32)
    hbuf[S:S + HALO, :] = jnp.zeros((HALO, D), f32)

    ident = (jax.lax.broadcasted_iota(jnp.int32, (128, 128), 0)
             == jax.lax.broadcasted_iota(jnp.int32, (128, 128), 1)).astype(f32).astype(bf16)

    def transpose_chunk(ic, _):
        pltpu.make_async_copy(stage.at[ic], stage.at[ic], tsems.at[ic]).wait()
        i = ic // NTC
        c = ic % NTC
        ro = pl.multiple_of(i * DHALF, DHALF)
        for n in range(D // 128):
            tile = _dot_nt(ident, stage[ic, :, n * 128:(n + 1) * 128]).astype(bf16)
            wt[n // 4, c, pl.ds(ro + (n % 4) * 128, 128), :] = tile
        return 0
    jax.lax.fori_loop(0, 2 * NTC, transpose_chunk, 0)

    cp_wk[1].start()
    cp_wo[1].start()
    cp_w1.start()
    cp_xr.start()
    cp_w2.start()
    for c in cp_w3:
        c.start()
    cp_w4.start()
    cp_x0.wait()
    cp_wk[0].wait()
    cp_wo[0].wait()

    def qmask(g, t):
        z = jnp.zeros((DH, 128), bf16)
        cols = []
        for h in range(4):
            qh = qt[g, h * DH:(h + 1) * DH, t * 128:(t + 1) * 128]
            cols.append(jnp.concatenate([qh if i == h else z for i in range(4)], axis=0))
        return jnp.concatenate(cols, axis=1)

    def attn_step(half, g, gn, fill=()):
        pr = None if g is None else g % 2
        pw = None if gn is None else gn % 2
        fill = list(fill)
        for t in range(NT_TILES):
            macc = None
            oacc = [None] * 4
            lacc = [None] * 4
            for j in range(t + 1):
                ks = slice(j * 128, (j + 1) * 128)
                if fill and (t, j) != (0, 0):
                    fill.pop(0)()
                if gn is not None:
                    s = _dot(kb[gn, ks, :], qmask(gn, t))
                    if j == t:
                        s = s + bias[...]
                    sbuf[t][pw, ks, :] = s
                    mx = _red8(s, jnp.maximum)
                    macc = mx if macc is None else jnp.maximum(macc, mx)
                if g is not None:
                    for h in range(4):
                        sl = slice(h * 128, (h + 1) * 128)
                        p = jnp.exp2(sbuf[t][pr, ks, sl] - mbuf[t][pr, :, sl])
                        lt = _red8(p, jnp.add)
                        lacc[h] = lt if lacc[h] is None else lacc[h] + lt
                        o = _dot(vt[g, h * DH:(h + 1) * DH, ks], p.astype(bf16))
                        oacc[h] = o if oacc[h] is None else oacc[h] + o
            if gn is not None:
                mbuf[t][pw] = jnp.max(macc, axis=0, keepdims=True)
            if g is not None:
                parts = []
                for h in range(4):
                    l = jnp.sum(lacc[h], axis=0, keepdims=True)
                    gh = gate[half, g * 4 + h:g * 4 + h + 1, :]
                    parts.append(oacc[h] * ((1.0 - gh) / l))
                ot = jnp.concatenate(parts, axis=0) + amem[g, :, t * 128:(t + 1) * 128]
                if g < GH - 1:
                    ob[g, t * 128:(t + 1) * 128, :] = ot.T.astype(bf16)
                else:
                    obl[half, t * 128:(t + 1) * 128, :] = ot.T.astype(bf16)

    rowh = jax.lax.broadcasted_iota(jnp.int32, (128, 128), 0) // DH
    colh = jax.lax.broadcasted_iota(jnp.int32, (128, 128), 1) // DH
    row16 = jax.lax.broadcasted_iota(jnp.int32, (16, 128), 0)
    col16 = jax.lax.broadcasted_iota(jnp.int32, (16, 128), 1) // DH

    def attn_half(layer, seg, half):
        r0 = pl.multiple_of(seg * L, L)

        @pl.when(jnp.logical_and(jnp.logical_and(layer == 0, seg == 0), half == 1))
        def _():
            cp_wk[1].wait()
            cp_wo[1].wait()
            cp_w1.wait()
            cp_xr.wait()

        xn = xna[...].astype(bf16)
        k = _dot(xn, wk[half])
        pk = _phi(k)
        for g in range(GH):
            kb[g] = k[:, g * 128:(g + 1) * 128].astype(bf16)
            pkb[g] = pk[:, g * 128:(g + 1) * 128].astype(bf16)
        zsum = jnp.sum(pk, axis=0, keepdims=True)
        w_t = jnp.concatenate([wt[half, c] for c in range(NTC)], axis=1)
        qv_t = _dot_nt(w_t, xn)
        for g in range(GH):
            qg = qv_t[g * 128:(g + 1) * 128, :]
            qt[g] = (qg * QSCALE).astype(bf16)
            pqt[g] = _phi(qg).astype(bf16)
            vt[g] = qv_t[DHALF + g * 128:DHALF + (g + 1) * 128, :].astype(bf16)

        zold = zrow[half]
        for g in range(GH):
            mold = mt[half, g]
            mbd = jnp.where(rowh == colh, mold, 0.0)
            zg = jnp.broadcast_to(zold[:, g * 128:(g + 1) * 128], (16, 128))
            zx = jnp.where(row16 == col16, zg, 0.0)
            lhs = jnp.concatenate([mbd, zx], axis=0).astype(bf16)
            ret = _dot(lhs, pqt[g])
            parts = []
            for h in range(4):
                gh = gate[half, g * 4 + h:g * 4 + h + 1, 0:1]
                den = ret[128 + h:129 + h, :] + 1e-6
                parts.append(ret[h * DH:(h + 1) * DH, :] * (gh / den))
            amem[g] = jnp.concatenate(parts, axis=0)
            mt[half, g] = mold + _dot(vt[g], pkb[g])
        zrow[half] = zold + zsum

        attn_step(half, None, 0)
        for g in range(GH - 1):
            attn_step(half, g, g + 1)
        kp = (GH - 1) * 128

        def wo_piece(i):
            off = (i // 2) * 128
            cs = slice((i % 2) * DHALF, (i % 2 + 1) * DHALF)
            rr = pl.ds(r0 + off, 128)
            o = jnp.concatenate([ob[g, off:off + 128, :] for g in range(GH - 1)], axis=1)
            big[rr, cs] = big[rr, cs] + _dot(o, wo[half, 0:kp, cs])

        attn_step(half, GH - 1, None, fill=[functools.partial(wo_piece, i) for i in range(8)])

    def phase_a(layer, seg):
        r0 = pl.multiple_of(seg * L, L)

        def half_body(half, _):
            attn_half(layer, seg, half)
            return 0
        jax.lax.fori_loop(0, 2, half_body, 0)

        hl = L // 2
        kp = (GH - 1) * 128

        def wo_rest(off, n):
            rr = pl.ds(r0 + off, n)
            o = jnp.concatenate([obl[0, off:off + n, :], obl[1, off:off + n, :]], axis=1)
            w = jnp.concatenate([wo[0, kp:DHALF, :], wo[1, kp:DHALF, :]], axis=0)
            big[rr, :] = big[rr, :] + _dot(o, w)

        def lnln(off, n):
            y, z = _ln_ln(big[pl.ds(r0 + off, n), :])
            yres[pl.ds(r0 + off, n), :] = y
            xnb[off:off + n, :] = z.astype(bf16)

        def up(off, n):
            cs = slice(n * 256, (n + 1) * 256)
            hh = _gelu(_dot(xnb[off:off + hl, :], w1[:, cs]))
            win = hbuf.at[pl.ds(r0 + off, hl + 2 * HALO), :]
            b = HALO + SHIFTS[n]
            win[b:b + hl, cs] = hh
            return [hh[0:8, 0:128], hh[hl - 8:hl, 0:128], hh[0:8, 128:256], hh[hl - 8:hl, 128:256]]

        def pin(v):
            big[pl.ds(PIN + pl.multiple_of(seg * 8, 8), 8), 0:128] = v

        n0 = pl.multiple_of(jnp.minimum(seg + 1, NSEG - 1) * L, L)
        fresh = jnp.logical_and(layer == 0, seg < NSEG - 1)

        def ln_next(off, n):
            rr = pl.ds(n0 + off, n)
            xv = jnp.where(fresh, xin[pl.ds(n0 + off, n), :].astype(f32), big[rr, :])
            big[rr, :] = xv
            xna[off:off + n, :] = _ln(xv)

        wo_rest(0, 128)
        lnln(0, 128)
        wo_rest(128, 128)
        lnln(128, 128)
        wo_rest(hl, hl)
        for n in range(4):
            marks = up(0, n)
            for i in range(4):
                lnln(hl + n * 64 + i * 16, 16)
                pin(marks[i])
        for n in range(4):
            marks = up(hl, n)
            for i in range(4):
                ln_next(n * 128 + i * 32, 32)
                pin(marks[i])

    def out_copy(blk, slot):
        return pltpu.make_async_copy(
            obuf.at[slot], out_hbm.at[0, pl.ds(blk * L, L), :], osems.at[slot])

    def phase_b(layer, blk):
        r0 = pl.multiple_of(blk * L, L)
        rows = pl.ds(r0, L)

        @pl.when(jnp.logical_and(layer == 0, blk == 0))
        def _():
            cp_w2.wait()
            for c in cp_w3:
                c.wait()
            cp_w4.wait()

        hl = L // 2

        def mix(off, cs):
            hs = hbuf[pl.ds(HALO + r0 + off, hl), :].astype(bf16)
            rr = pl.ds(r0 + off, hl)
            x1 = yres[rr, cs] + _dot(hs, w2[:, cs])
            yres[rr, cs] = x1
            big[rr, cs] = big[rr, cs] + x1

        def ln_mid(off, n):
            xnb[off:off + n, :] = _ln(yres[pl.ds(r0 + off, n), :]).astype(bf16)

        def ffn_up(c, slot, off=0, n=L):
            gh[slot, off:off + n, :] = _gelu(_dot(xnb[off:off + n, :], w3[c])).astype(bf16)

        def ffn_down(c, slot, cs=slice(0, D)):
            w = w4[pl.ds(pl.multiple_of(c * FC, FC), FC), cs]
            big[rows, cs] = big[rows, cs] + _dot(gh[slot], w)

        mix(0, slice(0, D))
        for n in range(4):
            ln_mid(n * 64, 64)
            mix(hl, slice(n * 256, (n + 1) * 256))
        ln_mid(hl, hl)
        ffn_up(0, 0, 0, hl)
        ffn_up(0, 0, hl, hl)

        def ffn(i, _):
            ffn_up(2 * i + 1, 1)
            ffn_down(2 * i, 0)
            ffn_up(2 * i + 2, 0)
            ffn_down(2 * i + 1, 1)
            return 0
        nc = F // FC
        jax.lax.fori_loop(0, nc // 2 - 1, ffn, 0)
        ffn_up(nc - 1, 1)
        ffn_down(nc - 2, 0)
        ffn_down(nc - 1, 1)

        @pl.when(layer == 1)
        def _():
            slot = blk % 2

            @pl.when(blk >= 2)
            def _():
                out_copy(blk - 2, slot).wait()
            obuf[slot] = big[rows, :].astype(bf16)
            out_copy(blk, slot).start()

    def layer_body(layer, _):
        mt[...] = jnp.zeros(mt.shape, f32)
        zrow[...] = jnp.zeros(zrow.shape, f32)

        def init_x(i, _):
            r = pl.multiple_of(i * 256, 256)
            xv = jnp.where(layer == 0, xin[pl.ds(r, 256), :].astype(f32), big[pl.ds(r, 256), :])
            big[pl.ds(r, 256), :] = xv
            xna[pl.ds(r, 256), :] = _ln(xv)
            return 0
        jax.lax.fori_loop(0, L // 256, init_x, 0)

        def a_body(seg, _):
            phase_a(layer, seg)
            return 0
        jax.lax.fori_loop(0, NSEG, a_body, 0)

        def b_body(blk, _):
            phase_b(layer, blk)
            return 0
        jax.lax.fori_loop(0, NSEG, b_body, 0)
        return 0
    jax.lax.fori_loop(0, 2, layer_body, 0)

    out_copy(NSEG - 2, 0).wait()
    out_copy(NSEG - 1, 1).wait()


@jax.jit
def pallas_interleave_layers__memory_aug_infini_attn__mixer_s_mlp__prompt_kernel(
    A_x: jax.Array,
    A_wq: jax.Array,
    A_wk: jax.Array,
    A_wv: jax.Array,
    A_wo: jax.Array,
    A_beta: jax.Array,
    B_x: jax.Array,
    B_w1: jax.Array,
    B_w2: jax.Array,
    B_w3: jax.Array,
    B_w4: jax.Array,
):
    del B_x
    hbm = pl.BlockSpec(memory_space=pl.ANY)
    vm = pltpu.VMEM
    scratch = [
        vm((S, D), bf16),
        vm((8, 256, D), bf16),
        vm((2, 4, D, 256), bf16),
        vm((2, D, DHALF), bf16),
        vm((2, DHALF, D), bf16),
        vm((D, D), bf16),
        vm((D, D), bf16),
        vm((F // FC, D, FC), bf16),
        vm((F, D), bf16),
        vm((BIG_ROWS, D), f32),
        vm((S, D), f32),
        vm((S + 2 * HALO, D), f32),
        vm((L, D), f32),
        vm((L, D), bf16),
        vm((2, L, FC), bf16),
        vm((GH, 128, L), bf16),
        vm((GH, 128, L), bf16),
        vm((GH, L, 128), bf16),
        vm((GH, L, 128), bf16),
        vm((GH, 128, L), bf16),
        vm((GH - 1, L, 128), bf16),
        vm((2, L, 128), bf16),
        vm((GH, 128, L), f32),
        vm((2, GH, 128, 128), f32),
        vm((2, 1, DHALF), f32),
        vm((2, H // 2, 128), f32),
        vm((128, 512), f32),
    ]
    scratch += [vm((2, 128 * (t + 1), 512), f32) for t in range(NT_TILES)]
    scratch += [vm((2, 1, 512), f32) for _ in range(NT_TILES)]
    scratch += [
        vm((2, L, D), bf16),
        pltpu.SemaphoreType.DMA((10,)),
        pltpu.SemaphoreType.DMA((8,)),
        pltpu.SemaphoreType.DMA((2,)),
    ]
    return pl.pallas_call(
        _kernel,
        out_shape=jax.ShapeDtypeStruct((1, S, D), bf16),
        in_specs=[hbm, hbm, hbm, hbm, hbm, pl.BlockSpec(memory_space=pltpu.VMEM),
                  hbm, hbm, hbm, hbm],
        out_specs=hbm,
        scratch_shapes=scratch,
        compiler_params=pltpu.CompilerParams(vmem_limit_bytes=120 * 1024 * 1024),
    )(A_x, A_wq, A_wk, A_wv, A_wo, A_beta.reshape(1, H), B_w1, B_w2, B_w3, B_w4)
```

```python
import functools
import math

import jax
import jax.numpy as jnp
import jax.experimental.pallas as pl
import jax.experimental.pallas.tpu as pltpu

S = 2048
D = 1024
F = 3584
H = 32
DH = 32
L = 512
NSEG = S // L
NG = D // 128
NT_TILES = L // 128
FC = 256
HALO = 8
GH = NG // 2
DHALF = D // 2
PIN = S
BIG_ROWS = PIN + 8 * NSEG
SHIFTS = (1, -1, 2, -2)

LOG2E = math.log2(math.e)
QSCALE = DH ** -0.5 * LOG2E
MASK_BIAS = -1e9 * LOG2E
EPS = 1e-5

f32 = jnp.float32
bf16 = jnp.bfloat16
NT_DIMS = (((1,), (1,)), ((), ()))


def _stats(x):
    m = jnp.mean(x, axis=-1, keepdims=True)
    xc = x - m
    return m, jnp.mean(xc * xc, axis=-1, keepdims=True)


def _ln(x):
    m, v = _stats(x)
    r = jax.lax.rsqrt(v + EPS)
    return x * r - m * r


def _ln_ln(x):
    m, v = _stats(x)
    r1 = jax.lax.rsqrt(v + EPS)
    y = x * r1 - m * r1
    return y, y * jax.lax.rsqrt(v * r1 * r1 + EPS)


def _gelu(x):
    c = math.sqrt(2.0 / math.pi)
    inner = x * (c + (c * 0.044715) * (x * x))
    hx = 0.5 * x
    return hx + hx * jnp.tanh(inner)


def _phi(t):
    return jnp.where(t > 0, t + 1.0, jnp.exp(t))


def _red8(x, op):
    return functools.reduce(op, [x[i * 8:(i + 1) * 8] for i in range(x.shape[0] // 8)])


def _dot(a, b):
    return jnp.dot(a, b, preferred_element_type=f32)


def _dot_nt(a, b):
    return jax.lax.dot_general(a, b, NT_DIMS, preferred_element_type=f32)


def _kernel(x_hbm, wq_hbm, wk_hbm, wv_hbm, wo_hbm, beta_ref, w1_hbm, w2_hbm, w3_hbm, w4_hbm,
            out_hbm,
            xin, stage, wt, wk, wo, w1, w2, w3, w4,
            big, yres, hbuf, xna, xnb, gh, qt, pqt, kb, pkb, vt, ob, obl, amem,
            mt, zrow, gate, bias,
            s0, s1, s2, s3, m0, m1, m2, m3,
            obuf, sems, tsems, osems):
    sbuf = (s0, s1, s2, s3)
    mbuf = (m0, m1, m2, m3)

    def seg_rows(s):
        return pl.ds(s * L, L)

    cp_x0 = pltpu.make_async_copy(x_hbm.at[0, seg_rows(0)], xin.at[seg_rows(0)], sems.at[0])
    cp_xr = pltpu.make_async_copy(x_hbm.at[0, pl.ds(L, S - L)], xin.at[pl.ds(L, S - L)], sems.at[1])
    cp_wk = [pltpu.make_async_copy(wk_hbm.at[:, pl.ds(i * DHALF, DHALF)], wk.at[i], sems.at[2 + i])
             for i in range(2)]
    cp_wo = [pltpu.make_async_copy(wo_hbm.at[pl.ds(i * DHALF, DHALF)], wo.at[i], sems.at[4 + i])
             for i in range(2)]
    cp_w1 = pltpu.make_async_copy(w1_hbm, w1, sems.at[6])
    cp_w2 = pltpu.make_async_copy(w2_hbm, w2, sems.at[7])
    cp_w3 = [pltpu.make_async_copy(w3_hbm.at[:, pl.ds(c * FC, FC)], w3.at[c], sems.at[8])
             for c in range(F // FC)]
    cp_w4 = pltpu.make_async_copy(w4_hbm, w4, sems.at[9])

    TC = 256
    NTC = D // TC

    def cp_stage(i, c):
        src = (wq_hbm, wv_hbm)[i]
        return pltpu.make_async_copy(src.at[pl.ds(c * TC, TC)], stage.at[i * NTC + c],
                                     tsems.at[i * NTC + c])

    cp_x0.start()
    for i in range(2):
        for c in range(NTC):
            cp_stage(i, c).start()
    cp_wk[0].start()
    cp_wo[0].start()

    kk = jax.lax.broadcasted_iota(jnp.int32, (128, 512), 0)
    qq = jax.lax.broadcasted_iota(jnp.int32, (128, 512), 1) % 128
    bias[...] = jnp.where(kk > qq, MASK_BIAS, 0.0).astype(f32)
    bt = jnp.broadcast_to(beta_ref[...].astype(f32), (H, H))
    eye = (jax.lax.broadcasted_iota(jnp.int32, (H, H), 0)
           == jax.lax.broadcasted_iota(jnp.int32, (H, H), 1))
    bcol = jnp.sum(jnp.where(eye, bt, 0.0), axis=1, keepdims=True)
    gsig = jnp.broadcast_to(jax.nn.sigmoid(bcol), (H, 128))
    gate[0] = gsig[0:H // 2]
    gate[1] = gsig[H // 2:H]
    hbuf[HALO:2 * HALO, :] = jnp.zeros((HALO, D), f32)
    hbuf[S:S + HALO, :] = jnp.zeros((HALO, D), f32)

    ident = (jax.lax.broadcasted_iota(jnp.int32, (128, 128), 0)
             == jax.lax.broadcasted_iota(jnp.int32, (128, 128), 1)).astype(f32).astype(bf16)

    def transpose_chunk(ic, _):
        pltpu.make_async_copy(stage.at[ic], stage.at[ic], tsems.at[ic]).wait()
        i = ic // NTC
        c = ic % NTC
        ro = pl.multiple_of(i * DHALF, DHALF)
        for n in range(D // 128):
            tile = _dot_nt(ident, stage[ic, :, n * 128:(n + 1) * 128]).astype(bf16)
            wt[n // 4, c, pl.ds(ro + (n % 4) * 128, 128), :] = tile
        return 0
    jax.lax.fori_loop(0, 2 * NTC, transpose_chunk, 0)

    cp_wk[1].start()
    cp_wo[1].start()
    cp_w1.start()
    cp_xr.start()
    cp_w2.start()
    for c in cp_w3:
        c.start()
    cp_w4.start()
    cp_x0.wait()
    cp_wk[0].wait()
    cp_wo[0].wait()

    def qmask(g, t):
        z = jnp.zeros((DH, 128), bf16)
        cols = []
        for h in range(4):
            qh = qt[g, h * DH:(h + 1) * DH, t * 128:(t + 1) * 128]
            cols.append(jnp.concatenate([qh if i == h else z for i in range(4)], axis=0))
        return jnp.concatenate(cols, axis=1)

    def attn_step(half, g, gn, fill=()):
        pr = None if g is None else g % 2
        pw = None if gn is None else gn % 2
        fill = list(fill)
        for t in range(NT_TILES):
            macc = None
            oacc = [None] * 4
            lacc = [None] * 4
            for j in range(t + 1):
                ks = slice(j * 128, (j + 1) * 128)
                if fill and (t, j) != (0, 0):
                    fill.pop(0)()
                if gn is not None:
                    s = _dot(kb[gn, ks, :], qmask(gn, t))
                    if j == t:
                        s = s + bias[...]
                    sbuf[t][pw, ks, :] = s
                    mx = _red8(s, jnp.maximum)
                    macc = mx if macc is None else jnp.maximum(macc, mx)
                if g is not None:
                    for h in range(4):
                        sl = slice(h * 128, (h + 1) * 128)
                        p = jnp.exp2(sbuf[t][pr, ks, sl] - mbuf[t][pr, :, sl])
                        lt = _red8(p, jnp.add)
                        lacc[h] = lt if lacc[h] is None else lacc[h] + lt
                        o = _dot(vt[g, h * DH:(h + 1) * DH, ks], p.astype(bf16))
                        oacc[h] = o if oacc[h] is None else oacc[h] + o
            if gn is not None:
                mbuf[t][pw] = jnp.max(macc, axis=0, keepdims=True)
            if g is not None:
                parts = []
                for h in range(4):
                    l = jnp.sum(lacc[h], axis=0, keepdims=True)
                    gh = gate[half, g * 4 + h:g * 4 + h + 1, :]
                    parts.append(oacc[h] * ((1.0 - gh) / l))
                ot = jnp.concatenate(parts, axis=0) + amem[g, :, t * 128:(t + 1) * 128]
                if g < GH - 1:
                    ob[g, t * 128:(t + 1) * 128, :] = ot.T.astype(bf16)
                else:
                    obl[half, t * 128:(t + 1) * 128, :] = ot.T.astype(bf16)

    rowh = jax.lax.broadcasted_iota(jnp.int32, (128, 128), 0) // DH
    colh = jax.lax.broadcasted_iota(jnp.int32, (128, 128), 1) // DH
    row16 = jax.lax.broadcasted_iota(jnp.int32, (16, 128), 0)
    col16 = jax.lax.broadcasted_iota(jnp.int32, (16, 128), 1) // DH

    def attn_half(layer, seg, half):
        r0 = pl.multiple_of(seg * L, L)

        @pl.when(jnp.logical_and(jnp.logical_and(layer == 0, seg == 0), half == 1))
        def _():
            cp_wk[1].wait()
            cp_wo[1].wait()
            cp_w1.wait()
            cp_xr.wait()

        def xn(c):
            return xna[c * 128:(c + 1) * 128, :].astype(bf16)

        zparts = {}

        def k_piece(g0, ng, c0, nc):
            lhs = jnp.concatenate([xn(c) for c in range(c0, c0 + nc)], axis=0)
            k = _dot(lhs, wk[half, :, g0 * 128:(g0 + ng) * 128])
            pk = _phi(k)
            rs = slice(c0 * 128, (c0 + nc) * 128)
            for i in range(ng):
                cs = slice(i * 128, (i + 1) * 128)
                kb[g0 + i, rs, :] = k[:, cs].astype(bf16)
                pkb[g0 + i, rs, :] = pk[:, cs].astype(bf16)
                zparts.setdefault(g0 + i, []).append(_red8(pk[:, cs], jnp.add))

        def qv_piece(qs, vs, c0, nc):
            offs = [g * 128 for g in qs] + [DHALF + g * 128 for g in vs]
            lhs = jnp.concatenate(
                [jnp.concatenate([wt[half, c, o:o + 128, :] for c in range(NTC)], axis=1)
                 for o in offs], axis=0)
            rhs = jnp.concatenate([xn(c) for c in range(c0, c0 + nc)], axis=0)
            r = _dot_nt(lhs, rhs)
            ts = slice(c0 * 128, (c0 + nc) * 128)
            for i, g in enumerate(qs):
                qg = r[i * 128:(i + 1) * 128, :]
                qt[g, :, ts] = (qg * QSCALE).astype(bf16)
                pqt[g, :, ts] = _phi(qg).astype(bf16)
            for i, g in enumerate(vs):
                o = (len(qs) + i) * 128
                vt[g, :, ts] = r[o:o + 128, :].astype(bf16)

        def mem(g):
            zold = zrow[half, g]
            mold = mt[half, g]
            mbd = jnp.where(rowh == colh, mold, 0.0)
            zx = jnp.where(row16 == col16, jnp.broadcast_to(zold, (16, 128)), 0.0)
            lhs = jnp.concatenate([mbd, zx], axis=0).astype(bf16)
            ret = _dot(lhs, pqt[g])
            parts = []
            for h in range(4):
                gh = gate[half, g * 4 + h:g * 4 + h + 1, 0:1]
                den = ret[128 + h:129 + h, :] + 1e-6
                parts.append(ret[h * DH:(h + 1) * DH, :] * (gh / den))
            amem[g] = jnp.concatenate(parts, axis=0)
            mt[half, g] = mold + _dot(vt[g], pkb[g])
            zsum = functools.reduce(jnp.add, zparts[g])
            zrow[half, g] = zold + jnp.sum(zsum, axis=0, keepdims=True)

        P = functools.partial
        skip = lambda: None
        k_piece(0, 2, 0, 4)
        qv_piece((0, 1), (0,), 0, 4)
        attn_step(half, None, 0)
        mem(0)
        for g in range(2):
            attn_step(half, g, g + 1, fill=[
                P(k_piece, g + 2, 1, 0, 2), skip, P(qv_piece, (g + 2,), (g + 1,), 0, 1),
                P(qv_piece, (g + 2,), (g + 1,), 1, 1), skip, P(k_piece, g + 2, 1, 2, 2),
                P(qv_piece, (g + 2,), (g + 1,), 2, 1), P(qv_piece, (g + 2,), (g + 1,), 3, 1),
                P(mem, g + 1)])
        attn_step(half, 2, 3, fill=[
            skip, P(qv_piece, (), (3,), 0, 1), skip, P(qv_piece, (), (3,), 1, 1), skip,
            P(qv_piece, (), (3,), 2, 1), P(qv_piece, (), (3,), 3, 1), skip, P(mem, 3)])
        kp = (GH - 1) * 128

        def wo_piece(i):
            off = (i // 2) * 128
            cs = slice((i % 2) * DHALF, (i % 2 + 1) * DHALF)
            rr = pl.ds(r0 + off, 128)
            o = jnp.concatenate([ob[g, off:off + 128, :] for g in range(GH - 1)], axis=1)
            big[rr, cs] = big[rr, cs] + _dot(o, wo[half, 0:kp, cs])

        attn_step(half, GH - 1, None, fill=[functools.partial(wo_piece, i) for i in range(8)])

    def phase_a(layer, seg):
        r0 = pl.multiple_of(seg * L, L)

        def half_body(half, _):
            attn_half(layer, seg, half)
            return 0
        jax.lax.fori_loop(0, 2, half_body, 0)

        hl = L // 2
        kp = (GH - 1) * 128

        def wo_rest(off, n):
            rr = pl.ds(r0 + off, n)
            o = jnp.concatenate([obl[0, off:off + n, :], obl[1, off:off + n, :]], axis=1)
            w = jnp.concatenate([wo[0, kp:DHALF, :], wo[1, kp:DHALF, :]], axis=0)
            big[rr, :] = big[rr, :] + _dot(o, w)

        def lnln(off, n):
            y, z = _ln_ln(big[pl.ds(r0 + off, n), :])
            yres[pl.ds(r0 + off, n), :] = y
            xnb[off:off + n, :] = z.astype(bf16)

        def up(off, n):
            cs = slice(n * 256, (n + 1) * 256)
            hh = _gelu(_dot(xnb[off:off + hl, :], w1[:, cs]))
            win = hbuf.at[pl.ds(r0 + off, hl + 2 * HALO), :]
            b = HALO + SHIFTS[n]
            win[b:b + hl, cs] = hh
            return [hh[0:8, 0:128], hh[hl - 8:hl, 0:128], hh[0:8, 128:256], hh[hl - 8:hl, 128:256]]

        def pin(v):
            big[pl.ds(PIN + pl.multiple_of(seg * 8, 8), 8), 0:128] = v

        n0 = pl.multiple_of(jnp.minimum(seg + 1, NSEG - 1) * L, L)
        fresh = jnp.logical_and(layer == 0, seg < NSEG - 1)

        def ln_next(off, n):
            rr = pl.ds(n0 + off, n)
            xv = jnp.where(fresh, xin[pl.ds(n0 + off, n), :].astype(f32), big[rr, :])
            big[rr, :] = xv
            xna[off:off + n, :] = _ln(xv)

        wo_rest(0, 128)
        lnln(0, 128)
        wo_rest(128, 128)
        lnln(128, 128)
        wo_rest(hl, hl)
        for n in range(4):
            marks = up(0, n)
            for i in range(4):
                lnln(hl + n * 64 + i * 16, 16)
                pin(marks[i])
        for n in range(4):
            marks = up(hl, n)
            for i in range(4):
                ln_next(n * 128 + i * 32, 32)
                pin(marks[i])

    def out_copy(blk, slot):
        return pltpu.make_async_copy(
            obuf.at[slot], out_hbm.at[0, pl.ds(blk * L, L), :], osems.at[slot])

    def phase_b(layer, blk):
        r0 = pl.multiple_of(blk * L, L)
        rows = pl.ds(r0, L)

        @pl.when(jnp.logical_and(layer == 0, blk == 0))
        def _():
            cp_w2.wait()
            for c in cp_w3:
                c.wait()
            cp_w4.wait()

        hl = L // 2

        def mix(off, cs):
            hs = hbuf[pl.ds(HALO + r0 + off, hl), :].astype(bf16)
            rr = pl.ds(r0 + off, hl)
            x1 = yres[rr, cs] + _dot(hs, w2[:, cs])
            yres[rr, cs] = x1
            big[rr, cs] = big[rr, cs] + x1

        def ln_mid(off, n):
            xnb[off:off + n, :] = _ln(yres[pl.ds(r0 + off, n), :]).astype(bf16)

        def ffn_up(c, slot, off=0, n=L):
            gh[slot, off:off + n, :] = _gelu(_dot(xnb[off:off + n, :], w3[c])).astype(bf16)

        def ffn_down(c, slot, cs=slice(0, D)):
            w = w4[pl.ds(pl.multiple_of(c * FC, FC), FC), cs]
            big[rows, cs] = big[rows, cs] + _dot(gh[slot], w)

        mix(0, slice(0, D))
        for n in range(4):
            ln_mid(n * 64, 64)
            mix(hl, slice(n * 256, (n + 1) * 256))
        ln_mid(hl, hl)
        ffn_up(0, 0, 0, hl)
        ffn_up(0, 0, hl, hl)

        def ffn(i, _):
            ffn_up(2 * i + 1, 1)
            ffn_down(2 * i, 0)
            ffn_up(2 * i + 2, 0)
            ffn_down(2 * i + 1, 1)
            return 0
        nc = F // FC
        jax.lax.fori_loop(0, nc // 2 - 1, ffn, 0)
        ffn_up(nc - 1, 1)
        ffn_down(nc - 2, 0)
        ffn_down(nc - 1, 1)

        @pl.when(layer == 1)
        def _():
            slot = blk % 2

            @pl.when(blk >= 2)
            def _():
                out_copy(blk - 2, slot).wait()
            obuf[slot] = big[rows, :].astype(bf16)
            out_copy(blk, slot).start()

    def layer_body(layer, _):
        mt[...] = jnp.zeros(mt.shape, f32)
        zrow[...] = jnp.zeros(zrow.shape, f32)

        def init_x(i, _):
            r = pl.multiple_of(i * 256, 256)
            xv = jnp.where(layer == 0, xin[pl.ds(r, 256), :].astype(f32), big[pl.ds(r, 256), :])
            big[pl.ds(r, 256), :] = xv
            xna[pl.ds(r, 256), :] = _ln(xv)
            return 0
        jax.lax.fori_loop(0, L // 256, init_x, 0)

        def a_body(seg, _):
            phase_a(layer, seg)
            return 0
        jax.lax.fori_loop(0, NSEG, a_body, 0)

        def b_body(blk, _):
            phase_b(layer, blk)
            return 0
        jax.lax.fori_loop(0, NSEG, b_body, 0)
        return 0
    jax.lax.fori_loop(0, 2, layer_body, 0)

    out_copy(NSEG - 2, 0).wait()
    out_copy(NSEG - 1, 1).wait()


@jax.jit
def pallas_interleave_layers__memory_aug_infini_attn__mixer_s_mlp__prompt_kernel(
    A_x: jax.Array,
    A_wq: jax.Array,
    A_wk: jax.Array,
    A_wv: jax.Array,
    A_wo: jax.Array,
    A_beta: jax.Array,
    B_x: jax.Array,
    B_w1: jax.Array,
    B_w2: jax.Array,
    B_w3: jax.Array,
    B_w4: jax.Array,
):
    del B_x
    hbm = pl.BlockSpec(memory_space=pl.ANY)
    vm = pltpu.VMEM
    scratch = [
        vm((S, D), bf16),
        vm((8, 256, D), bf16),
        vm((2, 4, D, 256), bf16),
        vm((2, D, DHALF), bf16),
        vm((2, DHALF, D), bf16),
        vm((D, D), bf16),
        vm((D, D), bf16),
        vm((F // FC, D, FC), bf16),
        vm((F, D), bf16),
        vm((BIG_ROWS, D), f32),
        vm((S, D), f32),
        vm((S + 2 * HALO, D), f32),
        vm((L, D), f32),
        vm((L, D), bf16),
        vm((2, L, FC), bf16),
        vm((GH, 128, L), bf16),
        vm((GH, 128, L), bf16),
        vm((GH, L, 128), bf16),
        vm((GH, L, 128), bf16),
        vm((GH, 128, L), bf16),
        vm((GH - 1, L, 128), bf16),
        vm((2, L, 128), bf16),
        vm((GH, 128, L), f32),
        vm((2, GH, 128, 128), f32),
        vm((2, GH, 1, 128), f32),
        vm((2, H // 2, 128), f32),
        vm((128, 512), f32),
    ]
    scratch += [vm((2, 128 * (t + 1), 512), f32) for t in range(NT_TILES)]
    scratch += [vm((2, 1, 512), f32) for _ in range(NT_TILES)]
    scratch += [
        vm((2, L, D), bf16),
        pltpu.SemaphoreType.DMA((10,)),
        pltpu.SemaphoreType.DMA((8,)),
        pltpu.SemaphoreType.DMA((2,)),
    ]
    return pl.pallas_call(
        _kernel,
        out_shape=jax.ShapeDtypeStruct((1, S, D), bf16),
        in_specs=[hbm, hbm, hbm, hbm, hbm, pl.BlockSpec(memory_space=pltpu.VMEM),
                  hbm, hbm, hbm, hbm],
        out_specs=hbm,
        scratch_shapes=scratch,
        compiler_params=pltpu.CompilerParams(vmem_limit_bytes=120 * 1024 * 1024),
    )(A_x, A_wq, A_wk, A_wv, A_wo, A_beta.reshape(1, H), B_w1, B_w2, B_w3, B_w4)
```

```python
import functools
import math

import jax
import jax.numpy as jnp
import jax.experimental.pallas as pl
import jax.experimental.pallas.tpu as pltpu

S = 2048
D = 1024
F = 3584
H = 32
DH = 32
L = 512
NSEG = S // L
NG = D // 128
NT_TILES = L // 128
FC = 256
HALO = 8
GH = NG // 2
DHALF = D // 2
PAD_ROWS = S + 2 * HALO
PIN = S + L + 2 * HALO
BIG_ROWS = PIN + 16 * NSEG
NC = F // FC
UNROLL = 4
SHIFTS = (1, -1, 2, -2)

LOG2E = math.log2(math.e)
QSCALE = DH ** -0.5 * LOG2E
MASK_BIAS = -1e9 * LOG2E
EPS = 1e-5

f32 = jnp.float32
bf16 = jnp.bfloat16
NT_DIMS = (((1,), (1,)), ((), ()))


def _stats(x):
    m = jnp.mean(x, axis=-1, keepdims=True)
    xc = x - m
    return m, jnp.mean(xc * xc, axis=-1, keepdims=True)


def _ln(x):
    m, v = _stats(x)
    r = jax.lax.rsqrt(v + EPS)
    return x * r - m * r


def _ln_ln(x):
    m, v = _stats(x)
    r1 = jax.lax.rsqrt(v + EPS)
    r2 = r1 * jax.lax.rsqrt(v * r1 * r1 + EPS)
    return r1, m * r1, x * r2 - m * r2


def _gelu(x):
    c = math.sqrt(2.0 / math.pi)
    inner = x * (c + (c * 0.044715) * (x * x))
    hx = 0.5 * x
    return hx + hx * jnp.tanh(inner)


def _phi(t):
    return jnp.where(t > 0, t + 1.0, jnp.exp(t))


def _red8(x, op):
    return functools.reduce(op, [x[i * 8:(i + 1) * 8] for i in range(x.shape[0] // 8)])


def _dot(a, b):
    return jnp.dot(a, b, preferred_element_type=f32)


def _dot_nt(a, b):
    return jax.lax.dot_general(a, b, NT_DIMS, preferred_element_type=f32)


def _kernel(x_hbm, wq_hbm, wk_hbm, wv_hbm, wo_hbm, beta_ref, w1_hbm, w2_hbm, w3_hbm, w4_hbm,
            out_hbm,
            xin, stage, wt, wk, wo, w1, w2, w3, w4,
            big, yres, hbuf, xna, xnb, xnc, gh, qt, pqt, kb, pkb, vt, ob, obl, amem,
            mt, zrow, gate, bias,
            s0, s1, s2, s3, m0, m1, m2, m3,
            obuf, sems, tsems, osems):
    sbuf = (s0, s1, s2, s3)
    mbuf = (m0, m1, m2, m3)

    def seg_rows(s):
        return pl.ds(s * L, L)

    cp_x0 = pltpu.make_async_copy(x_hbm.at[0, seg_rows(0)], xin.at[seg_rows(0)], sems.at[0])
    cp_xr = pltpu.make_async_copy(x_hbm.at[0, pl.ds(L, S - L)], xin.at[pl.ds(L, S - L)], sems.at[1])
    cp_wk = [pltpu.make_async_copy(wk_hbm.at[:, pl.ds(i * DHALF, DHALF)], wk.at[i], sems.at[2 + i])
             for i in range(2)]
    cp_wo = [pltpu.make_async_copy(wo_hbm.at[pl.ds(i * DHALF, DHALF)], wo.at[i], sems.at[4 + i])
             for i in range(2)]
    cp_w1 = pltpu.make_async_copy(w1_hbm, w1, sems.at[6])
    cp_w2 = pltpu.make_async_copy(w2_hbm, w2, sems.at[7])
    cp_w3 = [pltpu.make_async_copy(w3_hbm.at[:, pl.ds(c * FC, FC)], w3.at[c], sems.at[8])
             for c in range(F // FC)]
    cp_w4 = pltpu.make_async_copy(w4_hbm, w4, sems.at[9])

    TC = 256
    NTC = D // TC

    def cp_stage(i, c):
        src = (wq_hbm, wv_hbm)[i]
        return pltpu.make_async_copy(src.at[pl.ds(c * TC, TC)], stage.at[i * NTC + c],
                                     tsems.at[i * NTC + c])

    cp_x0.start()
    for i in range(2):
        for c in range(NTC):
            cp_stage(i, c).start()
    cp_wk[0].start()
    cp_wo[0].start()

    kk = jax.lax.broadcasted_iota(jnp.int32, (128, 512), 0)
    qq = jax.lax.broadcasted_iota(jnp.int32, (128, 512), 1) % 128
    bias[...] = jnp.where(kk > qq, MASK_BIAS, 0.0).astype(f32)
    bt = jnp.broadcast_to(beta_ref[...].astype(f32), (H, H))
    eye = (jax.lax.broadcasted_iota(jnp.int32, (H, H), 0)
           == jax.lax.broadcasted_iota(jnp.int32, (H, H), 1))
    bcol = jnp.sum(jnp.where(eye, bt, 0.0), axis=1, keepdims=True)
    gsig = jnp.broadcast_to(jax.nn.sigmoid(bcol), (H, 128))
    gate[0] = gsig[0:H // 2]
    gate[1] = gsig[H // 2:H]
    hbuf[0:2 * HALO, :] = jnp.zeros((2 * HALO, D), f32)
    hbuf[S:PAD_ROWS, :] = jnp.zeros((2 * HALO, D), f32)
    for ref in (big, yres):
        ref[0:HALO, :] = jnp.zeros((HALO, D), f32)
        ref[S + HALO:PAD_ROWS, :] = jnp.zeros((HALO, D), f32)

    ident = (jax.lax.broadcasted_iota(jnp.int32, (128, 128), 0)
             == jax.lax.broadcasted_iota(jnp.int32, (128, 128), 1)).astype(f32).astype(bf16)

    def transpose_chunk(ic, _):
        pltpu.make_async_copy(stage.at[ic], stage.at[ic], tsems.at[ic]).wait()
        i = ic // NTC
        c = ic % NTC
        ro = pl.multiple_of(i * DHALF, DHALF)
        for n in range(D // 128):
            tile = _dot_nt(ident, stage[ic, :, n * 128:(n + 1) * 128]).astype(bf16)
            wt[n // 4, c, pl.ds(ro + (n % 4) * 128, 128), :] = tile
        return 0
    jax.lax.fori_loop(0, 2 * NTC, transpose_chunk, 0)

    cp_wk[1].start()
    cp_wo[1].start()
    cp_w1.start()
    cp_xr.start()
    cp_w2.start()
    cp_x0.wait()

    def init_x(i, _):
        r = pl.multiple_of(i * 256, 256)
        xv = xin[pl.ds(r, 256), :].astype(f32)
        big[pl.ds(HALO + r, 256), :] = xv
        xna[pl.ds(r, 256), :] = _ln(xv)
        return 0
    jax.lax.fori_loop(0, L // 256, init_x, 0)
    cp_wk[0].wait()
    cp_wo[0].wait()

    def qmask(g, t):
        z = jnp.zeros((DH, 128), bf16)
        cols = []
        for h in range(4):
            qh = qt[g, h * DH:(h + 1) * DH, t * 128:(t + 1) * 128]
            cols.append(jnp.concatenate([qh if i == h else z for i in range(4)], axis=0))
        return jnp.concatenate(cols, axis=1)

    def attn_step(half, g, gn, fill=()):
        pr = None if g is None else g % 2
        pw = None if gn is None else gn % 2
        fill = list(fill)
        for t in range(NT_TILES):
            macc = None
            oacc = [None] * 4
            lacc = [None] * 4
            for j in range(t + 1):
                ks = slice(j * 128, (j + 1) * 128)
                if fill and (t, j) != (0, 0):
                    fill.pop(0)()
                if gn is not None:
                    s = _dot(kb[gn, ks, :], qmask(gn, t))
                    if j == t:
                        s = s + bias[...]
                    sbuf[t][pw, ks, :] = s
                    mx = _red8(s, jnp.maximum)
                    macc = mx if macc is None else jnp.maximum(macc, mx)
                if g is not None:
                    for h in range(4):
                        sl = slice(h * 128, (h + 1) * 128)
                        p = jnp.exp2(sbuf[t][pr, ks, sl] - mbuf[t][pr, :, sl])
                        lt = _red8(p, jnp.add)
                        lacc[h] = lt if lacc[h] is None else lacc[h] + lt
                        o = _dot(vt[g, h * DH:(h + 1) * DH, ks], p.astype(bf16))
                        oacc[h] = o if oacc[h] is None else oacc[h] + o
            if gn is not None:
                mbuf[t][pw] = jnp.max(macc, axis=0, keepdims=True)
            if g is not None:
                parts = []
                for h in range(4):
                    l = jnp.sum(lacc[h], axis=0, keepdims=True)
                    gh = gate[half, g * 4 + h:g * 4 + h + 1, :]
                    parts.append(oacc[h] * ((1.0 - gh) / l))
                ot = jnp.concatenate(parts, axis=0) + amem[g, :, t * 128:(t + 1) * 128]
                if g < GH - 1 or t < 2:
                    ob[g, t * 128:(t + 1) * 128, :] = ot.T.astype(bf16)
                else:
                    obl[half, (t - 2) * 128:(t - 1) * 128, :] = ot.T.astype(bf16)

    rowh = jax.lax.broadcasted_iota(jnp.int32, (128, 128), 0) // DH
    colh = jax.lax.broadcasted_iota(jnp.int32, (128, 128), 1) // DH
    row16 = jax.lax.broadcasted_iota(jnp.int32, (16, 128), 0)
    col16 = jax.lax.broadcasted_iota(jnp.int32, (16, 128), 1) // DH

    def attn_half(layer, seg, half):
        r0 = pl.multiple_of(seg * L, L)

        @pl.when(jnp.logical_and(jnp.logical_and(layer == 0, seg == 0), half == 1))
        def _():
            cp_wk[1].wait()
            cp_wo[1].wait()
            cp_w1.wait()
            cp_xr.wait()
            cp_w2.wait()
            for c in cp_w3:
                c.start()
            cp_w4.start()

        def xn(c):
            return xna[c * 128:(c + 1) * 128, :].astype(bf16)

        zparts = {}

        def k_piece(g0, ng, c0, nc):
            lhs = jnp.concatenate([xn(c) for c in range(c0, c0 + nc)], axis=0)
            k = _dot(lhs, wk[half, :, g0 * 128:(g0 + ng) * 128])
            pk = _phi(k)
            rs = slice(c0 * 128, (c0 + nc) * 128)
            for i in range(ng):
                cs = slice(i * 128, (i + 1) * 128)
                kb[g0 + i, rs, :] = k[:, cs].astype(bf16)
                pkb[g0 + i, rs, :] = pk[:, cs].astype(bf16)
                zparts.setdefault(g0 + i, []).append(_red8(pk[:, cs], jnp.add))

        def qv_piece(qs, vs, c0, nc):
            offs = [g * 128 for g in qs] + [DHALF + g * 128 for g in vs]
            lhs = jnp.concatenate(
                [jnp.concatenate([wt[half, c, o:o + 128, :] for c in range(NTC)], axis=1)
                 for o in offs], axis=0)
            rhs = jnp.concatenate([xn(c) for c in range(c0, c0 + nc)], axis=0)
            r = _dot_nt(lhs, rhs)
            ts = slice(c0 * 128, (c0 + nc) * 128)
            for i, g in enumerate(qs):
                qg = r[i * 128:(i + 1) * 128, :]
                qt[g, :, ts] = (qg * QSCALE).astype(bf16)
                pqt[g, :, ts] = _phi(qg).astype(bf16)
            for i, g in enumerate(vs):
                o = (len(qs) + i) * 128
                vt[g, :, ts] = r[o:o + 128, :].astype(bf16)

        def mem(g):
            zold = zrow[half, g]
            mold = mt[half, g]
            mbd = jnp.where(rowh == colh, mold, 0.0)
            zx = jnp.where(row16 == col16, jnp.broadcast_to(zold, (16, 128)), 0.0)
            lhs = jnp.concatenate([mbd, zx], axis=0).astype(bf16)
            ret = _dot(lhs, pqt[g])
            parts = []
            for h in range(4):
                gh = gate[half, g * 4 + h:g * 4 + h + 1, 0:1]
                den = ret[128 + h:129 + h, :] + 1e-6
                parts.append(ret[h * DH:(h + 1) * DH, :] * (gh / den))
            amem[g] = jnp.concatenate(parts, axis=0)
            mt[half, g] = mold + _dot(vt[g], pkb[g])
            zsum = functools.reduce(jnp.add, zparts[g])
            zrow[half, g] = zold + jnp.sum(zsum, axis=0, keepdims=True)

        P = functools.partial
        skip = lambda: None
        k_piece(0, 2, 0, 4)
        qv_piece((0, 1), (0,), 0, 4)
        attn_step(half, None, 0)
        mem(0)
        for g in range(2):
            attn_step(half, g, g + 1, fill=[
                P(k_piece, g + 2, 1, 0, 2), skip, P(qv_piece, (g + 2,), (g + 1,), 0, 1),
                P(qv_piece, (g + 2,), (g + 1,), 1, 1), skip, P(k_piece, g + 2, 1, 2, 2),
                P(qv_piece, (g + 2,), (g + 1,), 2, 1), P(qv_piece, (g + 2,), (g + 1,), 3, 1),
                P(mem, g + 1)])
        attn_step(half, 2, 3, fill=[
            skip, P(qv_piece, (), (3,), 0, 1), skip, P(qv_piece, (), (3,), 1, 1), skip,
            P(qv_piece, (), (3,), 2, 1), P(qv_piece, (), (3,), 3, 1), skip, P(mem, 3)])

        def wo_piece(t, n):
            off = t * 128
            cs = slice(n * DHALF, (n + 1) * DHALF)
            rr = pl.ds(r0 + (HALO + off), 128)
            ng = GH if t < 2 else GH - 1
            o = jnp.concatenate([ob[g, off:off + 128, :] for g in range(ng)], axis=1)
            big[rr, cs] = big[rr, cs] + _dot(o, wo[half, 0:ng * 128, cs])

        attn_step(half, GH - 1, None,
                  fill=[P(wo_piece, t, n) for t in (2, 3, 0, 1) for n in range(2)])

    def phase_a(layer, seg):
        r0 = pl.multiple_of(seg * L, L)

        def half_body(half, _):
            attn_half(layer, seg, half)
            return 0
        jax.lax.fori_loop(0, 2, half_body, 0)

        hl = L // 2
        kp = (GH - 1) * 128

        bw = big.at[pl.ds(r0, 2 * L + 2 * HALO), :]
        yw = yres.at[pl.ds(r0, L + 2 * HALO), :]
        hw = hbuf.at[pl.ds(r0, L + 2 * HALO), :]
        xw = xin.at[pl.ds(r0 + L, L), :]

        def wo_rest():
            rr = slice(HALO + hl, HALO + L)
            o = jnp.concatenate([obl[0], obl[1]], axis=1)
            w = jnp.concatenate([wo[0, kp:DHALF, :], wo[1, kp:DHALF, :]], axis=0)
            bw[rr, :] = bw[rr, :] + _dot(o, w)

        def lnln(off, n):
            rr = slice(HALO + off, HALO + off + n)
            r, mr, z = _ln_ln(bw[rr, :])
            yw[rr, D - 256:D - 128] = jnp.broadcast_to(r, (n, 128))
            yw[rr, D - 128:D] = jnp.broadcast_to(mr, (n, 128))
            xnb[off:off + n, :] = z.astype(bf16)

        def corners(v):
            return [v[0:8, 0:128], v[hl - 8:hl, 0:128], v[0:8, 128:256], v[hl - 8:hl, 128:256]]

        def up(off, n):
            cs = slice(n * 256, (n + 1) * 256)
            hh = _gelu(_dot(xnb[off:off + hl, :], w1[:, cs]))
            b = off + HALO + SHIFTS[n]
            hw[b:b + hl, cs] = hh
            return corners(hh)

        sink = PIN + pl.multiple_of(seg * 16, 16)

        def pin(ref, v):
            if ref.dtype == bf16:
                ref[pl.ds(sink, 16), 0:128] = jnp.concatenate([v, v], axis=0).astype(bf16)
            else:
                ref[pl.ds(sink, 8), 0:128] = v

        fresh = jnp.logical_and(layer == 0, seg < NSEG - 1)

        def ln_next(off, n):
            rr = slice(L + HALO + off, L + HALO + off + n)
            xv = jnp.where(fresh, xw[off:off + n, :].astype(f32), bw[rr, :])
            bw[rr, :] = xv
            xna[off:off + n, :] = _ln(xv)

        lnln(0, 128)
        lnln(128, 128)
        wo_rest()
        def mix_part(off, n):
            return corners(mix(hw, yw, bw, slice(off, off + hl), n))

        def fence():
            pin(yres, xna[pl.ds(pl.multiple_of(seg * 8, 8), 8), 0:128])

        late = list(range(hl, L, 16))
        nxt = list(range(0, L, 16))
        for n in range(4):
            marks = up(0, n)
            for i in (0, 1, 3):
                lnln(late.pop(0), 16)
                pin(big, marks[i])
        for n in range(4):
            marks = mix_part(0, n)
            for i in range(4):
                if late:
                    lnln(late.pop(0), 16)
                else:
                    ln_next(nxt.pop(0), 16)
                if n > 0 or i == 3:
                    pin(xin, marks[i])
        for n in range(4):
            marks = up(hl, n)
            for i in (0, 1, 3):
                ln_next(nxt.pop(0), 16)
                pin(xin, marks[i])
        for n in range(4):
            if n == 3:
                fence()
            marks = mix_part(hl, n)
            for i in range(4):
                if nxt:
                    ln_next(nxt.pop(0), 16)
                    pin(xin, marks[i])

    def mix(h_ref, y_ref, x_ref, rr, n):
        cs = slice(n * 256, (n + 1) * 256)
        r = y_ref[rr, D - 256:D - 128]
        mr = y_ref[rr, D - 128:D]
        x = x_ref[rr, cs]
        y = x * jnp.concatenate([r, r], axis=1) - jnp.concatenate([mr, mr], axis=1)
        x1 = y + _dot(h_ref[rr, :].astype(bf16), w2[:, cs])
        y_ref[rr, cs] = x1
        x_ref[rr, cs] = x + x1
        return x1

    def ln_mid(tok, n):
        xnc[pl.ds(tok, n), :] = _ln(yres[pl.ds(tok + HALO, n), :]).astype(bf16)

    def last_rows():
        for n in range(4):
            mix(hbuf, yres, big, slice(S, PAD_ROWS), n)
            ln_mid(n * 128, 128)

    def out_copy(blk):
        rows = pl.ds(blk * L, L)
        return pltpu.make_async_copy(obuf.at[rows], out_hbm.at[0, rows, :], osems.at[blk])

    def ffn(layer, it):
        blk = [(UNROLL * it + k) // NC for k in range(UNROLL)]
        chunk = [(UNROLL * it + k) % NC for k in range(UNROLL)]
        tok = [pl.multiple_of(b * L, L) for b in blk]

        def ffn_up(k):
            hh = _gelu(_dot(xnc[pl.ds(tok[k], L), :], w3[chunk[k]]))
            gh[k % 2] = hh.astype(bf16)
            return hh[L - 8:L, FC - 128:FC]

        def ffn_down(k):
            rows = pl.ds(tok[k] + HALO, L)
            w = w4[pl.ds(pl.multiple_of(chunk[k] * FC, FC), FC), :]
            big[rows, :] = big[rows, :] + _dot(gh[k % 2], w)

        def ln_ahead(k, mark):
            yres[pl.ds(PIN + pl.multiple_of(blk[0] * 16, 16), 8), 0:128] = mark
            nb = jnp.minimum(blk[k] + 1, NSEG - 1)
            ln_mid(pl.multiple_of(nb * L + jnp.minimum(chunk[k] * 40, L - 80), 16), 80)

        def ln_first():
            r = pl.multiple_of(jnp.clip((it - 4) * 64, 0, L - 64), 64)
            xna[pl.ds(r, 64), :] = _ln(big[pl.ds(r + HALO, 64), :])

        ffn_up(0)
        ln_ahead(0, ffn_up(1))
        ffn_down(0)
        ln_ahead(2, ffn_up(2))
        ffn_down(1)
        ln_first()
        ffn_up(3)
        ffn_down(2)
        ffn_down(3)

        done = (UNROLL * it + UNROLL) // NC

        @pl.when(jnp.logical_and(layer == 1, done != blk[0]))
        def _():
            r = pl.multiple_of((done - 1) * L, L)
            obuf[pl.ds(r, L), :] = big[pl.ds(r + HALO, L), :].astype(bf16)
            out_copy(done - 1).start()

    def layer_body(layer, _):
        mt[...] = jnp.zeros(mt.shape, f32)
        zrow[...] = jnp.zeros(zrow.shape, f32)

        def a_body(seg, _):
            phase_a(layer, seg)
            return 0
        jax.lax.fori_loop(0, NSEG, a_body, 0)

        last_rows()

        @pl.when(layer == 0)
        def _():
            for c in cp_w3:
                c.wait()
            cp_w4.wait()

        def b_body(it, _):
            ffn(layer, it)
            return 0
        jax.lax.fori_loop(0, NSEG * NC // UNROLL, b_body, 0)
        return 0
    jax.lax.fori_loop(0, 2, layer_body, 0)

    for blk in range(NSEG):
        out_copy(blk).wait()


@jax.jit
def pallas_interleave_layers__memory_aug_infini_attn__mixer_s_mlp__prompt_kernel(
    A_x: jax.Array,
    A_wq: jax.Array,
    A_wk: jax.Array,
    A_wv: jax.Array,
    A_wo: jax.Array,
    A_beta: jax.Array,
    B_x: jax.Array,
    B_w1: jax.Array,
    B_w2: jax.Array,
    B_w3: jax.Array,
    B_w4: jax.Array,
):
    del B_x
    hbm = pl.BlockSpec(memory_space=pl.ANY)
    vm = pltpu.VMEM
    scratch = [
        vm((BIG_ROWS, D), bf16),
        vm((8, 256, D), bf16),
        vm((2, 4, D, 256), bf16),
        vm((2, D, DHALF), bf16),
        vm((2, DHALF, D), bf16),
        vm((D, D), bf16),
        vm((D, D), bf16),
        vm((F // FC, D, FC), bf16),
        vm((F, D), bf16),
        vm((BIG_ROWS, D), f32),
        vm((BIG_ROWS, D), f32),
        vm((PAD_ROWS, D), f32),
        vm((L, D), f32),
        vm((L, D), bf16),
        vm((S, D), bf16),
        vm((2, L, FC), bf16),
        vm((GH, 128, L), bf16),
        vm((GH, 128, L), bf16),
        vm((GH, L, 128), bf16),
        vm((GH, L, 128), bf16),
        vm((GH, 128, L), bf16),
        vm((GH, L, 128), bf16),
        vm((2, L // 2, 128), bf16),
        vm((GH, 128, L), f32),
        vm((2, GH, 128, 128), f32),
        vm((2, GH, 1, 128), f32),
        vm((2, H // 2, 128), f32),
        vm((128, 512), f32),
    ]
    scratch += [vm((2, 128 * (t + 1), 512), f32) for t in range(NT_TILES)]
    scratch += [vm((2, 1, 512), f32) for _ in range(NT_TILES)]
    scratch += [
        vm((S, D), bf16),
        pltpu.SemaphoreType.DMA((10,)),
        pltpu.SemaphoreType.DMA((8,)),
        pltpu.SemaphoreType.DMA((NSEG,)),
    ]
    return pl.pallas_call(
        _kernel,
        out_shape=jax.ShapeDtypeStruct((1, S, D), bf16),
        in_specs=[hbm, hbm, hbm, hbm, hbm, pl.BlockSpec(memory_space=pltpu.VMEM),
                  hbm, hbm, hbm, hbm],
        out_specs=hbm,
        scratch_shapes=scratch,
        compiler_params=pltpu.CompilerParams(vmem_limit_bytes=120 * 1024 * 1024),
    )(A_x, A_wq, A_wk, A_wv, A_wo, A_beta.reshape(1, H), B_w1, B_w2, B_w3, B_w4)
```

```python
import functools
import math

import jax
import jax.numpy as jnp
import jax.experimental.pallas as pl
import jax.experimental.pallas.tpu as pltpu

S = 2048
D = 1024
F = 3584
H = 32
DH = 32
L = 512
NSEG = S // L
NG = D // 128
NT_TILES = L // 128
FC = 256
HALO = 8
GH = NG // 2
DHALF = D // 2
PAD_ROWS = S + 2 * HALO
PIN = S + L + 2 * HALO
BIG_ROWS = PIN + 16 * NSEG
NC = F // FC
UNROLL = 4
SHIFTS = (1, -1, 2, -2)

LOG2E = math.log2(math.e)
QSCALE = DH ** -0.5 * LOG2E
MASK_BIAS = -1e9 * LOG2E
EPS = 1e-5

f32 = jnp.float32
bf16 = jnp.bfloat16
u32 = jnp.uint32
NT_DIMS = (((1,), (1,)), ((), ()))


def _stats(x):
    m = jnp.mean(x, axis=-1, keepdims=True)
    xc = x - m
    return m, jnp.mean(xc * xc, axis=-1, keepdims=True)


def _ln(x):
    m, v = _stats(x)
    r = jax.lax.rsqrt(v + EPS)
    return x * r - m * r


def _ln_ln(x):
    m, v = _stats(x)
    r1 = jax.lax.rsqrt(v + EPS)
    r2 = r1 * jax.lax.rsqrt(v * r1 * r1 + EPS)
    return r1, m * r1, x * r2 - m * r2


def _gelu(x):
    c = math.sqrt(2.0 / math.pi)
    inner = x * (c + (c * 0.044715) * (x * x))
    hx = 0.5 * x
    return hx + hx * jnp.tanh(inner)


def _phi(t):
    return jnp.where(t > 0, t + 1.0, jnp.exp(t))


def _red8(x, op):
    return functools.reduce(op, [x[i * 8:(i + 1) * 8] for i in range(x.shape[0] // 8)])


def _pack(x):
    return pltpu.bitcast(x.astype(bf16), u32)


def _unpack(x):
    return pltpu.bitcast(x, bf16)


def _hs(start, n):
    if isinstance(start, int):
        return slice(start // 2, (start + n) // 2)
    return pl.ds(pl.multiple_of(start // 2, 8), n // 2)


def _dot(a, b):
    return jnp.dot(a, b, preferred_element_type=f32)


def _dot_nt(a, b):
    return jax.lax.dot_general(a, b, NT_DIMS, preferred_element_type=f32)


def _kernel(x_hbm, wq_hbm, wk_hbm, wv_hbm, wo_hbm, beta_ref, w1_hbm, w2_hbm, w3_hbm, w4_hbm,
            out_hbm,
            xin, stage, wt, wk, wo, w1, w2, w3, w4,
            big, yres, hbuf, xna, xnb, xnc, gh, qt, pqt, kb, pkb, vt, ob, obl, amem,
            mt, zrow, gate, bias,
            s0, s1, s2, s3, m0, m1, m2, m3,
            obuf, sems, tsems, osems):
    sbuf = (s0, s1, s2, s3)
    mbuf = (m0, m1, m2, m3)

    def seg_rows(s):
        return pl.ds(s * L, L)

    cp_x0 = pltpu.make_async_copy(x_hbm.at[0, seg_rows(0)], xin.at[seg_rows(0)], sems.at[0])
    cp_xr = pltpu.make_async_copy(x_hbm.at[0, pl.ds(L, S - L)], xin.at[pl.ds(L, S - L)], sems.at[1])
    cp_wk = [pltpu.make_async_copy(wk_hbm.at[:, pl.ds(i * DHALF, DHALF)], wk.at[i], sems.at[2 + i])
             for i in range(2)]
    cp_wo = [pltpu.make_async_copy(wo_hbm.at[pl.ds(i * DHALF, DHALF)], wo.at[i], sems.at[4 + i])
             for i in range(2)]
    cp_w1 = pltpu.make_async_copy(w1_hbm, w1, sems.at[6])
    cp_w2 = pltpu.make_async_copy(w2_hbm, w2, sems.at[7])
    cp_w3 = [pltpu.make_async_copy(w3_hbm.at[:, pl.ds(c * FC, FC)], w3.at[c], sems.at[8])
             for c in range(F // FC)]
    cp_w4 = pltpu.make_async_copy(w4_hbm, w4, sems.at[9])

    TC = 256
    NTC = D // TC

    def cp_stage(i, c):
        src = (wq_hbm, wv_hbm)[i]
        return pltpu.make_async_copy(src.at[pl.ds(c * TC, TC)], stage.at[i * NTC + c],
                                     tsems.at[i * NTC + c])

    cp_x0.start()
    for i in range(2):
        for c in range(NTC):
            cp_stage(i, c).start()
    cp_wk[0].start()
    cp_wo[0].start()

    kk = jax.lax.broadcasted_iota(jnp.int32, (128, 512), 0)
    qq = jax.lax.broadcasted_iota(jnp.int32, (128, 512), 1) % 128
    bias[...] = jnp.where(kk > qq, MASK_BIAS, 0.0).astype(f32)
    bt = jnp.broadcast_to(beta_ref[...].astype(f32), (H, H))
    eye = (jax.lax.broadcasted_iota(jnp.int32, (H, H), 0)
           == jax.lax.broadcasted_iota(jnp.int32, (H, H), 1))
    bcol = jnp.sum(jnp.where(eye, bt, 0.0), axis=1, keepdims=True)
    gsig = jnp.broadcast_to(jax.nn.sigmoid(bcol), (H, 128))
    gate[0] = gsig[0:H // 2]
    gate[1] = gsig[H // 2:H]
    hbuf[0:2 * HALO, :] = jnp.zeros((2 * HALO, D), f32)
    hbuf[S:PAD_ROWS, :] = jnp.zeros((2 * HALO, D), f32)
    for ref in (big, yres):
        ref[0:HALO, :] = jnp.zeros((HALO, D), f32)
        ref[S + HALO:PAD_ROWS, :] = jnp.zeros((HALO, D), f32)

    ident = (jax.lax.broadcasted_iota(jnp.int32, (128, 128), 0)
             == jax.lax.broadcasted_iota(jnp.int32, (128, 128), 1)).astype(f32).astype(bf16)

    def transpose_chunk(ic, _):
        pltpu.make_async_copy(stage.at[ic], stage.at[ic], tsems.at[ic]).wait()
        i = ic // NTC
        c = ic % NTC
        ro = pl.multiple_of(i * DHALF, DHALF)
        for n in range(D // 128):
            tile = _dot_nt(ident, stage[ic, :, n * 128:(n + 1) * 128])
            wt[n // 4, c, _hs(ro + (n % 4) * 128, 128), :] = _pack(tile)
        return 0
    jax.lax.fori_loop(0, 2 * NTC, transpose_chunk, 0)

    cp_wk[1].start()
    cp_wo[1].start()
    cp_w1.start()
    cp_xr.start()
    cp_w2.start()
    cp_x0.wait()

    def init_x(i, _):
        r = pl.multiple_of(i * 256, 256)
        xv = xin[pl.ds(r, 256), :].astype(f32)
        big[pl.ds(HALO + r, 256), :] = xv
        xna[_hs(r, 256), :] = _pack(_ln(xv))
        return 0
    jax.lax.fori_loop(0, L // 256, init_x, 0)
    cp_wk[0].wait()
    cp_wo[0].wait()

    def qmask(g, t):
        z = jnp.zeros((DH, 128), bf16)
        cols = []
        for h in range(4):
            qh = _unpack(qt[g, _hs(h * DH, DH), t * 128:(t + 1) * 128])
            cols.append(jnp.concatenate([qh if i == h else z for i in range(4)], axis=0))
        return jnp.concatenate(cols, axis=1)

    def attn_step(half, g, gn, fill=()):
        pr = None if g is None else g % 2
        pw = None if gn is None else gn % 2
        fill = list(fill)
        for t in range(NT_TILES):
            macc = None
            oacc = [None] * 4
            lacc = [None] * 4
            for j in range(t + 1):
                ks = slice(j * 128, (j + 1) * 128)
                if fill and (t, j) != (0, 0):
                    fill.pop(0)()
                if gn is not None:
                    s = _dot(_unpack(kb[gn, _hs(j * 128, 128), :]), qmask(gn, t))
                    if j == t:
                        s = s + bias[...]
                    sbuf[t][pw, ks, :] = s
                    mx = _red8(s, jnp.maximum)
                    macc = mx if macc is None else jnp.maximum(macc, mx)
                if g is not None:
                    for h in range(4):
                        sl = slice(h * 128, (h + 1) * 128)
                        p = jnp.exp2(sbuf[t][pr, ks, sl] - mbuf[t][pr, :, sl])
                        lt = _red8(p, jnp.add)
                        lacc[h] = lt if lacc[h] is None else lacc[h] + lt
                        o = _dot(_unpack(vt[g, _hs(h * DH, DH), ks]), p.astype(bf16))
                        oacc[h] = o if oacc[h] is None else oacc[h] + o
            if gn is not None:
                mbuf[t][pw] = jnp.max(macc, axis=0, keepdims=True)
            if g is not None:
                parts = []
                for h in range(4):
                    l = jnp.sum(lacc[h], axis=0, keepdims=True)
                    gh = gate[half, g * 4 + h:g * 4 + h + 1, :]
                    parts.append(oacc[h] * ((1.0 - gh) / l))
                ot = jnp.concatenate(parts, axis=0) + amem[g, :, t * 128:(t + 1) * 128]
                if g < GH - 1 or t < 2:
                    ob[g, _hs(t * 128, 128), :] = _pack(ot.T)
                else:
                    obl[half, _hs((t - 2) * 128, 128), :] = _pack(ot.T)

    rowh = jax.lax.broadcasted_iota(jnp.int32, (128, 128), 0) // DH
    colh = jax.lax.broadcasted_iota(jnp.int32, (128, 128), 1) // DH
    row16 = jax.lax.broadcasted_iota(jnp.int32, (16, 128), 0)
    col16 = jax.lax.broadcasted_iota(jnp.int32, (16, 128), 1) // DH

    def attn_half(layer, seg, half):
        r0 = pl.multiple_of(seg * L, L)

        @pl.when(jnp.logical_and(jnp.logical_and(layer == 0, seg == 0), half == 1))
        def _():
            cp_wk[1].wait()
            cp_wo[1].wait()
            cp_w1.wait()
            cp_xr.wait()
            cp_w2.wait()
            for c in cp_w3:
                c.start()
            cp_w4.start()

        def xn(c0, nc):
            return _unpack(xna[_hs(c0 * 128, nc * 128), :])

        zparts = {}

        def k_piece(g0, ng, c0, nc):
            k = _dot(xn(c0, nc), wk[half, :, g0 * 128:(g0 + ng) * 128])
            pk = _phi(k)
            rs = _hs(c0 * 128, nc * 128)
            for i in range(ng):
                cs = slice(i * 128, (i + 1) * 128)
                kb[g0 + i, rs, :] = _pack(k[:, cs])
                pkb[g0 + i, rs, :] = _pack(pk[:, cs])
                zparts.setdefault(g0 + i, []).append(_red8(pk[:, cs], jnp.add))

        def qv_piece(qs, vs, c0, nc):
            offs = [g * 128 for g in qs] + [DHALF + g * 128 for g in vs]
            lhs = jnp.concatenate(
                [jnp.concatenate([wt[half, c, _hs(o, 128), :] for c in range(NTC)], axis=1)
                 for o in offs], axis=0)
            r = _dot_nt(_unpack(lhs), xn(c0, nc))
            ts = slice(c0 * 128, (c0 + nc) * 128)
            for i, g in enumerate(qs):
                qg = r[i * 128:(i + 1) * 128, :]
                qt[g, :, ts] = _pack(qg * QSCALE)
                pqt[g, :, ts] = _pack(_phi(qg))
            for i, g in enumerate(vs):
                o = (len(qs) + i) * 128
                vt[g, :, ts] = _pack(r[o:o + 128, :])

        def mem(g):
            zold = zrow[half, g]
            mold = mt[half, g]
            mbd = jnp.where(rowh == colh, mold, 0.0)
            zx = jnp.where(row16 == col16, jnp.broadcast_to(zold, (16, 128)), 0.0)
            lhs = jnp.concatenate([mbd, zx], axis=0).astype(bf16)
            ret = _dot(lhs, _unpack(pqt[g]))
            parts = []
            for h in range(4):
                gh = gate[half, g * 4 + h:g * 4 + h + 1, 0:1]
                den = ret[128 + h:129 + h, :] + 1e-6
                parts.append(ret[h * DH:(h + 1) * DH, :] * (gh / den))
            amem[g] = jnp.concatenate(parts, axis=0)
            mt[half, g] = mold + _dot(_unpack(vt[g]), _unpack(pkb[g]))
            zsum = functools.reduce(jnp.add, zparts[g])
            zrow[half, g] = zold + jnp.sum(zsum, axis=0, keepdims=True)

        P = functools.partial
        skip = lambda: None
        k_piece(0, 2, 0, 4)
        qv_piece((0, 1), (0,), 0, 4)
        attn_step(half, None, 0)
        mem(0)
        for g in range(2):
            attn_step(half, g, g + 1, fill=[
                P(k_piece, g + 2, 1, 0, 2), skip, P(qv_piece, (g + 2,), (g + 1,), 0, 1),
                P(qv_piece, (g + 2,), (g + 1,), 1, 1), skip, P(k_piece, g + 2, 1, 2, 2),
                P(qv_piece, (g + 2,), (g + 1,), 2, 1), P(qv_piece, (g + 2,), (g + 1,), 3, 1),
                P(mem, g + 1)])
        attn_step(half, 2, 3, fill=[
            skip, P(qv_piece, (), (3,), 0, 1), skip, P(qv_piece, (), (3,), 1, 1), skip,
            P(qv_piece, (), (3,), 2, 1), P(qv_piece, (), (3,), 3, 1), skip, P(mem, 3)])

        def wo_piece(t, n):
            off = t * 128
            cs = slice(n * DHALF, (n + 1) * DHALF)
            rr = pl.ds(r0 + (HALO + off), 128)
            ng = GH if t < 2 else GH - 1
            o = jnp.concatenate([ob[g, _hs(off, 128), :] for g in range(ng)], axis=1)
            big[rr, cs] = big[rr, cs] + _dot(_unpack(o), wo[half, 0:ng * 128, cs])

        attn_step(half, GH - 1, None,
                  fill=[P(wo_piece, t, n) for t in (2, 3, 0, 1) for n in range(2)])

    def phase_a(layer, seg):
        r0 = pl.multiple_of(seg * L, L)

        def half_body(half, _):
            attn_half(layer, seg, half)
            return 0
        jax.lax.fori_loop(0, 2, half_body, 0)

        hl = L // 2
        kp = (GH - 1) * 128

        bw = big.at[pl.ds(r0, 2 * L + 2 * HALO), :]
        yw = yres.at[pl.ds(r0, L + 2 * HALO), :]
        hw = hbuf.at[pl.ds(r0, L + 2 * HALO), :]
        xw = xin.at[pl.ds(r0 + L, L), :]

        def wo_rest():
            rr = slice(HALO + hl, HALO + L)
            o = _unpack(jnp.concatenate([obl[0], obl[1]], axis=1))
            w = jnp.concatenate([wo[0, kp:DHALF, :], wo[1, kp:DHALF, :]], axis=0)
            bw[rr, :] = bw[rr, :] + _dot(o, w)

        def lnln(off, n):
            rr = slice(HALO + off, HALO + off + n)
            r, mr, z = _ln_ln(bw[rr, :])
            yw[rr, D - 256:D - 128] = jnp.broadcast_to(r, (n, 128))
            yw[rr, D - 128:D] = jnp.broadcast_to(mr, (n, 128))
            xnb[_hs(off, n), :] = _pack(z)

        def corners(v):
            return [v[0:8, 0:128], v[hl - 8:hl, 0:128], v[0:8, 128:256], v[hl - 8:hl, 128:256]]

        def up(off, n):
            cs = slice(n * 256, (n + 1) * 256)
            hh = _gelu(_dot(_unpack(xnb[_hs(off, hl), :]), w1[:, cs]))
            b = off + HALO + SHIFTS[n]
            hw[b:b + hl, cs] = hh
            return corners(hh)

        sink = PIN + pl.multiple_of(seg * 16, 16)

        def pin(ref, v):
            if ref.dtype == bf16:
                ref[pl.ds(sink, 16), 0:128] = jnp.concatenate([v, v], axis=0).astype(bf16)
            else:
                ref[pl.ds(sink, 8), 0:128] = v

        fresh = jnp.logical_and(layer == 0, seg < NSEG - 1)

        def ln_next(off, n):
            rr = slice(L + HALO + off, L + HALO + off + n)
            xv = jnp.where(fresh, xw[off:off + n, :].astype(f32), bw[rr, :])
            bw[rr, :] = xv
            xna[_hs(off, n), :] = _pack(_ln(xv))

        lnln(0, 128)
        lnln(128, 128)
        wo_rest()
        def mix_part(off, n):
            return corners(mix(hw, yw, bw, slice(off, off + hl), n))

        def fence():
            pin(yres, pltpu.bitcast(xna[pl.ds(pl.multiple_of(seg * 8, 8), 8), 0:128], f32))

        late = list(range(hl, L, 16))
        nxt = list(range(0, L, 16))
        for n in range(4):
            marks = up(0, n)
            for i in (0, 1, 3):
                lnln(late.pop(0), 16)
                pin(big, marks[i])
        for n in range(4):
            marks = mix_part(0, n)
            for i in range(4):
                if late:
                    lnln(late.pop(0), 16)
                else:
                    ln_next(nxt.pop(0), 16)
                if n > 0 or i == 3:
                    pin(xin, marks[i])
        for n in range(4):
            marks = up(hl, n)
            for i in (0, 1, 3):
                ln_next(nxt.pop(0), 16)
                pin(xin, marks[i])
        for n in range(4):
            if n == 3:
                fence()
            marks = mix_part(hl, n)
            for i in range(4):
                if nxt:
                    ln_next(nxt.pop(0), 16)
                    pin(xin, marks[i])

    def mix(h_ref, y_ref, x_ref, rr, n):
        cs = slice(n * 256, (n + 1) * 256)
        r = y_ref[rr, D - 256:D - 128]
        mr = y_ref[rr, D - 128:D]
        x = x_ref[rr, cs]
        y = x * jnp.concatenate([r, r], axis=1) - jnp.concatenate([mr, mr], axis=1)
        x1 = y + _dot(h_ref[rr, :].astype(bf16), w2[:, cs])
        y_ref[rr, cs] = x1
        x_ref[rr, cs] = x + x1
        return x1

    def ln_mid(tok, n):
        xnc[_hs(tok, n), :] = _pack(_ln(yres[pl.ds(tok + HALO, n), :]))

    def last_rows():
        for n in range(4):
            mix(hbuf, yres, big, slice(S, PAD_ROWS), n)
            ln_mid(n * 128, 128)

    def out_copy(blk):
        rows = pl.ds(blk * L, L)
        return pltpu.make_async_copy(obuf.at[rows], out_hbm.at[0, rows, :], osems.at[blk])

    def ffn(layer, it):
        blk = [(UNROLL * it + k) // NC for k in range(UNROLL)]
        chunk = [(UNROLL * it + k) % NC for k in range(UNROLL)]
        tok = [pl.multiple_of(b * L, L) for b in blk]

        def ffn_up(k):
            hh = _gelu(_dot(_unpack(xnc[_hs(tok[k], L), :]), w3[chunk[k]]))
            gh[k % 2] = _pack(hh)
            return hh[L - 8:L, FC - 128:FC]

        def ffn_down(k):
            rows = pl.ds(tok[k] + HALO, L)
            w = w4[pl.ds(pl.multiple_of(chunk[k] * FC, FC), FC), :]
            big[rows, :] = big[rows, :] + _dot(_unpack(gh[k % 2]), w)

        def ln_ahead(k, mark):
            yres[pl.ds(PIN + pl.multiple_of(blk[0] * 16, 16), 8), 0:128] = mark
            nb = jnp.minimum(blk[k] + 1, NSEG - 1)
            ln_mid(pl.multiple_of(nb * L + jnp.minimum(chunk[k] * 40, L - 80), 16), 80)

        def ln_first():
            r = pl.multiple_of(jnp.clip((it - 4) * 64, 0, L - 64), 64)
            xna[_hs(r, 64), :] = _pack(_ln(big[pl.ds(r + HALO, 64), :]))

        ffn_up(0)
        ln_ahead(0, ffn_up(1))
        ffn_down(0)
        ln_ahead(2, ffn_up(2))
        ffn_down(1)
        ln_first()
        ffn_up(3)
        ffn_down(2)
        ffn_down(3)

        done = (UNROLL * it + UNROLL) // NC

        @pl.when(jnp.logical_and(layer == 1, done != blk[0]))
        def _():
            r = pl.multiple_of((done - 1) * L, L)
            obuf[pl.ds(r, L), :] = big[pl.ds(r + HALO, L), :].astype(bf16)
            out_copy(done - 1).start()

    def layer_body(layer, _):
        mt[...] = jnp.zeros(mt.shape, f32)
        zrow[...] = jnp.zeros(zrow.shape, f32)

        def a_body(seg, _):
            phase_a(layer, seg)
            return 0
        jax.lax.fori_loop(0, NSEG, a_body, 0)

        last_rows()

        @pl.when(layer == 0)
        def _():
            for c in cp_w3:
                c.wait()
            cp_w4.wait()

        def b_body(it, _):
            ffn(layer, it)
            return 0
        jax.lax.fori_loop(0, NSEG * NC // UNROLL, b_body, 0)
        return 0
    jax.lax.fori_loop(0, 2, layer_body, 0)

    for blk in range(NSEG):
        out_copy(blk).wait()


@jax.jit
def pallas_interleave_layers__memory_aug_infini_attn__mixer_s_mlp__prompt_kernel(
    A_x: jax.Array,
    A_wq: jax.Array,
    A_wk: jax.Array,
    A_wv: jax.Array,
    A_wo: jax.Array,
    A_beta: jax.Array,
    B_x: jax.Array,
    B_w1: jax.Array,
    B_w2: jax.Array,
    B_w3: jax.Array,
    B_w4: jax.Array,
):
    del B_x
    hbm = pl.BlockSpec(memory_space=pl.ANY)
    vm = pltpu.VMEM
    scratch = [
        vm((BIG_ROWS, D), bf16),
        vm((8, 256, D), bf16),
        vm((2, 4, D // 2, 256), u32),
        vm((2, D, DHALF), bf16),
        vm((2, DHALF, D), bf16),
        vm((D, D), bf16),
        vm((D, D), bf16),
        vm((F // FC, D, FC), bf16),
        vm((F, D), bf16),
        vm((BIG_ROWS, D), f32),
        vm((BIG_ROWS, D), f32),
        vm((PAD_ROWS, D), f32),
        vm((L // 2, D), u32),
        vm((L // 2, D), u32),
        vm((S // 2, D), u32),
        vm((2, L // 2, FC), u32),
        vm((GH, 64, L), u32),
        vm((GH, 64, L), u32),
        vm((GH, L // 2, 128), u32),
        vm((GH, L // 2, 128), u32),
        vm((GH, 64, L), u32),
        vm((GH, L // 2, 128), u32),
        vm((2, L // 4, 128), u32),
        vm((GH, 128, L), f32),
        vm((2, GH, 128, 128), f32),
        vm((2, GH, 1, 128), f32),
        vm((2, H // 2, 128), f32),
        vm((128, 512), f32),
    ]
    scratch += [vm((2, 128 * (t + 1), 512), f32) for t in range(NT_TILES)]
    scratch += [vm((2, 1, 512), f32) for _ in range(NT_TILES)]
    scratch += [
        vm((S, D), bf16),
        pltpu.SemaphoreType.DMA((10,)),
        pltpu.SemaphoreType.DMA((8,)),
        pltpu.SemaphoreType.DMA((NSEG,)),
    ]
    return pl.pallas_call(
        _kernel,
        out_shape=jax.ShapeDtypeStruct((1, S, D), bf16),
        in_specs=[hbm, hbm, hbm, hbm, hbm, pl.BlockSpec(memory_space=pltpu.VMEM),
                  hbm, hbm, hbm, hbm],
        out_specs=hbm,
        scratch_shapes=scratch,
        compiler_params=pltpu.CompilerParams(vmem_limit_bytes=120 * 1024 * 1024),
    )(A_x, A_wq, A_wk, A_wv, A_wo, A_beta.reshape(1, H), B_w1, B_w2, B_w3, B_w4)
```

```python
import functools
import math

import jax
import jax.numpy as jnp
import jax.experimental.pallas as pl
import jax.experimental.pallas.tpu as pltpu

S = 2048
D = 1024
F = 3584
H = 32
DH = 32
L = 512
NSEG = S // L
NG = D // 128
NT_TILES = L // 128
FC = 256
HALO = 8
GH = NG // 2
DHALF = D // 2
PAD_ROWS = S + 2 * HALO
PIN = S + L + 2 * HALO
BIG_ROWS = PIN + 16 * NSEG
NC = F // FC
UNROLL = 4
SHIFTS = (1, -1, 2, -2)

LOG2E = math.log2(math.e)
QSCALE = DH ** -0.5 * LOG2E
MASK_BIAS = -1e9 * LOG2E
EPS = 1e-5

f32 = jnp.float32
bf16 = jnp.bfloat16
u32 = jnp.uint32
NT_DIMS = (((1,), (1,)), ((), ()))


def _stats(x):
    m = jnp.mean(x, axis=-1, keepdims=True)
    xc = x - m
    return m, jnp.mean(xc * xc, axis=-1, keepdims=True)


def _ln(x):
    m, v = _stats(x)
    r = jax.lax.rsqrt(v + EPS)
    return x * r - m * r


def _ln_ln(x):
    m, v = _stats(x)
    r1 = jax.lax.rsqrt(v + EPS)
    r2 = r1 * jax.lax.rsqrt(v * r1 * r1 + EPS)
    return r1, m * r1, x * r2 - m * r2


def _gelu(x):
    c = math.sqrt(2.0 / math.pi)
    inner = x * (c + (c * 0.044715) * (x * x))
    hx = 0.5 * x
    return hx + hx * jnp.tanh(inner)


def _phi(t):
    return jnp.where(t > 0, t + 1.0, jnp.exp(t))


def _red8(x, op):
    return functools.reduce(op, [x[i * 8:(i + 1) * 8] for i in range(x.shape[0] // 8)])


def _pack(x):
    return pltpu.bitcast(x.astype(bf16), u32)


def _unpack(x):
    return pltpu.bitcast(x, bf16)


def _hs(start, n):
    if isinstance(start, int):
        return slice(start // 2, (start + n) // 2)
    return pl.ds(pl.multiple_of(start // 2, 8), n // 2)


def _dot(a, b):
    return jnp.dot(a, b, preferred_element_type=f32)


def _dot_nt(a, b):
    return jax.lax.dot_general(a, b, NT_DIMS, preferred_element_type=f32)


def _kernel(x_hbm, wq_hbm, wk_hbm, wv_hbm, wo_hbm, beta_ref, w1_hbm, w2_hbm, w3_hbm, w4_hbm,
            out_hbm,
            xin, stage, wt, wk, wo, w1, w2, w3, w4,
            big, yres, hbuf, xna, xnb, xnc, gh, qt, pqt, kb, pkb, vt, ob, obl, amem,
            mt, zrow, gate, bias,
            s0, s1, s2, s3, m0, m1, m2, m3,
            obuf, sems, tsems, osems):
    sbuf = (s0, s1, s2, s3)
    mbuf = (m0, m1, m2, m3)

    def seg_rows(s):
        return pl.ds(s * L, L)

    cp_x0 = pltpu.make_async_copy(x_hbm.at[0, seg_rows(0)], xin.at[seg_rows(0)], sems.at[0])
    cp_xr = pltpu.make_async_copy(x_hbm.at[0, pl.ds(L, S - L)], xin.at[pl.ds(L, S - L)], sems.at[1])
    cp_wk = [pltpu.make_async_copy(wk_hbm.at[:, pl.ds(i * DHALF, DHALF)], wk.at[i].bitcast(bf16),
                                   sems.at[2 + i])
             for i in range(2)]
    cp_wo = [pltpu.make_async_copy(wo_hbm.at[pl.ds(i * DHALF, DHALF)], wo.at[i].bitcast(bf16),
                                   sems.at[4 + i])
             for i in range(2)]
    cp_w1 = pltpu.make_async_copy(w1_hbm, w1.bitcast(bf16), sems.at[6])
    cp_w2 = pltpu.make_async_copy(w2_hbm, w2.bitcast(bf16), sems.at[7])
    cp_w3 = [pltpu.make_async_copy(w3_hbm.at[:, pl.ds(c * FC, FC)], w3.at[c].bitcast(bf16),
                                   sems.at[8])
             for c in range(F // FC)]
    cp_w4 = pltpu.make_async_copy(w4_hbm, w4.bitcast(bf16), sems.at[9])

    TC = 256
    NTC = D // TC

    def cp_stage(i, c):
        src = (wq_hbm, wv_hbm)[i]
        return pltpu.make_async_copy(src.at[pl.ds(c * TC, TC)], stage.at[i * NTC + c],
                                     tsems.at[i * NTC + c])

    cp_x0.start()
    for i in range(2):
        for c in range(NTC):
            cp_stage(i, c).start()
    cp_wk[0].start()
    cp_wo[0].start()

    kk = jax.lax.broadcasted_iota(jnp.int32, (128, 512), 0)
    qq = jax.lax.broadcasted_iota(jnp.int32, (128, 512), 1) % 128
    bias[...] = jnp.where(kk > qq, MASK_BIAS, 0.0).astype(f32)
    bt = jnp.broadcast_to(beta_ref[...].astype(f32), (H, H))
    eye = (jax.lax.broadcasted_iota(jnp.int32, (H, H), 0)
           == jax.lax.broadcasted_iota(jnp.int32, (H, H), 1))
    bcol = jnp.sum(jnp.where(eye, bt, 0.0), axis=1, keepdims=True)
    gsig = jnp.broadcast_to(jax.nn.sigmoid(bcol), (H, 128))
    gate[0] = gsig[0:H // 2]
    gate[1] = gsig[H // 2:H]
    hbuf[0:2 * HALO, :] = jnp.zeros((2 * HALO, D), f32)
    hbuf[S:PAD_ROWS, :] = jnp.zeros((2 * HALO, D), f32)
    for ref in (big, yres):
        ref[0:HALO, :] = jnp.zeros((HALO, D), f32)
        ref[S + HALO:PAD_ROWS, :] = jnp.zeros((HALO, D), f32)

    ident = (jax.lax.broadcasted_iota(jnp.int32, (128, 128), 0)
             == jax.lax.broadcasted_iota(jnp.int32, (128, 128), 1)).astype(f32).astype(bf16)

    def transpose_chunk(ic, _):
        pltpu.make_async_copy(stage.at[ic], stage.at[ic], tsems.at[ic]).wait()
        i = ic // NTC
        c = ic % NTC
        ro = pl.multiple_of(i * DHALF, DHALF)
        for n in range(D // 128):
            tile = _dot_nt(ident, stage[ic, :, n * 128:(n + 1) * 128])
            wt[n // 4, c, _hs(ro + (n % 4) * 128, 128), :] = _pack(tile)
        return 0
    jax.lax.fori_loop(0, 2 * NTC, transpose_chunk, 0)

    cp_wk[1].start()
    cp_wo[1].start()
    cp_w1.start()
    cp_xr.start()
    cp_w2.start()
    cp_x0.wait()

    def init_x(i, _):
        r = pl.multiple_of(i * 256, 256)
        xv = xin[pl.ds(r, 256), :].astype(f32)
        big[pl.ds(HALO + r, 256), :] = xv
        xna[_hs(r, 256), :] = _pack(_ln(xv))
        return 0
    jax.lax.fori_loop(0, L // 256, init_x, 0)
    cp_wk[0].wait()
    cp_wo[0].wait()

    def qmask(g, t):
        z = jnp.zeros((DH, 128), bf16)
        cols = []
        for h in range(4):
            qh = _unpack(qt[g, _hs(h * DH, DH), t * 128:(t + 1) * 128])
            cols.append(jnp.concatenate([qh if i == h else z for i in range(4)], axis=0))
        return jnp.concatenate(cols, axis=1)

    def attn_step(half, g, gn, fill=()):
        pr = None if g is None else g % 2
        pw = None if gn is None else gn % 2
        fill = list(fill)
        for t in range(NT_TILES):
            macc = None
            oacc = [None] * 4
            lacc = [None] * 4
            for j in range(t + 1):
                ks = slice(j * 128, (j + 1) * 128)
                if fill and (t, j) != (0, 0):
                    fill.pop(0)()
                if gn is not None:
                    s = _dot(_unpack(kb[gn, _hs(j * 128, 128), :]), qmask(gn, t))
                    if j == t:
                        s = s + bias[...]
                    sbuf[t][pw, ks, :] = s
                    mx = _red8(s, jnp.maximum)
                    macc = mx if macc is None else jnp.maximum(macc, mx)
                if g is not None:
                    for h in range(4):
                        sl = slice(h * 128, (h + 1) * 128)
                        p = jnp.exp2(sbuf[t][pr, ks, sl] - mbuf[t][pr, :, sl])
                        lt = _red8(p, jnp.add)
                        lacc[h] = lt if lacc[h] is None else lacc[h] + lt
                        o = _dot(_unpack(vt[g, _hs(h * DH, DH), ks]), p.astype(bf16))
                        oacc[h] = o if oacc[h] is None else oacc[h] + o
            if gn is not None:
                mbuf[t][pw] = jnp.max(macc, axis=0, keepdims=True)
            if g is not None:
                parts = []
                for h in range(4):
                    l = jnp.sum(lacc[h], axis=0, keepdims=True)
                    gh = gate[half, g * 4 + h:g * 4 + h + 1, :]
                    parts.append(oacc[h] * ((1.0 - gh) / l))
                ot = jnp.concatenate(parts, axis=0) + amem[g, :, t * 128:(t + 1) * 128]
                if g < GH - 1 or t < 2:
                    ob[g, _hs(t * 128, 128), :] = _pack(ot.T)
                else:
                    obl[half, _hs((t - 2) * 128, 128), :] = _pack(ot.T)

    rowh = jax.lax.broadcasted_iota(jnp.int32, (128, 128), 0) // DH
    colh = jax.lax.broadcasted_iota(jnp.int32, (128, 128), 1) // DH
    row16 = jax.lax.broadcasted_iota(jnp.int32, (16, 128), 0)
    col16 = jax.lax.broadcasted_iota(jnp.int32, (16, 128), 1) // DH

    def attn_half(layer, seg, half):
        r0 = pl.multiple_of(seg * L, L)

        @pl.when(jnp.logical_and(jnp.logical_and(layer == 0, seg == 0), half == 1))
        def _():
            cp_wk[1].wait()
            cp_wo[1].wait()
            cp_w1.wait()
            cp_xr.wait()
            cp_w2.wait()
            for c in cp_w3:
                c.start()
            cp_w4.start()

        def xn(c0, nc):
            return _unpack(xna[_hs(c0 * 128, nc * 128), :])

        zparts = {}

        def k_piece(g0, ng, c0, nc):
            k = _dot(xn(c0, nc), _unpack(wk[half, :, g0 * 128:(g0 + ng) * 128]))
            pk = _phi(k)
            rs = _hs(c0 * 128, nc * 128)
            for i in range(ng):
                cs = slice(i * 128, (i + 1) * 128)
                kb[g0 + i, rs, :] = _pack(k[:, cs])
                pkb[g0 + i, rs, :] = _pack(pk[:, cs])
                zparts.setdefault(g0 + i, []).append(_red8(pk[:, cs], jnp.add))

        def qv_piece(qs, vs, c0, nc):
            offs = [g * 128 for g in qs] + [DHALF + g * 128 for g in vs]
            lhs = jnp.concatenate(
                [jnp.concatenate([wt[half, c, _hs(o, 128), :] for c in range(NTC)], axis=1)
                 for o in offs], axis=0)
            r = _dot_nt(_unpack(lhs), xn(c0, nc))
            ts = slice(c0 * 128, (c0 + nc) * 128)
            for i, g in enumerate(qs):
                qg = r[i * 128:(i + 1) * 128, :]
                qt[g, :, ts] = _pack(qg * QSCALE)
                pqt[g, :, ts] = _pack(_phi(qg))
            for i, g in enumerate(vs):
                o = (len(qs) + i) * 128
                vt[g, :, ts] = _pack(r[o:o + 128, :])

        def mem(g):
            zold = zrow[half, g]
            mold = mt[half, g]
            mbd = jnp.where(rowh == colh, mold, 0.0)
            zx = jnp.where(row16 == col16, jnp.broadcast_to(zold, (16, 128)), 0.0)
            lhs = jnp.concatenate([mbd, zx], axis=0).astype(bf16)
            ret = _dot(lhs, _unpack(pqt[g]))
            parts = []
            for h in range(4):
                gh = gate[half, g * 4 + h:g * 4 + h + 1, 0:1]
                den = ret[128 + h:129 + h, :] + 1e-6
                parts.append(ret[h * DH:(h + 1) * DH, :] * (gh / den))
            amem[g] = jnp.concatenate(parts, axis=0)
            mt[half, g] = mold + _dot(_unpack(vt[g]), _unpack(pkb[g]))
            zsum = functools.reduce(jnp.add, zparts[g])
            zrow[half, g] = zold + jnp.sum(zsum, axis=0, keepdims=True)

        P = functools.partial
        skip = lambda: None
        k_piece(0, 2, 0, 4)
        qv_piece((0, 1), (0,), 0, 4)
        attn_step(half, None, 0)
        mem(0)
        for g in range(2):
            attn_step(half, g, g + 1, fill=[
                P(k_piece, g + 2, 1, 0, 2), skip, P(qv_piece, (g + 2,), (g + 1,), 0, 1),
                P(qv_piece, (g + 2,), (g + 1,), 1, 1), skip, P(k_piece, g + 2, 1, 2, 2),
                P(qv_piece, (g + 2,), (g + 1,), 2, 1), P(qv_piece, (g + 2,), (g + 1,), 3, 1),
                P(mem, g + 1)])
        attn_step(half, 2, 3, fill=[
            skip, P(qv_piece, (), (3,), 0, 1), skip, P(qv_piece, (), (3,), 1, 1), skip,
            P(qv_piece, (), (3,), 2, 1), P(qv_piece, (), (3,), 3, 1), skip, P(mem, 3)])

        def wo_piece(t, n):
            off = t * 128
            cs = slice(n * DHALF, (n + 1) * DHALF)
            rr = pl.ds(r0 + (HALO + off), 128)
            ng = GH if t < 2 else GH - 1
            o = jnp.concatenate([ob[g, _hs(off, 128), :] for g in range(ng)], axis=1)
            big[rr, cs] = big[rr, cs] + _dot(_unpack(o), _unpack(wo[half, _hs(0, ng * 128), cs]))

        attn_step(half, GH - 1, None,
                  fill=[P(wo_piece, t, n) for t in (2, 3, 0, 1) for n in range(2)])

    def phase_a(layer, seg):
        r0 = pl.multiple_of(seg * L, L)

        def half_body(half, _):
            attn_half(layer, seg, half)
            return 0
        jax.lax.fori_loop(0, 2, half_body, 0)

        hl = L // 2
        kp = (GH - 1) * 128

        bw = big.at[pl.ds(r0, 2 * L + 2 * HALO), :]
        yw = yres.at[pl.ds(r0, L + 2 * HALO), :]
        hw = hbuf.at[pl.ds(r0, L + 2 * HALO), :]
        xw = xin.at[pl.ds(r0 + L, L), :]

        def wo_rest():
            rr = slice(HALO + hl, HALO + L)
            o = _unpack(jnp.concatenate([obl[0], obl[1]], axis=1))
            w = _unpack(jnp.concatenate([wo[i, _hs(kp, 128), :] for i in range(2)], axis=0))
            bw[rr, :] = bw[rr, :] + _dot(o, w)

        def lnln(off, n):
            rr = slice(HALO + off, HALO + off + n)
            r, mr, z = _ln_ln(bw[rr, :])
            yw[rr, D - 256:D - 128] = jnp.broadcast_to(r, (n, 128))
            yw[rr, D - 128:D] = jnp.broadcast_to(mr, (n, 128))
            xnb[_hs(off, n), :] = _pack(z)

        def corners(v):
            return [v[0:8, 0:128], v[hl - 8:hl, 0:128], v[0:8, 128:256], v[hl - 8:hl, 128:256]]

        def up(off, n):
            cs = slice(n * 256, (n + 1) * 256)
            hh = _gelu(_dot(_unpack(xnb[_hs(off, hl), :]), _unpack(w1[:, cs])))
            b = off + HALO + SHIFTS[n]
            hw[b:b + hl, cs] = hh
            return corners(hh)

        sink = PIN + pl.multiple_of(seg * 16, 16)

        def pin(ref, v):
            if ref.dtype == bf16:
                ref[pl.ds(sink, 16), 0:128] = jnp.concatenate([v, v], axis=0).astype(bf16)
            else:
                ref[pl.ds(sink, 8), 0:128] = v

        fresh = jnp.logical_and(layer == 0, seg < NSEG - 1)

        def ln_next(off, n):
            rr = slice(L + HALO + off, L + HALO + off + n)
            xv = jnp.where(fresh, xw[off:off + n, :].astype(f32), bw[rr, :])
            bw[rr, :] = xv
            xna[_hs(off, n), :] = _pack(_ln(xv))

        lnln(0, 128)
        lnln(128, 128)
        wo_rest()
        def mix_part(off, n):
            return corners(mix(hw, yw, bw, slice(off, off + hl), n))

        def fence():
            pin(yres, pltpu.bitcast(xna[pl.ds(pl.multiple_of(seg * 8, 8), 8), 0:128], f32))

        late = list(range(hl, L, 16))
        nxt = list(range(0, L, 16))
        for n in range(4):
            marks = up(0, n)
            for i in (0, 1, 3):
                lnln(late.pop(0), 16)
                pin(big, marks[i])
        for n in range(4):
            marks = mix_part(0, n)
            for i in range(4):
                if late:
                    lnln(late.pop(0), 16)
                else:
                    ln_next(nxt.pop(0), 16)
                if n > 0 or i == 3:
                    pin(xin, marks[i])
        for n in range(4):
            marks = up(hl, n)
            for i in (0, 1, 3):
                ln_next(nxt.pop(0), 16)
                pin(xin, marks[i])
        for n in range(4):
            if n == 3:
                fence()
            marks = mix_part(hl, n)
            for i in range(4):
                if nxt:
                    ln_next(nxt.pop(0), 16)
                    pin(xin, marks[i])

    def mix(h_ref, y_ref, x_ref, rr, n):
        cs = slice(n * 256, (n + 1) * 256)
        r = y_ref[rr, D - 256:D - 128]
        mr = y_ref[rr, D - 128:D]
        x = x_ref[rr, cs]
        y = x * jnp.concatenate([r, r], axis=1) - jnp.concatenate([mr, mr], axis=1)
        x1 = y + _dot(h_ref[rr, :].astype(bf16), _unpack(w2[:, cs]))
        y_ref[rr, cs] = x1
        x_ref[rr, cs] = x + x1
        return x1

    def ln_mid(tok, n):
        xnc[_hs(tok, n), :] = _pack(_ln(yres[pl.ds(tok + HALO, n), :]))

    def last_rows():
        for n in range(4):
            mix(hbuf, yres, big, slice(S, PAD_ROWS), n)
            ln_mid(n * 128, 128)

    def out_copy(blk):
        rows = pl.ds(blk * L, L)
        return pltpu.make_async_copy(obuf.at[rows], out_hbm.at[0, rows, :], osems.at[blk])

    def ffn(layer, it):
        blk = [(UNROLL * it + k) // NC for k in range(UNROLL)]
        chunk = [(UNROLL * it + k) % NC for k in range(UNROLL)]
        tok = [pl.multiple_of(b * L, L) for b in blk]

        def ffn_up(k):
            hh = _gelu(_dot(_unpack(xnc[_hs(tok[k], L), :]), _unpack(w3[chunk[k]])))
            gh[k % 2] = _pack(hh)
            return hh[L - 8:L, FC - 128:FC]

        def ffn_down(k):
            rows = pl.ds(tok[k] + HALO, L)
            w = _unpack(w4[_hs(chunk[k] * FC, FC), :])
            big[rows, :] = big[rows, :] + _dot(_unpack(gh[k % 2]), w)

        def ln_ahead(k, mark):
            yres[pl.ds(PIN + pl.multiple_of(blk[0] * 16, 16), 8), 0:128] = mark
            nb = jnp.minimum(blk[k] + 1, NSEG - 1)
            ln_mid(pl.multiple_of(nb * L + jnp.minimum(chunk[k] * 40, L - 80), 16), 80)

        def ln_first():
            r = pl.multiple_of(jnp.clip((it - 4) * 64, 0, L - 64), 64)
            xna[_hs(r, 64), :] = _pack(_ln(big[pl.ds(r + HALO, 64), :]))

        ffn_up(0)
        ln_ahead(0, ffn_up(1))
        ffn_down(0)
        ln_ahead(2, ffn_up(2))
        ffn_down(1)
        ln_first()
        ffn_up(3)
        ffn_down(2)
        ffn_down(3)

        done = (UNROLL * it + UNROLL) // NC

        @pl.when(jnp.logical_and(layer == 1, done != blk[0]))
        def _():
            r = pl.multiple_of((done - 1) * L, L)
            obuf[pl.ds(r, L), :] = big[pl.ds(r + HALO, L), :].astype(bf16)
            out_copy(done - 1).start()

    def layer_body(layer, _):
        mt[...] = jnp.zeros(mt.shape, f32)
        zrow[...] = jnp.zeros(zrow.shape, f32)

        def a_body(seg, _):
            phase_a(layer, seg)
            return 0
        jax.lax.fori_loop(0, NSEG, a_body, 0)

        last_rows()

        @pl.when(layer == 0)
        def _():
            for c in cp_w3:
                c.wait()
            cp_w4.wait()

        def b_body(it, _):
            ffn(layer, it)
            return 0
        jax.lax.fori_loop(0, NSEG * NC // UNROLL, b_body, 0)
        return 0
    jax.lax.fori_loop(0, 2, layer_body, 0)

    for blk in range(NSEG):
        out_copy(blk).wait()


@jax.jit
def pallas_interleave_layers__memory_aug_infini_attn__mixer_s_mlp__prompt_kernel(
    A_x: jax.Array,
    A_wq: jax.Array,
    A_wk: jax.Array,
    A_wv: jax.Array,
    A_wo: jax.Array,
    A_beta: jax.Array,
    B_x: jax.Array,
    B_w1: jax.Array,
    B_w2: jax.Array,
    B_w3: jax.Array,
    B_w4: jax.Array,
):
    del B_x
    hbm = pl.BlockSpec(memory_space=pl.ANY)
    vm = pltpu.VMEM
    scratch = [
        vm((BIG_ROWS, D), bf16),
        vm((8, 256, D), bf16),
        vm((2, 4, D // 2, 256), u32),
        vm((2, D // 2, DHALF), u32),
        vm((2, DHALF // 2, D), u32),
        vm((D // 2, D), u32),
        vm((D // 2, D), u32),
        vm((NC, D // 2, FC), u32),
        vm((F // 2, D), u32),
        vm((BIG_ROWS, D), f32),
        vm((BIG_ROWS, D), f32),
        vm((PAD_ROWS, D), f32),
        vm((L // 2, D), u32),
        vm((L // 2, D), u32),
        vm((S // 2, D), u32),
        vm((2, L // 2, FC), u32),
        vm((GH, 64, L), u32),
        vm((GH, 64, L), u32),
        vm((GH, L // 2, 128), u32),
        vm((GH, L // 2, 128), u32),
        vm((GH, 64, L), u32),
        vm((GH, L // 2, 128), u32),
        vm((2, L // 4, 128), u32),
        vm((GH, 128, L), f32),
        vm((2, GH, 128, 128), f32),
        vm((2, GH, 1, 128), f32),
        vm((2, H // 2, 128), f32),
        vm((128, 512), f32),
    ]
    scratch += [vm((2, 128 * (t + 1), 512), f32) for t in range(NT_TILES)]
    scratch += [vm((2, 1, 512), f32) for _ in range(NT_TILES)]
    scratch += [
        vm((S, D), bf16),
        pltpu.SemaphoreType.DMA((10,)),
        pltpu.SemaphoreType.DMA((8,)),
        pltpu.SemaphoreType.DMA((NSEG,)),
    ]
    return pl.pallas_call(
        _kernel,
        out_shape=jax.ShapeDtypeStruct((1, S, D), bf16),
        in_specs=[hbm, hbm, hbm, hbm, hbm, pl.BlockSpec(memory_space=pltpu.VMEM),
                  hbm, hbm, hbm, hbm],
        out_specs=hbm,
        scratch_shapes=scratch,
        compiler_params=pltpu.CompilerParams(vmem_limit_bytes=120 * 1024 * 1024),
    )(A_x, A_wq, A_wk, A_wv, A_wo, A_beta.reshape(1, H), B_w1, B_w2, B_w3, B_w4)
```

```python
import functools
import math

import jax
import jax.numpy as jnp
import jax.experimental.pallas as pl
import jax.experimental.pallas.tpu as pltpu

S = 2048
D = 1024
F = 3584
H = 32
DH = 32
L = 512
NSEG = S // L
NG = D // 128
NT_TILES = L // 128
FC = 256
HALO = 8
GH = NG // 2
DHALF = D // 2
PAD_ROWS = S + 2 * HALO
PIN = S + L + 2 * HALO
BIG_ROWS = PIN + 16 * NSEG
NC = F // FC
UNROLL = 4
SHIFTS = (1, -1, 2, -2)

LOG2E = math.log2(math.e)
QSCALE = DH ** -0.5 * LOG2E
MASK_BIAS = -1e9 * LOG2E
EPS = 1e-5

f32 = jnp.float32
bf16 = jnp.bfloat16
u32 = jnp.uint32
NT_DIMS = (((1,), (1,)), ((), ()))


def _stats(x):
    m = jnp.mean(x, axis=-1, keepdims=True)
    xc = x - m
    return m, jnp.mean(xc * xc, axis=-1, keepdims=True)


def _ln(x):
    m, v = _stats(x)
    r = jax.lax.rsqrt(v + EPS)
    return x * r - m * r


def _ln_ln(x):
    m, v = _stats(x)
    r1 = jax.lax.rsqrt(v + EPS)
    r2 = r1 * jax.lax.rsqrt(v * r1 * r1 + EPS)
    return r1, m * r1, x * r2 - m * r2


def _gelu(x):
    c = math.sqrt(2.0 / math.pi)
    inner = x * (c + (c * 0.044715) * (x * x))
    hx = 0.5 * x
    return hx + hx * jnp.tanh(inner)


def _phi(t):
    return jnp.where(t > 0, t + 1.0, jnp.exp(t))


def _red8(x, op):
    return functools.reduce(op, [x[i * 8:(i + 1) * 8] for i in range(x.shape[0] // 8)])


def _pack(x):
    return pltpu.bitcast(x.astype(bf16), u32)


def _unpack(x):
    return pltpu.bitcast(x, bf16)


def _hs(start, n):
    if isinstance(start, int):
        return slice(start // 2, (start + n) // 2)
    return pl.ds(pl.multiple_of(start >> 1, 8), n // 2)


def _dot(a, b):
    return jnp.dot(a, b, preferred_element_type=f32)


def _dot_nt(a, b):
    return jax.lax.dot_general(a, b, NT_DIMS, preferred_element_type=f32)


def _kernel(x_hbm, wq_hbm, wk_hbm, wv_hbm, wo_hbm, beta_ref, w1_hbm, w2_hbm, w3_hbm, w4_hbm,
            out_hbm,
            xin, stage, wt, wk, wo, w1, w2, w3, w4,
            big, yres, hbuf, xna, xnb, xnc, gh, qt, pqt, kb, pkb, vt, ob, obl, amem,
            mt, zrow, gate, bias,
            s0, s1, s2, s3, m0, m1, m2, m3,
            obuf, sems, tsems, osems):
    sbuf = (s0, s1, s2, s3)
    mbuf = (m0, m1, m2, m3)

    def seg_rows(s):
        return pl.ds(s * L, L)

    cp_x0 = pltpu.make_async_copy(x_hbm.at[0, seg_rows(0)], xin.at[seg_rows(0)], sems.at[0])
    cp_xr = pltpu.make_async_copy(x_hbm.at[0, pl.ds(L, S - L)], xin.at[pl.ds(L, S - L)], sems.at[1])
    cp_wk = [pltpu.make_async_copy(wk_hbm.at[:, pl.ds(i * DHALF, DHALF)], wk.at[i].bitcast(bf16),
                                   sems.at[2 + i])
             for i in range(2)]
    cp_wo = [pltpu.make_async_copy(wo_hbm.at[pl.ds(i * DHALF, DHALF)], wo.at[i].bitcast(bf16),
                                   sems.at[4 + i])
             for i in range(2)]
    cp_w1 = pltpu.make_async_copy(w1_hbm, w1.bitcast(bf16), sems.at[6])
    cp_w2 = pltpu.make_async_copy(w2_hbm, w2.bitcast(bf16), sems.at[7])
    cp_w3 = [pltpu.make_async_copy(w3_hbm.at[:, pl.ds(c * FC, FC)], w3.at[c].bitcast(bf16),
                                   sems.at[8])
             for c in range(F // FC)]
    cp_w4 = pltpu.make_async_copy(w4_hbm, w4.bitcast(bf16), sems.at[9])

    TC = 256
    NTC = D // TC

    def cp_stage(i, c):
        src = (wq_hbm, wv_hbm)[i]
        return pltpu.make_async_copy(src.at[pl.ds(c * TC, TC)], stage.at[i * NTC + c],
                                     tsems.at[i * NTC + c])

    cp_x0.start()
    for i in range(2):
        for c in range(NTC):
            cp_stage(i, c).start()
    cp_wk[0].start()
    cp_wo[0].start()

    kk = jax.lax.broadcasted_iota(jnp.int32, (128, 512), 0)
    qq = jax.lax.broadcasted_iota(jnp.int32, (128, 512), 1) % 128
    bias[...] = jnp.where(kk > qq, MASK_BIAS, 0.0).astype(f32)
    bt = jnp.broadcast_to(beta_ref[...].astype(f32), (H, H))
    eye = (jax.lax.broadcasted_iota(jnp.int32, (H, H), 0)
           == jax.lax.broadcasted_iota(jnp.int32, (H, H), 1))
    bcol = jnp.sum(jnp.where(eye, bt, 0.0), axis=1, keepdims=True)
    gsig = jnp.broadcast_to(jax.nn.sigmoid(bcol), (H, 128))
    gate[0] = gsig[0:H // 2]
    gate[1] = gsig[H // 2:H]
    hbuf[0:2 * HALO, :] = jnp.zeros((2 * HALO, D), f32)
    hbuf[S:PAD_ROWS, :] = jnp.zeros((2 * HALO, D), f32)
    for ref in (big, yres):
        ref[0:HALO, :] = jnp.zeros((HALO, D), f32)
        ref[S + HALO:PAD_ROWS, :] = jnp.zeros((HALO, D), f32)

    ident = (jax.lax.broadcasted_iota(jnp.int32, (128, 128), 0)
             == jax.lax.broadcasted_iota(jnp.int32, (128, 128), 1)).astype(f32).astype(bf16)

    def transpose_chunk(ic, _):
        pltpu.make_async_copy(stage.at[ic], stage.at[ic], tsems.at[ic]).wait()
        i = ic >> 2
        c = ic & 3
        ro = pl.multiple_of(i * DHALF, DHALF)
        for n in range(D // 128):
            tile = _dot_nt(ident, stage[ic, :, n * 128:(n + 1) * 128])
            wt[n // 4, c, _hs(ro + (n % 4) * 128, 128), :] = _pack(tile)
        return 0
    jax.lax.fori_loop(0, 2 * NTC, transpose_chunk, 0)

    cp_wk[1].start()
    cp_wo[1].start()
    cp_w1.start()
    cp_xr.start()
    cp_w2.start()
    cp_x0.wait()

    def init_x(i, _):
        r = pl.multiple_of(i * 256, 256)
        xv = xin[pl.ds(r, 256), :].astype(f32)
        big[pl.ds(HALO + r, 256), :] = xv
        xna[_hs(r, 256), :] = _pack(_ln(xv))
        return 0
    jax.lax.fori_loop(0, L // 256, init_x, 0)
    cp_wk[0].wait()
    cp_wo[0].wait()

    def qmask(g, t):
        z = jnp.zeros((DH, 128), bf16)
        cols = []
        for h in range(4):
            qh = _unpack(qt[g, _hs(h * DH, DH), t * 128:(t + 1) * 128])
            cols.append(jnp.concatenate([qh if i == h else z for i in range(4)], axis=0))
        return jnp.concatenate(cols, axis=1)

    def attn_step(half, g, gn, fill=()):
        pr = None if g is None else g % 2
        pw = None if gn is None else gn % 2
        fill = list(fill)
        for t in range(NT_TILES):
            macc = None
            oacc = [None] * 4
            lacc = [None] * 4
            for j in range(t + 1):
                ks = slice(j * 128, (j + 1) * 128)
                if fill and (t, j) != (0, 0):
                    fill.pop(0)()
                if gn is not None:
                    s = _dot(_unpack(kb[gn, _hs(j * 128, 128), :]), qmask(gn, t))
                    if j == t:
                        s = s + bias[...]
                    sbuf[t][pw, ks, :] = s
                    mx = _red8(s, jnp.maximum)
                    macc = mx if macc is None else jnp.maximum(macc, mx)
                if g is not None:
                    for h in range(4):
                        sl = slice(h * 128, (h + 1) * 128)
                        p = jnp.exp2(sbuf[t][pr, ks, sl] - mbuf[t][pr, :, sl])
                        lt = _red8(p, jnp.add)
                        lacc[h] = lt if lacc[h] is None else lacc[h] + lt
                        o = _dot(_unpack(vt[g, _hs(h * DH, DH), ks]), p.astype(bf16))
                        oacc[h] = o if oacc[h] is None else oacc[h] + o
            if gn is not None:
                mbuf[t][pw] = jnp.max(macc, axis=0, keepdims=True)
            if g is not None:
                parts = []
                for h in range(4):
                    l = jnp.sum(lacc[h], axis=0, keepdims=True)
                    gh = gate[half, g * 4 + h:g * 4 + h + 1, :]
                    parts.append(oacc[h] * ((1.0 - gh) / l))
                ot = jnp.concatenate(parts, axis=0) + amem[g, :, t * 128:(t + 1) * 128]
                if g < GH - 1 or t < 2:
                    ob[g, _hs(t * 128, 128), :] = _pack(ot.T)
                else:
                    obl[half, _hs((t - 2) * 128, 128), :] = _pack(ot.T)

    rowh = jax.lax.broadcasted_iota(jnp.int32, (128, 128), 0) // DH
    colh = jax.lax.broadcasted_iota(jnp.int32, (128, 128), 1) // DH
    row16 = jax.lax.broadcasted_iota(jnp.int32, (16, 128), 0)
    col16 = jax.lax.broadcasted_iota(jnp.int32, (16, 128), 1) // DH

    def attn_half(layer, seg, half):
        r0 = pl.multiple_of(seg * L, L)

        @pl.when(jnp.logical_and(jnp.logical_and(layer == 0, seg == 0), half == 1))
        def _():
            cp_wk[1].wait()
            cp_wo[1].wait()
            cp_w1.wait()
            cp_xr.wait()
            cp_w2.wait()
            for c in cp_w3:
                c.start()
            cp_w4.start()

        def xn(c0, nc):
            return _unpack(xna[_hs(c0 * 128, nc * 128), :])

        zparts = {}

        def k_piece(g0, ng, c0, nc):
            k = _dot(xn(c0, nc), _unpack(wk[half, :, g0 * 128:(g0 + ng) * 128]))
            pk = _phi(k)
            rs = _hs(c0 * 128, nc * 128)
            for i in range(ng):
                cs = slice(i * 128, (i + 1) * 128)
                kb[g0 + i, rs, :] = _pack(k[:, cs])
                pkb[g0 + i, rs, :] = _pack(pk[:, cs])
                zparts.setdefault(g0 + i, []).append(_red8(pk[:, cs], jnp.add))

        def qv_piece(qs, vs, c0, nc):
            offs = [g * 128 for g in qs] + [DHALF + g * 128 for g in vs]
            lhs = jnp.concatenate(
                [jnp.concatenate([wt[half, c, _hs(o, 128), :] for c in range(NTC)], axis=1)
                 for o in offs], axis=0)
            r = _dot_nt(_unpack(lhs), xn(c0, nc))
            ts = slice(c0 * 128, (c0 + nc) * 128)
            for i, g in enumerate(qs):
                qg = r[i * 128:(i + 1) * 128, :]
                qt[g, :, ts] = _pack(qg * QSCALE)
                pqt[g, :, ts] = _pack(_phi(qg))
            for i, g in enumerate(vs):
                o = (len(qs) + i) * 128
                vt[g, :, ts] = _pack(r[o:o + 128, :])

        def mem(g):
            zold = zrow[half, g]
            mold = mt[half, g]
            mbd = jnp.where(rowh == colh, mold, 0.0)
            zx = jnp.where(row16 == col16, jnp.broadcast_to(zold, (16, 128)), 0.0)
            lhs = jnp.concatenate([mbd, zx], axis=0).astype(bf16)
            ret = _dot(lhs, _unpack(pqt[g]))
            parts = []
            for h in range(4):
                gh = gate[half, g * 4 + h:g * 4 + h + 1, 0:1]
                den = ret[128 + h:129 + h, :] + 1e-6
                parts.append(ret[h * DH:(h + 1) * DH, :] * (gh / den))
            amem[g] = jnp.concatenate(parts, axis=0)
            mt[half, g] = mold + _dot(_unpack(vt[g]), _unpack(pkb[g]))
            zsum = functools.reduce(jnp.add, zparts[g])
            zrow[half, g] = zold + jnp.sum(zsum, axis=0, keepdims=True)

        P = functools.partial
        skip = lambda: None
        k_piece(0, 2, 0, 4)
        qv_piece((0, 1), (0,), 0, 4)
        attn_step(half, None, 0)
        mem(0)
        for g in range(2):
            attn_step(half, g, g + 1, fill=[
                P(k_piece, g + 2, 1, 0, 2), skip, P(qv_piece, (g + 2,), (g + 1,), 0, 1),
                P(qv_piece, (g + 2,), (g + 1,), 1, 1), skip, P(k_piece, g + 2, 1, 2, 2),
                P(qv_piece, (g + 2,), (g + 1,), 2, 1), P(qv_piece, (g + 2,), (g + 1,), 3, 1),
                P(mem, g + 1)])
        attn_step(half, 2, 3, fill=[
            skip, P(qv_piece, (), (3,), 0, 1), skip, P(qv_piece, (), (3,), 1, 1), skip,
            P(qv_piece, (), (3,), 2, 1), P(qv_piece, (), (3,), 3, 1), skip, P(mem, 3)])

        def wo_piece(t, n):
            off = t * 128
            cs = slice(n * DHALF, (n + 1) * DHALF)
            rr = pl.ds(r0 + (HALO + off), 128)
            ng = GH if t < 2 else GH - 1
            o = jnp.concatenate([ob[g, _hs(off, 128), :] for g in range(ng)], axis=1)
            big[rr, cs] = big[rr, cs] + _dot(_unpack(o), _unpack(wo[half, _hs(0, ng * 128), cs]))

        attn_step(half, GH - 1, None,
                  fill=[P(wo_piece, t, n) for t in (2, 3, 0, 1) for n in range(2)])

    def phase_a(layer, seg):
        r0 = pl.multiple_of(seg * L, L)

        def half_body(half, _):
            attn_half(layer, seg, half)
            return 0
        jax.lax.fori_loop(0, 2, half_body, 0)

        hl = L // 2
        kp = (GH - 1) * 128

        bw = big.at[pl.ds(r0, 2 * L + 2 * HALO), :]
        yw = yres.at[pl.ds(r0, L + 2 * HALO), :]
        hw = hbuf.at[pl.ds(r0, L + 2 * HALO), :]
        xw = xin.at[pl.ds(r0 + L, L), :]

        def wo_rest():
            rr = slice(HALO + hl, HALO + L)
            o = _unpack(jnp.concatenate([obl[0], obl[1]], axis=1))
            w = _unpack(jnp.concatenate([wo[i, _hs(kp, 128), :] for i in range(2)], axis=0))
            bw[rr, :] = bw[rr, :] + _dot(o, w)

        def lnln(off, n):
            rr = slice(HALO + off, HALO + off + n)
            r, mr, z = _ln_ln(bw[rr, :])
            yw[rr, D - 256:D - 128] = jnp.broadcast_to(r, (n, 128))
            yw[rr, D - 128:D] = jnp.broadcast_to(mr, (n, 128))
            xnb[_hs(off, n), :] = _pack(z)

        def corners(v):
            return [v[0:8, 0:128], v[hl - 8:hl, 0:128], v[0:8, 128:256], v[hl - 8:hl, 128:256]]

        def up(off, n):
            cs = slice(n * 256, (n + 1) * 256)
            hh = _gelu(_dot(_unpack(xnb[_hs(off, hl), :]), _unpack(w1[:, cs])))
            b = off + HALO + SHIFTS[n]
            hw[b:b + hl, cs] = hh
            return corners(hh)

        sink = PIN + pl.multiple_of(seg * 16, 16)

        def pin(ref, v):
            if ref.dtype == bf16:
                ref[pl.ds(sink, 16), 0:128] = jnp.concatenate([v, v], axis=0).astype(bf16)
            else:
                ref[pl.ds(sink, 8), 0:128] = v

        fresh = jnp.logical_and(layer == 0, seg < NSEG - 1)

        def ln_next(off, n):
            rr = slice(L + HALO + off, L + HALO + off + n)
            xv = jnp.where(fresh, xw[off:off + n, :].astype(f32), bw[rr, :])
            bw[rr, :] = xv
            xna[_hs(off, n), :] = _pack(_ln(xv))

        lnln(0, 128)
        lnln(128, 128)
        wo_rest()
        def mix_part(off, n):
            return corners(mix(hw, yw, bw, slice(off, off + hl), n))

        def fence():
            pin(yres, pltpu.bitcast(xna[pl.ds(pl.multiple_of(seg * 8, 8), 8), 0:128], f32))

        late = list(range(hl, L, 16))
        nxt = list(range(0, L, 16))
        for n in range(4):
            marks = up(0, n)
            for i in (0, 1, 3):
                lnln(late.pop(0), 16)
                pin(big, marks[i])
        for n in range(4):
            marks = mix_part(0, n)
            for i in range(4):
                if late:
                    lnln(late.pop(0), 16)
                else:
                    ln_next(nxt.pop(0), 16)
                if n > 0 or i == 3:
                    pin(xin, marks[i])
        for n in range(4):
            marks = up(hl, n)
            for i in (0, 1, 3):
                ln_next(nxt.pop(0), 16)
                pin(xin, marks[i])
        for n in range(4):
            if n == 3:
                fence()
            marks = mix_part(hl, n)
            for i in range(4):
                if nxt:
                    ln_next(nxt.pop(0), 16)
                    pin(xin, marks[i])

    def mix(h_ref, y_ref, x_ref, rr, n):
        cs = slice(n * 256, (n + 1) * 256)
        r = y_ref[rr, D - 256:D - 128]
        mr = y_ref[rr, D - 128:D]
        x = x_ref[rr, cs]
        y = x * jnp.concatenate([r, r], axis=1) - jnp.concatenate([mr, mr], axis=1)
        x1 = y + _dot(h_ref[rr, :].astype(bf16), _unpack(w2[:, cs]))
        y_ref[rr, cs] = x1
        x_ref[rr, cs] = x + x1
        return x1

    def ln_mid(tok, n):
        xnc[_hs(tok, n), :] = _pack(_ln(yres[pl.ds(tok + HALO, n), :]))

    def last_rows():
        for n in range(4):
            mix(hbuf, yres, big, slice(S, PAD_ROWS), n)
            ln_mid(n * 128, 128)

    def out_copy(blk):
        rows = pl.ds(blk * L, L)
        return pltpu.make_async_copy(obuf.at[rows], out_hbm.at[0, rows, :], osems.at[blk])

    def ffn(layer, it):
        def block_of(pair):
            return (pair * 37) >> 8

        blk, chunk, tok = [], [], []
        for h in range(UNROLL // 2):
            pair = (UNROLL // 2) * it + h
            b = block_of(pair)
            c = 2 * pair - NC * b
            t = pl.multiple_of(b * L, L)
            blk += [b, b]
            chunk += [c, c + 1]
            tok += [t, t]

        def ffn_up(k):
            hh = _gelu(_dot(_unpack(xnc[_hs(tok[k], L), :]), _unpack(w3[chunk[k]])))
            gh[k % 2] = _pack(hh)
            return hh[L - 8:L, FC - 128:FC]

        def ffn_down(k):
            rows = pl.ds(tok[k] + HALO, L)
            w = _unpack(w4[_hs(chunk[k] * FC, FC), :])
            big[rows, :] = big[rows, :] + _dot(_unpack(gh[k % 2]), w)

        def ln_ahead(k, mark):
            yres[pl.ds(PIN + pl.multiple_of(blk[0] * 16, 16), 8), 0:128] = mark
            nb = jnp.minimum(blk[k] + 1, NSEG - 1)
            ln_mid(pl.multiple_of(nb * L + jnp.minimum(chunk[k] * 40, L - 80), 16), 80)

        def ln_first():
            r = pl.multiple_of(jnp.clip((it - 4) * 64, 0, L - 64), 64)
            xna[_hs(r, 64), :] = _pack(_ln(big[pl.ds(r + HALO, 64), :]))

        ffn_up(0)
        ln_ahead(0, ffn_up(1))
        ffn_down(0)
        ln_ahead(2, ffn_up(2))
        ffn_down(1)
        ln_first()
        ffn_up(3)
        ffn_down(2)
        ffn_down(3)

        done = block_of((UNROLL // 2) * (it + 1))

        @pl.when(jnp.logical_and(layer == 1, done != blk[0]))
        def _():
            r = pl.multiple_of((done - 1) * L, L)
            obuf[pl.ds(r, L), :] = big[pl.ds(r + HALO, L), :].astype(bf16)
            out_copy(done - 1).start()

    def layer_body(layer, _):
        mt[...] = jnp.zeros(mt.shape, f32)
        zrow[...] = jnp.zeros(zrow.shape, f32)

        def a_body(seg, _):
            phase_a(layer, seg)
            return 0
        jax.lax.fori_loop(0, NSEG, a_body, 0)

        last_rows()

        @pl.when(layer == 0)
        def _():
            for c in cp_w3:
                c.wait()
            cp_w4.wait()

        def b_body(it, _):
            ffn(layer, it)
            return 0
        jax.lax.fori_loop(0, NSEG * NC // UNROLL, b_body, 0)
        return 0
    jax.lax.fori_loop(0, 2, layer_body, 0)

    for blk in range(NSEG):
        out_copy(blk).wait()


@jax.jit
def pallas_interleave_layers__memory_aug_infini_attn__mixer_s_mlp__prompt_kernel(
    A_x: jax.Array,
    A_wq: jax.Array,
    A_wk: jax.Array,
    A_wv: jax.Array,
    A_wo: jax.Array,
    A_beta: jax.Array,
    B_x: jax.Array,
    B_w1: jax.Array,
    B_w2: jax.Array,
    B_w3: jax.Array,
    B_w4: jax.Array,
):
    del B_x
    hbm = pl.BlockSpec(memory_space=pl.ANY)
    vm = pltpu.VMEM
    scratch = [
        vm((BIG_ROWS, D), bf16),
        vm((8, 256, D), bf16),
        vm((2, 4, D // 2, 256), u32),
        vm((2, D // 2, DHALF), u32),
        vm((2, DHALF // 2, D), u32),
        vm((D // 2, D), u32),
        vm((D // 2, D), u32),
        vm((NC, D // 2, FC), u32),
        vm((F // 2, D), u32),
        vm((BIG_ROWS, D), f32),
        vm((BIG_ROWS, D), f32),
        vm((PAD_ROWS, D), f32),
        vm((L // 2, D), u32),
        vm((L // 2, D), u32),
        vm((S // 2, D), u32),
        vm((2, L // 2, FC), u32),
        vm((GH, 64, L), u32),
        vm((GH, 64, L), u32),
        vm((GH, L // 2, 128), u32),
        vm((GH, L // 2, 128), u32),
        vm((GH, 64, L), u32),
        vm((GH, L // 2, 128), u32),
        vm((2, L // 4, 128), u32),
        vm((GH, 128, L), f32),
        vm((2, GH, 128, 128), f32),
        vm((2, GH, 1, 128), f32),
        vm((2, H // 2, 128), f32),
        vm((128, 512), f32),
    ]
    scratch += [vm((2, 128 * (t + 1), 512), f32) for t in range(NT_TILES)]
    scratch += [vm((2, 1, 512), f32) for _ in range(NT_TILES)]
    scratch += [
        vm((S, D), bf16),
        pltpu.SemaphoreType.DMA((10,)),
        pltpu.SemaphoreType.DMA((8,)),
        pltpu.SemaphoreType.DMA((NSEG,)),
    ]
    return pl.pallas_call(
        _kernel,
        out_shape=jax.ShapeDtypeStruct((1, S, D), bf16),
        in_specs=[hbm, hbm, hbm, hbm, hbm, pl.BlockSpec(memory_space=pltpu.VMEM),
                  hbm, hbm, hbm, hbm],
        out_specs=hbm,
        scratch_shapes=scratch,
        compiler_params=pltpu.CompilerParams(vmem_limit_bytes=120 * 1024 * 1024),
    )(A_x, A_wq, A_wk, A_wv, A_wo, A_beta.reshape(1, H), B_w1, B_w2, B_w3, B_w4)
```

```python
import functools
import math

import jax
import jax.numpy as jnp
import jax.experimental.pallas as pl
import jax.experimental.pallas.tpu as pltpu

S = 2048
D = 1024
F = 3584
H = 32
DH = 32
L = 512
NSEG = S // L
NG = D // 128
NT_TILES = L // 128
FC = 256
HALO = 8
GH = NG // 2
DHALF = D // 2
PAD_ROWS = S + 2 * HALO
PIN = S + L + 2 * HALO
BIG_ROWS = PIN + 16 * NSEG
NC = F // FC
UNROLL = 4
SHIFTS = (1, -1, 2, -2)

LOG2E = math.log2(math.e)
QSCALE = DH ** -0.5 * LOG2E
MASK_BIAS = -1e9 * LOG2E
EPS = 1e-5

f32 = jnp.float32
bf16 = jnp.bfloat16
u32 = jnp.uint32
NT_DIMS = (((1,), (1,)), ((), ()))


def _stats(x):
    m = jnp.mean(x, axis=-1, keepdims=True)
    xc = x - m
    return m, jnp.mean(xc * xc, axis=-1, keepdims=True)


def _ln(x):
    m, v = _stats(x)
    r = jax.lax.rsqrt(v + EPS)
    return x * r - m * r


def _ln_ln(x):
    m, v = _stats(x)
    r1 = jax.lax.rsqrt(v + EPS)
    r2 = r1 * jax.lax.rsqrt(v * r1 * r1 + EPS)
    return r1, m * r1, x * r2 - m * r2


def _gelu(x):
    c = math.sqrt(2.0 / math.pi)
    inner = x * (c + (c * 0.044715) * (x * x))
    hx = 0.5 * x
    return hx + hx * jnp.tanh(inner)


def _phi(t):
    return jnp.where(t > 0, t + 1.0, jnp.exp(t))


def _red8(x, op):
    return functools.reduce(op, [x[i * 8:(i + 1) * 8] for i in range(x.shape[0] // 8)])


def _pack(x):
    return pltpu.bitcast(x.astype(bf16), u32)


def _unpack(x):
    return pltpu.bitcast(x, bf16)


def _hs(start, n):
    if isinstance(start, int):
        return slice(start // 2, (start + n) // 2)
    return pl.ds(pl.multiple_of(start >> 1, 8), n // 2)


def _dot(a, b):
    return jnp.dot(a, b, preferred_element_type=f32)


def _dot_nt(a, b):
    return jax.lax.dot_general(a, b, NT_DIMS, preferred_element_type=f32)


def _kernel(x_hbm, wq_hbm, wk_hbm, wv_hbm, wo_hbm, beta_ref, w1_hbm, w2_hbm, w3_hbm, w4_hbm,
            out_hbm,
            xin, stage, wt, wk, wo, w1, w2, w3, w4,
            big, yres, hbuf, xna, xnb, xnc, gh, qt, pqt, kb, pkb, vt, ob, obl, amem,
            mt, zrow, gate, bias,
            s0, s1, s2, s3, m0, m1, m2, m3,
            obuf, sems, tsems, osems):
    sbuf = (s0, s1, s2, s3)
    mbuf = (m0, m1, m2, m3)

    def seg_rows(s):
        return pl.ds(s * L, L)

    cp_x0 = pltpu.make_async_copy(x_hbm.at[0, seg_rows(0)], xin.at[seg_rows(0)], sems.at[0])
    cp_xr = pltpu.make_async_copy(x_hbm.at[0, pl.ds(L, S - L)], xin.at[pl.ds(L, S - L)], sems.at[1])
    cp_wk = [pltpu.make_async_copy(wk_hbm.at[:, pl.ds(i * DHALF, DHALF)], wk.at[i].bitcast(bf16),
                                   sems.at[2 + i])
             for i in range(2)]
    cp_wo = [pltpu.make_async_copy(wo_hbm.at[pl.ds(i * DHALF, DHALF)], wo.at[i].bitcast(bf16),
                                   sems.at[4 + i])
             for i in range(2)]
    cp_w1 = pltpu.make_async_copy(w1_hbm, w1.bitcast(bf16), sems.at[6])
    cp_w2 = pltpu.make_async_copy(w2_hbm, w2.bitcast(bf16), sems.at[7])
    cp_w3 = [pltpu.make_async_copy(w3_hbm.at[:, pl.ds(c * FC, FC)], w3.at[c].bitcast(bf16),
                                   sems.at[8])
             for c in range(F // FC)]
    cp_w4 = pltpu.make_async_copy(w4_hbm, w4.bitcast(bf16), sems.at[9])

    TC = 256
    NTC = D // TC

    def cp_stage(i, c):
        src = (wq_hbm, wv_hbm)[i]
        return pltpu.make_async_copy(src.at[pl.ds(c * TC, TC)], stage.at[i * NTC + c],
                                     tsems.at[i * NTC + c])

    for i in range(2):
        for c in range(NTC):
            cp_stage(i, c).start()
    for cp in (cp_x0, cp_wk[0], cp_wo[0]):
        cp.start()

    kk = jax.lax.broadcasted_iota(jnp.int32, (128, 512), 0)
    qq = jax.lax.broadcasted_iota(jnp.int32, (128, 512), 1) % 128
    bias[...] = jnp.where(kk > qq, MASK_BIAS, 0.0).astype(f32)
    bt = jnp.broadcast_to(beta_ref[...].astype(f32), (H, H))
    eye = (jax.lax.broadcasted_iota(jnp.int32, (H, H), 0)
           == jax.lax.broadcasted_iota(jnp.int32, (H, H), 1))
    bcol = jnp.sum(jnp.where(eye, bt, 0.0), axis=1, keepdims=True)
    gsig = jnp.broadcast_to(jax.nn.sigmoid(bcol), (H, 128))
    gate[0] = gsig[0:H // 2]
    gate[1] = gsig[H // 2:H]
    hbuf[0:2 * HALO, :] = jnp.zeros((2 * HALO, D), f32)
    hbuf[S:PAD_ROWS, :] = jnp.zeros((2 * HALO, D), f32)
    for ref in (big, yres):
        ref[0:HALO, :] = jnp.zeros((HALO, D), f32)
        ref[S + HALO:PAD_ROWS, :] = jnp.zeros((HALO, D), f32)

    ident = (jax.lax.broadcasted_iota(jnp.int32, (128, 128), 0)
             == jax.lax.broadcasted_iota(jnp.int32, (128, 128), 1)).astype(f32).astype(bf16)

    def transpose_chunk(ic, _):
        pltpu.make_async_copy(stage.at[ic], stage.at[ic], tsems.at[ic]).wait()
        i = ic >> 2
        c = ic & 3
        ro = pl.multiple_of(i * DHALF, DHALF)
        for n in range(D // 128):
            tile = _dot_nt(ident, stage[ic, :, n * 128:(n + 1) * 128])
            wt[n // 4, c, _hs(ro + (n % 4) * 128, 128), :] = _pack(tile)
        return 0
    jax.lax.fori_loop(0, 2 * NTC, transpose_chunk, 0)

    cp_x0.wait()

    def init_x(i, _):
        r = pl.multiple_of(i * 256, 256)
        xv = xin[pl.ds(r, 256), :].astype(f32)
        big[pl.ds(HALO + r, 256), :] = xv
        xna[_hs(r, 256), :] = _pack(_ln(xv))
        return 0
    jax.lax.fori_loop(0, L // 256, init_x, 0)
    cp_wk[0].wait()
    for cp in [cp_wk[1], cp_wo[1], cp_w1, cp_xr, cp_w2] + cp_w3 + [cp_w4]:
        cp.start()

    def qmask(g, t):
        z = jnp.zeros((DH, 128), bf16)
        cols = []
        for h in range(4):
            qh = _unpack(qt[g, _hs(h * DH, DH), t * 128:(t + 1) * 128])
            cols.append(jnp.concatenate([qh if i == h else z for i in range(4)], axis=0))
        return jnp.concatenate(cols, axis=1)

    def attn_step(half, g, gn, fill=()):
        pr = None if g is None else g % 2
        pw = None if gn is None else gn % 2
        fill = list(fill)
        for t in range(NT_TILES):
            macc = None
            oacc = [None] * 4
            lacc = [None] * 4
            for j in range(t + 1):
                ks = slice(j * 128, (j + 1) * 128)
                if fill and (t, j) != (0, 0):
                    fill.pop(0)()
                if gn is not None:
                    s = _dot(_unpack(kb[gn, _hs(j * 128, 128), :]), qmask(gn, t))
                    if j == t:
                        s = s + bias[...]
                    sbuf[t][pw, ks, :] = s
                    mx = _red8(s, jnp.maximum)
                    macc = mx if macc is None else jnp.maximum(macc, mx)
                if g is not None:
                    for h in range(4):
                        sl = slice(h * 128, (h + 1) * 128)
                        p = jnp.exp2(sbuf[t][pr, ks, sl] - mbuf[t][pr, :, sl])
                        lt = _red8(p, jnp.add)
                        lacc[h] = lt if lacc[h] is None else lacc[h] + lt
                        o = _dot(_unpack(vt[g, _hs(h * DH, DH), ks]), p.astype(bf16))
                        oacc[h] = o if oacc[h] is None else oacc[h] + o
            if gn is not None:
                mbuf[t][pw] = jnp.max(macc, axis=0, keepdims=True)
            if g is not None:
                parts = []
                for h in range(4):
                    l = jnp.sum(lacc[h], axis=0, keepdims=True)
                    gh = gate[half, g * 4 + h:g * 4 + h + 1, :]
                    parts.append(oacc[h] * ((1.0 - gh) / l))
                ot = jnp.concatenate(parts, axis=0) + amem[g, :, t * 128:(t + 1) * 128]
                if g < GH - 1 or t < 2:
                    ob[g, _hs(t * 128, 128), :] = _pack(ot.T)
                else:
                    obl[half, _hs((t - 2) * 128, 128), :] = _pack(ot.T)

    rowh = jax.lax.broadcasted_iota(jnp.int32, (128, 128), 0) // DH
    colh = jax.lax.broadcasted_iota(jnp.int32, (128, 128), 1) // DH
    row16 = jax.lax.broadcasted_iota(jnp.int32, (16, 128), 0)
    col16 = jax.lax.broadcasted_iota(jnp.int32, (16, 128), 1) // DH

    def attn_half(layer, seg, half):
        r0 = pl.multiple_of(seg * L, L)

        @pl.when(jnp.logical_and(jnp.logical_and(layer == 0, seg == 0), half == 1))
        def _():
            cp_wk[1].wait()
            cp_wo[1].wait()
            cp_w1.wait()
            cp_xr.wait()
            cp_w2.wait()

        def xn(c0, nc):
            return _unpack(xna[_hs(c0 * 128, nc * 128), :])

        zparts = {}

        def k_piece(g0, ng, c0, nc):
            k = _dot(xn(c0, nc), _unpack(wk[half, :, g0 * 128:(g0 + ng) * 128]))
            pk = _phi(k)
            rs = _hs(c0 * 128, nc * 128)
            for i in range(ng):
                cs = slice(i * 128, (i + 1) * 128)
                kb[g0 + i, rs, :] = _pack(k[:, cs])
                pkb[g0 + i, rs, :] = _pack(pk[:, cs])
                zparts.setdefault(g0 + i, []).append(_red8(pk[:, cs], jnp.add))

        def qv_piece(qs, vs, c0, nc):
            offs = [g * 128 for g in qs] + [DHALF + g * 128 for g in vs]
            lhs = jnp.concatenate(
                [jnp.concatenate([wt[half, c, _hs(o, 128), :] for c in range(NTC)], axis=1)
                 for o in offs], axis=0)
            r = _dot_nt(_unpack(lhs), xn(c0, nc))
            ts = slice(c0 * 128, (c0 + nc) * 128)
            for i, g in enumerate(qs):
                qg = r[i * 128:(i + 1) * 128, :]
                qt[g, :, ts] = _pack(qg * QSCALE)
                pqt[g, :, ts] = _pack(_phi(qg))
            for i, g in enumerate(vs):
                o = (len(qs) + i) * 128
                vt[g, :, ts] = _pack(r[o:o + 128, :])

        def mem(g):
            zold = zrow[half, g]
            mold = mt[half, g]
            mbd = jnp.where(rowh == colh, mold, 0.0)
            zx = jnp.where(row16 == col16, jnp.broadcast_to(zold, (16, 128)), 0.0)
            lhs = jnp.concatenate([mbd, zx], axis=0).astype(bf16)
            ret = _dot(lhs, _unpack(pqt[g]))
            parts = []
            for h in range(4):
                gh = gate[half, g * 4 + h:g * 4 + h + 1, 0:1]
                den = ret[128 + h:129 + h, :] + 1e-6
                parts.append(ret[h * DH:(h + 1) * DH, :] * (gh / den))
            amem[g] = jnp.concatenate(parts, axis=0)
            mt[half, g] = mold + _dot(_unpack(vt[g]), _unpack(pkb[g]))
            zsum = functools.reduce(jnp.add, zparts[g])
            zrow[half, g] = zold + jnp.sum(zsum, axis=0, keepdims=True)

        P = functools.partial
        skip = lambda: None
        k_piece(0, 2, 0, 4)
        qv_piece((0, 1), (0,), 0, 4)

        @pl.when(jnp.logical_and(jnp.logical_and(layer == 0, seg == 0), half == 0))
        def _():
            cp_wo[0].wait()

        attn_step(half, None, 0)
        mem(0)
        for g in range(2):
            attn_step(half, g, g + 1, fill=[
                P(k_piece, g + 2, 1, 0, 2), skip, P(qv_piece, (g + 2,), (g + 1,), 0, 1),
                P(qv_piece, (g + 2,), (g + 1,), 1, 1), skip, P(k_piece, g + 2, 1, 2, 2),
                P(qv_piece, (g + 2,), (g + 1,), 2, 1), P(qv_piece, (g + 2,), (g + 1,), 3, 1),
                P(mem, g + 1)])
        attn_step(half, 2, 3, fill=[
            skip, P(qv_piece, (), (3,), 0, 1), skip, P(qv_piece, (), (3,), 1, 1), skip,
            P(qv_piece, (), (3,), 2, 1), P(qv_piece, (), (3,), 3, 1), skip, P(mem, 3)])

        def wo_piece(t, n):
            off = t * 128
            cs = slice(n * DHALF, (n + 1) * DHALF)
            rr = pl.ds(r0 + (HALO + off), 128)
            ng = GH if t < 2 else GH - 1
            o = jnp.concatenate([ob[g, _hs(off, 128), :] for g in range(ng)], axis=1)
            big[rr, cs] = big[rr, cs] + _dot(_unpack(o), _unpack(wo[half, _hs(0, ng * 128), cs]))

        attn_step(half, GH - 1, None,
                  fill=[P(wo_piece, t, n) for t in (2, 3, 0, 1) for n in range(2)])

    def phase_a(layer, seg):
        r0 = pl.multiple_of(seg * L, L)

        def half_body(half, _):
            attn_half(layer, seg, half)
            return 0
        jax.lax.fori_loop(0, 2, half_body, 0)

        hl = L // 2
        kp = (GH - 1) * 128

        bw = big.at[pl.ds(r0, 2 * L + 2 * HALO), :]
        yw = yres.at[pl.ds(r0, L + 2 * HALO), :]
        hw = hbuf.at[pl.ds(r0, L + 2 * HALO), :]
        xw = xin.at[pl.ds(r0 + L, L), :]

        def wo_rest():
            rr = slice(HALO + hl, HALO + L)
            o = _unpack(jnp.concatenate([obl[0], obl[1]], axis=1))
            w = _unpack(jnp.concatenate([wo[i, _hs(kp, 128), :] for i in range(2)], axis=0))
            bw[rr, :] = bw[rr, :] + _dot(o, w)

        def lnln(off, n):
            rr = slice(HALO + off, HALO + off + n)
            r, mr, z = _ln_ln(bw[rr, :])
            yw[rr, D - 256:D - 128] = jnp.broadcast_to(r, (n, 128))
            yw[rr, D - 128:D] = jnp.broadcast_to(mr, (n, 128))
            xnb[_hs(off, n), :] = _pack(z)

        def corners(v):
            return [v[0:8, 0:128], v[hl - 8:hl, 0:128], v[0:8, 128:256], v[hl - 8:hl, 128:256]]

        def up(off, n):
            cs = slice(n * 256, (n + 1) * 256)
            hh = _gelu(_dot(_unpack(xnb[_hs(off, hl), :]), _unpack(w1[:, cs])))
            b = off + HALO + SHIFTS[n]
            hw[b:b + hl, cs] = hh
            return corners(hh)

        sink = PIN + pl.multiple_of(seg * 16, 16)

        def pin(ref, v):
            if ref.dtype == bf16:
                ref[pl.ds(sink, 16), 0:128] = jnp.concatenate([v, v], axis=0).astype(bf16)
            else:
                ref[pl.ds(sink, 8), 0:128] = v

        fresh = jnp.logical_and(layer == 0, seg < NSEG - 1)

        def ln_next(off, n):
            rr = slice(L + HALO + off, L + HALO + off + n)
            xv = jnp.where(fresh, xw[off:off + n, :].astype(f32), bw[rr, :])
            bw[rr, :] = xv
            xna[_hs(off, n), :] = _pack(_ln(xv))

        lnln(0, 128)
        lnln(128, 128)
        wo_rest()
        def mix_part(off, n):
            return corners(mix(hw, yw, bw, slice(off, off + hl), n))

        def fence():
            pin(yres, pltpu.bitcast(xna[pl.ds(pl.multiple_of(seg * 8, 8), 8), 0:128], f32))

        late = list(range(hl, L, 16))
        nxt = list(range(0, L, 16))
        for n in range(4):
            marks = up(0, n)
            for i in (0, 1, 3):
                lnln(late.pop(0), 16)
                pin(big, marks[i])
        for n in range(4):
            marks = mix_part(0, n)
            for i in range(4):
                if late:
                    lnln(late.pop(0), 16)
                else:
                    ln_next(nxt.pop(0), 16)
                if n > 0 or i == 3:
                    pin(xin, marks[i])
        for n in range(4):
            marks = up(hl, n)
            for i in (0, 1, 3):
                ln_next(nxt.pop(0), 16)
                pin(xin, marks[i])
        for n in range(4):
            if n == 3:
                fence()
            marks = mix_part(hl, n)
            for i in range(4):
                if nxt:
                    ln_next(nxt.pop(0), 16)
                    pin(xin, marks[i])

    def mix(h_ref, y_ref, x_ref, rr, n):
        cs = slice(n * 256, (n + 1) * 256)
        r = y_ref[rr, D - 256:D - 128]
        mr = y_ref[rr, D - 128:D]
        x = x_ref[rr, cs]
        y = x * jnp.concatenate([r, r], axis=1) - jnp.concatenate([mr, mr], axis=1)
        x1 = y + _dot(h_ref[rr, :].astype(bf16), _unpack(w2[:, cs]))
        y_ref[rr, cs] = x1
        x_ref[rr, cs] = x + x1
        return x1

    def ln_mid(tok, n):
        xnc[_hs(tok, n), :] = _pack(_ln(yres[pl.ds(tok + HALO, n), :]))

    def last_rows():
        for n in range(4):
            mix(hbuf, yres, big, slice(S, PAD_ROWS), n)
            ln_mid(n * 128, 128)

    def out_copy(blk):
        rows = pl.ds(blk * L, L)
        return pltpu.make_async_copy(obuf.at[rows], out_hbm.at[0, rows, :], osems.at[blk])

    def ffn(layer, it):
        def block_of(pair):
            return (pair * 37) >> 8

        blk, chunk, tok = [], [], []
        for h in range(UNROLL // 2):
            pair = (UNROLL // 2) * it + h
            b = block_of(pair)
            c = 2 * pair - NC * b
            t = pl.multiple_of(b * L, L)
            blk += [b, b]
            chunk += [c, c + 1]
            tok += [t, t]

        def ffn_up(k):
            hh = _gelu(_dot(_unpack(xnc[_hs(tok[k], L), :]), _unpack(w3[chunk[k]])))
            gh[k % 2] = _pack(hh)
            return hh[L - 8:L, FC - 128:FC]

        def ffn_down(k):
            rows = pl.ds(tok[k] + HALO, L)
            w = _unpack(w4[_hs(chunk[k] * FC, FC), :])
            big[rows, :] = big[rows, :] + _dot(_unpack(gh[k % 2]), w)

        def ln_ahead(k, mark):
            yres[pl.ds(PIN + pl.multiple_of(blk[0] * 16, 16), 8), 0:128] = mark
            nb = jnp.minimum(blk[k] + 1, NSEG - 1)
            ln_mid(pl.multiple_of(nb * L + jnp.minimum(chunk[k] * 40, L - 80), 16), 80)

        def ln_first():
            r = pl.multiple_of(jnp.clip((it - 4) * 64, 0, L - 64), 64)
            xna[_hs(r, 64), :] = _pack(_ln(big[pl.ds(r + HALO, 64), :]))

        ffn_up(0)
        ln_ahead(0, ffn_up(1))
        ffn_down(0)
        ln_ahead(2, ffn_up(2))
        ffn_down(1)
        ln_first()
        ffn_up(3)
        ffn_down(2)
        ffn_down(3)

        done = block_of((UNROLL // 2) * (it + 1))

        @pl.when(jnp.logical_and(layer == 1, done != blk[0]))
        def _():
            r = pl.multiple_of((done - 1) * L, L)
            obuf[pl.ds(r, L), :] = big[pl.ds(r + HALO, L), :].astype(bf16)
            out_copy(done - 1).start()

    def layer_body(layer, _):
        mt[...] = jnp.zeros(mt.shape, f32)
        zrow[...] = jnp.zeros(zrow.shape, f32)

        def a_body(seg, _):
            phase_a(layer, seg)
            return 0
        jax.lax.fori_loop(0, NSEG, a_body, 0)

        last_rows()

        @pl.when(layer == 0)
        def _():
            for c in cp_w3:
                c.wait()
            cp_w4.wait()

        def b_body(it, _):
            ffn(layer, it)
            return 0
        jax.lax.fori_loop(0, NSEG * NC // UNROLL, b_body, 0)
        return 0
    jax.lax.fori_loop(0, 2, layer_body, 0)

    for blk in range(NSEG):
        out_copy(blk).wait()


@jax.jit
def pallas_interleave_layers__memory_aug_infini_attn__mixer_s_mlp__prompt_kernel(
    A_x: jax.Array,
    A_wq: jax.Array,
    A_wk: jax.Array,
    A_wv: jax.Array,
    A_wo: jax.Array,
    A_beta: jax.Array,
    B_x: jax.Array,
    B_w1: jax.Array,
    B_w2: jax.Array,
    B_w3: jax.Array,
    B_w4: jax.Array,
):
    del B_x
    hbm = pl.BlockSpec(memory_space=pl.ANY)
    vm = pltpu.VMEM
    scratch = [
        vm((BIG_ROWS, D), bf16),
        vm((8, 256, D), bf16),
        vm((2, 4, D // 2, 256), u32),
        vm((2, D // 2, DHALF), u32),
        vm((2, DHALF // 2, D), u32),
        vm((D // 2, D), u32),
        vm((D // 2, D), u32),
        vm((NC, D // 2, FC), u32),
        vm((F // 2, D), u32),
        vm((BIG_ROWS, D), f32),
        vm((BIG_ROWS, D), f32),
        vm((PAD_ROWS, D), f32),
        vm((L // 2, D), u32),
        vm((L // 2, D), u32),
        vm((S // 2, D), u32),
        vm((2, L // 2, FC), u32),
        vm((GH, 64, L), u32),
        vm((GH, 64, L), u32),
        vm((GH, L // 2, 128), u32),
        vm((GH, L // 2, 128), u32),
        vm((GH, 64, L), u32),
        vm((GH, L // 2, 128), u32),
        vm((2, L // 4, 128), u32),
        vm((GH, 128, L), f32),
        vm((2, GH, 128, 128), f32),
        vm((2, GH, 1, 128), f32),
        vm((2, H // 2, 128), f32),
        vm((128, 512), f32),
    ]
    scratch += [vm((2, 128 * (t + 1), 512), f32) for t in range(NT_TILES)]
    scratch += [vm((2, 1, 512), f32) for _ in range(NT_TILES)]
    scratch += [
        vm((S, D), bf16),
        pltpu.SemaphoreType.DMA((10,)),
        pltpu.SemaphoreType.DMA((8,)),
        pltpu.SemaphoreType.DMA((NSEG,)),
    ]
    return pl.pallas_call(
        _kernel,
        out_shape=jax.ShapeDtypeStruct((1, S, D), bf16),
        in_specs=[hbm, hbm, hbm, hbm, hbm, pl.BlockSpec(memory_space=pltpu.VMEM),
                  hbm, hbm, hbm, hbm],
        out_specs=hbm,
        scratch_shapes=scratch,
        compiler_params=pltpu.CompilerParams(vmem_limit_bytes=120 * 1024 * 1024),
    )(A_x, A_wq, A_wk, A_wv, A_wo, A_beta.reshape(1, H), B_w1, B_w2, B_w3, B_w4)
```

```python
import functools
import math

import jax
import jax.numpy as jnp
import jax.experimental.pallas as pl
import jax.experimental.pallas.tpu as pltpu

S = 2048
D = 1024
F = 3584
H = 32
DH = 32
L = 512
NSEG = S // L
NG = D // 128
NT_TILES = L // 128
FC = 256
HALO = 8
GH = NG // 2
DHALF = D // 2
PAD_ROWS = S + 2 * HALO
PIN = S + L + 2 * HALO
BIG_ROWS = PIN + 16 * NSEG
NC = F // FC
UNROLL = 4
SHIFTS = (1, -1, 2, -2)

LOG2E = math.log2(math.e)
QSCALE = DH ** -0.5 * LOG2E
MASK_BIAS = -1e9 * LOG2E
EPS = 1e-5

f32 = jnp.float32
bf16 = jnp.bfloat16
u32 = jnp.uint32
NT_DIMS = (((1,), (1,)), ((), ()))


def _stats(x):
    m = jnp.mean(x, axis=-1, keepdims=True)
    xc = x - m
    return m, jnp.mean(xc * xc, axis=-1, keepdims=True)


def _ln(x):
    m, v = _stats(x)
    r = jax.lax.rsqrt(v + EPS)
    return x * r - m * r


def _ln_ln(x):
    m, v = _stats(x)
    r1 = jax.lax.rsqrt(v + EPS)
    r2 = r1 * jax.lax.rsqrt(v * r1 * r1 + EPS)
    return r1, m * r1, x * r2 - m * r2


def _gelu(x):
    c = math.sqrt(2.0 / math.pi)
    inner = x * (c + (c * 0.044715) * (x * x))
    hx = 0.5 * x
    return hx + hx * jnp.tanh(inner)


def _phi(t):
    return jnp.where(t > 0, t + 1.0, jnp.exp(t))


def _red8(x, op):
    return functools.reduce(op, [x[i * 8:(i + 1) * 8] for i in range(x.shape[0] // 8)])


def _pack(x):
    return pltpu.bitcast(x.astype(bf16), u32)


def _unpack(x):
    return pltpu.bitcast(x, bf16)


def _hs(start, n):
    if isinstance(start, int):
        return slice(start // 2, (start + n) // 2)
    return pl.ds(pl.multiple_of(start >> 1, 8), n // 2)


def _dot(a, b):
    return jnp.dot(a, b, preferred_element_type=f32)


def _dot_nt(a, b):
    return jax.lax.dot_general(a, b, NT_DIMS, preferred_element_type=f32)


def _kernel(x_hbm, wq_hbm, wk_hbm, wv_hbm, wo_hbm, beta_ref, w1_hbm, w2_hbm, w3_hbm, w4_hbm,
            out_hbm,
            xin, stage, wt, wk, wo, w1, w2, w3, w4,
            big, yres, hbuf, xna, xnb, xnc, gh, qt, pqt, kb, pkb, vt, ob, obl, amem,
            mt, zrow, gate, bias,
            s0, s1, s2, s3, s4, s5, s6, s7, m0, m1, m2, m3,
            obuf, sems, tsems, osems):
    sbuf = ((s0, s1, s2, s3), (s4, s5, s6, s7))
    mbuf = (m0, m1, m2, m3)

    def seg_rows(s):
        return pl.ds(s * L, L)

    cp_x0 = pltpu.make_async_copy(x_hbm.at[0, seg_rows(0)], xin.at[seg_rows(0)], sems.at[0])
    cp_xr = pltpu.make_async_copy(x_hbm.at[0, pl.ds(L, S - L)], xin.at[pl.ds(L, S - L)], sems.at[1])
    cp_wk = [pltpu.make_async_copy(wk_hbm.at[:, pl.ds(i * DHALF, DHALF)], wk.at[i].bitcast(bf16),
                                   sems.at[2 + i])
             for i in range(2)]
    cp_wo = [pltpu.make_async_copy(wo_hbm.at[pl.ds(i * DHALF, DHALF)], wo.at[i].bitcast(bf16),
                                   sems.at[4 + i])
             for i in range(2)]
    cp_w1 = pltpu.make_async_copy(w1_hbm, w1.bitcast(bf16), sems.at[6])
    cp_w2 = pltpu.make_async_copy(w2_hbm, w2.bitcast(bf16), sems.at[7])
    cp_w3 = [pltpu.make_async_copy(w3_hbm.at[:, pl.ds(c * FC, FC)], w3.at[c].bitcast(bf16),
                                   sems.at[8])
             for c in range(F // FC)]
    cp_w4 = pltpu.make_async_copy(w4_hbm, w4.bitcast(bf16), sems.at[9])

    TC = 256
    NTC = D // TC

    def cp_stage(i, c):
        src = (wq_hbm, wv_hbm)[i]
        return pltpu.make_async_copy(src.at[pl.ds(c * TC, TC)], stage.at[i * NTC + c],
                                     tsems.at[i * NTC + c])

    for i in range(2):
        for c in range(NTC):
            cp_stage(i, c).start()
    for cp in (cp_x0, cp_wk[0], cp_wo[0]):
        cp.start()

    kk = jax.lax.broadcasted_iota(jnp.int32, (128, 512), 0)
    qq = jax.lax.broadcasted_iota(jnp.int32, (128, 512), 1) % 128
    bias[...] = jnp.where(kk > qq, MASK_BIAS, 0.0).astype(f32)
    bt = jnp.broadcast_to(beta_ref[...].astype(f32), (H, H))
    eye = (jax.lax.broadcasted_iota(jnp.int32, (H, H), 0)
           == jax.lax.broadcasted_iota(jnp.int32, (H, H), 1))
    bcol = jnp.sum(jnp.where(eye, bt, 0.0), axis=1, keepdims=True)
    gsig = jnp.broadcast_to(jax.nn.sigmoid(bcol), (H, 128))
    gate[0] = gsig[0:H // 2]
    gate[1] = gsig[H // 2:H]
    hbuf[0:2 * HALO, :] = jnp.zeros((2 * HALO, D), f32)
    hbuf[S:PAD_ROWS, :] = jnp.zeros((2 * HALO, D), f32)
    for ref in (big, yres):
        ref[0:HALO, :] = jnp.zeros((HALO, D), f32)
        ref[S + HALO:PAD_ROWS, :] = jnp.zeros((HALO, D), f32)

    ident = (jax.lax.broadcasted_iota(jnp.int32, (128, 128), 0)
             == jax.lax.broadcasted_iota(jnp.int32, (128, 128), 1)).astype(f32).astype(bf16)

    def transpose_chunk(ic, _):
        pltpu.make_async_copy(stage.at[ic], stage.at[ic], tsems.at[ic]).wait()
        i = ic >> 2
        c = ic & 3
        ro = pl.multiple_of(i * DHALF, DHALF)
        for n in range(D // 128):
            tile = _dot_nt(ident, stage[ic, :, n * 128:(n + 1) * 128])
            wt[n // 4, c, _hs(ro + (n % 4) * 128, 128), :] = _pack(tile)
        return 0
    jax.lax.fori_loop(0, 2 * NTC, transpose_chunk, 0)

    cp_x0.wait()

    def init_x(i, _):
        r = pl.multiple_of(i * 256, 256)
        xv = xin[pl.ds(r, 256), :].astype(f32)
        big[pl.ds(HALO + r, 256), :] = xv
        xna[_hs(r, 256), :] = _pack(_ln(xv))
        return 0
    jax.lax.fori_loop(0, L // 256, init_x, 0)
    cp_wk[0].wait()
    for cp in [cp_wk[1], cp_wo[1], cp_w1, cp_xr, cp_w2] + cp_w3 + [cp_w4]:
        cp.start()

    def qmask(g, t):
        z = jnp.zeros((DH, 128), bf16)
        cols = []
        for h in range(4):
            qh = _unpack(qt[g, _hs(h * DH, DH), t * 128:(t + 1) * 128])
            cols.append(jnp.concatenate([qh if i == h else z for i in range(4)], axis=0))
        return jnp.concatenate(cols, axis=1)

    def attn_step(half, g, gn, fill=()):
        pr = None if g is None else g % 2
        pw = None if gn is None else gn % 2
        fill = list(fill)
        for t in range(NT_TILES):
            macc = None
            oacc = [None] * 4
            lacc = [None] * 4
            for j in range(t + 1):
                ks = slice(j * 128, (j + 1) * 128)
                if fill and (t, j) != (0, 0):
                    fill.pop(0)()
                if gn is not None:
                    s = _dot(_unpack(kb[gn, _hs(j * 128, 128), :]), qmask(gn, t))
                    if j == t:
                        s = s + bias[...]
                    sbuf[pw][t][0, ks, :] = s
                    mx = _red8(s, jnp.maximum)
                    macc = mx if macc is None else jnp.maximum(macc, mx)
                if g is not None:
                    for h in range(4):
                        sl = slice(h * 128, (h + 1) * 128)
                        p = jnp.exp2(sbuf[pr][t][half >> 1, ks, sl] - mbuf[t][pr, :, sl])
                        lt = _red8(p, jnp.add)
                        lacc[h] = lt if lacc[h] is None else lacc[h] + lt
                        o = _dot(_unpack(vt[g, _hs(h * DH, DH), ks]), p.astype(bf16))
                        oacc[h] = o if oacc[h] is None else oacc[h] + o
            if gn is not None:
                mbuf[t][pw] = jnp.max(macc, axis=0, keepdims=True)
            if g is not None:
                parts = []
                for h in range(4):
                    l = jnp.sum(lacc[h], axis=0, keepdims=True)
                    gh = gate[half, g * 4 + h:g * 4 + h + 1, :]
                    parts.append(oacc[h] * ((1.0 - gh) / l))
                ot = jnp.concatenate(parts, axis=0) + amem[g, :, t * 128:(t + 1) * 128]
                if g < GH - 1 or t < 2:
                    ob[g, _hs(t * 128, 128), :] = _pack(ot.T)
                else:
                    obl[half, _hs((t - 2) * 128, 128), :] = _pack(ot.T)

    rowh = jax.lax.broadcasted_iota(jnp.int32, (128, 128), 0) // DH
    colh = jax.lax.broadcasted_iota(jnp.int32, (128, 128), 1) // DH
    row16 = jax.lax.broadcasted_iota(jnp.int32, (16, 128), 0)
    col16 = jax.lax.broadcasted_iota(jnp.int32, (16, 128), 1) // DH

    def attn_half(layer, seg, half):
        r0 = pl.multiple_of(seg * L, L)

        @pl.when(jnp.logical_and(jnp.logical_and(layer == 0, seg == 0), half == 1))
        def _():
            cp_wk[1].wait()
            cp_wo[1].wait()
            cp_w1.wait()
            cp_xr.wait()
            cp_w2.wait()

        def xn(c0, nc):
            return _unpack(xna[_hs(c0 * 128, nc * 128), :])

        zparts = {}

        def k_piece(g0, ng, c0, nc):
            k = _dot(xn(c0, nc), _unpack(wk[half, :, g0 * 128:(g0 + ng) * 128]))
            pk = _phi(k)
            rs = _hs(c0 * 128, nc * 128)
            for i in range(ng):
                cs = slice(i * 128, (i + 1) * 128)
                kb[g0 + i, rs, :] = _pack(k[:, cs])
                pkb[g0 + i, rs, :] = _pack(pk[:, cs])
                zparts.setdefault(g0 + i, []).append(_red8(pk[:, cs], jnp.add))

        def qv_piece(qs, vs, c0, nc):
            offs = [g * 128 for g in qs] + [DHALF + g * 128 for g in vs]
            lhs = jnp.concatenate(
                [jnp.concatenate([wt[half, c, _hs(o, 128), :] for c in range(NTC)], axis=1)
                 for o in offs], axis=0)
            r = _dot_nt(_unpack(lhs), xn(c0, nc))
            ts = slice(c0 * 128, (c0 + nc) * 128)
            for i, g in enumerate(qs):
                qg = r[i * 128:(i + 1) * 128, :]
                qt[g, :, ts] = _pack(qg * QSCALE)
                pqt[g, :, ts] = _pack(_phi(qg))
            for i, g in enumerate(vs):
                o = (len(qs) + i) * 128
                vt[g, :, ts] = _pack(r[o:o + 128, :])

        def mem(g):
            zold = zrow[half, g]
            mold = mt[half, g]
            mbd = jnp.where(rowh == colh, mold, 0.0)
            zx = jnp.where(row16 == col16, jnp.broadcast_to(zold, (16, 128)), 0.0)
            lhs = jnp.concatenate([mbd, zx], axis=0).astype(bf16)
            ret = _dot(lhs, _unpack(pqt[g]))
            parts = []
            for h in range(4):
                gh = gate[half, g * 4 + h:g * 4 + h + 1, 0:1]
                den = ret[128 + h:129 + h, :] + 1e-6
                parts.append(ret[h * DH:(h + 1) * DH, :] * (gh / den))
            amem[g] = jnp.concatenate(parts, axis=0)
            mt[half, g] = mold + _dot(_unpack(vt[g]), _unpack(pkb[g]))
            zsum = functools.reduce(jnp.add, zparts[g])
            zrow[half, g] = zold + jnp.sum(zsum, axis=0, keepdims=True)

        P = functools.partial
        skip = lambda: None
        k_piece(0, 2, 0, 4)
        qv_piece((0, 1), (0,), 0, 4)

        @pl.when(jnp.logical_and(jnp.logical_and(layer == 0, seg == 0), half == 0))
        def _():
            cp_wo[0].wait()

        attn_step(half, None, 0)
        mem(0)
        for g in range(2):
            attn_step(half, g, g + 1, fill=[
                P(k_piece, g + 2, 1, 0, 2), skip, P(qv_piece, (g + 2,), (g + 1,), 0, 1),
                P(qv_piece, (g + 2,), (g + 1,), 1, 1), skip, P(k_piece, g + 2, 1, 2, 2),
                P(qv_piece, (g + 2,), (g + 1,), 2, 1), P(qv_piece, (g + 2,), (g + 1,), 3, 1),
                P(mem, g + 1)])
        attn_step(half, 2, 3, fill=[
            skip, P(qv_piece, (), (3,), 0, 1), skip, P(qv_piece, (), (3,), 1, 1), skip,
            P(qv_piece, (), (3,), 2, 1), P(qv_piece, (), (3,), 3, 1), skip, P(mem, 3)])

        def wo_piece(t, n):
            off = t * 128
            cs = slice(n * DHALF, (n + 1) * DHALF)
            rr = pl.ds(r0 + (HALO + off), 128)
            ng = GH if t < 2 else GH - 1
            o = jnp.concatenate([ob[g, _hs(off, 128), :] for g in range(ng)], axis=1)
            big[rr, cs] = big[rr, cs] + _dot(_unpack(o), _unpack(wo[half, _hs(0, ng * 128), cs]))

        attn_step(half, GH - 1, None,
                  fill=[P(wo_piece, t, n) for t in (2, 3, 0, 1) for n in range(2)])

    def phase_a(layer, seg):
        r0 = pl.multiple_of(seg * L, L)

        def half_body(half, _):
            attn_half(layer, seg, half)
            return 0
        jax.lax.fori_loop(0, 2, half_body, 0)

        hl = L // 2
        kp = (GH - 1) * 128

        bw = big.at[pl.ds(r0, 2 * L + 2 * HALO), :]
        yw = yres.at[pl.ds(r0, L + 2 * HALO), :]
        hw = hbuf.at[pl.ds(r0, L + 2 * HALO), :]
        xw = xin.at[pl.ds(r0 + L, L), :]

        def wo_rest():
            rr = slice(HALO + hl, HALO + L)
            o = _unpack(jnp.concatenate([obl[0], obl[1]], axis=1))
            w = _unpack(jnp.concatenate([wo[i, _hs(kp, 128), :] for i in range(2)], axis=0))
            bw[rr, :] = bw[rr, :] + _dot(o, w)

        def lnln(off, n):
            rr = slice(HALO + off, HALO + off + n)
            r, mr, z = _ln_ln(bw[rr, :])
            yw[rr, D - 256:D - 128] = jnp.broadcast_to(r, (n, 128))
            yw[rr, D - 128:D] = jnp.broadcast_to(mr, (n, 128))
            xnb[_hs(off, n), :] = _pack(z)

        def corners(v):
            return [v[0:8, 0:128], v[hl - 8:hl, 0:128], v[0:8, 128:256], v[hl - 8:hl, 128:256]]

        def up(off, n):
            cs = slice(n * 256, (n + 1) * 256)
            hh = _gelu(_dot(_unpack(xnb[_hs(off, hl), :]), _unpack(w1[:, cs])))
            b = off + HALO + SHIFTS[n]
            hw[b:b + hl, cs] = hh
            return corners(hh)

        sink = PIN + pl.multiple_of(seg * 16, 16)

        def pin(ref, v):
            if ref.dtype == bf16:
                ref[pl.ds(sink, 16), 0:128] = jnp.concatenate([v, v], axis=0).astype(bf16)
            else:
                ref[pl.ds(sink, 8), 0:128] = v

        fresh = jnp.logical_and(layer == 0, seg < NSEG - 1)

        def ln_next(off, n):
            rr = slice(L + HALO + off, L + HALO + off + n)
            xv = jnp.where(fresh, xw[off:off + n, :].astype(f32), bw[rr, :])
            bw[rr, :] = xv
            xna[_hs(off, n), :] = _pack(_ln(xv))

        lnln(0, 128)
        lnln(128, 128)
        wo_rest()
        def mix_part(off, n):
            return corners(mix(hw, yw, bw, slice(off, off + hl), n))

        def fence():
            pin(yres, pltpu.bitcast(xna[pl.ds(pl.multiple_of(seg * 8, 8), 8), 0:128], f32))

        late = list(range(hl, L, 16))
        nxt = list(range(0, L, 16))
        for n in range(4):
            marks = up(0, n)
            for i in (0, 1, 3):
                lnln(late.pop(0), 16)
                pin(big, marks[i])
        for n in range(4):
            marks = mix_part(0, n)
            for i in range(4):
                if late:
                    lnln(late.pop(0), 16)
                else:
                    ln_next(nxt.pop(0), 16)
                if n > 0 or i == 3:
                    pin(xin, marks[i])
        for n in range(4):
            marks = up(hl, n)
            for i in (0, 1, 3):
                ln_next(nxt.pop(0), 16)
                pin(xin, marks[i])
        for n in range(4):
            if n == 3:
                fence()
            marks = mix_part(hl, n)
            for i in range(4):
                if nxt:
                    ln_next(nxt.pop(0), 16)
                    pin(xin, marks[i])

    def mix(h_ref, y_ref, x_ref, rr, n):
        cs = slice(n * 256, (n + 1) * 256)
        r = y_ref[rr, D - 256:D - 128]
        mr = y_ref[rr, D - 128:D]
        x = x_ref[rr, cs]
        y = x * jnp.concatenate([r, r], axis=1) - jnp.concatenate([mr, mr], axis=1)
        x1 = y + _dot(h_ref[rr, :].astype(bf16), _unpack(w2[:, cs]))
        y_ref[rr, cs] = x1
        x_ref[rr, cs] = x + x1
        return x1

    def ln_mid(tok, n):
        xnc[_hs(tok, n), :] = _pack(_ln(yres[pl.ds(tok + HALO, n), :]))

    def last_rows():
        for n in range(4):
            mix(hbuf, yres, big, slice(S, PAD_ROWS), n)
            ln_mid(n * 128, 128)

    def out_copy(blk):
        rows = pl.ds(blk * L, L)
        return pltpu.make_async_copy(obuf.at[rows], out_hbm.at[0, rows, :], osems.at[blk])

    def ffn(layer, it):
        def block_of(pair):
            return (pair * 37) >> 8

        blk, chunk, tok = [], [], []
        for h in range(UNROLL // 2):
            pair = (UNROLL // 2) * it + h
            b = block_of(pair)
            c = 2 * pair - NC * b
            t = pl.multiple_of(b * L, L)
            blk += [b, b]
            chunk += [c, c + 1]
            tok += [t, t]

        def ffn_up(k):
            hh = _gelu(_dot(_unpack(xnc[_hs(tok[k], L), :]), _unpack(w3[chunk[k]])))
            gh[k % 2] = _pack(hh)
            return hh[L - 8:L, FC - 128:FC]

        def ffn_down(k):
            rows = pl.ds(tok[k] + HALO, L)
            w = _unpack(w4[_hs(chunk[k] * FC, FC), :])
            big[rows, :] = big[rows, :] + _dot(_unpack(gh[k % 2]), w)

        def ln_ahead(k, mark):
            yres[pl.ds(PIN + pl.multiple_of(blk[0] * 16, 16), 8), 0:128] = mark
            nb = jnp.minimum(blk[k] + 1, NSEG - 1)
            ln_mid(pl.multiple_of(nb * L + jnp.minimum(chunk[k] * 40, L - 80), 16), 80)

        def ln_first():
            r = pl.multiple_of(jnp.clip((it - 4) * 64, 0, L - 64), 64)
            xna[_hs(r, 64), :] = _pack(_ln(big[pl.ds(r + HALO, 64), :]))

        ffn_up(0)
        ln_ahead(0, ffn_up(1))
        ffn_down(0)
        ln_ahead(2, ffn_up(2))
        ffn_down(1)
        ln_first()
        ffn_up(3)
        ffn_down(2)
        ffn_down(3)

        done = block_of((UNROLL // 2) * (it + 1))

        @pl.when(jnp.logical_and(layer == 1, done != blk[0]))
        def _():
            r = pl.multiple_of((done - 1) * L, L)
            obuf[pl.ds(r, L), :] = big[pl.ds(r + HALO, L), :].astype(bf16)
            out_copy(done - 1).start()

    def layer_body(layer, _):
        mt[...] = jnp.zeros(mt.shape, f32)
        zrow[...] = jnp.zeros(zrow.shape, f32)

        def a_body(seg, _):
            phase_a(layer, seg)
            return 0
        jax.lax.fori_loop(0, NSEG, a_body, 0)

        last_rows()

        @pl.when(layer == 0)
        def _():
            for c in cp_w3:
                c.wait()
            cp_w4.wait()

        def b_body(it, _):
            ffn(layer, it)
            return 0
        jax.lax.fori_loop(0, NSEG * NC // UNROLL, b_body, 0)
        return 0
    jax.lax.fori_loop(0, 2, layer_body, 0)

    for blk in range(NSEG):
        out_copy(blk).wait()


@jax.jit
def pallas_interleave_layers__memory_aug_infini_attn__mixer_s_mlp__prompt_kernel(
    A_x: jax.Array,
    A_wq: jax.Array,
    A_wk: jax.Array,
    A_wv: jax.Array,
    A_wo: jax.Array,
    A_beta: jax.Array,
    B_x: jax.Array,
    B_w1: jax.Array,
    B_w2: jax.Array,
    B_w3: jax.Array,
    B_w4: jax.Array,
):
    del B_x
    hbm = pl.BlockSpec(memory_space=pl.ANY)
    vm = pltpu.VMEM
    scratch = [
        vm((BIG_ROWS, D), bf16),
        vm((8, 256, D), bf16),
        vm((2, 4, D // 2, 256), u32),
        vm((2, D // 2, DHALF), u32),
        vm((2, DHALF // 2, D), u32),
        vm((D // 2, D), u32),
        vm((D // 2, D), u32),
        vm((NC, D // 2, FC), u32),
        vm((F // 2, D), u32),
        vm((BIG_ROWS, D), f32),
        vm((BIG_ROWS, D), f32),
        vm((PAD_ROWS, D), f32),
        vm((L // 2, D), u32),
        vm((L // 2, D), u32),
        vm((S // 2, D), u32),
        vm((2, L // 2, FC), u32),
        vm((GH, 64, L), u32),
        vm((GH, 64, L), u32),
        vm((GH, L // 2, 128), u32),
        vm((GH, L // 2, 128), u32),
        vm((GH, 64, L), u32),
        vm((GH, L // 2, 128), u32),
        vm((2, L // 4, 128), u32),
        vm((GH, 128, L), f32),
        vm((2, GH, 128, 128), f32),
        vm((2, GH, 1, 128), f32),
        vm((2, H // 2, 128), f32),
        vm((128, 512), f32),
    ]
    scratch += [vm((1, 128 * (t + 1), 512), f32) for _ in range(2) for t in range(NT_TILES)]
    scratch += [vm((2, 1, 512), f32) for _ in range(NT_TILES)]
    scratch += [
        vm((S, D), bf16),
        pltpu.SemaphoreType.DMA((10,)),
        pltpu.SemaphoreType.DMA((8,)),
        pltpu.SemaphoreType.DMA((NSEG,)),
    ]
    return pl.pallas_call(
        _kernel,
        out_shape=jax.ShapeDtypeStruct((1, S, D), bf16),
        in_specs=[hbm, hbm, hbm, hbm, hbm, pl.BlockSpec(memory_space=pltpu.VMEM),
                  hbm, hbm, hbm, hbm],
        out_specs=hbm,
        scratch_shapes=scratch,
        compiler_params=pltpu.CompilerParams(vmem_limit_bytes=120 * 1024 * 1024),
    )(A_x, A_wq, A_wk, A_wv, A_wo, A_beta.reshape(1, H), B_w1, B_w2, B_w3, B_w4)
```

```python
import functools
import math

import jax
import jax.numpy as jnp
import jax.experimental.pallas as pl
import jax.experimental.pallas.tpu as pltpu

S = 2048
D = 1024
F = 3584
H = 32
DH = 32
L = 512
NSEG = S // L
NG = D // 128
NT_TILES = L // 128
FC = 256
HALO = 8
GH = NG // 2
DHALF = D // 2
PAD_ROWS = S + 2 * HALO
PIN = S + L + 2 * HALO
BIG_ROWS = PIN + 16 * NSEG
NC = F // FC
UNROLL = 4
SHIFTS = (1, -1, 2, -2)

LOG2E = math.log2(math.e)
QSCALE = DH ** -0.5 * LOG2E
MASK_BIAS = -1e9 * LOG2E
EPS = 1e-5

f32 = jnp.float32
bf16 = jnp.bfloat16
u32 = jnp.uint32
NT_DIMS = (((1,), (1,)), ((), ()))


def _stats(x):
    m = jnp.mean(x, axis=-1, keepdims=True)
    xc = x - m
    return m, jnp.mean(xc * xc, axis=-1, keepdims=True)


def _ln(x):
    m, v = _stats(x)
    r = jax.lax.rsqrt(v + EPS)
    return x * r - m * r


def _ln_ln(x):
    m, v = _stats(x)
    r1 = jax.lax.rsqrt(v + EPS)
    r2 = r1 * jax.lax.rsqrt(v * r1 * r1 + EPS)
    return r1, m * r1, x * r2 - m * r2


def _gelu(x):
    c = math.sqrt(2.0 / math.pi)
    inner = x * (c + (c * 0.044715) * (x * x))
    hx = 0.5 * x
    return hx + hx * jnp.tanh(inner)


def _phi(t):
    return jnp.where(t > 0, t + 1.0, jnp.exp(t))


def _red8(x, op):
    return functools.reduce(op, [x[i * 8:(i + 1) * 8] for i in range(x.shape[0] // 8)])


def _pack(x):
    return pltpu.bitcast(x.astype(bf16), u32)


def _unpack(x):
    return pltpu.bitcast(x, bf16)


def _hs(start, n):
    if isinstance(start, int):
        return slice(start // 2, (start + n) // 2)
    return pl.ds(pl.multiple_of(start >> 1, 8), n // 2)


def _dot(a, b):
    return jnp.dot(a, b, preferred_element_type=f32)


def _dot_nt(a, b):
    return jax.lax.dot_general(a, b, NT_DIMS, preferred_element_type=f32)


def _kernel(x_hbm, wq_hbm, wk_hbm, wv_hbm, wo_hbm, beta_ref, w1_hbm, w2_hbm, w3_hbm, w4_hbm,
            out_hbm,
            xin, stage, wt, wk, wo, w1, w2, w3, w4,
            big, yres, hbuf, xna, xnb, xnc, gh, qt, pqt, kb, pkb, vt, ob, obl, amem,
            mt, zrow, gate, bias,
            s0, s1, s2, s3, s4, s5, s6, s7, m0, m1, m2, m3,
            obuf, sems, tsems, osems):
    sbuf = ((s0, s1, s2, s3), (s4, s5, s6, s7))
    mbuf = (m0, m1, m2, m3)

    def seg_rows(s):
        return pl.ds(s * L, L)

    cp_x0 = pltpu.make_async_copy(x_hbm.at[0, seg_rows(0)], xin.at[seg_rows(0)], sems.at[0])
    cp_xr = pltpu.make_async_copy(x_hbm.at[0, pl.ds(L, S - L)], xin.at[pl.ds(L, S - L)], sems.at[1])
    cp_wk = [pltpu.make_async_copy(wk_hbm.at[:, pl.ds(i * DHALF, DHALF)], wk.at[i].bitcast(bf16),
                                   sems.at[2 + i])
             for i in range(2)]
    cp_wo = [pltpu.make_async_copy(wo_hbm.at[pl.ds(i * DHALF, DHALF)], wo.at[i].bitcast(bf16),
                                   sems.at[4 + i])
             for i in range(2)]
    cp_w1 = pltpu.make_async_copy(w1_hbm, w1.bitcast(bf16), sems.at[6])
    cp_w2 = pltpu.make_async_copy(w2_hbm, w2.bitcast(bf16), sems.at[7])
    cp_w3 = [pltpu.make_async_copy(w3_hbm.at[:, pl.ds(c * FC, FC)], w3.at[c].bitcast(bf16),
                                   sems.at[8])
             for c in range(F // FC)]
    cp_w4 = pltpu.make_async_copy(w4_hbm, w4.bitcast(bf16), sems.at[9])

    TC = 256
    NTC = D // TC

    def cp_stage(i, c):
        src = (wq_hbm, wv_hbm)[i]
        return pltpu.make_async_copy(src.at[pl.ds(c * TC, TC)], stage.at[i * NTC + c],
                                     tsems.at[i * NTC + c])

    for i in range(2):
        for c in range(NTC):
            cp_stage(i, c).start()
    for cp in (cp_x0, cp_wk[0], cp_wo[0]):
        cp.start()

    kk = jax.lax.broadcasted_iota(jnp.int32, (128, 512), 0)
    qq = jax.lax.broadcasted_iota(jnp.int32, (128, 512), 1) % 128
    bias[...] = jnp.where(kk > qq, MASK_BIAS, 0.0).astype(f32)
    bt = jnp.broadcast_to(beta_ref[...].astype(f32), (H, H))
    eye = (jax.lax.broadcasted_iota(jnp.int32, (H, H), 0)
           == jax.lax.broadcasted_iota(jnp.int32, (H, H), 1))
    bcol = jnp.sum(jnp.where(eye, bt, 0.0), axis=1, keepdims=True)
    gsig = jnp.broadcast_to(jax.nn.sigmoid(bcol), (H, 128))
    gate[0] = gsig[0:H // 2]
    gate[1] = gsig[H // 2:H]
    hbuf[0:2 * HALO, :] = jnp.zeros((2 * HALO, D), f32)
    hbuf[S:PAD_ROWS, :] = jnp.zeros((2 * HALO, D), f32)
    for ref in (big, yres):
        ref[0:HALO, :] = jnp.zeros((HALO, D), f32)
        ref[S + HALO:PAD_ROWS, :] = jnp.zeros((HALO, D), f32)

    ident = (jax.lax.broadcasted_iota(jnp.int32, (128, 128), 0)
             == jax.lax.broadcasted_iota(jnp.int32, (128, 128), 1)).astype(f32).astype(bf16)

    def transpose_chunk(ic, _):
        pltpu.make_async_copy(stage.at[ic], stage.at[ic], tsems.at[ic]).wait()
        i = ic >> 2
        c = ic & 3
        ro = pl.multiple_of(i * DHALF, DHALF)
        for n in range(D // 128):
            tile = _dot_nt(ident, stage[ic, :, n * 128:(n + 1) * 128])
            wt[n // 4, c, _hs(ro + (n % 4) * 128, 128), :] = _pack(tile)
        return 0
    jax.lax.fori_loop(0, 2 * NTC, transpose_chunk, 0)

    cp_x0.wait()

    def init_x(i, _):
        r = pl.multiple_of(i * 256, 256)
        xv = xin[pl.ds(r, 256), :].astype(f32)
        big[pl.ds(HALO + r, 256), :] = xv
        xna[_hs(r, 256), :] = _pack(_ln(xv))
        return 0
    jax.lax.fori_loop(0, L // 256, init_x, 0)
    cp_wk[0].wait()
    for cp in [cp_wk[1], cp_wo[1], cp_w1, cp_xr, cp_w2] + cp_w3 + [cp_w4]:
        cp.start()
    cp_wo[0].wait()

    def qmask(g, t):
        z = jnp.zeros((DH, 128), bf16)
        cols = []
        for h in range(4):
            qh = _unpack(qt[g, _hs(h * DH, DH), t * 128:(t + 1) * 128])
            cols.append(jnp.concatenate([qh if i == h else z for i in range(4)], axis=0))
        return jnp.concatenate(cols, axis=1)

    def attn_step(half, g, gn, last, fill=()):
        pr = None if g is None else g % 2
        pw = None if gn is None else gn % 2
        fill = list(fill)
        for t in range(NT_TILES):
            macc = None
            oacc = [None] * 4
            lacc = [None] * 4
            for j in range(t + 1):
                ks = slice(j * 128, (j + 1) * 128)
                filled = fill.pop(0) if fill else None
                if filled:
                    filled()
                    last["pace"] = last["o"]
                elif gn is not None and g is not None:
                    last["pace"] = last["s"]
                if g is not None:
                    sbuf[pr][t][0, (t + 1) * 128:(t + 1) * 128 + 8, 0:128] = last["pace"]
                if gn is not None:
                    s = _dot(_unpack(kb[gn, _hs(j * 128, 128), :]), qmask(gn, t))
                    if j == t:
                        s = s + bias[...]
                    sbuf[pw][t][0, ks, :] = s
                    last["s"] = s[0:8, 0:128]
                    mx = _red8(s, jnp.maximum)
                    macc = mx if macc is None else jnp.maximum(macc, mx)
                if g is not None:
                    for h in range(4):
                        sl = slice(h * 128, (h + 1) * 128)
                        p = jnp.exp2(sbuf[pr][t][half >> 1, ks, sl] - mbuf[t][pr, :, sl])
                        lt = _red8(p, jnp.add)
                        lacc[h] = lt if lacc[h] is None else lacc[h] + lt
                        o = _dot(_unpack(vt[g, _hs(h * DH, DH), ks]), p.astype(bf16))
                        oacc[h] = o if oacc[h] is None else oacc[h] + o
                        if h == 0:
                            last["o"] = o[0:8, :]
            if gn is not None:
                mbuf[t][pw] = jnp.max(macc, axis=0, keepdims=True)
            if g is not None:
                parts = []
                for h in range(4):
                    l = jnp.sum(lacc[h], axis=0, keepdims=True)
                    gh = gate[half, g * 4 + h:g * 4 + h + 1, :]
                    parts.append(oacc[h] * ((1.0 - gh) / l))
                ot = jnp.concatenate(parts, axis=0) + amem[g, :, t * 128:(t + 1) * 128]
                if g < GH - 1 or t < 2:
                    ob[g, _hs(t * 128, 128), :] = _pack(ot.T)
                else:
                    obl[half, _hs((t - 2) * 128, 128), :] = _pack(ot.T)

    rowh = jax.lax.broadcasted_iota(jnp.int32, (128, 128), 0) // DH
    colh = jax.lax.broadcasted_iota(jnp.int32, (128, 128), 1) // DH
    row16 = jax.lax.broadcasted_iota(jnp.int32, (16, 128), 0)
    col16 = jax.lax.broadcasted_iota(jnp.int32, (16, 128), 1) // DH

    def attn_half(layer, seg, half):
        r0 = pl.multiple_of(seg * L, L)

        @pl.when(jnp.logical_and(jnp.logical_and(layer == 0, seg == 0), half == 1))
        def _():
            cp_wk[1].wait()
            cp_wo[1].wait()
            cp_w1.wait()
            cp_xr.wait()
            cp_w2.wait()

        def xn(c0, nc):
            return _unpack(xna[_hs(c0 * 128, nc * 128), :])

        zparts = {}

        def k_piece(g0, ng, c0, nc):
            k = _dot(xn(c0, nc), _unpack(wk[half, :, g0 * 128:(g0 + ng) * 128]))
            pk = _phi(k)
            rs = _hs(c0 * 128, nc * 128)
            for i in range(ng):
                cs = slice(i * 128, (i + 1) * 128)
                kb[g0 + i, rs, :] = _pack(k[:, cs])
                pkb[g0 + i, rs, :] = _pack(pk[:, cs])
                zparts.setdefault(g0 + i, []).append(_red8(pk[:, cs], jnp.add))

        def qv_piece(qs, vs, c0, nc):
            offs = [g * 128 for g in qs] + [DHALF + g * 128 for g in vs]
            lhs = jnp.concatenate(
                [jnp.concatenate([wt[half, c, _hs(o, 128), :] for c in range(NTC)], axis=1)
                 for o in offs], axis=0)
            r = _dot_nt(_unpack(lhs), xn(c0, nc))
            ts = slice(c0 * 128, (c0 + nc) * 128)
            for i, g in enumerate(qs):
                qg = r[i * 128:(i + 1) * 128, :]
                qt[g, :, ts] = _pack(qg * QSCALE)
                pqt[g, :, ts] = _pack(_phi(qg))
            for i, g in enumerate(vs):
                o = (len(qs) + i) * 128
                vt[g, :, ts] = _pack(r[o:o + 128, :])

        def mem(g):
            zold = zrow[half, g]
            mold = mt[half, g]
            mbd = jnp.where(rowh == colh, mold, 0.0)
            zx = jnp.where(row16 == col16, jnp.broadcast_to(zold, (16, 128)), 0.0)
            lhs = jnp.concatenate([mbd, zx], axis=0).astype(bf16)
            ret = _dot(lhs, _unpack(pqt[g]))
            parts = []
            for h in range(4):
                gh = gate[half, g * 4 + h:g * 4 + h + 1, 0:1]
                den = ret[128 + h:129 + h, :] + 1e-6
                parts.append(ret[h * DH:(h + 1) * DH, :] * (gh / den))
            amem[g] = jnp.concatenate(parts, axis=0)
            mt[half, g] = mold + _dot(_unpack(vt[g]), _unpack(pkb[g]))
            zsum = functools.reduce(jnp.add, zparts[g])
            zrow[half, g] = zold + jnp.sum(zsum, axis=0, keepdims=True)

        P = functools.partial
        skip = None
        last = {}
        k_piece(0, 2, 0, 4)
        qv_piece((0, 1), (0,), 0, 4)
        attn_step(half, None, 0, last)
        mem(0)
        for g in range(2):
            attn_step(half, g, g + 1, last, fill=[
                skip, P(k_piece, g + 2, 1, 0, 2), skip, P(qv_piece, (g + 2,), (g + 1,), 0, 1),
                P(qv_piece, (g + 2,), (g + 1,), 1, 1), skip, P(k_piece, g + 2, 1, 2, 2),
                P(qv_piece, (g + 2,), (g + 1,), 2, 1), P(qv_piece, (g + 2,), (g + 1,), 3, 1),
                P(mem, g + 1)])
        attn_step(half, 2, 3, last, fill=[
            skip, skip, P(qv_piece, (), (3,), 0, 1), skip, P(qv_piece, (), (3,), 1, 1), skip,
            P(qv_piece, (), (3,), 2, 1), P(qv_piece, (), (3,), 3, 1), skip, P(mem, 3)])

        def wo_piece(t, n):
            off = t * 128
            cs = slice(n * DHALF, (n + 1) * DHALF)
            rr = pl.ds(r0 + (HALO + off), 128)
            ng = GH if t < 2 else GH - 1
            o = jnp.concatenate([ob[g, _hs(off, 128), :] for g in range(ng)], axis=1)
            big[rr, cs] = big[rr, cs] + _dot(_unpack(o), _unpack(wo[half, _hs(0, ng * 128), cs]))

        attn_step(half, GH - 1, None, last, fill=[
            P(wo_piece, 2, 0), P(wo_piece, 2, 1), P(wo_piece, 3, 0), skip, P(wo_piece, 3, 1),
            P(wo_piece, 0, 0), skip, P(wo_piece, 0, 1), P(wo_piece, 1, 0), skip])
        wo_piece(1, 1)

    def phase_a(layer, seg):
        r0 = pl.multiple_of(seg * L, L)

        def half_body(half, _):
            attn_half(layer, seg, half)
            return 0
        jax.lax.fori_loop(0, 2, half_body, 0)

        hl = L // 2
        kp = (GH - 1) * 128

        bw = big.at[pl.ds(r0, 2 * L + 2 * HALO), :]
        yw = yres.at[pl.ds(r0, L + 2 * HALO), :]
        hw = hbuf.at[pl.ds(r0, L + 2 * HALO), :]
        xw = xin.at[pl.ds(r0 + L, L), :]

        def wo_rest():
            rr = slice(HALO + hl, HALO + L)
            o = _unpack(jnp.concatenate([obl[0], obl[1]], axis=1))
            w = _unpack(jnp.concatenate([wo[i, _hs(kp, 128), :] for i in range(2)], axis=0))
            bw[rr, :] = bw[rr, :] + _dot(o, w)

        def lnln(off, n):
            rr = slice(HALO + off, HALO + off + n)
            r, mr, z = _ln_ln(bw[rr, :])
            yw[rr, D - 256:D - 128] = jnp.broadcast_to(r, (n, 128))
            yw[rr, D - 128:D] = jnp.broadcast_to(mr, (n, 128))
            xnb[_hs(off, n), :] = _pack(z)

        def corners(v):
            return [v[0:8, 0:128], v[hl - 8:hl, 0:128], v[0:8, 128:256], v[hl - 8:hl, 128:256]]

        def up(off, n):
            cs = slice(n * 256, (n + 1) * 256)
            hh = _gelu(_dot(_unpack(xnb[_hs(off, hl), :]), _unpack(w1[:, cs])))
            b = off + HALO + SHIFTS[n]
            hw[b:b + hl, cs] = hh
            return corners(hh)

        sink = PIN + pl.multiple_of(seg * 16, 16)

        def pin(ref, v):
            if ref.dtype == bf16:
                ref[pl.ds(sink, 16), 0:128] = jnp.concatenate([v, v], axis=0).astype(bf16)
            else:
                ref[pl.ds(sink, 8), 0:128] = v

        fresh = jnp.logical_and(layer == 0, seg < NSEG - 1)

        def ln_next(off, n):
            rr = slice(L + HALO + off, L + HALO + off + n)
            xv = jnp.where(fresh, xw[off:off + n, :].astype(f32), bw[rr, :])
            bw[rr, :] = xv
            xna[_hs(off, n), :] = _pack(_ln(xv))

        lnln(0, 128)
        lnln(128, 128)
        wo_rest()
        def mix_part(off, n):
            return corners(mix(hw, yw, bw, slice(off, off + hl), n))

        def fence():
            pin(yres, pltpu.bitcast(xna[pl.ds(pl.multiple_of(seg * 8, 8), 8), 0:128], f32))

        late = list(range(hl, L, 16))
        nxt = list(range(0, L, 16))
        for n in range(4):
            marks = up(0, n)
            for i in (0, 1, 3):
                lnln(late.pop(0), 16)
                pin(big, marks[i])
        for n in range(4):
            marks = mix_part(0, n)
            for i in range(4):
                if late:
                    lnln(late.pop(0), 16)
                else:
                    ln_next(nxt.pop(0), 16)
                if n > 0 or i == 3:
                    pin(xin, marks[i])
        for n in range(4):
            marks = up(hl, n)
            for i in (0, 1, 3):
                ln_next(nxt.pop(0), 16)
                pin(xin, marks[i])
        for n in range(4):
            if n == 3:
                fence()
            marks = mix_part(hl, n)
            for i in range(4):
                if nxt:
                    ln_next(nxt.pop(0), 16)
                    pin(xin, marks[i])

    def mix(h_ref, y_ref, x_ref, rr, n):
        cs = slice(n * 256, (n + 1) * 256)
        r = y_ref[rr, D - 256:D - 128]
        mr = y_ref[rr, D - 128:D]
        x = x_ref[rr, cs]
        y = x * jnp.concatenate([r, r], axis=1) - jnp.concatenate([mr, mr], axis=1)
        x1 = y + _dot(h_ref[rr, :].astype(bf16), _unpack(w2[:, cs]))
        y_ref[rr, cs] = x1
        x_ref[rr, cs] = x + x1
        return x1

    def ln_mid(tok, n):
        xnc[_hs(tok, n), :] = _pack(_ln(yres[pl.ds(tok + HALO, n), :]))

    def last_rows():
        for n in range(4):
            mix(hbuf, yres, big, slice(S, PAD_ROWS), n)
            ln_mid(n * 128, 128)

    def out_copy(blk):
        rows = pl.ds(blk * L, L)
        return pltpu.make_async_copy(obuf.at[rows], out_hbm.at[0, rows, :], osems.at[blk])

    def ffn(layer, it):
        def block_of(pair):
            return (pair * 37) >> 8

        blk, chunk, tok = [], [], []
        for h in range(UNROLL // 2):
            pair = (UNROLL // 2) * it + h
            b = block_of(pair)
            c = 2 * pair - NC * b
            t = pl.multiple_of(b * L, L)
            blk += [b, b]
            chunk += [c, c + 1]
            tok += [t, t]

        def ffn_up(k):
            hh = _gelu(_dot(_unpack(xnc[_hs(tok[k], L), :]), _unpack(w3[chunk[k]])))
            gh[k % 2] = _pack(hh)
            return hh[L - 8:L, FC - 128:FC]

        def ffn_down(k):
            rows = pl.ds(tok[k] + HALO, L)
            w = _unpack(w4[_hs(chunk[k] * FC, FC), :])
            big[rows, :] = big[rows, :] + _dot(_unpack(gh[k % 2]), w)

        def ln_ahead(k, mark):
            yres[pl.ds(PIN + pl.multiple_of(blk[0] * 16, 16), 8), 0:128] = mark
            nb = jnp.minimum(blk[k] + 1, NSEG - 1)
            ln_mid(pl.multiple_of(nb * L + jnp.minimum(chunk[k] * 40, L - 80), 16), 80)

        def ln_first():
            r = pl.multiple_of(jnp.clip((it - 4) * 64, 0, L - 64), 64)
            xna[_hs(r, 64), :] = _pack(_ln(big[pl.ds(r + HALO, 64), :]))

        ffn_up(0)
        ln_ahead(0, ffn_up(1))
        ffn_down(0)
        ln_ahead(2, ffn_up(2))
        ffn_down(1)
        ln_first()
        ffn_up(3)
        ffn_down(2)
        ffn_down(3)

        done = block_of((UNROLL // 2) * (it + 1))

        @pl.when(jnp.logical_and(layer == 1, done != blk[0]))
        def _():
            r = pl.multiple_of((done - 1) * L, L)
            obuf[pl.ds(r, L), :] = big[pl.ds(r + HALO, L), :].astype(bf16)
            out_copy(done - 1).start()

    def layer_body(layer, _):
        mt[...] = jnp.zeros(mt.shape, f32)
        zrow[...] = jnp.zeros(zrow.shape, f32)

        def a_body(seg, _):
            phase_a(layer, seg)
            return 0
        jax.lax.fori_loop(0, NSEG, a_body, 0)

        last_rows()

        @pl.when(layer == 0)
        def _():
            for c in cp_w3:
                c.wait()
            cp_w4.wait()

        def b_body(it, _):
            ffn(layer, it)
            return 0
        jax.lax.fori_loop(0, NSEG * NC // UNROLL, b_body, 0)
        return 0
    jax.lax.fori_loop(0, 2, layer_body, 0)

    for blk in range(NSEG):
        out_copy(blk).wait()


@jax.jit
def pallas_interleave_layers__memory_aug_infini_attn__mixer_s_mlp__prompt_kernel(
    A_x: jax.Array,
    A_wq: jax.Array,
    A_wk: jax.Array,
    A_wv: jax.Array,
    A_wo: jax.Array,
    A_beta: jax.Array,
    B_x: jax.Array,
    B_w1: jax.Array,
    B_w2: jax.Array,
    B_w3: jax.Array,
    B_w4: jax.Array,
):
    del B_x
    hbm = pl.BlockSpec(memory_space=pl.ANY)
    vm = pltpu.VMEM
    scratch = [
        vm((BIG_ROWS, D), bf16),
        vm((8, 256, D), bf16),
        vm((2, 4, D // 2, 256), u32),
        vm((2, D // 2, DHALF), u32),
        vm((2, DHALF // 2, D), u32),
        vm((D // 2, D), u32),
        vm((D // 2, D), u32),
        vm((NC, D // 2, FC), u32),
        vm((F // 2, D), u32),
        vm((BIG_ROWS, D), f32),
        vm((BIG_ROWS, D), f32),
        vm((PAD_ROWS, D), f32),
        vm((L // 2, D), u32),
        vm((L // 2, D), u32),
        vm((S // 2, D), u32),
        vm((2, L // 2, FC), u32),
        vm((GH, 64, L), u32),
        vm((GH, 64, L), u32),
        vm((GH, L // 2, 128), u32),
        vm((GH, L // 2, 128), u32),
        vm((GH, 64, L), u32),
        vm((GH, L // 2, 128), u32),
        vm((2, L // 4, 128), u32),
        vm((GH, 128, L), f32),
        vm((2, GH, 128, 128), f32),
        vm((2, GH, 1, 128), f32),
        vm((2, H // 2, 128), f32),
        vm((128, 512), f32),
    ]
    scratch += [vm((1, 128 * (t + 1) + 8, 512), f32) for _ in range(2) for t in range(NT_TILES)]
    scratch += [vm((2, 1, 512), f32) for _ in range(NT_TILES)]
    scratch += [
        vm((S, D), bf16),
        pltpu.SemaphoreType.DMA((10,)),
        pltpu.SemaphoreType.DMA((8,)),
        pltpu.SemaphoreType.DMA((NSEG,)),
    ]
    return pl.pallas_call(
        _kernel,
        out_shape=jax.ShapeDtypeStruct((1, S, D), bf16),
        in_specs=[hbm, hbm, hbm, hbm, hbm, pl.BlockSpec(memory_space=pltpu.VMEM),
                  hbm, hbm, hbm, hbm],
        out_specs=hbm,
        scratch_shapes=scratch,
        compiler_params=pltpu.CompilerParams(vmem_limit_bytes=120 * 1024 * 1024),
    )(A_x, A_wq, A_wk, A_wv, A_wo, A_beta.reshape(1, H), B_w1, B_w2, B_w3, B_w4)
```

```python
import functools
import math

import jax
import jax.numpy as jnp
import jax.experimental.pallas as pl
import jax.experimental.pallas.tpu as pltpu

S = 2048
D = 1024
F = 3584
H = 32
DH = 32
L = 512
NSEG = S // L
NG = D // 128
NT_TILES = L // 128
FC = 256
HALO = 8
GH = NG // 2
DHALF = D // 2
PAD_ROWS = S + 2 * HALO
PIN = S + L + 2 * HALO
BIG_ROWS = PIN + 16 * NSEG
NC = F // FC
UNROLL = 4
SHIFTS = (1, -1, 2, -2)

LOG2E = math.log2(math.e)
QSCALE = DH ** -0.5 * LOG2E
MASK_BIAS = -1e9 * LOG2E
EPS = 1e-5

f32 = jnp.float32
bf16 = jnp.bfloat16
u32 = jnp.uint32
NT_DIMS = (((1,), (1,)), ((), ()))


def _stats(x):
    m = jnp.mean(x, axis=-1, keepdims=True)
    xc = x - m
    return m, jnp.mean(xc * xc, axis=-1, keepdims=True)


def _ln(x):
    m, v = _stats(x)
    r = jax.lax.rsqrt(v + EPS)
    return x * r - m * r


def _ln_ln(x):
    m, v = _stats(x)
    r1 = jax.lax.rsqrt(v + EPS)
    r2 = r1 * jax.lax.rsqrt(v * r1 * r1 + EPS)
    return r1, m * r1, x * r2 - m * r2


def _gelu(x):
    c = math.sqrt(2.0 / math.pi)
    inner = x * (c + (c * 0.044715) * (x * x))
    hx = 0.5 * x
    return hx + hx * jnp.tanh(inner)


def _phi(t):
    return jnp.where(t > 0, t + 1.0, jnp.exp(t))


def _red8(x, op):
    return functools.reduce(op, [x[i * 8:(i + 1) * 8] for i in range(x.shape[0] // 8)])


def _pack(x):
    return pltpu.bitcast(x.astype(bf16), u32)


def _unpack(x):
    return pltpu.bitcast(x, bf16)


def _hs(start, n):
    if isinstance(start, int):
        return slice(start // 2, (start + n) // 2)
    return pl.ds(pl.multiple_of(start >> 1, 8), n // 2)


def _dot(a, b):
    return jnp.dot(a, b, preferred_element_type=f32)


def _dot_nt(a, b):
    return jax.lax.dot_general(a, b, NT_DIMS, preferred_element_type=f32)


def _kernel(x_hbm, wq_hbm, wk_hbm, wv_hbm, wo_hbm, beta_ref, w1_hbm, w2_hbm, w3_hbm, w4_hbm,
            out_hbm,
            xin, stage, wt, wk, wo, w1, w2, w3, w4,
            big, yres, hbuf, xna, xnb, xnc, gh, qt, pqt, kb, pkb, vt, ob, obl, amem,
            mt, zrow, gate, bias,
            s0, s1, s2, s3, s4, s5, s6, s7, m0, m1, m2, m3,
            obuf, sems, tsems, osems):
    sbuf = ((s0, s1, s2, s3), (s4, s5, s6, s7))
    mbuf = (m0, m1, m2, m3)

    def seg_rows(s):
        return pl.ds(s * L, L)

    cp_x0 = pltpu.make_async_copy(x_hbm.at[0, seg_rows(0)], xin.at[seg_rows(0)], sems.at[0])
    cp_xr = pltpu.make_async_copy(x_hbm.at[0, pl.ds(L, S - L)], xin.at[pl.ds(L, S - L)], sems.at[1])
    cp_wk = [pltpu.make_async_copy(wk_hbm.at[:, pl.ds(i * DHALF, DHALF)], wk.at[i].bitcast(bf16),
                                   sems.at[2 + i])
             for i in range(2)]
    cp_wo = [pltpu.make_async_copy(wo_hbm.at[pl.ds(i * DHALF, DHALF)], wo.at[i].bitcast(bf16),
                                   sems.at[4 + i])
             for i in range(2)]
    cp_w1 = pltpu.make_async_copy(w1_hbm, w1.bitcast(bf16), sems.at[6])
    cp_w2 = pltpu.make_async_copy(w2_hbm, w2.bitcast(bf16), sems.at[7])
    cp_w3 = [pltpu.make_async_copy(w3_hbm.at[:, pl.ds(c * FC, FC)], w3.at[c].bitcast(bf16),
                                   sems.at[8])
             for c in range(F // FC)]
    cp_w4 = pltpu.make_async_copy(w4_hbm, w4.bitcast(bf16), sems.at[9])

    TC = 256
    NTC = D // TC

    def cp_stage(i, c):
        src = (wq_hbm, wv_hbm)[i]
        return pltpu.make_async_copy(src.at[pl.ds(c * TC, TC)], stage.at[i * NTC + c],
                                     tsems.at[i * NTC + c])

    for i in range(2):
        for c in range(NTC):
            cp_stage(i, c).start()
    for cp in (cp_x0, cp_wk[0], cp_wo[0]):
        cp.start()

    kk = jax.lax.broadcasted_iota(jnp.int32, (128, 512), 0)
    ll = jax.lax.broadcasted_iota(jnp.int32, (128, 512), 1)
    qq = jnp.where(kk < 64, (ll + ((ll >> 7) & 1) * 64) & 127, 64 + (ll & 63))
    bias[...] = jnp.where(kk > qq, MASK_BIAS, 0.0).astype(f32)
    bt = jnp.broadcast_to(beta_ref[...].astype(f32), (H, H))
    eye = (jax.lax.broadcasted_iota(jnp.int32, (H, H), 0)
           == jax.lax.broadcasted_iota(jnp.int32, (H, H), 1))
    bcol = jnp.sum(jnp.where(eye, bt, 0.0), axis=1, keepdims=True)
    gsig = jnp.broadcast_to(jax.nn.sigmoid(bcol), (H, 128))
    gate[0] = gsig[0:H // 2]
    gate[1] = gsig[H // 2:H]
    hbuf[0:2 * HALO, :] = jnp.zeros((2 * HALO, D), f32)
    hbuf[S:PAD_ROWS, :] = jnp.zeros((2 * HALO, D), f32)
    for ref in (big, yres):
        ref[0:HALO, :] = jnp.zeros((HALO, D), f32)
        ref[S + HALO:PAD_ROWS, :] = jnp.zeros((HALO, D), f32)

    ident = (jax.lax.broadcasted_iota(jnp.int32, (128, 128), 0)
             == jax.lax.broadcasted_iota(jnp.int32, (128, 128), 1)).astype(f32).astype(bf16)

    def transpose_chunk(ic, _):
        pltpu.make_async_copy(stage.at[ic], stage.at[ic], tsems.at[ic]).wait()
        i = ic >> 2
        c = ic & 3
        ro = pl.multiple_of(i * DHALF, DHALF)
        for n in range(D // 128):
            tile = _dot_nt(ident, stage[ic, :, n * 128:(n + 1) * 128])
            wt[n // 4, c, _hs(ro + (n % 4) * 128, 128), :] = _pack(tile)
        return 0
    jax.lax.fori_loop(0, 2 * NTC, transpose_chunk, 0)

    cp_x0.wait()

    def init_x(i, _):
        r = pl.multiple_of(i * 256, 256)
        xv = xin[pl.ds(r, 256), :].astype(f32)
        big[pl.ds(HALO + r, 256), :] = xv
        xna[_hs(r, 256), :] = _pack(_ln(xv))
        return 0
    jax.lax.fori_loop(0, L // 256, init_x, 0)
    cp_wk[0].wait()
    for cp in [cp_wk[1], cp_wo[1], cp_w1, cp_xr, cp_w2] + cp_w3 + [cp_w4]:
        cp.start()
    cp_wo[0].wait()

    def qmask(g, t):
        z = jnp.zeros((DH, 128), bf16)
        cols = []
        for h in range(4):
            qh = _unpack(qt[g, _hs(h * DH, DH), t * 128:(t + 1) * 128])
            cols.append(jnp.concatenate([qh if i == h else z for i in range(4)], axis=0))
        return jnp.concatenate(cols, axis=1)

    def upper(x, h, other):
        lane = jax.lax.broadcasted_iota(jnp.int32, x.shape, 1)
        return jnp.where(lane < 64 if h % 2 else lane >= 64, x, other)

    def qpair(g, t):
        z = jnp.zeros((DH, 128), u32)
        qs = [upper(qt[g, _hs(h * DH, DH), t * 128:(t + 1) * 128], h, u32(0)) for h in range(4)]
        cols = [jnp.concatenate(qs[0:2] + [z], axis=0), jnp.concatenate([z] + qs[2:4], axis=0)]
        return _unpack(jnp.concatenate(cols, axis=1))

    def attn_step(half, g, gn, last, fill=()):
        pr = None if g is None else g % 2
        pw = None if gn is None else gn % 2
        fill = list(fill)
        for t in range(NT_TILES):
            macc = None
            oacc = [None] * 4
            lacc = [None] * 4
            for j in range(t + 1):
                ks = slice(j * 128, (j + 1) * 128)
                nk = 64 if j == t else 128
                kl = slice(j * 128, j * 128 + nk)
                ku = slice(j * 128 + 64, (j + 1) * 128)
                filled = fill.pop(0) if fill else None
                if filled:
                    filled()
                    last["pace"] = last["o"]
                elif gn is not None and g is not None:
                    last["pace"] = last["s"]
                if g is not None:
                    sbuf[pr][t][0, (t + 1) * 128:(t + 1) * 128 + 8, 0:128] = last["pace"]
                if gn is not None:
                    s = _dot(_unpack(kb[gn, _hs(j * 128, nk), :]), qmask(gn, t))
                    if j == t:
                        s = s + bias[0:64, :]
                    sbuf[pw][t][0, kl, :] = s
                    last["s"] = s[0:8, 0:128]
                    mx = _red8(s, jnp.maximum)
                    if j == t:
                        su = _dot(_unpack(kb[gn, _hs(j * 128 + 64, 64), :]), qpair(gn, t))
                        su = su + bias[64:128, 0:256]
                        sbuf[pw][t][0, ku, 0:256] = su
                        mu = _red8(su, jnp.maximum)
                        mx = jnp.concatenate(
                            [jnp.maximum(mx[:, h * 128:(h + 1) * 128],
                                         upper(mu[:, (h // 2) * 128:(h // 2 + 1) * 128], h,
                                               mx[:, h * 128:(h + 1) * 128]))
                             for h in range(4)], axis=1)
                    macc = mx if macc is None else jnp.maximum(macc, mx)
                if g is not None:
                    for h in range(4):
                        sl = slice(h * 128, (h + 1) * 128)
                        p = jnp.exp2(sbuf[pr][t][half >> 1, kl, sl] - mbuf[t][pr, :, sl])
                        lt = _red8(p, jnp.add)
                        p = p.astype(bf16)
                        if j == t:
                            if h % 2 == 0:
                                mu = upper(mbuf[t][pr, :, sl], h,
                                           mbuf[t][pr, :, (h + 1) * 128:(h + 2) * 128])
                                pu = jnp.exp2(
                                    sbuf[pr][t][half >> 1, ku, h * 64:h * 64 + 128] - mu)
                                lu = _red8(pu, jnp.add)
                                pu = _pack(pu)
                            lt = lt + upper(lu, h, 0.0)
                            p = _unpack(jnp.concatenate(
                                [pltpu.bitcast(p, u32), upper(pu, h, u32(0))], axis=0))
                        lacc[h] = lt if lacc[h] is None else lacc[h] + lt
                        o = _dot(_unpack(vt[g, _hs(h * DH, DH), ks]), p)
                        oacc[h] = o if oacc[h] is None else oacc[h] + o
                        if h == 0:
                            last["o"] = o[0:8, :]
            if gn is not None:
                mbuf[t][pw] = jnp.max(macc, axis=0, keepdims=True)
            if g is not None:
                parts = []
                for h in range(4):
                    l = jnp.sum(lacc[h], axis=0, keepdims=True)
                    gh = gate[half, g * 4 + h:g * 4 + h + 1, :]
                    oh = oacc[h] * ((1.0 - gh) / l)
                    parts.append(pltpu.roll(oh, 64, 1) if h % 2 else oh)
                ot = jnp.concatenate(parts, axis=0) + amem[g, :, t * 128:(t + 1) * 128]
                if g < GH - 1 or t < 2:
                    ob[g, _hs(t * 128, 128), :] = _pack(ot.T)
                else:
                    obl[half, _hs((t - 2) * 128, 128), :] = _pack(ot.T)

    rowh = jax.lax.broadcasted_iota(jnp.int32, (128, 128), 0) // DH
    colh = jax.lax.broadcasted_iota(jnp.int32, (128, 128), 1) // DH
    row16 = jax.lax.broadcasted_iota(jnp.int32, (16, 128), 0)
    col16 = jax.lax.broadcasted_iota(jnp.int32, (16, 128), 1) // DH

    def attn_half(layer, seg, half):
        r0 = pl.multiple_of(seg * L, L)

        @pl.when(jnp.logical_and(jnp.logical_and(layer == 0, seg == 0), half == 1))
        def _():
            cp_wk[1].wait()
            cp_wo[1].wait()
            cp_w1.wait()
            cp_xr.wait()
            cp_w2.wait()

        def xn(c0, nc):
            return _unpack(xna[_hs(c0 * 128, nc * 128), :])

        zparts = {}

        def k_piece(g0, ng, c0, nc):
            k = _dot(xn(c0, nc), _unpack(wk[half, :, g0 * 128:(g0 + ng) * 128]))
            pk = _phi(k)
            rs = _hs(c0 * 128, nc * 128)
            for i in range(ng):
                cs = slice(i * 128, (i + 1) * 128)
                kb[g0 + i, rs, :] = _pack(k[:, cs])
                pkb[g0 + i, rs, :] = _pack(pk[:, cs])
                zparts.setdefault(g0 + i, []).append(_red8(pk[:, cs], jnp.add))

        def qv_piece(qs, vs, c0, nc):
            offs = [g * 128 for g in qs] + [DHALF + g * 128 for g in vs]
            lhs = jnp.concatenate(
                [jnp.concatenate([wt[half, c, _hs(o, 128), :] for c in range(NTC)], axis=1)
                 for o in offs], axis=0)
            r = _dot_nt(_unpack(lhs), xn(c0, nc))
            ts = slice(c0 * 128, (c0 + nc) * 128)
            for i, g in enumerate(qs):
                qg = r[i * 128:(i + 1) * 128, :]
                qp = _pack(qg * QSCALE)
                for c in range(nc):
                    for h in range(4):
                        qh = qp[_hs(h * DH, DH), c * 128:(c + 1) * 128]
                        qt[g, _hs(h * DH, DH), (c0 + c) * 128:(c0 + c + 1) * 128] = (
                            pltpu.roll(qh, 64, 1) if h % 2 else qh)
                pqt[g, :, ts] = _pack(_phi(qg))
            for i, g in enumerate(vs):
                o = (len(qs) + i) * 128
                vt[g, :, ts] = _pack(r[o:o + 128, :])

        def mem(g):
            zold = zrow[half, g]
            mold = mt[half, g]
            mbd = jnp.where(rowh == colh, mold, 0.0)
            zx = jnp.where(row16 == col16, jnp.broadcast_to(zold, (16, 128)), 0.0)
            lhs = jnp.concatenate([mbd, zx], axis=0).astype(bf16)
            ret = _dot(lhs, _unpack(pqt[g]))
            parts = []
            for h in range(4):
                gh = gate[half, g * 4 + h:g * 4 + h + 1, 0:1]
                den = ret[128 + h:129 + h, :] + 1e-6
                parts.append(ret[h * DH:(h + 1) * DH, :] * (gh / den))
            amem[g] = jnp.concatenate(parts, axis=0)
            zsum = functools.reduce(jnp.add, zparts[g])
            zrow[half, g] = zold + jnp.sum(zsum, axis=0, keepdims=True)

        def upd(g):
            mt[half, g] = mt[half, g] + _dot(_unpack(vt[g]), _unpack(pkb[g]))

        def mem_upd(g):
            mem(g)
            upd(g)

        P = functools.partial
        skip = None
        last = {}
        k_piece(0, 2, 0, 4)
        qv_piece((0, 1), (0,), 0, 4)
        attn_step(half, None, 0, last)
        mem(0)
        for g in range(2):
            attn_step(half, g, g + 1, last, fill=[
                skip, P(k_piece, g + 2, 1, 0, 2), skip, P(qv_piece, (g + 2,), (g + 1,), 0, 1),
                P(qv_piece, (g + 2,), (g + 1,), 1, 1), skip, P(k_piece, g + 2, 1, 2, 2),
                P(qv_piece, (g + 2,), (g + 1,), 2, 1), P(qv_piece, (g + 2,), (g + 1,), 3, 1),
                P(mem_upd, g + 1)])
        attn_step(half, 2, 3, last, fill=[
            P(upd, 0), skip, P(qv_piece, (), (3,), 0, 1), skip, P(qv_piece, (), (3,), 1, 1),
            skip, P(qv_piece, (), (3,), 2, 1), P(qv_piece, (), (3,), 3, 1), skip, P(mem_upd, 3)])

        def wo_piece(t, n):
            off = t * 128
            cs = slice(n * DHALF, (n + 1) * DHALF)
            rr = pl.ds(r0 + (HALO + off), 128)
            ng = GH if t < 2 else GH - 1
            o = jnp.concatenate([ob[g, _hs(off, 128), :] for g in range(ng)], axis=1)
            big[rr, cs] = big[rr, cs] + _dot(_unpack(o), _unpack(wo[half, _hs(0, ng * 128), cs]))

        attn_step(half, GH - 1, None, last, fill=[
            P(wo_piece, 2, 0), P(wo_piece, 2, 1), P(wo_piece, 3, 0), skip, P(wo_piece, 3, 1),
            P(wo_piece, 0, 0), skip, P(wo_piece, 0, 1), P(wo_piece, 1, 0), skip])
        wo_piece(1, 1)

    def phase_a(layer, seg):
        r0 = pl.multiple_of(seg * L, L)

        def half_body(half, _):
            attn_half(layer, seg, half)
            return 0
        jax.lax.fori_loop(0, 2, half_body, 0)

        hl = L // 2
        kp = (GH - 1) * 128

        bw = big.at[pl.ds(r0, 2 * L + 2 * HALO), :]
        yw = yres.at[pl.ds(r0, L + 2 * HALO), :]
        hw = hbuf.at[pl.ds(r0, L + 2 * HALO), :]
        xw = xin.at[pl.ds(r0 + L, L), :]

        def wo_rest():
            rr = slice(HALO + hl, HALO + L)
            o = _unpack(jnp.concatenate([obl[0], obl[1]], axis=1))
            w = _unpack(jnp.concatenate([wo[i, _hs(kp, 128), :] for i in range(2)], axis=0))
            bw[rr, :] = bw[rr, :] + _dot(o, w)

        def lnln(off, n):
            rr = slice(HALO + off, HALO + off + n)
            r, mr, z = _ln_ln(bw[rr, :])
            yw[rr, D - 256:D - 128] = jnp.broadcast_to(r, (n, 128))
            yw[rr, D - 128:D] = jnp.broadcast_to(mr, (n, 128))
            xnb[_hs(off, n), :] = _pack(z)

        def corners(v):
            return [v[0:8, 0:128], v[hl - 8:hl, 0:128], v[0:8, 128:256], v[hl - 8:hl, 128:256]]

        def up(off, n):
            cs = slice(n * 256, (n + 1) * 256)
            hh = _gelu(_dot(_unpack(xnb[_hs(off, hl), :]), _unpack(w1[:, cs])))
            b = off + HALO + SHIFTS[n]
            hw[b:b + hl, cs] = hh
            return corners(hh)

        sink = PIN + pl.multiple_of(seg * 16, 16)

        def pin(ref, v):
            if ref.dtype == bf16:
                ref[pl.ds(sink, 16), 0:128] = jnp.concatenate([v, v], axis=0).astype(bf16)
            else:
                ref[pl.ds(sink, 8), 0:128] = v

        fresh = jnp.logical_and(layer == 0, seg < NSEG - 1)

        def ln_next(off, n):
            rr = slice(L + HALO + off, L + HALO + off + n)
            xv = jnp.where(fresh, xw[off:off + n, :].astype(f32), bw[rr, :])
            bw[rr, :] = xv
            xna[_hs(off, n), :] = _pack(_ln(xv))

        lnln(0, 128)
        lnln(128, 128)
        wo_rest()
        def mix_part(off, n):
            return corners(mix(hw, yw, bw, slice(off, off + hl), n))

        def fence():
            pin(yres, pltpu.bitcast(xna[pl.ds(pl.multiple_of(seg * 8, 8), 8), 0:128], f32))

        late = list(range(hl, L, 16))
        nxt = list(range(0, L, 16))
        for n in range(4):
            marks = up(0, n)
            for i in (0, 1, 3):
                lnln(late.pop(0), 16)
                pin(big, marks[i])
        for n in range(4):
            marks = mix_part(0, n)
            for i in range(4):
                if late:
                    lnln(late.pop(0), 16)
                else:
                    ln_next(nxt.pop(0), 16)
                if n > 0 or i == 3:
                    pin(xin, marks[i])
        for n in range(4):
            marks = up(hl, n)
            for i in (0, 1, 3):
                ln_next(nxt.pop(0), 16)
                pin(xin, marks[i])
        for n in range(4):
            if n == 3:
                fence()
            marks = mix_part(hl, n)
            for i in range(4):
                if nxt:
                    ln_next(nxt.pop(0), 16)
                    pin(xin, marks[i])

    def mix(h_ref, y_ref, x_ref, rr, n):
        cs = slice(n * 256, (n + 1) * 256)
        r = y_ref[rr, D - 256:D - 128]
        mr = y_ref[rr, D - 128:D]
        x = x_ref[rr, cs]
        y = x * jnp.concatenate([r, r], axis=1) - jnp.concatenate([mr, mr], axis=1)
        x1 = y + _dot(h_ref[rr, :].astype(bf16), _unpack(w2[:, cs]))
        y_ref[rr, cs] = x1
        x_ref[rr, cs] = x + x1
        return x1

    def ln_mid(tok, n):
        xnc[_hs(tok, n), :] = _pack(_ln(yres[pl.ds(tok + HALO, n), :]))

    def last_rows():
        for n in range(4):
            mix(hbuf, yres, big, slice(S, PAD_ROWS), n)
            ln_mid(n * 128, 128)

    def out_copy(blk):
        rows = pl.ds(blk * L, L)
        return pltpu.make_async_copy(obuf.at[rows], out_hbm.at[0, rows, :], osems.at[blk])

    def ffn(layer, it):
        def block_of(pair):
            return (pair * 37) >> 8

        blk, chunk, tok = [], [], []
        for h in range(UNROLL // 2):
            pair = (UNROLL // 2) * it + h
            b = block_of(pair)
            c = 2 * pair - NC * b
            t = pl.multiple_of(b * L, L)
            blk += [b, b]
            chunk += [c, c + 1]
            tok += [t, t]

        def ffn_up(k):
            hh = _gelu(_dot(_unpack(xnc[_hs(tok[k], L), :]), _unpack(w3[chunk[k]])))
            gh[k % 2] = _pack(hh)
            return hh[L - 8:L, FC - 128:FC]

        def ffn_down(k):
            rows = pl.ds(tok[k] + HALO, L)
            w = _unpack(w4[_hs(chunk[k] * FC, FC), :])
            big[rows, :] = big[rows, :] + _dot(_unpack(gh[k % 2]), w)

        def ln_ahead(k, mark):
            yres[pl.ds(PIN + pl.multiple_of(blk[0] * 16, 16), 8), 0:128] = mark
            nb = jnp.minimum(blk[k] + 1, NSEG - 1)
            ln_mid(pl.multiple_of(nb * L + jnp.minimum(chunk[k] * 40, L - 80), 16), 80)

        def ln_first():
            r = pl.multiple_of(jnp.clip((it - 4) * 64, 0, L - 64), 64)
            xna[_hs(r, 64), :] = _pack(_ln(big[pl.ds(r + HALO, 64), :]))

        ffn_up(0)
        ln_ahead(0, ffn_up(1))
        ffn_down(0)
        ln_ahead(2, ffn_up(2))
        ffn_down(1)
        ln_first()
        ffn_up(3)
        ffn_down(2)
        ffn_down(3)

        done = block_of((UNROLL // 2) * (it + 1))

        @pl.when(jnp.logical_and(layer == 1, done != blk[0]))
        def _():
            r = pl.multiple_of((done - 1) * L, L)
            obuf[pl.ds(r, L), :] = big[pl.ds(r + HALO, L), :].astype(bf16)
            out_copy(done - 1).start()

    def layer_body(layer, _):
        mt[...] = jnp.zeros(mt.shape, f32)
        zrow[...] = jnp.zeros(zrow.shape, f32)

        def a_body(seg, _):
            phase_a(layer, seg)
            return 0
        jax.lax.fori_loop(0, NSEG, a_body, 0)

        last_rows()

        @pl.when(layer == 0)
        def _():
            for c in cp_w3:
                c.wait()
            cp_w4.wait()

        def b_body(it, _):
            ffn(layer, it)
            return 0
        jax.lax.fori_loop(0, NSEG * NC // UNROLL, b_body, 0)
        return 0
    jax.lax.fori_loop(0, 2, layer_body, 0)

    for blk in range(NSEG):
        out_copy(blk).wait()


@jax.jit
def pallas_interleave_layers__memory_aug_infini_attn__mixer_s_mlp__prompt_kernel(
    A_x: jax.Array,
    A_wq: jax.Array,
    A_wk: jax.Array,
    A_wv: jax.Array,
    A_wo: jax.Array,
    A_beta: jax.Array,
    B_x: jax.Array,
    B_w1: jax.Array,
    B_w2: jax.Array,
    B_w3: jax.Array,
    B_w4: jax.Array,
):
    del B_x
    hbm = pl.BlockSpec(memory_space=pl.ANY)
    vm = pltpu.VMEM
    scratch = [
        vm((BIG_ROWS, D), bf16),
        vm((8, 256, D), bf16),
        vm((2, 4, D // 2, 256), u32),
        vm((2, D // 2, DHALF), u32),
        vm((2, DHALF // 2, D), u32),
        vm((D // 2, D), u32),
        vm((D // 2, D), u32),
        vm((NC, D // 2, FC), u32),
        vm((F // 2, D), u32),
        vm((BIG_ROWS, D), f32),
        vm((BIG_ROWS, D), f32),
        vm((PAD_ROWS, D), f32),
        vm((L // 2, D), u32),
        vm((L // 2, D), u32),
        vm((S // 2, D), u32),
        vm((2, L // 2, FC), u32),
        vm((GH, 64, L), u32),
        vm((GH, 64, L), u32),
        vm((GH, L // 2, 128), u32),
        vm((GH, L // 2, 128), u32),
        vm((GH, 64, L), u32),
        vm((GH, L // 2, 128), u32),
        vm((2, L // 4, 128), u32),
        vm((GH, 128, L), f32),
        vm((2, GH, 128, 128), f32),
        vm((2, GH, 1, 128), f32),
        vm((2, H // 2, 128), f32),
        vm((128, 512), f32),
    ]
    scratch += [vm((1, 128 * (t + 1) + 8, 512), f32) for _ in range(2) for t in range(NT_TILES)]
    scratch += [vm((2, 1, 512), f32) for _ in range(NT_TILES)]
    scratch += [
        vm((S, D), bf16),
        pltpu.SemaphoreType.DMA((10,)),
        pltpu.SemaphoreType.DMA((8,)),
        pltpu.SemaphoreType.DMA((NSEG,)),
    ]
    return pl.pallas_call(
        _kernel,
        out_shape=jax.ShapeDtypeStruct((1, S, D), bf16),
        in_specs=[hbm, hbm, hbm, hbm, hbm, pl.BlockSpec(memory_space=pltpu.VMEM),
                  hbm, hbm, hbm, hbm],
        out_specs=hbm,
        scratch_shapes=scratch,
        compiler_params=pltpu.CompilerParams(vmem_limit_bytes=120 * 1024 * 1024),
    )(A_x, A_wq, A_wk, A_wv, A_wo, A_beta.reshape(1, H), B_w1, B_w2, B_w3, B_w4)
```

```python
import functools
import math

import jax
import jax.numpy as jnp
import jax.experimental.pallas as pl
import jax.experimental.pallas.tpu as pltpu

S = 2048
D = 1024
F = 3584
H = 32
DH = 32
L = 512
NSEG = S // L
NG = D // 128
NT_TILES = L // 128
FC = 256
HALO = 8
GH = NG // 2
DHALF = D // 2
PAD_ROWS = S + 2 * HALO
PIN = S + L + 2 * HALO
BIG_ROWS = PIN + 16 * NSEG
NC = F // FC
UNROLL = 4
SHIFTS = (1, -1, 2, -2)
ROT = (0, 2, 1, 3)
OWNER = (((0,) * 4, (1,) * 4, (2,) * 4, (3,) * 4),
         ((3, 0, 0, 0), (1, 1, 3, 1), (2, 3, 2, 2)),
         ((1, 1, 0, 0), (2, 3, 3, 2)),
         ((2, 1, 3, 0),))

LOG2E = math.log2(math.e)
QSCALE = DH ** -0.5 * LOG2E
MASK_BIAS = -1e9 * LOG2E
EPS = 1e-5

f32 = jnp.float32
bf16 = jnp.bfloat16
u32 = jnp.uint32
NT_DIMS = (((1,), (1,)), ((), ()))


def _stats(x):
    m = jnp.mean(x, axis=-1, keepdims=True)
    xc = x - m
    return m, jnp.mean(xc * xc, axis=-1, keepdims=True)


def _ln(x):
    m, v = _stats(x)
    r = jax.lax.rsqrt(v + EPS)
    return x * r - m * r


def _ln_ln(x):
    m, v = _stats(x)
    r1 = jax.lax.rsqrt(v + EPS)
    r2 = r1 * jax.lax.rsqrt(v * r1 * r1 + EPS)
    return r1, m * r1, x * r2 - m * r2


def _gelu(x):
    c = math.sqrt(2.0 / math.pi)
    inner = x * (c + (c * 0.044715) * (x * x))
    hx = 0.5 * x
    return hx + hx * jnp.tanh(inner)


def _phi(t):
    return jnp.where(t > 0, t + 1.0, jnp.exp(t))


def _red8(x, op):
    return functools.reduce(op, [x[i * 8:(i + 1) * 8] for i in range(x.shape[0] // 8)])


def _pick(pos, x, other):
    if len(pos) == 4:
        return x
    lane = jax.lax.broadcasted_iota(jnp.int32, x.shape, 1)
    if len(pos) == 2:
        low = lane < 64 if pos in ((0, 1), (2, 3)) else ((lane + 32) & 127) < 64
        return jnp.where(low, x, other) if 0 in pos else jnp.where(low, other, x)
    if len(pos) == 1:
        return jnp.where((lane >> 5) == pos[0], x, other)
    return jnp.where((lane >> 5) == 6 - sum(pos), other, x)


def _owned(b, i, h):
    return tuple(p for p in range(4) if OWNER[b][i][p] == h)


def _of_head(tiles, b, h, other):
    for i, x in enumerate(tiles):
        if _owned(b, i, h):
            other = _pick(_owned(b, i, h), x, other)
    return other


def _of_tile(heads, b, i):
    out = None
    for h in sorted(set(OWNER[b][i]), key=lambda h: -len(_owned(b, i, h))):
        out = heads[h] if out is None else _pick(_owned(b, i, h), heads[h], out)
    return out


def _pack(x):
    return pltpu.bitcast(x.astype(bf16), u32)


def _unpack(x):
    return pltpu.bitcast(x, bf16)


def _hs(start, n):
    if isinstance(start, int):
        return slice(start // 2, (start + n) // 2)
    return pl.ds(pl.multiple_of(start >> 1, 8), n // 2)


def _dot(a, b):
    return jnp.dot(a, b, preferred_element_type=f32)


def _dot_nt(a, b):
    return jax.lax.dot_general(a, b, NT_DIMS, preferred_element_type=f32)


def _kernel(x_hbm, wq_hbm, wk_hbm, wv_hbm, wo_hbm, beta_ref, w1_hbm, w2_hbm, w3_hbm, w4_hbm,
            out_hbm,
            xin, stage, wt, wk, wo, w1, w2, w3, w4,
            big, yres, hbuf, xna, xnb, xnc, gh, qt, pqt, kb, pkb, vt, ob, obl, amem,
            mt, zrow, gate, bias,
            s0, s1, s2, s3, s4, s5, s6, s7, m0, m1, m2, m3,
            obuf, sems, tsems, osems):
    sbuf = ((s0, s1, s2, s3), (s4, s5, s6, s7))
    mbuf = (m0, m1, m2, m3)

    def seg_rows(s):
        return pl.ds(s * L, L)

    cp_x0 = pltpu.make_async_copy(x_hbm.at[0, seg_rows(0)], xin.at[seg_rows(0)], sems.at[0])
    cp_xr = pltpu.make_async_copy(x_hbm.at[0, pl.ds(L, S - L)], xin.at[pl.ds(L, S - L)], sems.at[1])
    cp_wk = [pltpu.make_async_copy(wk_hbm.at[:, pl.ds(i * DHALF, DHALF)], wk.at[i].bitcast(bf16),
                                   sems.at[2 + i])
             for i in range(2)]
    cp_wo = [pltpu.make_async_copy(wo_hbm.at[pl.ds(i * DHALF, DHALF)], wo.at[i].bitcast(bf16),
                                   sems.at[4 + i])
             for i in range(2)]
    cp_w1 = pltpu.make_async_copy(w1_hbm, w1.bitcast(bf16), sems.at[6])
    cp_w2 = pltpu.make_async_copy(w2_hbm, w2.bitcast(bf16), sems.at[7])
    cp_w3 = [pltpu.make_async_copy(w3_hbm.at[:, pl.ds(c * FC, FC)], w3.at[c].bitcast(bf16),
                                   sems.at[8])
             for c in range(F // FC)]
    cp_w4 = pltpu.make_async_copy(w4_hbm, w4.bitcast(bf16), sems.at[9])

    TC = 256
    NTC = D // TC

    cp_stage = [pltpu.make_async_copy(
        (wq_hbm, wv_hbm)[(ic >> 1) & 1].at[pl.ds((ic & 1) * DHALF, DHALF),
                                           pl.ds((ic >> 2) * DHALF, DHALF)],
        stage.at[ic], tsems.at[ic]) for ic in range(8)]

    for cp in cp_stage[0:4]:
        cp.start()
    for cp in (cp_x0, cp_wk[0], cp_wo[0]):
        cp.start()

    kk = jax.lax.broadcasted_iota(jnp.int32, (DH, 128), 0)
    ll = jax.lax.broadcasted_iota(jnp.int32, (DH, 128), 1)
    qq = [(ll + (128 - DH * r)) & 127 for r in ROT]
    for b in range(4):
        for i in range(4 - b):
            bias[b * DH:(b + 1) * DH, i * 128:(i + 1) * 128] = jnp.where(
                kk + b * DH > _of_tile(qq, b, i), MASK_BIAS, 0.0).astype(f32)
    bt = jnp.broadcast_to(beta_ref[...].astype(f32), (H, H))
    eye = (jax.lax.broadcasted_iota(jnp.int32, (H, H), 0)
           == jax.lax.broadcasted_iota(jnp.int32, (H, H), 1))
    bcol = jnp.sum(jnp.where(eye, bt, 0.0), axis=1, keepdims=True)
    gsig = jnp.broadcast_to(jax.nn.sigmoid(bcol), (H, 128))
    gate[0] = gsig[0:H // 2]
    gate[1] = gsig[H // 2:H]
    hbuf[0:2 * HALO, :] = jnp.zeros((2 * HALO, D), f32)
    hbuf[S:PAD_ROWS, :] = jnp.zeros((2 * HALO, D), f32)
    for ref in (big, yres):
        ref[0:HALO, :] = jnp.zeros((HALO, D), f32)
        ref[S + HALO:PAD_ROWS, :] = jnp.zeros((HALO, D), f32)

    ident = (jax.lax.broadcasted_iota(jnp.int32, (128, 128), 0)
             == jax.lax.broadcasted_iota(jnp.int32, (128, 128), 1)).astype(f32).astype(bf16)

    def transpose(hf, ic, ro, c0):
        for c in range(2):
            for n in range(GH):
                tile = _dot_nt(ident, stage[ic, c * TC:(c + 1) * TC, n * 128:(n + 1) * 128])
                wt[hf, c0 + c, _hs(ro + n * 128, 128), :] = _pack(tile)

    def transpose_chunk(ic, _):
        pltpu.make_async_copy(stage.at[ic], stage.at[ic], tsems.at[ic]).wait()
        transpose(0, ic, pl.multiple_of((ic >> 1) * DHALF, DHALF), (ic & 1) * 2)
        return 0
    jax.lax.fori_loop(0, 4, transpose_chunk, 0)

    cp_x0.wait()

    def init_x(i, _):
        r = pl.multiple_of(i * 256, 256)
        xv = xin[pl.ds(r, 256), :].astype(f32)
        big[pl.ds(HALO + r, 256), :] = xv
        xna[_hs(r, 256), :] = _pack(_ln(xv))
        return 0
    jax.lax.fori_loop(0, L // 256, init_x, 0)
    cp_wk[0].wait()
    for cp in cp_stage[4:8] + [cp_wk[1], cp_wo[1], cp_w1, cp_xr, cp_w2] + cp_w3 + [cp_w4]:
        cp.start()
    cp_wo[0].wait()

    def qmask(g, t, b=0):
        z = jnp.zeros((DH // 2, 128), u32)
        qs = [qt[g, _hs(h * DH, DH), t * 128:(t + 1) * 128] for h in range(4)]
        cols = [jnp.concatenate([_pick(_owned(b, i, h), qs[h], z) if _owned(b, i, h) else z
                                 for h in range(4)], axis=0) for i in range(4 - b)]
        return _unpack(jnp.concatenate(cols, axis=1))

    def tiles(x):
        return [x[:, i * 128:(i + 1) * 128] for i in range(x.shape[1] // 128)]

    def attn_step(half, g, gn, last, fill=()):
        pr = None if g is None else g % 2
        pw = None if gn is None else gn % 2
        fill = list(fill)
        for t in range(NT_TILES):
            macc = None
            oacc = [None] * 4
            lacc = [None] * 4
            for j in range(t + 1):
                ks = slice(j * 128, (j + 1) * 128)
                nk = DH if j == t else 128
                kl = slice(j * 128, j * 128 + nk)
                filled = fill.pop(0) if fill else None
                if filled:
                    filled()
                    last["pace"] = last.get("o", last["s"])
                elif gn is not None and g is not None:
                    last["pace"] = last["s"]
                if g is not None:
                    sbuf[pr][t][0, (t + 1) * 128:(t + 1) * 128 + 8, 0:128] = last["pace"]
                if gn is not None:
                    s = _dot(_unpack(kb[gn, _hs(j * 128, nk), :]), qmask(gn, t))
                    if j == t:
                        s = s + bias[0:DH, :]
                    sbuf[pw][t][0, kl, :] = s
                    last["s"] = s[0:8, 0:128]
                    mx = _red8(s, jnp.maximum)
                    if j == t:
                        mx = tiles(mx)
                        for b in range(1, 4):
                            k0 = j * 128 + b * DH
                            su = _dot(_unpack(kb[gn, _hs(k0, DH), :]), qmask(gn, t, b))
                            su = su + bias[b * DH:(b + 1) * DH, 0:(4 - b) * 128]
                            sbuf[pw][t][0, k0:k0 + DH, 0:(4 - b) * 128] = su
                            mu = tiles(_red8(su, jnp.maximum))
                            mx = [jnp.maximum(mx[h], _of_head(mu, b, h, mx[h])) for h in range(4)]
                        mx = jnp.concatenate(mx, axis=1)
                    macc = mx if macc is None else jnp.maximum(macc, mx)
                if g is not None:
                    ms = tiles(mbuf[t][pr])
                    pu, lu = {}, {}
                    for h in range(4):
                        sl = slice(h * 128, (h + 1) * 128)
                        p = jnp.exp2(sbuf[pr][t][half >> 1, kl, sl] - ms[h])
                        lt = _red8(p, jnp.add)
                        p = p.astype(bf16)
                        if j == t:
                            rows = [pltpu.bitcast(p, u32)]
                            for b in range(1, 4):
                                k0 = j * 128 + b * DH
                                for i in range(4 - b):
                                    if _owned(b, i, h) and (b, i) not in pu:
                                        e = jnp.exp2(sbuf[pr][t][half >> 1, k0:k0 + DH,
                                                                 i * 128:(i + 1) * 128]
                                                     - _of_tile(ms, b, i))
                                        lu[b, i] = _red8(e, jnp.add)
                                        pu[b, i] = _pack(e)
                                at = [(b, i) for i in range(4 - b)]
                                lt = lt + _of_head([lu.get(k) for k in at], b, h, 0.0)
                                rows.append(_of_head([pu.get(k) for k in at], b, h, u32(0)))
                            p = _unpack(jnp.concatenate(rows, axis=0))
                        lacc[h] = lt if lacc[h] is None else lacc[h] + lt
                        o = _dot(_unpack(vt[g, _hs(h * DH, DH), ks]), p)
                        oacc[h] = o if oacc[h] is None else oacc[h] + o
                        if h == 0:
                            last["o"] = o[0:8, :]
            if gn is not None:
                mbuf[t][pw] = jnp.max(macc, axis=0, keepdims=True)
            if g is not None:
                parts = []
                for h in range(4):
                    l = jnp.sum(lacc[h], axis=0, keepdims=True)
                    gh = gate[half, g * 4 + h:g * 4 + h + 1, :]
                    oh = oacc[h] * ((1.0 - gh) / l)
                    parts.append(pltpu.roll(oh, 128 - DH * ROT[h], 1) if h else oh)
                ot = jnp.concatenate(parts, axis=0) + amem[g, :, t * 128:(t + 1) * 128]
                if g < GH - 1 or t < 2:
                    ob[g, _hs(t * 128, 128), :] = _pack(ot.T)
                else:
                    obl[half, _hs((t - 2) * 128, 128), :] = _pack(ot.T)

    rowh = jax.lax.broadcasted_iota(jnp.int32, (128, 128), 0) // DH
    colh = jax.lax.broadcasted_iota(jnp.int32, (128, 128), 1) // DH
    row16 = jax.lax.broadcasted_iota(jnp.int32, (16, 128), 0)
    col16 = jax.lax.broadcasted_iota(jnp.int32, (16, 128), 1) // DH

    def attn_half(layer, seg, half):
        r0 = pl.multiple_of(seg * L, L)

        @pl.when(jnp.logical_and(jnp.logical_and(layer == 0, seg == 0), half == 1))
        def _():
            cp_wk[1].wait()
            cp_wo[1].wait()
            cp_w1.wait()
            cp_xr.wait()
            cp_w2.wait()
            for cp in cp_stage[4:8]:
                cp.wait()
            for ic in range(4):
                transpose(1, 4 + ic, (ic >> 1) * DHALF, (ic & 1) * 2)

        def xn(c0, nc):
            return _unpack(xna[_hs(c0 * 128, nc * 128), :])

        zparts = {}

        def k_piece(g0, ng, c0, nc):
            k = _dot(xn(c0, nc), _unpack(wk[half, :, g0 * 128:(g0 + ng) * 128]))
            pk = _phi(k)
            rs = _hs(c0 * 128, nc * 128)
            for i in range(ng):
                cs = slice(i * 128, (i + 1) * 128)
                kb[g0 + i, rs, :] = _pack(k[:, cs])
                pkb[g0 + i, rs, :] = _pack(pk[:, cs])
                zparts.setdefault(g0 + i, []).append(_red8(pk[:, cs], jnp.add))

        def qv_piece(qs, vs, c0, nc):
            offs = [g * 128 for g in qs] + [DHALF + g * 128 for g in vs]
            lhs = jnp.concatenate(
                [jnp.concatenate([wt[half, c, _hs(o, 128), :] for c in range(NTC)], axis=1)
                 for o in offs], axis=0)
            r = _dot_nt(_unpack(lhs), xn(c0, nc))
            ts = slice(c0 * 128, (c0 + nc) * 128)
            for i, g in enumerate(qs):
                qg = r[i * 128:(i + 1) * 128, :]
                qp = _pack(qg * QSCALE)
                for c in range(nc):
                    for h in range(4):
                        qh = qp[_hs(h * DH, DH), c * 128:(c + 1) * 128]
                        qt[g, _hs(h * DH, DH), (c0 + c) * 128:(c0 + c + 1) * 128] = (
                            pltpu.roll(qh, DH * ROT[h], 1) if h else qh)
                pqt[g, :, ts] = _pack(_phi(qg))
            for i, g in enumerate(vs):
                o = (len(qs) + i) * 128
                vt[g, :, ts] = _pack(r[o:o + 128, :])

        def mem(g):
            zold = zrow[half, g]
            mold = mt[half, g]
            mbd = jnp.where(rowh == colh, mold, 0.0)
            zx = jnp.where(row16 == col16, jnp.broadcast_to(zold, (16, 128)), 0.0)
            lhs = jnp.concatenate([mbd, zx], axis=0).astype(bf16)
            ret = _dot(lhs, _unpack(pqt[g]))
            parts = []
            for h in range(4):
                gh = gate[half, g * 4 + h:g * 4 + h + 1, 0:1]
                den = ret[128 + h:129 + h, :] + 1e-6
                parts.append(ret[h * DH:(h + 1) * DH, :] * (gh / den))
            amem[g] = jnp.concatenate(parts, axis=0)
            zsum = functools.reduce(jnp.add, zparts[g])
            zrow[half, g] = zold + jnp.sum(zsum, axis=0, keepdims=True)

        def upd(g):
            mt[half, g] = mt[half, g] + _dot(_unpack(vt[g]), _unpack(pkb[g]))

        def mem_upd(g):
            mem(g)
            upd(g)

        P = functools.partial
        skip = None
        last = {}
        k_piece(0, 2, 0, 4)
        qv_piece((0, 1), (0,), 0, 4)
        attn_step(half, None, 0, last)
        mem(0)
        for g in range(2):
            attn_step(half, g, g + 1, last, fill=[
                skip, P(k_piece, g + 2, 1, 0, 2), skip, P(qv_piece, (g + 2,), (g + 1,), 0, 1),
                P(qv_piece, (g + 2,), (g + 1,), 1, 1), skip, P(k_piece, g + 2, 1, 2, 2),
                P(qv_piece, (g + 2,), (g + 1,), 2, 1), P(qv_piece, (g + 2,), (g + 1,), 3, 1),
                P(mem_upd, g + 1)])
        attn_step(half, 2, 3, last, fill=[
            P(upd, 0), skip, P(qv_piece, (), (3,), 0, 1), skip, P(qv_piece, (), (3,), 1, 1),
            skip, P(qv_piece, (), (3,), 2, 1), P(qv_piece, (), (3,), 3, 1), skip, P(mem_upd, 3)])

        def wo_piece(t, n):
            off = t * 128
            cs = slice(n * DHALF, (n + 1) * DHALF)
            rr = pl.ds(r0 + (HALO + off), 128)
            ng = GH if t < 2 else GH - 1
            o = jnp.concatenate([ob[g, _hs(off, 128), :] for g in range(ng)], axis=1)
            big[rr, cs] = big[rr, cs] + _dot(_unpack(o), _unpack(wo[half, _hs(0, ng * 128), cs]))

        attn_step(half, GH - 1, None, last, fill=[
            P(wo_piece, 2, 0), P(wo_piece, 2, 1), P(wo_piece, 3, 0), skip, P(wo_piece, 3, 1),
            P(wo_piece, 0, 0), skip, P(wo_piece, 0, 1), P(wo_piece, 1, 0), skip])
        wo_piece(1, 1)

    def phase_a(layer, seg):
        r0 = pl.multiple_of(seg * L, L)

        def half_body(half, _):
            attn_half(layer, seg, half)
            return 0
        jax.lax.fori_loop(0, 2, half_body, 0)

        hl = L // 2
        kp = (GH - 1) * 128

        bw = big.at[pl.ds(r0, 2 * L + 2 * HALO), :]
        yw = yres.at[pl.ds(r0, L + 2 * HALO), :]
        hw = hbuf.at[pl.ds(r0, L + 2 * HALO), :]
        xw = xin.at[pl.ds(r0 + L, L), :]

        def wo_rest():
            rr = slice(HALO + hl, HALO + L)
            o = _unpack(jnp.concatenate([obl[0], obl[1]], axis=1))
            w = _unpack(jnp.concatenate([wo[i, _hs(kp, 128), :] for i in range(2)], axis=0))
            bw[rr, :] = bw[rr, :] + _dot(o, w)

        def lnln(off, n):
            rr = slice(HALO + off, HALO + off + n)
            r, mr, z = _ln_ln(bw[rr, :])
            yw[rr, D - 256:D - 128] = jnp.broadcast_to(r, (n, 128))
            yw[rr, D - 128:D] = jnp.broadcast_to(mr, (n, 128))
            xnb[_hs(off, n), :] = _pack(z)

        def corners(v):
            return [v[0:8, 0:128], v[hl - 8:hl, 0:128], v[0:8, 128:256], v[hl - 8:hl, 128:256]]

        def up(off, n):
            cs = slice(n * 256, (n + 1) * 256)
            hh = _gelu(_dot(_unpack(xnb[_hs(off, hl), :]), _unpack(w1[:, cs])))
            b = off + HALO + SHIFTS[n]
            hw[b:b + hl, cs] = hh
            return corners(hh)

        sink = PIN + pl.multiple_of(seg * 16, 16)

        def pin(ref, v):
            if ref.dtype == bf16:
                ref[pl.ds(sink, 16), 0:128] = jnp.concatenate([v, v], axis=0).astype(bf16)
            else:
                ref[pl.ds(sink, 8), 0:128] = v

        fresh = jnp.logical_and(layer == 0, seg < NSEG - 1)

        def ln_next(off, n):
            rr = slice(L + HALO + off, L + HALO + off + n)
            xv = jnp.where(fresh, xw[off:off + n, :].astype(f32), bw[rr, :])
            bw[rr, :] = xv
            xna[_hs(off, n), :] = _pack(_ln(xv))

        lnln(0, 128)
        lnln(128, 128)
        wo_rest()
        def mix_part(off, n):
            return corners(mix(hw, yw, bw, slice(off, off + hl), n))

        def fence():
            pin(yres, pltpu.bitcast(xna[pl.ds(pl.multiple_of(seg * 8, 8), 8), 0:128], f32))

        late = list(range(hl, L, 16))
        nxt = list(range(0, L, 16))
        for n in range(4):
            marks = up(0, n)
            for i in (0, 1, 3):
                lnln(late.pop(0), 16)
                pin(big, marks[i])
        for n in range(4):
            marks = mix_part(0, n)
            for i in range(4):
                if late:
                    lnln(late.pop(0), 16)
                else:
                    ln_next(nxt.pop(0), 16)
                if n > 0 or i == 3:
                    pin(xin, marks[i])
        for n in range(4):
            marks = up(hl, n)
            for i in (0, 1, 3):
                ln_next(nxt.pop(0), 16)
                pin(xin, marks[i])
        for n in range(4):
            if n == 3:
                fence()
            marks = mix_part(hl, n)
            for i in range(4):
                if nxt:
                    ln_next(nxt.pop(0), 16)
                    pin(xin, marks[i])

    def mix(h_ref, y_ref, x_ref, rr, n):
        cs = slice(n * 256, (n + 1) * 256)
        r = y_ref[rr, D - 256:D - 128]
        mr = y_ref[rr, D - 128:D]
        x = x_ref[rr, cs]
        y = x * jnp.concatenate([r, r], axis=1) - jnp.concatenate([mr, mr], axis=1)
        x1 = y + _dot(h_ref[rr, :].astype(bf16), _unpack(w2[:, cs]))
        y_ref[rr, cs] = x1
        x_ref[rr, cs] = x + x1
        return x1

    def ln_mid(tok, n):
        xnc[_hs(tok, n), :] = _pack(_ln(yres[pl.ds(tok + HALO, n), :]))

    def last_rows():
        for n in range(4):
            mix(hbuf, yres, big, slice(S, PAD_ROWS), n)
            ln_mid(n * 128, 128)

    def out_copy(blk):
        rows = pl.ds(blk * L, L)
        return pltpu.make_async_copy(obuf.at[rows], out_hbm.at[0, rows, :], osems.at[blk])

    def ffn(layer, it):
        def block_of(pair):
            return (pair * 37) >> 8

        blk, chunk, tok = [], [], []
        for h in range(UNROLL // 2):
            pair = (UNROLL // 2) * it + h
            b = block_of(pair)
            c = 2 * pair - NC * b
            t = pl.multiple_of(b * L, L)
            blk += [b, b]
            chunk += [c, c + 1]
            tok += [t, t]

        def ffn_up(k):
            hh = _gelu(_dot(_unpack(xnc[_hs(tok[k], L), :]), _unpack(w3[chunk[k]])))
            gh[k % 2] = _pack(hh)
            return hh[L - 8:L, FC - 128:FC]

        def ffn_down(k):
            rows = pl.ds(tok[k] + HALO, L)
            w = _unpack(w4[_hs(chunk[k] * FC, FC), :])
            big[rows, :] = big[rows, :] + _dot(_unpack(gh[k % 2]), w)

        def ln_ahead(k, mark):
            yres[pl.ds(PIN + pl.multiple_of(blk[0] * 16, 16), 8), 0:128] = mark
            nb = jnp.minimum(blk[k] + 1, NSEG - 1)
            ln_mid(pl.multiple_of(nb * L + jnp.minimum(chunk[k] * 40, L - 80), 16), 80)

        def ln_first():
            r = pl.multiple_of(jnp.clip((it - 4) * 64, 0, L - 64), 64)
            xna[_hs(r, 64), :] = _pack(_ln(big[pl.ds(r + HALO, 64), :]))

        ffn_up(0)
        ln_ahead(0, ffn_up(1))
        ffn_down(0)
        ln_ahead(2, ffn_up(2))
        ffn_down(1)
        ln_first()
        ffn_up(3)
        ffn_down(2)
        ffn_down(3)

        done = block_of((UNROLL // 2) * (it + 1))

        @pl.when(jnp.logical_and(layer == 1, done != blk[0]))
        def _():
            r = pl.multiple_of((done - 1) * L, L)
            obuf[pl.ds(r, L), :] = big[pl.ds(r + HALO, L), :].astype(bf16)
            out_copy(done - 1).start()

    def layer_body(layer, _):
        mt[...] = jnp.zeros(mt.shape, f32)
        zrow[...] = jnp.zeros(zrow.shape, f32)

        def a_body(seg, _):
            phase_a(layer, seg)
            return 0
        jax.lax.fori_loop(0, NSEG, a_body, 0)

        last_rows()

        @pl.when(layer == 0)
        def _():
            for c in cp_w3:
                c.wait()
            cp_w4.wait()

        def b_body(it, _):
            ffn(layer, it)
            return 0
        jax.lax.fori_loop(0, NSEG * NC // UNROLL, b_body, 0)
        return 0
    jax.lax.fori_loop(0, 2, layer_body, 0)

    for blk in range(NSEG):
        out_copy(blk).wait()


@jax.jit
def pallas_interleave_layers__memory_aug_infini_attn__mixer_s_mlp__prompt_kernel(
    A_x: jax.Array,
    A_wq: jax.Array,
    A_wk: jax.Array,
    A_wv: jax.Array,
    A_wo: jax.Array,
    A_beta: jax.Array,
    B_x: jax.Array,
    B_w1: jax.Array,
    B_w2: jax.Array,
    B_w3: jax.Array,
    B_w4: jax.Array,
):
    del B_x
    hbm = pl.BlockSpec(memory_space=pl.ANY)
    vm = pltpu.VMEM
    scratch = [
        vm((BIG_ROWS, D), bf16),
        vm((8, DHALF, DHALF), bf16),
        vm((2, 4, D // 2, 256), u32),
        vm((2, D // 2, DHALF), u32),
        vm((2, DHALF // 2, D), u32),
        vm((D // 2, D), u32),
        vm((D // 2, D), u32),
        vm((NC, D // 2, FC), u32),
        vm((F // 2, D), u32),
        vm((BIG_ROWS, D), f32),
        vm((BIG_ROWS, D), f32),
        vm((PAD_ROWS, D), f32),
        vm((L // 2, D), u32),
        vm((L // 2, D), u32),
        vm((S // 2, D), u32),
        vm((2, L // 2, FC), u32),
        vm((GH, 64, L), u32),
        vm((GH, 64, L), u32),
        vm((GH, L // 2, 128), u32),
        vm((GH, L // 2, 128), u32),
        vm((GH, 64, L), u32),
        vm((GH, L // 2, 128), u32),
        vm((2, L // 4, 128), u32),
        vm((GH, 128, L), f32),
        vm((2, GH, 128, 128), f32),
        vm((2, GH, 1, 128), f32),
        vm((2, H // 2, 128), f32),
        vm((128, 512), f32),
    ]
    scratch += [vm((1, 128 * (t + 1) + 8, 512), f32) for _ in range(2) for t in range(NT_TILES)]
    scratch += [vm((2, 1, 512), f32) for _ in range(NT_TILES)]
    scratch += [
        vm((S, D), bf16),
        pltpu.SemaphoreType.DMA((10,)),
        pltpu.SemaphoreType.DMA((8,)),
        pltpu.SemaphoreType.DMA((NSEG,)),
    ]
    return pl.pallas_call(
        _kernel,
        out_shape=jax.ShapeDtypeStruct((1, S, D), bf16),
        in_specs=[hbm, hbm, hbm, hbm, hbm, pl.BlockSpec(memory_space=pltpu.VMEM),
                  hbm, hbm, hbm, hbm],
        out_specs=hbm,
        scratch_shapes=scratch,
        compiler_params=pltpu.CompilerParams(vmem_limit_bytes=120 * 1024 * 1024),
    )(A_x, A_wq, A_wk, A_wv, A_wo, A_beta.reshape(1, H), B_w1, B_w2, B_w3, B_w4)
```

```python
import functools
import math

import jax
import jax.numpy as jnp
import jax.experimental.pallas as pl
import jax.experimental.pallas.tpu as pltpu

S = 2048
D = 1024
F = 3584
H = 32
DH = 32
L = 512
NSEG = S // L
NG = D // 128
NT_TILES = L // 128
FC = 256
HALO = 8
GH = NG // 2
DHALF = D // 2
PAD_ROWS = S + 2 * HALO
PIN = S + L + 2 * HALO
BIG_ROWS = PIN + 16 * NSEG
NC = F // FC
UNROLL = 4
SHIFTS = (1, -1, 2, -2)
ROT = (0, 2, 1, 3)
OWNER = (((0,) * 4, (1,) * 4, (2,) * 4, (3,) * 4),
         ((3, 0, 0, 0), (1, 1, 3, 1), (2, 3, 2, 2)),
         ((1, 1, 0, 0), (2, 3, 3, 2)),
         ((2, 1, 3, 0),))

LOG2E = math.log2(math.e)
QSCALE = DH ** -0.5 * LOG2E
MASK_BIAS = -1e9 * LOG2E
EPS = 1e-5

f32 = jnp.float32
bf16 = jnp.bfloat16
u32 = jnp.uint32
NT_DIMS = (((1,), (1,)), ((), ()))


def _stats(x):
    m = jnp.mean(x, axis=-1, keepdims=True)
    xc = x - m
    return m, jnp.mean(xc * xc, axis=-1, keepdims=True)


def _ln(x):
    m, v = _stats(x)
    r = jax.lax.rsqrt(v + EPS)
    return x * r - m * r


def _ln_ln(x):
    m, v = _stats(x)
    r1 = jax.lax.rsqrt(v + EPS)
    r2 = r1 * jax.lax.rsqrt(v * r1 * r1 + EPS)
    return r1, m * r1, x * r2 - m * r2


def _gelu(x):
    c = math.sqrt(2.0 / math.pi)
    inner = x * (c + (c * 0.044715) * (x * x))
    hx = 0.5 * x
    return hx + hx * jnp.tanh(inner)


def _phi(t):
    return jnp.where(t > 0, t + 1.0, jnp.exp(t))


def _red8(x, op):
    return functools.reduce(op, [x[i * 8:(i + 1) * 8] for i in range(x.shape[0] // 8)])


def _pick(pos, x, other):
    if len(pos) == 4:
        return x
    lane = jax.lax.broadcasted_iota(jnp.int32, x.shape, 1)
    if len(pos) == 2:
        low = lane < 64 if pos in ((0, 1), (2, 3)) else ((lane + 32) & 127) < 64
        return jnp.where(low, x, other) if 0 in pos else jnp.where(low, other, x)
    if len(pos) == 1:
        return jnp.where((lane >> 5) == pos[0], x, other)
    return jnp.where((lane >> 5) == 6 - sum(pos), other, x)


def _owned(b, i, h):
    return tuple(p for p in range(4) if OWNER[b][i][p] == h)


def _of_head(tiles, b, h, other):
    for i, x in enumerate(tiles):
        if _owned(b, i, h):
            other = _pick(_owned(b, i, h), x, other)
    return other


def _of_tile(heads, b, i):
    out = None
    for h in sorted(set(OWNER[b][i]), key=lambda h: -len(_owned(b, i, h))):
        out = heads[h] if out is None else _pick(_owned(b, i, h), heads[h], out)
    return out


def _pack(x):
    return pltpu.bitcast(x.astype(bf16), u32)


def _unpack(x):
    return pltpu.bitcast(x, bf16)


def _hs(start, n):
    if isinstance(start, int):
        return slice(start // 2, (start + n) // 2)
    return pl.ds(pl.multiple_of(start >> 1, 8), n // 2)


def _dot(a, b):
    return jnp.dot(a, b, preferred_element_type=f32)


def _dot_nt(a, b):
    return jax.lax.dot_general(a, b, NT_DIMS, preferred_element_type=f32)


def _kernel(x_hbm, wq_hbm, wk_hbm, wv_hbm, wo_hbm, beta_ref, w1_hbm, w2_hbm, w3_hbm, w4_hbm,
            out_hbm,
            xin, stage, wt, wk, wo, w1, w2, w3, w4,
            big, yres, hbuf, xna, xnb, xnc, gh, qt, pqt, kb, pkb, vt, ob, obl, amem,
            mt, zrow, gate, bias,
            s0, s1, s2, s3, s4, s5, s6, s7, m0, m1, m2, m3,
            obuf, sems, tsems, osems):
    sbuf = ((s0, s1, s2, s3), (s4, s5, s6, s7))
    mbuf = (m0, m1, m2, m3)

    def seg_rows(s):
        return pl.ds(s * L, L)

    cp_x0 = pltpu.make_async_copy(x_hbm.at[0, seg_rows(0)], xin.at[seg_rows(0)], sems.at[0])
    cp_xr = pltpu.make_async_copy(x_hbm.at[0, pl.ds(L, S - L)], xin.at[pl.ds(L, S - L)], sems.at[1])
    cp_wk = [pltpu.make_async_copy(wk_hbm.at[:, pl.ds(i * DHALF, DHALF)], wk.at[i].bitcast(bf16),
                                   sems.at[2 + i])
             for i in range(2)]
    cp_wo = [pltpu.make_async_copy(wo_hbm.at[pl.ds(i * DHALF, DHALF)], wo.at[i].bitcast(bf16),
                                   sems.at[4 + i])
             for i in range(2)]
    cp_w1 = pltpu.make_async_copy(w1_hbm, w1.bitcast(bf16), sems.at[6])
    cp_w2 = pltpu.make_async_copy(w2_hbm, w2.bitcast(bf16), sems.at[7])
    cp_w3 = [pltpu.make_async_copy(w3_hbm.at[:, pl.ds(c * FC, FC)], w3.at[c].bitcast(bf16),
                                   sems.at[8])
             for c in range(F // FC)]
    cp_w4 = pltpu.make_async_copy(w4_hbm, w4.bitcast(bf16), sems.at[9])

    TC = 256
    NTC = D // TC

    cp_stage = [pltpu.make_async_copy(
        (wq_hbm, wv_hbm)[(ic >> 1) & 1].at[pl.ds((ic & 1) * DHALF, DHALF),
                                           pl.ds((ic >> 2) * DHALF, DHALF)],
        stage.at[ic], tsems.at[ic]) for ic in range(8)]

    for cp in cp_stage[0:4]:
        cp.start()
    for cp in (cp_x0, cp_wk[0], cp_wo[0]):
        cp.start()

    kk = jax.lax.broadcasted_iota(jnp.int32, (DH, 128), 0)
    ll = jax.lax.broadcasted_iota(jnp.int32, (DH, 128), 1)
    qq = [(ll + (128 - DH * r)) & 127 for r in ROT]
    for b in range(4):
        for i in range(4 - b):
            bias[b * DH:(b + 1) * DH, i * 128:(i + 1) * 128] = jnp.where(
                kk + b * DH > _of_tile(qq, b, i), MASK_BIAS, 0.0).astype(f32)
    bt = jnp.broadcast_to(beta_ref[...].astype(f32), (H, H))
    eye = (jax.lax.broadcasted_iota(jnp.int32, (H, H), 0)
           == jax.lax.broadcasted_iota(jnp.int32, (H, H), 1))
    bcol = jnp.sum(jnp.where(eye, bt, 0.0), axis=1, keepdims=True)
    gsig = jnp.broadcast_to(jax.nn.sigmoid(bcol), (H, 128))
    gate[0] = gsig[0:H // 2]
    gate[1] = gsig[H // 2:H]
    hbuf[0:2 * HALO, :] = jnp.zeros((2 * HALO, D), f32)
    hbuf[S:PAD_ROWS, :] = jnp.zeros((2 * HALO, D), f32)
    for ref in (big, yres):
        ref[0:HALO, :] = jnp.zeros((HALO, D), f32)
        ref[S + HALO:PAD_ROWS, :] = jnp.zeros((HALO, D), f32)

    ident = (jax.lax.broadcasted_iota(jnp.int32, (128, 128), 0)
             == jax.lax.broadcasted_iota(jnp.int32, (128, 128), 1)).astype(f32).astype(bf16)

    def transpose(hf, ic, ro, c0):
        for c in range(2):
            for n in range(GH):
                tile = _dot_nt(ident, stage[ic, c * TC:(c + 1) * TC, n * 128:(n + 1) * 128])
                wt[hf, c0 + c, _hs(ro + n * 128, 128), :] = _pack(tile)

    def transpose_chunk(ic, _):
        pltpu.make_async_copy(stage.at[ic], stage.at[ic], tsems.at[ic]).wait()
        transpose(0, ic, pl.multiple_of((ic >> 1) * DHALF, DHALF), (ic & 1) * 2)
        return 0
    jax.lax.fori_loop(0, 4, transpose_chunk, 0)

    cp_x0.wait()

    def init_x(i, _):
        r = pl.multiple_of(i * 256, 256)
        xv = xin[pl.ds(r, 256), :].astype(f32)
        big[pl.ds(HALO + r, 256), :] = xv
        xna[_hs(r, 256), :] = _pack(_ln(xv))
        return 0
    jax.lax.fori_loop(0, L // 256, init_x, 0)
    cp_wk[0].wait()
    for cp in cp_stage[4:8] + [cp_wk[1], cp_wo[1], cp_w1, cp_xr, cp_w2] + cp_w3 + [cp_w4]:
        cp.start()
    cp_wo[0].wait()

    def qmask(g, t, b=0):
        z = jnp.zeros((DH // 2, 128), u32)
        qs = [qt[g, _hs(h * DH, DH), t * 128:(t + 1) * 128] for h in range(4)]
        cols = [jnp.concatenate([_pick(_owned(b, i, h), qs[h], z) if _owned(b, i, h) else z
                                 for h in range(4)], axis=0) for i in range(4 - b)]
        return _unpack(jnp.concatenate(cols, axis=1))

    def tiles(x):
        return [x[:, i * 128:(i + 1) * 128] for i in range(x.shape[1] // 128)]

    def attn_step(half, g, gn, last, fill=()):
        pr = None if g is None else g % 2
        pw = None if gn is None else gn % 2
        fill = list(fill)
        for t in range(NT_TILES):
            macc = None
            oacc = [None] * 4
            lacc = [None] * 4
            for j in range(t + 1):
                ks = slice(j * 128, (j + 1) * 128)
                nk = DH if j == t else 128
                kl = slice(j * 128, j * 128 + nk)
                filled = fill.pop(0) if fill else None
                if filled:
                    filled()
                    last["pace"] = last.get("o", last["s"])
                elif gn is not None and g is not None:
                    last["pace"] = last["s"]
                if g is not None:
                    sbuf[pr][t][0, (t + 1) * 128:(t + 1) * 128 + 8, 0:128] = last["pace"]
                if gn is not None:
                    s = _dot(_unpack(kb[gn, _hs(j * 128, nk), :]), qmask(gn, t))
                    if j == t:
                        s = s + bias[0:DH, :]
                    sbuf[pw][t][0, kl, :] = s
                    last["s"] = s[0:8, 0:128]
                    mx = _red8(s, jnp.maximum)
                    if j == t:
                        mx = tiles(mx)
                        for b in range(1, 4):
                            k0 = j * 128 + b * DH
                            su = _dot(_unpack(kb[gn, _hs(k0, DH), :]), qmask(gn, t, b))
                            su = su + bias[b * DH:(b + 1) * DH, 0:(4 - b) * 128]
                            sbuf[pw][t][0, k0:k0 + DH, 0:(4 - b) * 128] = su
                            mu = tiles(_red8(su, jnp.maximum))
                            mx = [jnp.maximum(mx[h], _of_head(mu, b, h, mx[h])) for h in range(4)]
                        mx = jnp.concatenate(mx, axis=1)
                    macc = mx if macc is None else jnp.maximum(macc, mx)
                if g is not None:
                    ms = tiles(mbuf[t][pr])
                    pu, lu = {}, {}
                    for h in range(4):
                        sl = slice(h * 128, (h + 1) * 128)
                        p = jnp.exp2(sbuf[pr][t][half >> 1, kl, sl] - ms[h])
                        lt = _red8(p, jnp.add)
                        p = p.astype(bf16)
                        if j == t:
                            rows = [pltpu.bitcast(p, u32)]
                            for b in range(1, 4):
                                k0 = j * 128 + b * DH
                                for i in range(4 - b):
                                    if _owned(b, i, h) and (b, i) not in pu:
                                        e = jnp.exp2(sbuf[pr][t][half >> 1, k0:k0 + DH,
                                                                 i * 128:(i + 1) * 128]
                                                     - _of_tile(ms, b, i))
                                        lu[b, i] = _red8(e, jnp.add)
                                        pu[b, i] = _pack(e)
                                at = [(b, i) for i in range(4 - b)]
                                lt = lt + _of_head([lu.get(k) for k in at], b, h, 0.0)
                                rows.append(_of_head([pu.get(k) for k in at], b, h, u32(0)))
                            p = _unpack(jnp.concatenate(rows, axis=0))
                        lacc[h] = lt if lacc[h] is None else lacc[h] + lt
                        o = _dot(_unpack(vt[g, _hs(h * DH, DH), ks]), p)
                        oacc[h] = o if oacc[h] is None else oacc[h] + o
                        if h == 0:
                            last["o"] = o[0:8, :]
            if gn is not None:
                mbuf[t][pw] = jnp.max(macc, axis=0, keepdims=True)
            if g is not None:
                parts = []
                for h in range(4):
                    l = jnp.sum(lacc[h], axis=0, keepdims=True)
                    gh = gate[half, g * 4 + h:g * 4 + h + 1, :]
                    oh = oacc[h] * ((1.0 - gh) / l)
                    parts.append(pltpu.roll(oh, 128 - DH * ROT[h], 1) if h else oh)
                ot = jnp.concatenate(parts, axis=0) + amem[g, :, t * 128:(t + 1) * 128]
                if g < GH - 1 or t < 2:
                    ob[g, _hs(t * 128, 128), :] = _pack(ot.T)
                else:
                    obl[half, _hs((t - 2) * 128, 128), :] = _pack(ot.T)

    rowh = jax.lax.broadcasted_iota(jnp.int32, (128, 128), 0) // DH
    colh = jax.lax.broadcasted_iota(jnp.int32, (128, 128), 1) // DH
    row16 = jax.lax.broadcasted_iota(jnp.int32, (16, 128), 0)
    col16 = jax.lax.broadcasted_iota(jnp.int32, (16, 128), 1) // DH

    def attn_half(layer, seg, half):
        r0 = pl.multiple_of(seg * L, L)

        @pl.when(jnp.logical_and(jnp.logical_and(layer == 0, seg == 0), half == 1))
        def _():
            cp_wk[1].wait()
            cp_wo[1].wait()
            cp_w1.wait()
            cp_xr.wait()
            cp_w2.wait()
            for cp in cp_stage[4:8]:
                cp.wait()
            for ic in range(4):
                transpose(1, 4 + ic, (ic >> 1) * DHALF, (ic & 1) * 2)

        def xn(c0, nc):
            return _unpack(xna[_hs(c0 * 128, nc * 128), :])

        zparts = {}

        def k_piece(g0, ng, c0, nc):
            k = _dot(xn(c0, nc), _unpack(wk[half, :, g0 * 128:(g0 + ng) * 128]))
            pk = _phi(k)
            rs = _hs(c0 * 128, nc * 128)
            for i in range(ng):
                cs = slice(i * 128, (i + 1) * 128)
                kb[g0 + i, rs, :] = _pack(k[:, cs])
                pkb[g0 + i, rs, :] = _pack(pk[:, cs])
                zparts.setdefault(g0 + i, []).append(_red8(pk[:, cs], jnp.add))

        def qv_piece(qs, vs, c0, nc):
            offs = [g * 128 for g in qs] + [DHALF + g * 128 for g in vs]
            lhs = jnp.concatenate(
                [jnp.concatenate([wt[half, c, _hs(o, 128), :] for c in range(NTC)], axis=1)
                 for o in offs], axis=0)
            r = _dot_nt(_unpack(lhs), xn(c0, nc))
            ts = slice(c0 * 128, (c0 + nc) * 128)
            for i, g in enumerate(qs):
                qg = r[i * 128:(i + 1) * 128, :]
                qp = _pack(qg * QSCALE)
                for c in range(nc):
                    for h in range(4):
                        qh = qp[_hs(h * DH, DH), c * 128:(c + 1) * 128]
                        qt[g, _hs(h * DH, DH), (c0 + c) * 128:(c0 + c + 1) * 128] = (
                            pltpu.roll(qh, DH * ROT[h], 1) if h else qh)
                pqt[g, :, ts] = _pack(_phi(qg))
            for i, g in enumerate(vs):
                o = (len(qs) + i) * 128
                vt[g, :, ts] = _pack(r[o:o + 128, :])

        def mem(g):
            zold = zrow[half, g]
            mold = mt[half, g]
            mbd = jnp.where(rowh == colh, mold, 0.0)
            zx = jnp.where(row16 == col16, jnp.broadcast_to(zold, (16, 128)), 0.0)
            lhs = jnp.concatenate([mbd, zx], axis=0).astype(bf16)
            ret = _dot(lhs, _unpack(pqt[g]))
            parts = []
            for h in range(4):
                gh = gate[half, g * 4 + h:g * 4 + h + 1, 0:1]
                den = ret[128 + h:129 + h, :] + 1e-6
                parts.append(ret[h * DH:(h + 1) * DH, :] * (gh / den))
            amem[g] = jnp.concatenate(parts, axis=0)
            zsum = functools.reduce(jnp.add, zparts[g])
            zrow[half, g] = zold + jnp.sum(zsum, axis=0, keepdims=True)

        def upd(g):
            mt[half, g] = mt[half, g] + _dot(_unpack(vt[g]), _unpack(pkb[g]))

        def mem_upd(g):
            mem(g)
            upd(g)

        P = functools.partial
        skip = None
        last = {}
        k_piece(0, 2, 0, 4)
        qv_piece((0, 1), (0,), 0, 4)
        attn_step(half, None, 0, last)
        mem(0)
        for g in range(2):
            attn_step(half, g, g + 1, last, fill=[
                skip, P(k_piece, g + 2, 1, 0, 2), skip, P(qv_piece, (g + 2,), (g + 1,), 0, 1),
                P(qv_piece, (g + 2,), (g + 1,), 1, 1), skip, P(k_piece, g + 2, 1, 2, 2),
                P(qv_piece, (g + 2,), (g + 1,), 2, 1), P(qv_piece, (g + 2,), (g + 1,), 3, 1),
                P(mem_upd, g + 1)])
        attn_step(half, 2, 3, last, fill=[
            P(upd, 0), skip, P(qv_piece, (), (3,), 0, 1), skip, P(qv_piece, (), (3,), 1, 1),
            skip, P(qv_piece, (), (3,), 2, 1), P(qv_piece, (), (3,), 3, 1), skip, P(mem_upd, 3)])

        def wo_piece(t, n):
            off = t * 128
            cs = slice(n * DHALF, (n + 1) * DHALF)
            rr = pl.ds(r0 + (HALO + off), 128)
            ng = GH if t < 2 else GH - 1
            o = jnp.concatenate([ob[g, _hs(off, 128), :] for g in range(ng)], axis=1)
            big[rr, cs] = big[rr, cs] + _dot(_unpack(o), _unpack(wo[half, _hs(0, ng * 128), cs]))

        attn_step(half, GH - 1, None, last, fill=[
            P(wo_piece, 2, 0), P(wo_piece, 2, 1), P(wo_piece, 3, 0), skip, P(wo_piece, 3, 1),
            P(wo_piece, 0, 0), skip, P(wo_piece, 0, 1), P(wo_piece, 1, 0), skip])
        wo_piece(1, 1)

    def phase_a(layer, seg):
        r0 = pl.multiple_of(seg * L, L)

        def half_body(half, _):
            attn_half(layer, seg, half)
            return 0
        jax.lax.fori_loop(0, 2, half_body, 0)

        hl = L // 2
        kp = (GH - 1) * 128

        bw = big.at[pl.ds(r0, 2 * L + 2 * HALO), :]
        yw = yres.at[pl.ds(r0, L + 2 * HALO), :]
        hw = hbuf.at[pl.ds(r0, L + 2 * HALO), :]
        xw = xin.at[pl.ds(r0 + L, L), :]

        def wo_rest():
            rr = slice(HALO + hl, HALO + L)
            o = _unpack(jnp.concatenate([obl[0], obl[1]], axis=1))
            w = _unpack(jnp.concatenate([wo[i, _hs(kp, 128), :] for i in range(2)], axis=0))
            bw[rr, :] = bw[rr, :] + _dot(o, w)

        def lnln(off, n):
            rr = slice(HALO + off, HALO + off + n)
            r, mr, z = _ln_ln(bw[rr, :])
            yw[rr, D - 256:D - 128] = jnp.broadcast_to(r, (n, 128))
            yw[rr, D - 128:D] = jnp.broadcast_to(mr, (n, 128))
            xnb[_hs(off, n), :] = _pack(z)

        def corners(v):
            return [v[0:8, 0:128], v[hl - 8:hl, 0:128], v[0:8, 128:256], v[hl - 8:hl, 128:256]]

        def up(off, n):
            cs = slice(n * 256, (n + 1) * 256)
            hh = _gelu(_dot(_unpack(xnb[_hs(off, hl), :]), _unpack(w1[:, cs])))
            b = off + HALO + SHIFTS[n]
            hw[b:b + hl, cs] = hh
            return corners(hh)

        sink = PIN + pl.multiple_of(seg * 16, 16)

        def pin(ref, v):
            if ref.dtype == bf16:
                ref[pl.ds(sink, 16), 0:128] = jnp.concatenate([v, v], axis=0).astype(bf16)
            else:
                ref[pl.ds(sink, 8), 0:128] = v

        fresh = jnp.logical_and(layer == 0, seg < NSEG - 1)

        def ln_next(off, n):
            rr = slice(L + HALO + off, L + HALO + off + n)
            xv = jnp.where(fresh, xw[off:off + n, :].astype(f32), bw[rr, :])
            bw[rr, :] = xv
            xna[_hs(off, n), :] = _pack(_ln(xv))

        lnln(0, 128)
        lnln(128, 128)
        wo_rest()
        def mix_part(off, n):
            return corners(mix(hw, yw, bw, slice(off, off + hl), n))

        def fence():
            pin(yres, pltpu.bitcast(xna[pl.ds(pl.multiple_of(seg * 8, 8), 8), 0:128], f32))

        late = list(range(hl, L, 16))
        nxt = list(range(0, L, 16))
        for n in range(4):
            for mark in up(0, n):
                lnln(late.pop(0), 16)
                pin(big, mark)
        for n in range(4):
            for mark in mix_part(0, n):
                ln_next(nxt.pop(0), 16)
                pin(xin, mark)
        for n in range(4):
            for mark in up(hl, n)[1::2]:
                ln_next(nxt.pop(0), 16)
                pin(xin, mark)
        for n in range(4):
            if n == 3:
                fence()
            marks = mix_part(hl, n)
            for i in range(4):
                if nxt:
                    ln_next(nxt.pop(0), 16)
                    pin(xin, marks[i])

    def mix(h_ref, y_ref, x_ref, rr, n):
        cs = slice(n * 256, (n + 1) * 256)
        r = y_ref[rr, D - 256:D - 128]
        mr = y_ref[rr, D - 128:D]
        x = x_ref[rr, cs]
        y = x * jnp.concatenate([r, r], axis=1) - jnp.concatenate([mr, mr], axis=1)
        x1 = y + _dot(h_ref[rr, :].astype(bf16), _unpack(w2[:, cs]))
        y_ref[rr, cs] = x1
        x_ref[rr, cs] = x + x1
        return x1

    def ln_mid(tok, n):
        xnc[_hs(tok, n), :] = _pack(_ln(yres[pl.ds(tok + HALO, n), :]))

    def last_rows():
        for n in range(4):
            mix(hbuf, yres, big, slice(S, PAD_ROWS), n)
            ln_mid(n * 128, 128)

    def out_copy(blk):
        rows = pl.ds(blk * L, L)
        return pltpu.make_async_copy(obuf.at[rows], out_hbm.at[0, rows, :], osems.at[blk])

    def ffn(layer, it):
        def block_of(pair):
            return (pair * 37) >> 8

        blk, chunk, tok = [], [], []
        for h in range(UNROLL // 2):
            pair = (UNROLL // 2) * it + h
            b = block_of(pair)
            c = 2 * pair - NC * b
            t = pl.multiple_of(b * L, L)
            blk += [b, b]
            chunk += [c, c + 1]
            tok += [t, t]

        def ffn_up(k):
            hh = _gelu(_dot(_unpack(xnc[_hs(tok[k], L), :]), _unpack(w3[chunk[k]])))
            gh[k % 2] = _pack(hh)
            return hh[L - 8:L, FC - 128:FC]

        def ffn_down(k):
            rows = pl.ds(tok[k] + HALO, L)
            w = _unpack(w4[_hs(chunk[k] * FC, FC), :])
            big[rows, :] = big[rows, :] + _dot(_unpack(gh[k % 2]), w)

        def ln_ahead(k, mark):
            yres[pl.ds(PIN + pl.multiple_of(blk[0] * 16, 16), 8), 0:128] = mark
            nb = jnp.minimum(blk[k] + 1, NSEG - 1)
            ln_mid(pl.multiple_of(nb * L + jnp.minimum(chunk[k] * 40, L - 80), 16), 80)

        def ln_first():
            r = pl.multiple_of(jnp.clip((it - 3) * 48, 0, L - 48), 16)
            xna[_hs(r, 48), :] = _pack(_ln(big[pl.ds(r + HALO, 48), :]))

        ffn_up(0)
        ln_ahead(0, ffn_up(1))
        ffn_down(0)
        ln_ahead(2, ffn_up(2))
        ffn_down(1)
        ffn_up(3)
        ln_first()
        ffn_down(2)
        ffn_down(3)

        done = block_of((UNROLL // 2) * (it + 1))

        @pl.when(jnp.logical_and(layer == 1, done != blk[0]))
        def _():
            r = pl.multiple_of((done - 1) * L, L)
            obuf[pl.ds(r, L), :] = big[pl.ds(r + HALO, L), :].astype(bf16)
            out_copy(done - 1).start()

    def layer_body(layer, _):
        mt[...] = jnp.zeros(mt.shape, f32)
        zrow[...] = jnp.zeros(zrow.shape, f32)

        def a_body(seg, _):
            phase_a(layer, seg)
            return 0
        jax.lax.fori_loop(0, NSEG, a_body, 0)

        last_rows()

        @pl.when(layer == 0)
        def _():
            for c in cp_w3:
                c.wait()
            cp_w4.wait()

        def b_body(it, _):
            ffn(layer, it)
            return 0
        jax.lax.fori_loop(0, NSEG * NC // UNROLL, b_body, 0)
        return 0
    jax.lax.fori_loop(0, 2, layer_body, 0)

    for blk in range(NSEG):
        out_copy(blk).wait()


@jax.jit
def pallas_interleave_layers__memory_aug_infini_attn__mixer_s_mlp__prompt_kernel(
    A_x: jax.Array,
    A_wq: jax.Array,
    A_wk: jax.Array,
    A_wv: jax.Array,
    A_wo: jax.Array,
    A_beta: jax.Array,
    B_x: jax.Array,
    B_w1: jax.Array,
    B_w2: jax.Array,
    B_w3: jax.Array,
    B_w4: jax.Array,
):
    del B_x
    hbm = pl.BlockSpec(memory_space=pl.ANY)
    vm = pltpu.VMEM
    scratch = [
        vm((BIG_ROWS, D), bf16),
        vm((8, DHALF, DHALF), bf16),
        vm((2, 4, D // 2, 256), u32),
        vm((2, D // 2, DHALF), u32),
        vm((2, DHALF // 2, D), u32),
        vm((D // 2, D), u32),
        vm((D // 2, D), u32),
        vm((NC, D // 2, FC), u32),
        vm((F // 2, D), u32),
        vm((BIG_ROWS, D), f32),
        vm((BIG_ROWS, D), f32),
        vm((PAD_ROWS, D), f32),
        vm((L // 2, D), u32),
        vm((L // 2, D), u32),
        vm((S // 2, D), u32),
        vm((2, L // 2, FC), u32),
        vm((GH, 64, L), u32),
        vm((GH, 64, L), u32),
        vm((GH, L // 2, 128), u32),
        vm((GH, L // 2, 128), u32),
        vm((GH, 64, L), u32),
        vm((GH, L // 2, 128), u32),
        vm((2, L // 4, 128), u32),
        vm((GH, 128, L), f32),
        vm((2, GH, 128, 128), f32),
        vm((2, GH, 1, 128), f32),
        vm((2, H // 2, 128), f32),
        vm((128, 512), f32),
    ]
    scratch += [vm((1, 128 * (t + 1) + 8, 512), f32) for _ in range(2) for t in range(NT_TILES)]
    scratch += [vm((2, 1, 512), f32) for _ in range(NT_TILES)]
    scratch += [
        vm((S, D), bf16),
        pltpu.SemaphoreType.DMA((10,)),
        pltpu.SemaphoreType.DMA((8,)),
        pltpu.SemaphoreType.DMA((NSEG,)),
    ]
    return pl.pallas_call(
        _kernel,
        out_shape=jax.ShapeDtypeStruct((1, S, D), bf16),
        in_specs=[hbm, hbm, hbm, hbm, hbm, pl.BlockSpec(memory_space=pltpu.VMEM),
                  hbm, hbm, hbm, hbm],
        out_specs=hbm,
        scratch_shapes=scratch,
        compiler_params=pltpu.CompilerParams(vmem_limit_bytes=120 * 1024 * 1024),
    )(A_x, A_wq, A_wk, A_wv, A_wo, A_beta.reshape(1, H), B_w1, B_w2, B_w3, B_w4)
```

```python
import functools
import math

import jax
import jax.numpy as jnp
import jax.experimental.pallas as pl
import jax.experimental.pallas.tpu as pltpu

S = 2048
D = 1024
F = 3584
H = 32
DH = 32
L = 512
NSEG = S // L
NG = D // 128
NT_TILES = L // 128
FC = 256
HALO = 8
GH = NG // 2
DHALF = D // 2
PAD_ROWS = S + 2 * HALO
PIN = S + L + 2 * HALO
BIG_ROWS = PIN + 16 * NSEG
NC = F // FC
UNROLL = 4
SHIFTS = (1, -1, 2, -2)
ROT = (0, 2, 1, 3)
OWNER = (((0,) * 4, (1,) * 4, (2,) * 4, (3,) * 4),
         ((3, 0, 0, 0), (1, 1, 3, 1), (2, 3, 2, 2)),
         ((1, 1, 0, 0), (2, 3, 3, 2)),
         ((2, 1, 3, 0),))

LOG2E = math.log2(math.e)
QSCALE = DH ** -0.5 * LOG2E
MASK_BIAS = -1e9 * LOG2E
EPS = 1e-5

f32 = jnp.float32
bf16 = jnp.bfloat16
u32 = jnp.uint32
NT_DIMS = (((1,), (1,)), ((), ()))


def _stats(x):
    m = jnp.mean(x, axis=-1, keepdims=True)
    xc = x - m
    return m, jnp.mean(xc * xc, axis=-1, keepdims=True)


def _ln(x):
    m, v = _stats(x)
    r = jax.lax.rsqrt(v + EPS)
    return x * r - m * r


def _ln_ln(x):
    m, v = _stats(x)
    r1 = jax.lax.rsqrt(v + EPS)
    r2 = r1 * jax.lax.rsqrt(v * r1 * r1 + EPS)
    return r1, m * r1, x * r2 - m * r2


def _gelu(x):
    c = math.sqrt(2.0 / math.pi)
    inner = x * (c + (c * 0.044715) * (x * x))
    hx = 0.5 * x
    return hx + hx * jnp.tanh(inner)


def _phi(t):
    return jnp.where(t > 0, t + 1.0, jnp.exp(t))


def _red8(x, op):
    return functools.reduce(op, [x[i * 8:(i + 1) * 8] for i in range(x.shape[0] // 8)])


def _pick(pos, x, other):
    if len(pos) == 4:
        return x
    lane = jax.lax.broadcasted_iota(jnp.int32, x.shape, 1)
    if len(pos) == 2:
        low = lane < 64 if pos in ((0, 1), (2, 3)) else ((lane + 32) & 127) < 64
        return jnp.where(low, x, other) if 0 in pos else jnp.where(low, other, x)
    if len(pos) == 1:
        return jnp.where((lane >> 5) == pos[0], x, other)
    return jnp.where((lane >> 5) == 6 - sum(pos), other, x)


def _owned(b, i, h):
    return tuple(p for p in range(4) if OWNER[b][i][p] == h)


def _of_head(tiles, b, h, other):
    for i, x in enumerate(tiles):
        if _owned(b, i, h):
            other = _pick(_owned(b, i, h), x, other)
    return other


def _of_tile(heads, b, i):
    out = None
    for h in sorted(set(OWNER[b][i]), key=lambda h: -len(_owned(b, i, h))):
        out = heads[h] if out is None else _pick(_owned(b, i, h), heads[h], out)
    return out


def _pack(x):
    return pltpu.bitcast(x.astype(bf16), u32)


def _unpack(x):
    return pltpu.bitcast(x, bf16)


def _hs(start, n):
    if isinstance(start, int):
        return slice(start // 2, (start + n) // 2)
    return pl.ds(pl.multiple_of(start >> 1, 8), n // 2)


def _dot(a, b):
    return jnp.dot(a, b, preferred_element_type=f32)


def _dot_nt(a, b):
    return jax.lax.dot_general(a, b, NT_DIMS, preferred_element_type=f32)


def _kernel(x_hbm, wq_hbm, wk_hbm, wv_hbm, wo_hbm, beta_ref, w1_hbm, w2_hbm, w3_hbm, w4_hbm,
            out_hbm,
            xin, stage, wt, wk, wo, w1, w2, w3, w4,
            big, yres, hbuf, xna, xnb, xnc, gh, qt, pqt, kb, pkb, vt, ob, obl, amem,
            mt, zrow, gate, bias,
            s0, s1, s2, s3, s4, s5, s6, s7, m0, m1, m2, m3,
            obuf, sems, tsems, osems):
    sbuf = ((s0, s1, s2, s3), (s4, s5, s6, s7))
    mbuf = (m0, m1, m2, m3)

    def seg_rows(s):
        return pl.ds(s * L, L)

    cp_x0 = pltpu.make_async_copy(x_hbm.at[0, seg_rows(0)], xin.at[seg_rows(0)], sems.at[0])
    cp_xr = pltpu.make_async_copy(x_hbm.at[0, pl.ds(L, S - L)], xin.at[pl.ds(L, S - L)], sems.at[1])
    cp_wk = [pltpu.make_async_copy(wk_hbm.at[:, pl.ds(i * DHALF, DHALF)], wk.at[i].bitcast(bf16),
                                   sems.at[2 + i])
             for i in range(2)]
    cp_wo = [pltpu.make_async_copy(wo_hbm.at[pl.ds(i * DHALF, DHALF)], wo.at[i].bitcast(bf16),
                                   sems.at[4 + i])
             for i in range(2)]
    cp_w1 = pltpu.make_async_copy(w1_hbm, w1.bitcast(bf16), sems.at[6])
    cp_w2 = pltpu.make_async_copy(w2_hbm, w2.bitcast(bf16), sems.at[7])
    cp_w3 = [pltpu.make_async_copy(w3_hbm.at[:, pl.ds(c * FC, FC)], w3.at[c].bitcast(bf16),
                                   sems.at[8])
             for c in range(F // FC)]
    cp_w4 = pltpu.make_async_copy(w4_hbm, w4.bitcast(bf16), sems.at[9])

    TC = 256
    NTC = D // TC

    cp_stage = [pltpu.make_async_copy(
        (wq_hbm, wv_hbm)[(ic >> 1) & 1].at[pl.ds((ic & 1) * DHALF, DHALF),
                                           pl.ds((ic >> 2) * DHALF, DHALF)],
        stage.at[ic], tsems.at[ic]) for ic in range(8)]

    for cp in cp_stage[0:4]:
        cp.start()
    for cp in (cp_x0, cp_wk[0], cp_wo[0]):
        cp.start()

    kk = jax.lax.broadcasted_iota(jnp.int32, (DH, 128), 0)
    ll = jax.lax.broadcasted_iota(jnp.int32, (DH, 128), 1)
    qq = [(ll + (128 - DH * r)) & 127 for r in ROT]
    for b in range(4):
        for i in range(4 - b):
            bias[b * DH:(b + 1) * DH, i * 128:(i + 1) * 128] = jnp.where(
                kk + b * DH > _of_tile(qq, b, i), MASK_BIAS, 0.0).astype(f32)
    bt = jnp.broadcast_to(beta_ref[...].astype(f32), (H, H))
    eye = (jax.lax.broadcasted_iota(jnp.int32, (H, H), 0)
           == jax.lax.broadcasted_iota(jnp.int32, (H, H), 1))
    bcol = jnp.sum(jnp.where(eye, bt, 0.0), axis=1, keepdims=True)
    gsig = jnp.broadcast_to(jax.nn.sigmoid(bcol), (H, 128))
    gate[0] = gsig[0:H // 2]
    gate[1] = gsig[H // 2:H]
    hbuf[0:2 * HALO, :] = jnp.zeros((2 * HALO, D), f32)
    hbuf[S:PAD_ROWS, :] = jnp.zeros((2 * HALO, D), f32)
    for ref in (big, yres):
        ref[0:HALO, :] = jnp.zeros((HALO, D), f32)
        ref[S + HALO:PAD_ROWS, :] = jnp.zeros((HALO, D), f32)

    ident = (jax.lax.broadcasted_iota(jnp.int32, (128, 128), 0)
             == jax.lax.broadcasted_iota(jnp.int32, (128, 128), 1)).astype(f32).astype(bf16)

    def transpose(hf, ic, ro, c0):
        for c in range(2):
            for n in range(GH):
                tile = _dot_nt(ident, stage[ic, c * TC:(c + 1) * TC, n * 128:(n + 1) * 128])
                wt[hf, c0 + c, _hs(ro + n * 128, 128), :] = _pack(tile)

    def transpose_chunk(ic, _):
        pltpu.make_async_copy(stage.at[ic], stage.at[ic], tsems.at[ic]).wait()
        transpose(0, ic, pl.multiple_of((ic >> 1) * DHALF, DHALF), (ic & 1) * 2)
        return 0
    jax.lax.fori_loop(0, 4, transpose_chunk, 0)

    cp_x0.wait()

    def init_x(i, _):
        r = pl.multiple_of(i * 256, 256)
        xv = xin[pl.ds(r, 256), :].astype(f32)
        big[pl.ds(HALO + r, 256), :] = xv
        xna[_hs(r, 256), :] = _pack(_ln(xv))
        return 0
    jax.lax.fori_loop(0, L // 256, init_x, 0)
    cp_wk[0].wait()
    for cp in cp_stage[4:8] + [cp_wk[1], cp_wo[1], cp_w1, cp_xr, cp_w2] + cp_w3 + [cp_w4]:
        cp.start()
    cp_wo[0].wait()

    def qmask(g, t, b=0):
        z = jnp.zeros((DH // 2, 128), u32)
        qs = [qt[g, _hs(h * DH, DH), t * 128:(t + 1) * 128] for h in range(4)]
        cols = [jnp.concatenate([_pick(_owned(b, i, h), qs[h], z) if _owned(b, i, h) else z
                                 for h in range(4)], axis=0) for i in range(4 - b)]
        return _unpack(jnp.concatenate(cols, axis=1))

    def tiles(x):
        return [x[:, i * 128:(i + 1) * 128] for i in range(x.shape[1] // 128)]

    def attn_step(half, g, gn, last, fill=()):
        pr = None if g is None else g % 2
        pw = None if gn is None else gn % 2
        fill = list(fill)
        for t in range(NT_TILES):
            macc = None
            oacc = [None] * 4
            lacc = [None] * 4
            for j in range(t + 1):
                ks = slice(j * 128, (j + 1) * 128)
                nk = DH if j == t else 128
                kl = slice(j * 128, j * 128 + nk)
                filled = fill.pop(0) if fill else None
                if filled:
                    filled()
                    last["pace"] = last.get("o", last["s"])
                elif gn is not None and g is not None:
                    last["pace"] = last["s"]
                if g is not None:
                    sbuf[pr][t][0, (t + 1) * 128:(t + 1) * 128 + 8, 0:128] = last["pace"]
                if gn is not None:
                    s = _dot(_unpack(kb[gn, _hs(j * 128, nk), :]), qmask(gn, t))
                    if j == t:
                        s = s + bias[0:DH, :]
                    sbuf[pw][t][0, kl, :] = s
                    last["s"] = s[0:8, 0:128]
                    mx = _red8(s, jnp.maximum)
                    if j == t:
                        mx = tiles(mx)
                        for b in range(1, 4):
                            k0 = j * 128 + b * DH
                            su = _dot(_unpack(kb[gn, _hs(k0, DH), :]), qmask(gn, t, b))
                            su = su + bias[b * DH:(b + 1) * DH, 0:(4 - b) * 128]
                            sbuf[pw][t][0, k0:k0 + DH, 0:(4 - b) * 128] = su
                            mu = tiles(_red8(su, jnp.maximum))
                            mx = [jnp.maximum(mx[h], _of_head(mu, b, h, mx[h])) for h in range(4)]
                        mx = jnp.concatenate(mx, axis=1)
                    macc = mx if macc is None else jnp.maximum(macc, mx)
                if g is not None:
                    ms = tiles(mbuf[t][pr])
                    pu, lu = {}, {}
                    for h in range(4):
                        sl = slice(h * 128, (h + 1) * 128)
                        p = jnp.exp2(sbuf[pr][t][half >> 1, kl, sl] - ms[h])
                        lt = _red8(p, jnp.add)
                        p = p.astype(bf16)
                        if j == t:
                            rows = [pltpu.bitcast(p, u32)]
                            for b in range(1, 4):
                                k0 = j * 128 + b * DH
                                for i in range(4 - b):
                                    if _owned(b, i, h) and (b, i) not in pu:
                                        e = jnp.exp2(sbuf[pr][t][half >> 1, k0:k0 + DH,
                                                                 i * 128:(i + 1) * 128]
                                                     - _of_tile(ms, b, i))
                                        lu[b, i] = _red8(e, jnp.add)
                                        pu[b, i] = _pack(e)
                                at = [(b, i) for i in range(4 - b)]
                                lt = lt + _of_head([lu.get(k) for k in at], b, h, 0.0)
                                rows.append(_of_head([pu.get(k) for k in at], b, h, u32(0)))
                            p = _unpack(jnp.concatenate(rows, axis=0))
                        lacc[h] = lt if lacc[h] is None else lacc[h] + lt
                        o = _dot(_unpack(vt[g, _hs(h * DH, DH), ks]), p)
                        oacc[h] = o if oacc[h] is None else oacc[h] + o
                        if h == 0:
                            last["o"] = o[0:8, :]
            if gn is not None:
                mbuf[t][pw] = jnp.max(macc, axis=0, keepdims=True)
            if g is not None:
                parts = []
                for h in range(4):
                    l = jnp.sum(lacc[h], axis=0, keepdims=True)
                    gh = gate[half, g * 4 + h:g * 4 + h + 1, :]
                    oh = oacc[h] * ((1.0 - gh) / l)
                    parts.append(pltpu.roll(oh, 128 - DH * ROT[h], 1) if h else oh)
                ot = jnp.concatenate(parts, axis=0) + amem[g, :, t * 128:(t + 1) * 128]
                if g < GH - 1 or t < 2:
                    ob[g, _hs(t * 128, 128), :] = _pack(ot.T)
                else:
                    obl[half, _hs((t - 2) * 128, 128), :] = _pack(ot.T)

    rowh = jax.lax.broadcasted_iota(jnp.int32, (128, 128), 0) // DH
    colh = jax.lax.broadcasted_iota(jnp.int32, (128, 128), 1) // DH
    row16 = jax.lax.broadcasted_iota(jnp.int32, (16, 128), 0)
    col16 = jax.lax.broadcasted_iota(jnp.int32, (16, 128), 1) // DH

    def attn_half(layer, seg, half):
        r0 = pl.multiple_of(seg * L, L)

        @pl.when(jnp.logical_and(jnp.logical_and(layer == 0, seg == 0), half == 1))
        def _():
            cp_wk[1].wait()
            cp_wo[1].wait()
            cp_w1.wait()
            cp_xr.wait()
            cp_w2.wait()
            for cp in cp_stage[4:8]:
                cp.wait()
            for ic in range(4):
                transpose(1, 4 + ic, (ic >> 1) * DHALF, (ic & 1) * 2)

        def xn(c0, nc):
            return _unpack(xna[_hs(c0 * 128, nc * 128), :])

        zparts = {}

        def k_piece(g0, ng, c0, nc):
            k = _dot(xn(c0, nc), _unpack(wk[half, :, g0 * 128:(g0 + ng) * 128]))
            pk = _phi(k)
            rs = _hs(c0 * 128, nc * 128)
            for i in range(ng):
                cs = slice(i * 128, (i + 1) * 128)
                kb[g0 + i, rs, :] = _pack(k[:, cs])
                pkb[g0 + i, rs, :] = _pack(pk[:, cs])
                zparts.setdefault(g0 + i, []).append(_red8(pk[:, cs], jnp.add))

        def qv_piece(qs, vs, c0, nc):
            offs = [g * 128 for g in qs] + [DHALF + g * 128 for g in vs]
            lhs = jnp.concatenate(
                [jnp.concatenate([wt[half, c, _hs(o, 128), :] for c in range(NTC)], axis=1)
                 for o in offs], axis=0)
            r = _dot_nt(_unpack(lhs), xn(c0, nc))
            ts = slice(c0 * 128, (c0 + nc) * 128)
            for i, g in enumerate(qs):
                qg = r[i * 128:(i + 1) * 128, :]
                qp = _pack(qg * QSCALE)
                for c in range(nc):
                    for h in range(4):
                        qh = qp[_hs(h * DH, DH), c * 128:(c + 1) * 128]
                        qt[g, _hs(h * DH, DH), (c0 + c) * 128:(c0 + c + 1) * 128] = (
                            pltpu.roll(qh, DH * ROT[h], 1) if h else qh)
                pqt[g, :, ts] = _pack(_phi(qg))
            for i, g in enumerate(vs):
                o = (len(qs) + i) * 128
                vt[g, :, ts] = _pack(r[o:o + 128, :])

        def mem(g):
            zold = zrow[half, g]
            mold = mt[half, g]
            mbd = jnp.where(rowh == colh, mold, 0.0)
            zx = jnp.where(row16 == col16, jnp.broadcast_to(zold, (16, 128)), 0.0)
            lhs = jnp.concatenate([mbd, zx], axis=0).astype(bf16)
            ret = _dot(lhs, _unpack(pqt[g]))
            parts = []
            for h in range(4):
                gh = gate[half, g * 4 + h:g * 4 + h + 1, 0:1]
                den = ret[128 + h:129 + h, :] + 1e-6
                parts.append(ret[h * DH:(h + 1) * DH, :] * (gh / den))
            amem[g] = jnp.concatenate(parts, axis=0)
            zsum = functools.reduce(jnp.add, zparts[g])
            zrow[half, g] = zold + jnp.sum(zsum, axis=0, keepdims=True)

        def upd(g):
            mt[half, g] = mt[half, g] + _dot(_unpack(vt[g]), _unpack(pkb[g]))

        def mem_upd(g):
            mem(g)
            upd(g)

        P = functools.partial
        skip = None
        last = {}
        k_piece(0, 2, 0, 4)
        qv_piece((0, 1), (0,), 0, 4)
        attn_step(half, None, 0, last)
        mem(0)
        for g in range(2):
            attn_step(half, g, g + 1, last, fill=[
                skip, P(k_piece, g + 2, 1, 0, 2), skip, P(qv_piece, (g + 2,), (g + 1,), 0, 1),
                P(qv_piece, (g + 2,), (g + 1,), 1, 1), skip, P(k_piece, g + 2, 1, 2, 2),
                P(qv_piece, (g + 2,), (g + 1,), 2, 1), P(qv_piece, (g + 2,), (g + 1,), 3, 1),
                P(mem_upd, g + 1)])
        attn_step(half, 2, 3, last, fill=[
            P(upd, 0), skip, P(qv_piece, (), (3,), 0, 1), skip, P(qv_piece, (), (3,), 1, 1),
            skip, P(qv_piece, (), (3,), 2, 1), P(qv_piece, (), (3,), 3, 1), skip, P(mem_upd, 3)])

        def wo_piece(t, n):
            off = t * 128
            cs = slice(n * DHALF, (n + 1) * DHALF)
            rr = pl.ds(r0 + (HALO + off), 128)
            ng = GH if t < 2 else GH - 1
            o = jnp.concatenate([ob[g, _hs(off, 128), :] for g in range(ng)], axis=1)
            big[rr, cs] = big[rr, cs] + _dot(_unpack(o), _unpack(wo[half, _hs(0, ng * 128), cs]))

        attn_step(half, GH - 1, None, last, fill=[
            P(wo_piece, 2, 0), P(wo_piece, 2, 1), P(wo_piece, 3, 0), skip, P(wo_piece, 3, 1),
            P(wo_piece, 0, 0), skip, P(wo_piece, 0, 1), P(wo_piece, 1, 0), skip])
        wo_piece(1, 1)

    def phase_a(layer, seg):
        r0 = pl.multiple_of(seg * L, L)

        def half_body(half, _):
            attn_half(layer, seg, half)
            return 0
        jax.lax.fori_loop(0, 2, half_body, 0)

        hl = L // 2
        kp = (GH - 1) * 128

        bw = big.at[pl.ds(r0, 2 * L + 2 * HALO), :]
        yw = yres.at[pl.ds(r0, L + 2 * HALO), :]
        hw = hbuf.at[pl.ds(r0, L + 2 * HALO), :]
        xw = xin.at[pl.ds(r0 + L, L), :]

        def wo_rest():
            rr = slice(HALO + hl, HALO + L)
            o = _unpack(jnp.concatenate([obl[0], obl[1]], axis=1))
            w = _unpack(jnp.concatenate([wo[i, _hs(kp, 128), :] for i in range(2)], axis=0))
            bw[rr, :] = bw[rr, :] + _dot(o, w)

        def lnln(off, n):
            rr = slice(HALO + off, HALO + off + n)
            r, mr, z = _ln_ln(bw[rr, :])
            yw[rr, D - 256:D - 128] = jnp.broadcast_to(r, (n, 128))
            yw[rr, D - 128:D] = jnp.broadcast_to(mr, (n, 128))
            xnb[_hs(off, n), :] = _pack(z)

        def corners(v):
            return [v[0:8, 0:128], v[hl - 8:hl, 0:128], v[0:8, 128:256], v[hl - 8:hl, 128:256]]

        def up(off, n):
            cs = slice(n * 256, (n + 1) * 256)
            hh = _gelu(_dot(_unpack(xnb[_hs(off, hl), :]), _unpack(w1[:, cs])))
            b = off + HALO + SHIFTS[n]
            hw[b:b + hl, cs] = hh
            return corners(hh)

        sink = PIN + pl.multiple_of(seg * 16, 16)

        def pin(ref, v):
            if ref.dtype == bf16:
                ref[pl.ds(sink, 16), 0:128] = jnp.concatenate([v, v], axis=0).astype(bf16)
            else:
                ref[pl.ds(sink, 8), 0:128] = v

        fresh = jnp.logical_and(layer == 0, seg < NSEG - 1)

        def ln_next(off, n):
            rr = slice(L + HALO + off, L + HALO + off + n)
            xv = jnp.where(fresh, xw[off:off + n, :].astype(f32), bw[rr, :])
            bw[rr, :] = xv
            xna[_hs(off, n), :] = _pack(_ln(xv))

        lnln(0, 128)
        lnln(128, 128)
        wo_rest()
        def mix_part(off, n):
            return corners(mix(hw, yw, bw, slice(off, off + hl), n))

        def fence():
            pin(yres, pltpu.bitcast(xna[pl.ds(pl.multiple_of(seg * 8, 8), 8), 0:128], f32))

        late = list(range(hl, L, 16))
        nxt = list(range(0, L, 16))
        for n in range(4):
            for mark in up(0, n):
                lnln(late.pop(0), 16)
                pin(big, mark)
        for n in range(4):
            for mark in mix_part(0, n):
                ln_next(nxt.pop(0), 16)
                pin(xin, mark)
        for n in range(4):
            for mark in up(hl, n)[1::2]:
                ln_next(nxt.pop(0), 16)
                pin(xin, mark)
        for n in range(4):
            if n == 3:
                fence()
            marks = mix_part(hl, n)
            for i in range(4):
                if nxt:
                    ln_next(nxt.pop(0), 16)
                    pin(xin, marks[i])

    def mix(h_ref, y_ref, x_ref, rr, n):
        cs = slice(n * 256, (n + 1) * 256)
        r = y_ref[rr, D - 256:D - 128]
        mr = y_ref[rr, D - 128:D]
        x = x_ref[rr, cs]
        y = x * jnp.concatenate([r, r], axis=1) - jnp.concatenate([mr, mr], axis=1)
        x1 = y + _dot(h_ref[rr, :].astype(bf16), _unpack(w2[:, cs]))
        y_ref[rr, cs] = x1
        x_ref[rr, cs] = x + x1
        return x1

    def ln_mid(tok, n):
        xnc[_hs(tok, n), :] = _pack(_ln(yres[pl.ds(tok + HALO, n), :]))

    def last_rows():
        for n in range(4):
            mix(hbuf, yres, big, slice(S, PAD_ROWS), n)
            ln_mid(n * 128, 128)

    def out_copy(blk):
        rows = pl.ds(blk * L, L)
        return pltpu.make_async_copy(obuf.at[rows], out_hbm.at[0, rows, :], osems.at[blk])

    def ffn(layer, it):
        def block_of(pair):
            return (pair * 37) >> 8

        blk, chunk, tok = [], [], []
        for h in range(UNROLL // 2):
            pair = (UNROLL // 2) * it + h
            b = block_of(pair)
            c = 2 * pair - NC * b
            t = pl.multiple_of(b * L, L)
            blk += [b, b]
            chunk += [c, c + 1]
            tok += [t, t]

        def ffn_up(k):
            hh = _gelu(_dot(_unpack(xnc[_hs(tok[k], L), :]), _unpack(w3[chunk[k]])))
            gh[k % 2] = _pack(hh)
            return [hh[r:r + 8, FC - 128:FC] for r in (0, 256, L - 8)]

        def ffn_down(k):
            rows = pl.ds(tok[k] + HALO, L)
            w = _unpack(w4[_hs(chunk[k] * FC, FC), :])
            y = big[rows, :] + _dot(_unpack(gh[k % 2]), w)
            big[rows, :] = y
            return [y[r:r + 8, c:c + 128]
                    for r, c in ((0, 0), (256, 0), (504, 0), (0, 512), (256, 512))]

        sink = pl.ds(PIN + pl.multiple_of(blk[0] * 16, 16), 8)

        def ln_ahead(k, marks):
            nb = jnp.minimum(blk[k] + 1, NSEG - 1)
            r = nb * L + jnp.minimum(chunk[k] * 40, L - 80)
            n = 80 // len(marks)
            for i, mark in enumerate(marks):
                yres[sink, 0:128] = mark
                ln_mid(pl.multiple_of(r + i * n, 16), n)

        def ln_first(marks):
            r0 = jnp.clip((it - 3) * 48, 0, L - 48)
            for i, mark in enumerate(marks):
                r = pl.multiple_of(r0 + i * 16, 16)
                xna[_hs(r, 16), :] = _pack(_ln(big[pl.ds(r + HALO, 16), :]))
                if i < 2:
                    big[sink, 0:128] = mark

        ffn_up(0)
        ffn_up(1)
        ln_ahead(0, ffn_down(0))
        ffn_up(2)
        ffn_down(1)
        ln_first(ffn_up(3))
        ln_ahead(2, ffn_down(2))
        ffn_down(3)

        done = block_of((UNROLL // 2) * (it + 1))

        @pl.when(jnp.logical_and(layer == 1, done != blk[0]))
        def _():
            r = pl.multiple_of((done - 1) * L, L)
            obuf[pl.ds(r, L), :] = big[pl.ds(r + HALO, L), :].astype(bf16)
            out_copy(done - 1).start()

    def layer_body(layer, _):
        mt[...] = jnp.zeros(mt.shape, f32)
        zrow[...] = jnp.zeros(zrow.shape, f32)

        def a_body(seg, _):
            phase_a(layer, seg)
            return 0
        jax.lax.fori_loop(0, NSEG, a_body, 0)

        last_rows()

        @pl.when(layer == 0)
        def _():
            for c in cp_w3:
                c.wait()
            cp_w4.wait()

        def b_body(it, _):
            ffn(layer, it)
            return 0
        jax.lax.fori_loop(0, NSEG * NC // UNROLL, b_body, 0)
        return 0
    jax.lax.fori_loop(0, 2, layer_body, 0)

    for blk in range(NSEG):
        out_copy(blk).wait()


@jax.jit
def pallas_interleave_layers__memory_aug_infini_attn__mixer_s_mlp__prompt_kernel(
    A_x: jax.Array,
    A_wq: jax.Array,
    A_wk: jax.Array,
    A_wv: jax.Array,
    A_wo: jax.Array,
    A_beta: jax.Array,
    B_x: jax.Array,
    B_w1: jax.Array,
    B_w2: jax.Array,
    B_w3: jax.Array,
    B_w4: jax.Array,
):
    del B_x
    hbm = pl.BlockSpec(memory_space=pl.ANY)
    vm = pltpu.VMEM
    scratch = [
        vm((BIG_ROWS, D), bf16),
        vm((8, DHALF, DHALF), bf16),
        vm((2, 4, D // 2, 256), u32),
        vm((2, D // 2, DHALF), u32),
        vm((2, DHALF // 2, D), u32),
        vm((D // 2, D), u32),
        vm((D // 2, D), u32),
        vm((NC, D // 2, FC), u32),
        vm((F // 2, D), u32),
        vm((BIG_ROWS, D), f32),
        vm((BIG_ROWS, D), f32),
        vm((PAD_ROWS, D), f32),
        vm((L // 2, D), u32),
        vm((L // 2, D), u32),
        vm((S // 2, D), u32),
        vm((2, L // 2, FC), u32),
        vm((GH, 64, L), u32),
        vm((GH, 64, L), u32),
        vm((GH, L // 2, 128), u32),
        vm((GH, L // 2, 128), u32),
        vm((GH, 64, L), u32),
        vm((GH, L // 2, 128), u32),
        vm((2, L // 4, 128), u32),
        vm((GH, 128, L), f32),
        vm((2, GH, 128, 128), f32),
        vm((2, GH, 1, 128), f32),
        vm((2, H // 2, 128), f32),
        vm((128, 512), f32),
    ]
    scratch += [vm((1, 128 * (t + 1) + 8, 512), f32) for _ in range(2) for t in range(NT_TILES)]
    scratch += [vm((2, 1, 512), f32) for _ in range(NT_TILES)]
    scratch += [
        vm((S, D), bf16),
        pltpu.SemaphoreType.DMA((10,)),
        pltpu.SemaphoreType.DMA((8,)),
        pltpu.SemaphoreType.DMA((NSEG,)),
    ]
    return pl.pallas_call(
        _kernel,
        out_shape=jax.ShapeDtypeStruct((1, S, D), bf16),
        in_specs=[hbm, hbm, hbm, hbm, hbm, pl.BlockSpec(memory_space=pltpu.VMEM),
                  hbm, hbm, hbm, hbm],
        out_specs=hbm,
        scratch_shapes=scratch,
        compiler_params=pltpu.CompilerParams(vmem_limit_bytes=120 * 1024 * 1024),
    )(A_x, A_wq, A_wk, A_wv, A_wo, A_beta.reshape(1, H), B_w1, B_w2, B_w3, B_w4)
```

```python
import functools
import math

import jax
import jax.numpy as jnp
import jax.experimental.pallas as pl
import jax.experimental.pallas.tpu as pltpu

S = 2048
D = 1024
F = 3584
H = 32
DH = 32
L = 512
NSEG = S // L
NG = D // 128
NT_TILES = L // 128
FC = 256
HALO = 8
GH = NG // 2
DHALF = D // 2
PAD_ROWS = S + 2 * HALO
PIN = S + L + 2 * HALO
BIG_ROWS = PIN + 16 * NSEG
NC = F // FC
UNROLL = 4
SHIFTS = (1, -1, 2, -2)
ROT = (0, 2, 1, 3)
OWNER = (((0,) * 4, (1,) * 4, (2,) * 4, (3,) * 4),
         ((3, 0, 0, 0), (1, 1, 3, 1), (2, 3, 2, 2)),
         ((1, 1, 0, 0), (2, 3, 3, 2)),
         ((2, 1, 3, 0),))

LOG2E = math.log2(math.e)
QSCALE = DH ** -0.5 * LOG2E
MASK_BIAS = -1e9 * LOG2E
EPS = 1e-5

f32 = jnp.float32
bf16 = jnp.bfloat16
u32 = jnp.uint32
NT_DIMS = (((1,), (1,)), ((), ()))


def _stats(x):
    m = jnp.mean(x, axis=-1, keepdims=True)
    xc = x - m
    return m, jnp.mean(xc * xc, axis=-1, keepdims=True)


def _ln(x):
    m, v = _stats(x)
    r = jax.lax.rsqrt(v + EPS)
    return x * r - m * r


def _ln_ln(x):
    m, v = _stats(x)
    r1 = jax.lax.rsqrt(v + EPS)
    r2 = r1 * jax.lax.rsqrt(v * r1 * r1 + EPS)
    return r1, m * r1, x * r2 - m * r2


def _gelu(x):
    c = math.sqrt(2.0 / math.pi)
    inner = x * (c + (c * 0.044715) * (x * x))
    hx = 0.5 * x
    return hx + hx * jnp.tanh(inner)


def _phi(t):
    return jnp.where(t > 0, t + 1.0, jnp.exp(t))


def _red8(x, op):
    return functools.reduce(op, [x[i * 8:(i + 1) * 8] for i in range(x.shape[0] // 8)])


def _pick(pos, x, other):
    if len(pos) == 4:
        return x
    lane = jax.lax.broadcasted_iota(jnp.int32, x.shape, 1)
    if len(pos) == 2:
        low = lane < 64 if pos in ((0, 1), (2, 3)) else ((lane + 32) & 127) < 64
        return jnp.where(low, x, other) if 0 in pos else jnp.where(low, other, x)
    if len(pos) == 1:
        return jnp.where((lane >> 5) == pos[0], x, other)
    return jnp.where((lane >> 5) == 6 - sum(pos), other, x)


def _owned(b, i, h):
    return tuple(p for p in range(4) if OWNER[b][i][p] == h)


def _of_head(tiles, b, h, other):
    for i, x in enumerate(tiles):
        if _owned(b, i, h):
            other = _pick(_owned(b, i, h), x, other)
    return other


def _of_tile(heads, b, i):
    out = None
    for h in sorted(set(OWNER[b][i]), key=lambda h: -len(_owned(b, i, h))):
        out = heads[h] if out is None else _pick(_owned(b, i, h), heads[h], out)
    return out


def _pack(x):
    return pltpu.bitcast(x.astype(bf16), u32)


def _unpack(x):
    return pltpu.bitcast(x, bf16)


def _hs(start, n):
    if isinstance(start, int):
        return slice(start // 2, (start + n) // 2)
    return pl.ds(pl.multiple_of(start >> 1, 8), n // 2)


def _dot(a, b):
    return jnp.dot(a, b, preferred_element_type=f32)


def _dot_nt(a, b):
    return jax.lax.dot_general(a, b, NT_DIMS, preferred_element_type=f32)


def _kernel(x_hbm, wq_hbm, wk_hbm, wv_hbm, wo_hbm, beta_ref, w1_hbm, w2_hbm, w3_hbm, w4_hbm,
            out_hbm,
            xin, stage, wt, wk, wo, w1, w2, w3, w4,
            big, yres, hbuf, xna, xnb, xnc, gh, qt, pqt, kb, pkb, vt, ob, obl, amem,
            mt, zrow, gate, bias,
            s0, s1, s2, s3, s4, s5, s6, s7, m0, m1, m2, m3,
            obuf, sems, tsems, osems):
    sbuf = ((s0, s1, s2, s3), (s4, s5, s6, s7))
    mbuf = (m0, m1, m2, m3)

    def seg_rows(s):
        return pl.ds(s * L, L)

    cp_x0 = pltpu.make_async_copy(x_hbm.at[0, seg_rows(0)], xin.at[seg_rows(0)], sems.at[0])
    cp_xr = pltpu.make_async_copy(x_hbm.at[0, pl.ds(L, S - L)], xin.at[pl.ds(L, S - L)], sems.at[1])
    cp_wk = [pltpu.make_async_copy(wk_hbm.at[:, pl.ds(i * DHALF, DHALF)], wk.at[i].bitcast(bf16),
                                   sems.at[2 + i])
             for i in range(2)]
    cp_wo = [pltpu.make_async_copy(wo_hbm.at[pl.ds(i * DHALF, DHALF)], wo.at[i].bitcast(bf16),
                                   sems.at[4 + i])
             for i in range(2)]
    cp_w1 = pltpu.make_async_copy(w1_hbm, w1.bitcast(bf16), sems.at[6])
    cp_w2 = pltpu.make_async_copy(w2_hbm, w2.bitcast(bf16), sems.at[7])
    cp_w3 = [pltpu.make_async_copy(w3_hbm.at[:, pl.ds(c * FC, FC)], w3.at[c].bitcast(bf16),
                                   sems.at[8])
             for c in range(F // FC)]
    cp_w4 = pltpu.make_async_copy(w4_hbm, w4.bitcast(bf16), sems.at[9])

    TC = 256
    NTC = D // TC

    cp_stage = [pltpu.make_async_copy(
        (wq_hbm, wv_hbm)[(ic >> 1) & 1].at[pl.ds((ic & 1) * DHALF, DHALF),
                                           pl.ds((ic >> 2) * DHALF, DHALF)],
        stage.at[ic], tsems.at[ic]) for ic in range(8)]

    for cp in cp_stage[0:4]:
        cp.start()
    for cp in (cp_x0, cp_wk[0], cp_wo[0]):
        cp.start()

    kk = jax.lax.broadcasted_iota(jnp.int32, (DH, 128), 0)
    ll = jax.lax.broadcasted_iota(jnp.int32, (DH, 128), 1)
    qq = [(ll + (128 - DH * r)) & 127 for r in ROT]
    for b in range(4):
        for i in range(4 - b):
            bias[b * DH:(b + 1) * DH, i * 128:(i + 1) * 128] = jnp.where(
                kk + b * DH > _of_tile(qq, b, i), MASK_BIAS, 0.0).astype(f32)
    bt = jnp.broadcast_to(beta_ref[...].astype(f32), (H, H))
    eye = (jax.lax.broadcasted_iota(jnp.int32, (H, H), 0)
           == jax.lax.broadcasted_iota(jnp.int32, (H, H), 1))
    bcol = jnp.sum(jnp.where(eye, bt, 0.0), axis=1, keepdims=True)
    gsig = jnp.broadcast_to(jax.nn.sigmoid(bcol), (H, 128))
    gate[0] = gsig[0:H // 2]
    gate[1] = gsig[H // 2:H]
    hbuf[0:2 * HALO, :] = jnp.zeros((2 * HALO, D), f32)
    hbuf[S:PAD_ROWS, :] = jnp.zeros((2 * HALO, D), f32)
    for ref in (big, yres):
        ref[0:HALO, :] = jnp.zeros((HALO, D), f32)
        ref[S + HALO:PAD_ROWS, :] = jnp.zeros((HALO, D), f32)

    ident = (jax.lax.broadcasted_iota(jnp.int32, (128, 128), 0)
             == jax.lax.broadcasted_iota(jnp.int32, (128, 128), 1)).astype(f32).astype(bf16)

    def transpose(hf, ic, ro, c0):
        for c in range(2):
            for n in range(GH):
                tile = _dot_nt(ident, stage[ic, c * TC:(c + 1) * TC, n * 128:(n + 1) * 128])
                wt[hf, c0 + c, _hs(ro + n * 128, 128), :] = _pack(tile)

    def transpose_chunk(ic, _):
        pltpu.make_async_copy(stage.at[ic], stage.at[ic], tsems.at[ic]).wait()
        transpose(0, ic, pl.multiple_of((ic >> 1) * DHALF, DHALF), (ic & 1) * 2)
        return 0
    jax.lax.fori_loop(0, 4, transpose_chunk, 0)

    cp_x0.wait()

    def init_x(i, _):
        r = pl.multiple_of(i * 256, 256)
        xv = xin[pl.ds(r, 256), :].astype(f32)
        big[pl.ds(HALO + r, 256), :] = xv
        xna[_hs(r, 256), :] = _pack(_ln(xv))
        return 0
    jax.lax.fori_loop(0, L // 256, init_x, 0)
    cp_wk[0].wait()
    for cp in cp_stage[4:8] + [cp_wk[1], cp_wo[1], cp_w1, cp_xr, cp_w2] + cp_w3 + [cp_w4]:
        cp.start()
    cp_wo[0].wait()

    def qmask(g, t, b=0):
        z = jnp.zeros((DH // 2, 128), u32)
        qs = [qt[g, _hs(h * DH, DH), t * 128:(t + 1) * 128] for h in range(4)]
        cols = [jnp.concatenate([_pick(_owned(b, i, h), qs[h], z) if _owned(b, i, h) else z
                                 for h in range(4)], axis=0) for i in range(4 - b)]
        return _unpack(jnp.concatenate(cols, axis=1))

    def tiles(x):
        return [x[:, i * 128:(i + 1) * 128] for i in range(x.shape[1] // 128)]

    def attn_step(half, g, gn, last, fill=()):
        pr = None if g is None else g % 2
        pw = None if gn is None else gn % 2
        fill = list(fill)
        for t in range(NT_TILES):
            macc = None
            oacc = [None] * 4
            lacc = [None] * 4
            for j in range(t + 1):
                ks = slice(j * 128, (j + 1) * 128)
                nk = DH if j == t else 128
                kl = slice(j * 128, j * 128 + nk)
                filled = fill.pop(0) if fill else None
                if filled:
                    filled()
                    last["pace"] = last.get("o", last["s"])
                elif gn is not None and g is not None:
                    last["pace"] = last["s"]
                if g is not None:
                    sbuf[pr][t][0, (t + 1) * 128:(t + 1) * 128 + 8, 0:128] = last["pace"]
                if gn is not None:
                    s = _dot(_unpack(kb[gn, _hs(j * 128, nk), :]), qmask(gn, t))
                    if j == t:
                        s = s + bias[0:DH, :]
                    sbuf[pw][t][0, kl, :] = s
                    last["s"] = s[0:8, 0:128]
                    mx = _red8(s, jnp.maximum)
                    if j == t:
                        mx = tiles(mx)
                        for b in range(1, 4):
                            k0 = j * 128 + b * DH
                            su = _dot(_unpack(kb[gn, _hs(k0, DH), :]), qmask(gn, t, b))
                            su = su + bias[b * DH:(b + 1) * DH, 0:(4 - b) * 128]
                            sbuf[pw][t][0, k0:k0 + DH, 0:(4 - b) * 128] = su
                            mu = tiles(_red8(su, jnp.maximum))
                            mx = [jnp.maximum(mx[h], _of_head(mu, b, h, mx[h])) for h in range(4)]
                        mx = jnp.concatenate(mx, axis=1)
                    macc = mx if macc is None else jnp.maximum(macc, mx)
                if g is not None:
                    ms = tiles(mbuf[t][pr])
                    pu, lu = {}, {}
                    for h in range(4):
                        sl = slice(h * 128, (h + 1) * 128)
                        p = jnp.exp2(sbuf[pr][t][half >> 1, kl, sl] - ms[h])
                        lt = _red8(p, jnp.add)
                        p = p.astype(bf16)
                        if j == t:
                            rows = [pltpu.bitcast(p, u32)]
                            for b in range(1, 4):
                                k0 = j * 128 + b * DH
                                for i in range(4 - b):
                                    if _owned(b, i, h) and (b, i) not in pu:
                                        e = jnp.exp2(sbuf[pr][t][half >> 1, k0:k0 + DH,
                                                                 i * 128:(i + 1) * 128]
                                                     - _of_tile(ms, b, i))
                                        lu[b, i] = _red8(e, jnp.add)
                                        pu[b, i] = _pack(e)
                                at = [(b, i) for i in range(4 - b)]
                                lt = lt + _of_head([lu.get(k) for k in at], b, h, 0.0)
                                rows.append(_of_head([pu.get(k) for k in at], b, h, u32(0)))
                            p = _unpack(jnp.concatenate(rows, axis=0))
                        lacc[h] = lt if lacc[h] is None else lacc[h] + lt
                        o = _dot(_unpack(vt[g, _hs(h * DH, DH), ks]), p)
                        oacc[h] = o if oacc[h] is None else oacc[h] + o
                        if h == 0:
                            last["o"] = o[0:8, :]
            if gn is not None:
                mbuf[t][pw] = jnp.max(macc, axis=0, keepdims=True)
            if g is not None:
                parts = []
                for h in range(4):
                    l = jnp.sum(lacc[h], axis=0, keepdims=True)
                    gh = gate[half, g * 4 + h:g * 4 + h + 1, :]
                    oh = oacc[h] * ((1.0 - gh) / l)
                    parts.append(pltpu.roll(oh, 128 - DH * ROT[h], 1) if h else oh)
                ot = jnp.concatenate(parts, axis=0) + amem[g, :, t * 128:(t + 1) * 128]
                if g < GH - 1 or t < 2:
                    ob[g, _hs(t * 128, 128), :] = _pack(ot.T)
                else:
                    obl[half, _hs((t - 2) * 128, 128), :] = _pack(ot.T)

    rowh = jax.lax.broadcasted_iota(jnp.int32, (128, 128), 0) // DH
    colh = jax.lax.broadcasted_iota(jnp.int32, (128, 128), 1) // DH
    row16 = jax.lax.broadcasted_iota(jnp.int32, (16, 128), 0)
    col16 = jax.lax.broadcasted_iota(jnp.int32, (16, 128), 1) // DH

    def attn_half(layer, seg, half):
        r0 = pl.multiple_of(seg * L, L)

        @pl.when(jnp.logical_and(jnp.logical_and(layer == 0, seg == 0), half == 1))
        def _():
            cp_wk[1].wait()
            cp_wo[1].wait()
            cp_w1.wait()
            cp_xr.wait()
            cp_w2.wait()
            for cp in cp_stage[4:8]:
                cp.wait()
            for ic in range(4):
                transpose(1, 4 + ic, (ic >> 1) * DHALF, (ic & 1) * 2)

        def xn(c0, nc):
            return _unpack(xna[_hs(c0 * 128, nc * 128), :])

        zparts = {}

        def k_piece(g0, ng, c0, nc):
            k = _dot(xn(c0, nc), _unpack(wk[half, :, g0 * 128:(g0 + ng) * 128]))
            pk = _phi(k)
            rs = _hs(c0 * 128, nc * 128)
            for i in range(ng):
                cs = slice(i * 128, (i + 1) * 128)
                kb[g0 + i, rs, :] = _pack(k[:, cs])
                pkb[g0 + i, rs, :] = _pack(pk[:, cs])
                zparts.setdefault(g0 + i, []).append(_red8(pk[:, cs], jnp.add))

        def qv_piece(qs, vs, c0, nc):
            offs = [g * 128 for g in qs] + [DHALF + g * 128 for g in vs]
            lhs = jnp.concatenate(
                [jnp.concatenate([wt[half, c, _hs(o, 128), :] for c in range(NTC)], axis=1)
                 for o in offs], axis=0)
            r = _dot_nt(_unpack(lhs), xn(c0, nc))
            ts = slice(c0 * 128, (c0 + nc) * 128)
            for i, g in enumerate(qs):
                qg = r[i * 128:(i + 1) * 128, :]
                qp = _pack(qg * QSCALE)
                for c in range(nc):
                    for h in range(4):
                        qh = qp[_hs(h * DH, DH), c * 128:(c + 1) * 128]
                        qt[g, _hs(h * DH, DH), (c0 + c) * 128:(c0 + c + 1) * 128] = (
                            pltpu.roll(qh, DH * ROT[h], 1) if h else qh)
                pqt[g, :, ts] = _pack(_phi(qg))
            for i, g in enumerate(vs):
                o = (len(qs) + i) * 128
                vt[g, :, ts] = _pack(r[o:o + 128, :])

        def mem(g):
            zold = zrow[half, g]
            mold = mt[half, g]
            mbd = jnp.where(rowh == colh, mold, 0.0)
            zx = jnp.where(row16 == col16, jnp.broadcast_to(zold, (16, 128)), 0.0)
            lhs = jnp.concatenate([mbd, zx], axis=0).astype(bf16)
            ret = _dot(lhs, _unpack(pqt[g]))
            parts = []
            for h in range(4):
                gh = gate[half, g * 4 + h:g * 4 + h + 1, 0:1]
                den = ret[128 + h:129 + h, :] + 1e-6
                parts.append(ret[h * DH:(h + 1) * DH, :] * (gh / den))
            amem[g] = jnp.concatenate(parts, axis=0)
            zsum = functools.reduce(jnp.add, zparts[g])
            zrow[half, g] = zold + jnp.sum(zsum, axis=0, keepdims=True)

        def upd(g):
            mt[half, g] = mt[half, g] + _dot(_unpack(vt[g]), _unpack(pkb[g]))

        def mem_upd(g):
            mem(g)
            upd(g)

        P = functools.partial
        skip = None
        last = {}
        k_piece(0, 2, 0, 4)
        qv_piece((0, 1), (0,), 0, 4)
        attn_step(half, None, 0, last)
        mem(0)
        for g in range(2):
            attn_step(half, g, g + 1, last, fill=[
                skip, P(k_piece, g + 2, 1, 0, 2), skip, P(qv_piece, (g + 2,), (g + 1,), 0, 1),
                P(qv_piece, (g + 2,), (g + 1,), 1, 1), skip, P(k_piece, g + 2, 1, 2, 2),
                P(qv_piece, (g + 2,), (g + 1,), 2, 1), P(qv_piece, (g + 2,), (g + 1,), 3, 1),
                P(mem_upd, g + 1)])
        attn_step(half, 2, 3, last, fill=[
            P(upd, 0), skip, P(qv_piece, (), (3,), 0, 1), skip, P(qv_piece, (), (3,), 1, 1),
            skip, P(qv_piece, (), (3,), 2, 1), P(qv_piece, (), (3,), 3, 1), skip, P(mem_upd, 3)])

        def wo_piece(t, n):
            off = t * 128
            cs = slice(n * DHALF, (n + 1) * DHALF)
            rr = pl.ds(r0 + (HALO + off), 128)
            ng = GH if t < 2 else GH - 1
            o = jnp.concatenate([ob[g, _hs(off, 128), :] for g in range(ng)], axis=1)
            big[rr, cs] = big[rr, cs] + _dot(_unpack(o), _unpack(wo[half, _hs(0, ng * 128), cs]))

        attn_step(half, GH - 1, None, last, fill=[
            P(wo_piece, 2, 0), P(wo_piece, 2, 1), P(wo_piece, 3, 0), skip, P(wo_piece, 3, 1),
            P(wo_piece, 0, 0), skip, P(wo_piece, 0, 1), P(wo_piece, 1, 0), skip])
        wo_piece(1, 1)

    def phase_a(layer, seg):
        r0 = pl.multiple_of(seg * L, L)

        def half_body(half, _):
            attn_half(layer, seg, half)
            return 0
        jax.lax.fori_loop(0, 2, half_body, 0)

        hl = L // 2
        kp = (GH - 1) * 128

        bw = big.at[pl.ds(r0, 2 * L + 2 * HALO), :]
        yw = yres.at[pl.ds(r0, L + 2 * HALO), :]
        hw = hbuf.at[pl.ds(r0, L + 2 * HALO), :]
        xw = xin.at[pl.ds(r0 + L, L), :]

        def wo_rest():
            rr = slice(HALO + hl, HALO + L)
            o = _unpack(jnp.concatenate([obl[0], obl[1]], axis=1))
            w = _unpack(jnp.concatenate([wo[i, _hs(kp, 128), :] for i in range(2)], axis=0))
            bw[rr, :] = bw[rr, :] + _dot(o, w)

        def lnln(off, n):
            rr = slice(HALO + off, HALO + off + n)
            r, mr, z = _ln_ln(bw[rr, :])
            yw[rr, D - 256:D - 128] = jnp.broadcast_to(r, (n, 128))
            yw[rr, D - 128:D] = jnp.broadcast_to(mr, (n, 128))
            xnb[_hs(off, n), :] = _pack(z)

        def corners(v):
            return [v[0:8, 0:128], v[hl - 8:hl, 0:128], v[0:8, 128:256], v[hl - 8:hl, 128:256]]

        def up(off, n):
            cs = slice(n * 256, (n + 1) * 256)
            hh = _gelu(_dot(_unpack(xnb[_hs(off, hl), :]), _unpack(w1[:, cs])))
            b = off + HALO + SHIFTS[n]
            hw[b:b + hl, cs] = hh
            return corners(hh)

        sink = PIN + pl.multiple_of(seg * 16, 16)

        def pin(ref, v):
            if ref.dtype == bf16:
                ref[pl.ds(sink, 16), 0:128] = jnp.concatenate([v, v], axis=0).astype(bf16)
            else:
                ref[pl.ds(sink, 8), 0:128] = v

        fresh = jnp.logical_and(layer == 0, seg < NSEG - 1)

        def ln_next(off, n):
            rr = slice(L + HALO + off, L + HALO + off + n)
            xv = jnp.where(fresh, xw[off:off + n, :].astype(f32), bw[rr, :])
            bw[rr, :] = xv
            xna[_hs(off, n), :] = _pack(_ln(xv))

        lnln(0, 128)
        lnln(128, 128)
        wo_rest()
        def mix_part(off, n):
            return corners(mix(hw, yw, bw, slice(off, off + hl), n))

        def probe():
            return pltpu.bitcast(xna[pl.ds(pl.multiple_of(seg * 8, 8), 8), 0:128], f32)

        late = list(range(hl, L, 16))
        nxt = list(range(0, L, 16))

        def next_piece(mark):
            done = probe()
            ln_next(nxt.pop(0), 16)
            pin(xin, mark + done)

        for n in range(4):
            for mark in up(0, n):
                lnln(late.pop(0), 16)
                pin(big, mark)
        for n in range(4):
            for mark in mix_part(0, n):
                next_piece(mark)
        for n in range(4):
            for mark in up(hl, n)[1:]:
                next_piece(mark)
        for n in range(4):
            if n == 3:
                pin(yres, probe())
            for mark in mix_part(hl, n):
                if nxt:
                    next_piece(mark)

    def mix(h_ref, y_ref, x_ref, rr, n):
        cs = slice(n * 256, (n + 1) * 256)
        r = y_ref[rr, D - 256:D - 128]
        mr = y_ref[rr, D - 128:D]
        x = x_ref[rr, cs]
        y = x * jnp.concatenate([r, r], axis=1) - jnp.concatenate([mr, mr], axis=1)
        x1 = y + _dot(h_ref[rr, :].astype(bf16), _unpack(w2[:, cs]))
        y_ref[rr, cs] = x1
        x_ref[rr, cs] = x + x1
        return x1

    def ln_mid(tok, n):
        xnc[_hs(tok, n), :] = _pack(_ln(yres[pl.ds(tok + HALO, n), :]))

    def last_rows():
        for n in range(4):
            mix(hbuf, yres, big, slice(S, PAD_ROWS), n)
            ln_mid(n * 128, 128)

    def out_copy(blk):
        rows = pl.ds(blk * L, L)
        return pltpu.make_async_copy(obuf.at[rows], out_hbm.at[0, rows, :], osems.at[blk])

    def ffn(layer, it):
        def block_of(pair):
            return (pair * 37) >> 8

        blk, chunk, tok = [], [], []
        for h in range(UNROLL // 2):
            pair = (UNROLL // 2) * it + h
            b = block_of(pair)
            c = 2 * pair - NC * b
            t = pl.multiple_of(b * L, L)
            blk += [b, b]
            chunk += [c, c + 1]
            tok += [t, t]

        def ffn_up(k):
            hh = _gelu(_dot(_unpack(xnc[_hs(tok[k], L), :]), _unpack(w3[chunk[k]])))
            gh[k % 2] = _pack(hh)
            return [hh[r:r + 8, FC - 128:FC] for r in (0, 256, L - 8)]

        def ffn_down(k):
            rows = pl.ds(tok[k] + HALO, L)
            w = _unpack(w4[_hs(chunk[k] * FC, FC), :])
            y = big[rows, :] + _dot(_unpack(gh[k % 2]), w)
            big[rows, :] = y
            return [y[r:r + 8, c:c + 128]
                    for r, c in ((0, 0), (256, 0), (504, 0), (0, 512), (256, 512))]

        sink = pl.ds(PIN + pl.multiple_of(blk[0] * 16, 16), 8)

        def ln_ahead(k, marks):
            nb = jnp.minimum(blk[k] + 1, NSEG - 1)
            r = nb * L + jnp.minimum(chunk[k] * 40, L - 80)
            n = 80 // len(marks)
            for i, mark in enumerate(marks):
                yres[sink, 0:128] = mark
                ln_mid(pl.multiple_of(r + i * n, 16), n)

        def ln_first(marks):
            r0 = jnp.clip((it - 3) * 48, 0, L - 48)
            for i, mark in enumerate(marks):
                r = pl.multiple_of(r0 + i * 16, 16)
                xna[_hs(r, 16), :] = _pack(_ln(big[pl.ds(r + HALO, 16), :]))
                if i < 2:
                    big[sink, 0:128] = mark

        ffn_up(0)
        ffn_up(1)
        ln_ahead(0, ffn_down(0))
        ffn_up(2)
        ffn_down(1)
        ln_first(ffn_up(3))
        ln_ahead(2, ffn_down(2))
        ffn_down(3)

        done = block_of((UNROLL // 2) * (it + 1))

        @pl.when(jnp.logical_and(layer == 1, done != blk[0]))
        def _():
            r = pl.multiple_of((done - 1) * L, L)
            obuf[pl.ds(r, L), :] = big[pl.ds(r + HALO, L), :].astype(bf16)
            out_copy(done - 1).start()

    def layer_body(layer, _):
        mt[...] = jnp.zeros(mt.shape, f32)
        zrow[...] = jnp.zeros(zrow.shape, f32)

        def a_body(seg, _):
            phase_a(layer, seg)
            return 0
        jax.lax.fori_loop(0, NSEG, a_body, 0)

        last_rows()

        @pl.when(layer == 0)
        def _():
            for c in cp_w3:
                c.wait()
            cp_w4.wait()

        def b_body(it, _):
            ffn(layer, it)
            return 0
        jax.lax.fori_loop(0, NSEG * NC // UNROLL, b_body, 0)
        return 0
    jax.lax.fori_loop(0, 2, layer_body, 0)

    for blk in range(NSEG):
        out_copy(blk).wait()


@jax.jit
def pallas_interleave_layers__memory_aug_infini_attn__mixer_s_mlp__prompt_kernel(
    A_x: jax.Array,
    A_wq: jax.Array,
    A_wk: jax.Array,
    A_wv: jax.Array,
    A_wo: jax.Array,
    A_beta: jax.Array,
    B_x: jax.Array,
    B_w1: jax.Array,
    B_w2: jax.Array,
    B_w3: jax.Array,
    B_w4: jax.Array,
):
    del B_x
    hbm = pl.BlockSpec(memory_space=pl.ANY)
    vm = pltpu.VMEM
    scratch = [
        vm((BIG_ROWS, D), bf16),
        vm((8, DHALF, DHALF), bf16),
        vm((2, 4, D // 2, 256), u32),
        vm((2, D // 2, DHALF), u32),
        vm((2, DHALF // 2, D), u32),
        vm((D // 2, D), u32),
        vm((D // 2, D), u32),
        vm((NC, D // 2, FC), u32),
        vm((F // 2, D), u32),
        vm((BIG_ROWS, D), f32),
        vm((BIG_ROWS, D), f32),
        vm((PAD_ROWS, D), f32),
        vm((L // 2, D), u32),
        vm((L // 2, D), u32),
        vm((S // 2, D), u32),
        vm((2, L // 2, FC), u32),
        vm((GH, 64, L), u32),
        vm((GH, 64, L), u32),
        vm((GH, L // 2, 128), u32),
        vm((GH, L // 2, 128), u32),
        vm((GH, 64, L), u32),
        vm((GH, L // 2, 128), u32),
        vm((2, L // 4, 128), u32),
        vm((GH, 128, L), f32),
        vm((2, GH, 128, 128), f32),
        vm((2, GH, 1, 128), f32),
        vm((2, H // 2, 128), f32),
        vm((128, 512), f32),
    ]
    scratch += [vm((1, 128 * (t + 1) + 8, 512), f32) for _ in range(2) for t in range(NT_TILES)]
    scratch += [vm((2, 1, 512), f32) for _ in range(NT_TILES)]
    scratch += [
        vm((S, D), bf16),
        pltpu.SemaphoreType.DMA((10,)),
        pltpu.SemaphoreType.DMA((8,)),
        pltpu.SemaphoreType.DMA((NSEG,)),
    ]
    return pl.pallas_call(
        _kernel,
        out_shape=jax.ShapeDtypeStruct((1, S, D), bf16),
        in_specs=[hbm, hbm, hbm, hbm, hbm, pl.BlockSpec(memory_space=pltpu.VMEM),
                  hbm, hbm, hbm, hbm],
        out_specs=hbm,
        scratch_shapes=scratch,
        compiler_params=pltpu.CompilerParams(vmem_limit_bytes=120 * 1024 * 1024),
    )(A_x, A_wq, A_wk, A_wv, A_wo, A_beta.reshape(1, H), B_w1, B_w2, B_w3, B_w4)
```

```python
import functools
import math

import jax
import jax.numpy as jnp
import jax.experimental.pallas as pl
import jax.experimental.pallas.tpu as pltpu

S = 2048
D = 1024
F = 3584
H = 32
DH = 32
L = 512
NSEG = S // L
NG = D // 128
NT_TILES = L // 128
FC = 256
HALO = 8
GH = NG // 2
DHALF = D // 2
PAD_ROWS = S + 2 * HALO
PIN = S + L + 2 * HALO
BIG_ROWS = PIN + 16 * NSEG
NC = F // FC
UNROLL = 4
SHIFTS = (1, -1, 2, -2)
ROT = (0, 2, 1, 3)
OWNER = (((0,) * 4, (1,) * 4, (2,) * 4, (3,) * 4),
         ((3, 0, 0, 0), (1, 1, 3, 1), (2, 3, 2, 2)),
         ((1, 1, 0, 0), (2, 3, 3, 2)),
         ((2, 1, 3, 0),))

LOG2E = math.log2(math.e)
QSCALE = DH ** -0.5 * LOG2E
MASK_BIAS = -1e9 * LOG2E
EPS = 1e-5

f32 = jnp.float32
bf16 = jnp.bfloat16
u32 = jnp.uint32
NT_DIMS = (((1,), (1,)), ((), ()))


def _stats(x):
    m = jnp.mean(x, axis=-1, keepdims=True)
    xc = x - m
    return m, jnp.mean(xc * xc, axis=-1, keepdims=True)


def _ln(x):
    m, v = _stats(x)
    r = jax.lax.rsqrt(v + EPS)
    return x * r - m * r


def _ln_ln(x):
    m, v = _stats(x)
    r1 = jax.lax.rsqrt(v + EPS)
    r2 = r1 * jax.lax.rsqrt(v * r1 * r1 + EPS)
    return r1, m * r1, x * r2 - m * r2


def _gelu(x):
    c = math.sqrt(2.0 / math.pi)
    inner = x * (c + (c * 0.044715) * (x * x))
    hx = 0.5 * x
    return hx + hx * jnp.tanh(inner)


def _phi(t):
    return jnp.where(t > 0, t + 1.0, jnp.exp(t))


def _red8(x, op):
    return functools.reduce(op, [x[i * 8:(i + 1) * 8] for i in range(x.shape[0] // 8)])


def _pick(pos, x, other):
    if len(pos) == 4:
        return x
    lane = jax.lax.broadcasted_iota(jnp.int32, x.shape, 1)
    if len(pos) == 2:
        low = lane < 64 if pos in ((0, 1), (2, 3)) else ((lane + 32) & 127) < 64
        return jnp.where(low, x, other) if 0 in pos else jnp.where(low, other, x)
    if len(pos) == 1:
        return jnp.where((lane >> 5) == pos[0], x, other)
    return jnp.where((lane >> 5) == 6 - sum(pos), other, x)


def _owned(b, i, h):
    return tuple(p for p in range(4) if OWNER[b][i][p] == h)


def _of_head(tiles, b, h, other):
    for i, x in enumerate(tiles):
        if _owned(b, i, h):
            other = _pick(_owned(b, i, h), x, other)
    return other


def _of_tile(heads, b, i):
    out = None
    for h in sorted(set(OWNER[b][i]), key=lambda h: -len(_owned(b, i, h))):
        out = heads[h] if out is None else _pick(_owned(b, i, h), heads[h], out)
    return out


def _pack(x):
    return pltpu.bitcast(x.astype(bf16), u32)


def _unpack(x):
    return pltpu.bitcast(x, bf16)


def _hs(start, n):
    if isinstance(start, int):
        return slice(start // 2, (start + n) // 2)
    return pl.ds(pl.multiple_of(start >> 1, 8), n // 2)


def _dot(a, b):
    return jnp.dot(a, b, preferred_element_type=f32)


def _dot_nt(a, b):
    return jax.lax.dot_general(a, b, NT_DIMS, preferred_element_type=f32)


def _kernel(x_hbm, wq_hbm, wk_hbm, wv_hbm, wo_hbm, beta_ref, w1_hbm, w2_hbm, w3_hbm, w4_hbm,
            out_hbm,
            xin, stage, wt, wk, wo, w1, w2, w3, w4,
            big, yres, hbuf, xna, xnb, xnc, gh, qt, pqt, kb, pkb, vt, ob, obl, amem,
            mt, zrow, gate, bias,
            s0, s1, s2, s3, s4, s5, s6, s7, m0, m1, m2, m3,
            obuf, sems, tsems, osems):
    sbuf = ((s0, s1, s2, s3), (s4, s5, s6, s7))
    mbuf = (m0, m1, m2, m3)

    def seg_rows(s):
        return pl.ds(s * L, L)

    cp_x0 = pltpu.make_async_copy(x_hbm.at[0, seg_rows(0)], xin.at[seg_rows(0)], sems.at[0])
    cp_xr = pltpu.make_async_copy(x_hbm.at[0, pl.ds(L, S - L)], xin.at[pl.ds(L, S - L)], sems.at[1])
    cp_wk = [pltpu.make_async_copy(wk_hbm.at[:, pl.ds(i * DHALF, DHALF)], wk.at[i].bitcast(bf16),
                                   sems.at[2 + i])
             for i in range(2)]
    cp_wo = [pltpu.make_async_copy(wo_hbm.at[pl.ds(i * DHALF, DHALF)], wo.at[i].bitcast(bf16),
                                   sems.at[4 + i])
             for i in range(2)]
    cp_w1 = pltpu.make_async_copy(w1_hbm, w1.bitcast(bf16), sems.at[6])
    cp_w2 = pltpu.make_async_copy(w2_hbm, w2.bitcast(bf16), sems.at[7])
    cp_w3 = [pltpu.make_async_copy(w3_hbm.at[:, pl.ds(c * FC, FC)], w3.at[c].bitcast(bf16),
                                   sems.at[8])
             for c in range(F // FC)]
    cp_w4 = pltpu.make_async_copy(w4_hbm, w4.bitcast(bf16), sems.at[9])

    TC = 256
    NTC = D // TC

    cp_stage = [pltpu.make_async_copy(
        (wq_hbm, wv_hbm)[(ic >> 1) & 1].at[pl.ds((ic & 1) * DHALF, DHALF),
                                           pl.ds((ic >> 2) * DHALF, DHALF)],
        stage.at[ic], tsems.at[ic]) for ic in range(8)]

    for cp in cp_stage[0:4]:
        cp.start()
    for cp in (cp_x0, cp_wk[0], cp_wo[0]):
        cp.start()

    kk = jax.lax.broadcasted_iota(jnp.int32, (DH, 128), 0)
    ll = jax.lax.broadcasted_iota(jnp.int32, (DH, 128), 1)
    qq = [(ll + (128 - DH * r)) & 127 for r in ROT]
    for b in range(4):
        for i in range(4 - b):
            bias[b * DH:(b + 1) * DH, i * 128:(i + 1) * 128] = jnp.where(
                kk + b * DH > _of_tile(qq, b, i), MASK_BIAS, 0.0).astype(f32)
    bt = jnp.broadcast_to(beta_ref[...].astype(f32), (H, H))
    eye = (jax.lax.broadcasted_iota(jnp.int32, (H, H), 0)
           == jax.lax.broadcasted_iota(jnp.int32, (H, H), 1))
    bcol = jnp.sum(jnp.where(eye, bt, 0.0), axis=1, keepdims=True)
    gsig = jnp.broadcast_to(jax.nn.sigmoid(bcol), (H, 128))
    gate[0] = gsig[0:H // 2]
    gate[1] = gsig[H // 2:H]
    hbuf[0:2 * HALO, :] = jnp.zeros((2 * HALO, D), f32)
    hbuf[S:PAD_ROWS, :] = jnp.zeros((2 * HALO, D), f32)
    for ref in (big, yres):
        ref[0:HALO, :] = jnp.zeros((HALO, D), f32)
        ref[S + HALO:PAD_ROWS, :] = jnp.zeros((HALO, D), f32)

    ident = (jax.lax.broadcasted_iota(jnp.int32, (128, 128), 0)
             == jax.lax.broadcasted_iota(jnp.int32, (128, 128), 1)).astype(f32).astype(bf16)

    def transpose(hf, ic, ro, c0):
        for c in range(2):
            for n in range(GH):
                tile = _dot_nt(ident, stage[ic, c * TC:(c + 1) * TC, n * 128:(n + 1) * 128])
                wt[hf, c0 + c, _hs(ro + n * 128, 128), :] = _pack(tile)

    def transpose_chunk(ic, _):
        pltpu.make_async_copy(stage.at[ic], stage.at[ic], tsems.at[ic]).wait()
        transpose(0, ic, pl.multiple_of((ic >> 1) * DHALF, DHALF), (ic & 1) * 2)
        return 0
    jax.lax.fori_loop(0, 4, transpose_chunk, 0)

    cp_x0.wait()

    def init_x(i, _):
        r = pl.multiple_of(i * 256, 256)
        xv = xin[pl.ds(r, 256), :].astype(f32)
        big[pl.ds(HALO + r, 256), :] = xv
        xna[_hs(r, 256), :] = _pack(_ln(xv))
        return 0
    jax.lax.fori_loop(0, L // 256, init_x, 0)
    cp_wk[0].wait()
    for cp in cp_stage[4:8] + [cp_wk[1], cp_wo[1], cp_w1, cp_xr, cp_w2] + cp_w3 + [cp_w4]:
        cp.start()
    cp_wo[0].wait()

    def qmask(g, t, b=0):
        z = jnp.zeros((DH // 2, 128), u32)
        qs = [qt[g, _hs(h * DH, DH), t * 128:(t + 1) * 128] for h in range(4)]
        cols = [jnp.concatenate([_pick(_owned(b, i, h), qs[h], z) if _owned(b, i, h) else z
                                 for h in range(4)], axis=0) for i in range(4 - b)]
        return _unpack(jnp.concatenate(cols, axis=1))

    def tiles(x):
        return [x[:, i * 128:(i + 1) * 128] for i in range(x.shape[1] // 128)]

    def attn_step(half, g, gn, last, fill=()):
        pr = None if g is None else g % 2
        pw = None if gn is None else gn % 2
        fill = list(fill)
        for t in range(NT_TILES):
            macc = None
            oacc = [None] * 4
            lacc = [None] * 4
            for j in range(t + 1):
                ks = slice(j * 128, (j + 1) * 128)
                nk = DH if j == t else 128
                kl = slice(j * 128, j * 128 + nk)
                filled = fill.pop(0) if fill else None
                if filled:
                    filled()
                    last["pace"] = last.get("o", last["s"])
                elif gn is not None and g is not None:
                    last["pace"] = last["s"]
                if g is not None:
                    sbuf[pr][t][0, (t + 1) * 128:(t + 1) * 128 + 8, 0:128] = last["pace"]
                if gn is not None:
                    s = _dot(_unpack(kb[gn, _hs(j * 128, nk), :]), qmask(gn, t))
                    if j == t:
                        s = s + bias[0:DH, :]
                    sbuf[pw][t][0, kl, :] = s
                    last["s"] = s[0:8, 0:128]
                    mx = _red8(s, jnp.maximum)
                    if j == t:
                        mx = tiles(mx)
                        for b in range(1, 4):
                            k0 = j * 128 + b * DH
                            su = _dot(_unpack(kb[gn, _hs(k0, DH), :]), qmask(gn, t, b))
                            su = su + bias[b * DH:(b + 1) * DH, 0:(4 - b) * 128]
                            sbuf[pw][t][0, k0:k0 + DH, 0:(4 - b) * 128] = su
                            mu = tiles(_red8(su, jnp.maximum))
                            mx = [jnp.maximum(mx[h], _of_head(mu, b, h, mx[h])) for h in range(4)]
                        mx = jnp.concatenate(mx, axis=1)
                    macc = mx if macc is None else jnp.maximum(macc, mx)
                if g is not None:
                    ms = tiles(mbuf[t][pr])
                    pu, lu = {}, {}
                    for h in range(4):
                        sl = slice(h * 128, (h + 1) * 128)
                        p = jnp.exp2(sbuf[pr][t][half >> 1, kl, sl] - ms[h])
                        lt = _red8(p, jnp.add)
                        p = p.astype(bf16)
                        if j == t:
                            rows = [pltpu.bitcast(p, u32)]
                            for b in range(1, 4):
                                k0 = j * 128 + b * DH
                                for i in range(4 - b):
                                    if _owned(b, i, h) and (b, i) not in pu:
                                        e = jnp.exp2(sbuf[pr][t][half >> 1, k0:k0 + DH,
                                                                 i * 128:(i + 1) * 128]
                                                     - _of_tile(ms, b, i))
                                        lu[b, i] = _red8(e, jnp.add)
                                        pu[b, i] = _pack(e)
                                at = [(b, i) for i in range(4 - b)]
                                lt = lt + _of_head([lu.get(k) for k in at], b, h, 0.0)
                                rows.append(_of_head([pu.get(k) for k in at], b, h, u32(0)))
                            p = _unpack(jnp.concatenate(rows, axis=0))
                        lacc[h] = lt if lacc[h] is None else lacc[h] + lt
                        o = _dot(_unpack(vt[g, _hs(h * DH, DH), ks]), p)
                        oacc[h] = o if oacc[h] is None else oacc[h] + o
                        if h == 0:
                            last["o"] = o[0:8, :]
            if gn is not None:
                mbuf[t][pw] = jnp.max(macc, axis=0, keepdims=True)
            if g is not None:
                parts = []
                for h in range(4):
                    l = jnp.sum(lacc[h], axis=0, keepdims=True)
                    gh = gate[half, g * 4 + h:g * 4 + h + 1, :]
                    oh = oacc[h] * ((1.0 - gh) / l)
                    parts.append(pltpu.roll(oh, 128 - DH * ROT[h], 1) if h else oh)
                ot = jnp.concatenate(parts, axis=0) + amem[g, :, t * 128:(t + 1) * 128]
                if g < GH - 1 or t < 2:
                    ob[g, _hs(t * 128, 128), :] = _pack(ot.T)
                else:
                    obl[half, _hs((t - 2) * 128, 128), :] = _pack(ot.T)

    rowh = jax.lax.broadcasted_iota(jnp.int32, (128, 128), 0) // DH
    colh = jax.lax.broadcasted_iota(jnp.int32, (128, 128), 1) // DH
    row16 = jax.lax.broadcasted_iota(jnp.int32, (16, 128), 0)
    col16 = jax.lax.broadcasted_iota(jnp.int32, (16, 128), 1) // DH

    def attn_half(layer, seg, half):
        r0 = pl.multiple_of(seg * L, L)

        @pl.when(jnp.logical_and(jnp.logical_and(layer == 0, seg == 0), half == 1))
        def _():
            cp_wk[1].wait()
            cp_wo[1].wait()
            cp_w1.wait()
            cp_xr.wait()
            cp_w2.wait()
            for cp in cp_stage[4:8]:
                cp.wait()
            for ic in range(4):
                transpose(1, 4 + ic, (ic >> 1) * DHALF, (ic & 1) * 2)

        def xn(c0, nc):
            return _unpack(xna[_hs(c0 * 128, nc * 128), :])

        zparts = {}

        def k_piece(g0, ng, c0, nc):
            k = _dot(xn(c0, nc), _unpack(wk[half, :, g0 * 128:(g0 + ng) * 128]))
            pk = _phi(k)
            rs = _hs(c0 * 128, nc * 128)
            for i in range(ng):
                cs = slice(i * 128, (i + 1) * 128)
                kb[g0 + i, rs, :] = _pack(k[:, cs])
                pkb[g0 + i, rs, :] = _pack(pk[:, cs])
                zparts.setdefault(g0 + i, []).append(_red8(pk[:, cs], jnp.add))
            return k

        def qv_piece(qs, vs, c0, nc):
            offs = [g * 128 for g in qs] + [DHALF + g * 128 for g in vs]
            lhs = jnp.concatenate(
                [jnp.concatenate([wt[half, c, _hs(o, 128), :] for c in range(NTC)], axis=1)
                 for o in offs], axis=0)
            r = _dot_nt(_unpack(lhs), xn(c0, nc))
            ts = slice(c0 * 128, (c0 + nc) * 128)
            for i, g in enumerate(qs):
                qg = r[i * 128:(i + 1) * 128, :]
                qp = _pack(qg * QSCALE)
                for c in range(nc):
                    for h in range(4):
                        qh = qp[_hs(h * DH, DH), c * 128:(c + 1) * 128]
                        qt[g, _hs(h * DH, DH), (c0 + c) * 128:(c0 + c + 1) * 128] = (
                            pltpu.roll(qh, DH * ROT[h], 1) if h else qh)
                pqt[g, :, ts] = _pack(_phi(qg))
            for i, g in enumerate(vs):
                o = (len(qs) + i) * 128
                vt[g, :, ts] = _pack(r[o:o + 128, :])

        def mem(g):
            zold = zrow[half, g]
            mold = mt[half, g]
            mbd = jnp.where(rowh == colh, mold, 0.0)
            zx = jnp.where(row16 == col16, jnp.broadcast_to(zold, (16, 128)), 0.0)
            lhs = jnp.concatenate([mbd, zx], axis=0).astype(bf16)
            ret = _dot(lhs, _unpack(pqt[g]))
            parts = []
            for h in range(4):
                gh = gate[half, g * 4 + h:g * 4 + h + 1, 0:1]
                den = ret[128 + h:129 + h, :] + 1e-6
                parts.append(ret[h * DH:(h + 1) * DH, :] * (gh / den))
            amem[g] = jnp.concatenate(parts, axis=0)
            zsum = functools.reduce(jnp.add, zparts[g])
            zrow[half, g] = zold + jnp.sum(zsum, axis=0, keepdims=True)

        def upd(g):
            mt[half, g] = mt[half, g] + _dot(_unpack(vt[g]), _unpack(pkb[g]))

        def mem_upd(g):
            mem(g)
            upd(g)

        P = functools.partial
        skip = None
        last = {}
        k = k_piece(0, 2, 0, 4)
        qv_piece((0, 1), (0,), 0, 4)
        f0 = jnp.clip((2 * seg + half - 2) * 96, 0, L - 96)
        ysink = pl.ds(PIN + pl.multiple_of(seg * 16, 16), 8)
        xprobe = pl.ds(pl.multiple_of(f0 >> 1, 8), 8)
        done = [k[0:8, 0:128], k[L - 8:L, 128:256]]
        for i in range(6):
            yres[ysink, 0:128] = done[i]
            ln_mid(pl.multiple_of(f0 + i * 16, 16), 16)
            done.append(pltpu.bitcast(xnc[xprobe, 0:128], f32))
        kb[0, 0:8, :] = jnp.where(half < 2, kb[0, 0:8, :], xnc[xprobe, 0:128])
        attn_step(half, None, 0, last)
        mem(0)
        for g in range(2):
            attn_step(half, g, g + 1, last, fill=[
                skip, P(k_piece, g + 2, 1, 0, 2), skip, P(qv_piece, (g + 2,), (g + 1,), 0, 1),
                P(qv_piece, (g + 2,), (g + 1,), 1, 1), skip, P(k_piece, g + 2, 1, 2, 2),
                P(qv_piece, (g + 2,), (g + 1,), 2, 1), P(qv_piece, (g + 2,), (g + 1,), 3, 1),
                P(mem_upd, g + 1)])
        attn_step(half, 2, 3, last, fill=[
            P(upd, 0), skip, P(qv_piece, (), (3,), 0, 1), skip, P(qv_piece, (), (3,), 1, 1),
            skip, P(qv_piece, (), (3,), 2, 1), P(qv_piece, (), (3,), 3, 1), skip, P(mem_upd, 3)])

        def wo_piece(t, n):
            off = t * 128
            cs = slice(n * DHALF, (n + 1) * DHALF)
            rr = pl.ds(r0 + (HALO + off), 128)
            ng = GH if t < 2 else GH - 1
            o = jnp.concatenate([ob[g, _hs(off, 128), :] for g in range(ng)], axis=1)
            big[rr, cs] = big[rr, cs] + _dot(_unpack(o), _unpack(wo[half, _hs(0, ng * 128), cs]))

        attn_step(half, GH - 1, None, last, fill=[
            P(wo_piece, 2, 0), P(wo_piece, 2, 1), P(wo_piece, 3, 0), skip, P(wo_piece, 3, 1),
            P(wo_piece, 0, 0), skip, P(wo_piece, 0, 1), P(wo_piece, 1, 0), skip])
        wo_piece(1, 1)

    def phase_a(layer, seg):
        r0 = pl.multiple_of(seg * L, L)

        def half_body(half, _):
            attn_half(layer, seg, half)
            return 0
        jax.lax.fori_loop(0, 2, half_body, 0)

        hl = L // 2
        kp = (GH - 1) * 128

        bw = big.at[pl.ds(r0, 2 * L + 2 * HALO), :]
        yw = yres.at[pl.ds(r0, L + 2 * HALO), :]
        hw = hbuf.at[pl.ds(r0, L + 2 * HALO), :]
        xw = xin.at[pl.ds(r0 + L, L), :]

        def wo_rest():
            rr = slice(HALO + hl, HALO + L)
            o = _unpack(jnp.concatenate([obl[0], obl[1]], axis=1))
            w = _unpack(jnp.concatenate([wo[i, _hs(kp, 128), :] for i in range(2)], axis=0))
            bw[rr, :] = bw[rr, :] + _dot(o, w)

        def lnln(off, n):
            rr = slice(HALO + off, HALO + off + n)
            r, mr, z = _ln_ln(bw[rr, :])
            yw[rr, D - 256:D - 128] = jnp.broadcast_to(r, (n, 128))
            yw[rr, D - 128:D] = jnp.broadcast_to(mr, (n, 128))
            xnb[_hs(off, n), :] = _pack(z)

        def corners(v):
            return [v[0:8, 0:128], v[hl - 8:hl, 0:128], v[0:8, 128:256], v[hl - 8:hl, 128:256]]

        def up(off, n):
            cs = slice(n * 256, (n + 1) * 256)
            hh = _gelu(_dot(_unpack(xnb[_hs(off, hl), :]), _unpack(w1[:, cs])))
            b = off + HALO + SHIFTS[n]
            hw[b:b + hl, cs] = hh
            return corners(hh)

        sink = PIN + pl.multiple_of(seg * 16, 16)

        def pin(ref, v):
            if ref.dtype == bf16:
                ref[pl.ds(sink, 16), 0:128] = jnp.concatenate([v, v], axis=0).astype(bf16)
            else:
                ref[pl.ds(sink, 8), 0:128] = v

        fresh = jnp.logical_and(layer == 0, seg < NSEG - 1)

        def ln_next(off, n):
            rr = slice(L + HALO + off, L + HALO + off + n)
            xv = jnp.where(fresh, xw[off:off + n, :].astype(f32), bw[rr, :])
            bw[rr, :] = xv
            xna[_hs(off, n), :] = _pack(_ln(xv))

        lnln(0, 128)
        lnln(128, 128)
        wo_rest()
        def mix_part(off, n):
            return corners(mix(hw, yw, bw, slice(off, off + hl), n))

        def probe():
            return pltpu.bitcast(xna[pl.ds(pl.multiple_of(seg * 8, 8), 8), 0:128], f32)

        late = list(range(hl, L, 16))
        nxt = list(range(0, L, 16))

        def next_piece(mark):
            done = probe()
            ln_next(nxt.pop(0), 16)
            pin(xin, mark + done)

        for n in range(4):
            for mark in up(0, n):
                lnln(late.pop(0), 16)
                pin(big, mark)
        for n in range(4):
            for mark in mix_part(0, n):
                next_piece(mark)
        for n in range(4):
            for mark in up(hl, n)[1:]:
                next_piece(mark)
        for n in range(4):
            if n == 3:
                pin(yres, probe())
            for mark in mix_part(hl, n):
                if nxt:
                    next_piece(mark)

    def mix(h_ref, y_ref, x_ref, rr, n):
        cs = slice(n * 256, (n + 1) * 256)
        r = y_ref[rr, D - 256:D - 128]
        mr = y_ref[rr, D - 128:D]
        x = x_ref[rr, cs]
        y = x * jnp.concatenate([r, r], axis=1) - jnp.concatenate([mr, mr], axis=1)
        x1 = y + _dot(h_ref[rr, :].astype(bf16), _unpack(w2[:, cs]))
        y_ref[rr, cs] = x1
        x_ref[rr, cs] = x + x1
        return x1

    def ln_mid(tok, n):
        xnc[_hs(tok, n), :] = _pack(_ln(yres[pl.ds(tok + HALO, n), :]))

    def last_rows():
        for n in range(4):
            mix(hbuf, yres, big, slice(S, PAD_ROWS), n)

    def out_copy(blk):
        rows = pl.ds(blk * L, L)
        return pltpu.make_async_copy(obuf.at[rows], out_hbm.at[0, rows, :], osems.at[blk])

    def ffn(layer, it):
        def block_of(pair):
            return (pair * 37) >> 8

        blk, chunk, tok = [], [], []
        for h in range(UNROLL // 2):
            pair = (UNROLL // 2) * it + h
            b = block_of(pair)
            c = 2 * pair - NC * b
            t = pl.multiple_of(b * L, L)
            blk += [b, b]
            chunk += [c, c + 1]
            tok += [t, t]

        def ffn_up(k):
            hh = _gelu(_dot(_unpack(xnc[_hs(tok[k], L), :]), _unpack(w3[chunk[k]])))
            gh[k % 2] = _pack(hh)
            return [hh[r:r + 8, FC - 128:FC] for r in (0, 256, L - 8)]

        def ffn_down(k):
            rows = pl.ds(tok[k] + HALO, L)
            w = _unpack(w4[_hs(chunk[k] * FC, FC), :])
            y = big[rows, :] + _dot(_unpack(gh[k % 2]), w)
            big[rows, :] = y
            return [y[r:r + 8, c:c + 128]
                    for r, c in ((0, 0), (256, 0), (504, 0), (0, 512), (256, 512))]

        sink = pl.ds(PIN + pl.multiple_of(blk[0] * 16, 16), 8)

        def ln_ahead(k, marks):
            nb = jnp.minimum(blk[k] + 1, NSEG - 1)
            r = nb * L + jnp.minimum(chunk[k] * 40, L - 80)
            n = 80 // len(marks)
            for i, mark in enumerate(marks):
                yres[sink, 0:128] = mark
                ln_mid(pl.multiple_of(r + i * n, 16), n)

        def ln_first(marks):
            r0 = jnp.clip((it - 3) * 48, 0, L - 48)
            for i, mark in enumerate(marks):
                r = pl.multiple_of(r0 + i * 16, 16)
                xna[_hs(r, 16), :] = _pack(_ln(big[pl.ds(r + HALO, 16), :]))
                if i < 2:
                    big[sink, 0:128] = mark

        ffn_up(0)
        ffn_up(1)
        ln_ahead(0, ffn_down(0))
        ffn_up(2)
        ffn_down(1)
        ln_first(ffn_up(3))
        ln_ahead(2, ffn_down(2))
        ffn_down(3)

        done = block_of((UNROLL // 2) * (it + 1))

        @pl.when(jnp.logical_and(layer == 1, done != blk[0]))
        def _():
            r = pl.multiple_of((done - 1) * L, L)
            obuf[pl.ds(r, L), :] = big[pl.ds(r + HALO, L), :].astype(bf16)
            out_copy(done - 1).start()

    def layer_body(layer, _):
        mt[...] = jnp.zeros(mt.shape, f32)
        zrow[...] = jnp.zeros(zrow.shape, f32)

        def a_body(seg, _):
            phase_a(layer, seg)
            return 0
        jax.lax.fori_loop(0, NSEG, a_body, 0)

        last_rows()

        @pl.when(layer == 0)
        def _():
            for c in cp_w3:
                c.wait()
            cp_w4.wait()

        def b_body(it, _):
            ffn(layer, it)
            return 0
        jax.lax.fori_loop(0, NSEG * NC // UNROLL, b_body, 0)
        return 0
    jax.lax.fori_loop(0, 2, layer_body, 0)

    for blk in range(NSEG):
        out_copy(blk).wait()


@jax.jit
def pallas_interleave_layers__memory_aug_infini_attn__mixer_s_mlp__prompt_kernel(
    A_x: jax.Array,
    A_wq: jax.Array,
    A_wk: jax.Array,
    A_wv: jax.Array,
    A_wo: jax.Array,
    A_beta: jax.Array,
    B_x: jax.Array,
    B_w1: jax.Array,
    B_w2: jax.Array,
    B_w3: jax.Array,
    B_w4: jax.Array,
):
    del B_x
    hbm = pl.BlockSpec(memory_space=pl.ANY)
    vm = pltpu.VMEM
    scratch = [
        vm((BIG_ROWS, D), bf16),
        vm((8, DHALF, DHALF), bf16),
        vm((2, 4, D // 2, 256), u32),
        vm((2, D // 2, DHALF), u32),
        vm((2, DHALF // 2, D), u32),
        vm((D // 2, D), u32),
        vm((D // 2, D), u32),
        vm((NC, D // 2, FC), u32),
        vm((F // 2, D), u32),
        vm((BIG_ROWS, D), f32),
        vm((BIG_ROWS, D), f32),
        vm((PAD_ROWS, D), f32),
        vm((L // 2, D), u32),
        vm((L // 2, D), u32),
        vm((S // 2, D), u32),
        vm((2, L // 2, FC), u32),
        vm((GH, 64, L), u32),
        vm((GH, 64, L), u32),
        vm((GH, L // 2, 128), u32),
        vm((GH, L // 2, 128), u32),
        vm((GH, 64, L), u32),
        vm((GH, L // 2, 128), u32),
        vm((2, L // 4, 128), u32),
        vm((GH, 128, L), f32),
        vm((2, GH, 128, 128), f32),
        vm((2, GH, 1, 128), f32),
        vm((2, H // 2, 128), f32),
        vm((128, 512), f32),
    ]
    scratch += [vm((1, 128 * (t + 1) + 8, 512), f32) for _ in range(2) for t in range(NT_TILES)]
    scratch += [vm((2, 1, 512), f32) for _ in range(NT_TILES)]
    scratch += [
        vm((S, D), bf16),
        pltpu.SemaphoreType.DMA((10,)),
        pltpu.SemaphoreType.DMA((8,)),
        pltpu.SemaphoreType.DMA((NSEG,)),
    ]
    return pl.pallas_call(
        _kernel,
        out_shape=jax.ShapeDtypeStruct((1, S, D), bf16),
        in_specs=[hbm, hbm, hbm, hbm, hbm, pl.BlockSpec(memory_space=pltpu.VMEM),
                  hbm, hbm, hbm, hbm],
        out_specs=hbm,
        scratch_shapes=scratch,
        compiler_params=pltpu.CompilerParams(vmem_limit_bytes=120 * 1024 * 1024),
    )(A_x, A_wq, A_wk, A_wv, A_wo, A_beta.reshape(1, H), B_w1, B_w2, B_w3, B_w4)
```
